```python
import jax
import jax.numpy as jnp

def _softmax(x, axis=-1):
    return jax.nn.softmax(x, axis=axis)

def _gelu(x):
    return jax.nn.gelu(x, approximate=True)

def _silu(x):
    return jax.nn.silu(x)

def _sigmoid(x):
    return jax.nn.sigmoid(x)

def _layernorm(x, axis=-1, eps=1e-05):
    m = jnp.mean(x, axis=axis, keepdims=True)
    v = jnp.var(x, axis=axis, keepdims=True)
    return (x - m) / jnp.sqrt(v + eps)

def _scatter_add(tgt, idx, src, axis=0):
    return tgt.at[idx].add(src)

def _segment_sum(src, seg, n):
    return jax.ops.segment_sum(src, seg, n)

class _Rng:

    def __init__(self, key):
        self._k = key

    def _next(self):
        self._k, sub = jax.random.split(self._k)
        return sub

    def normal(self, shape):
        return jax.random.normal(self._next(), shape, dtype=jnp.bfloat16)

    def randint(self, lo, hi, shape):
        return jax.random.randint(self._next(), shape, lo, hi, dtype=jnp.int32)

    def uniform(self, shape, lo=0.0, hi=1.0):
        return jax.random.uniform(self._next(), shape, jnp.bfloat16, lo, hi)

    def permutation(self, n):
        return jax.random.permutation(self._next(), n)
kernel_name = 'concat_heads__sliding_local_dilated__memory_aug_recurrent_mem_tr__prompt'

def setup_inputs():
    _rng = _Rng(jax.random.key(int.from_bytes(__import__("os").urandom(4), "little")))
    _w = lambda a: (lambda t: t.astype(jnp.bfloat16) if jnp.issubdtype(t.dtype, jnp.floating) else t)(jnp.asarray(a))

    def _A_setup():
        B, S, D = (1, 2048, 640)
        return {'x': _w((lambda *s: _rng.normal(s) * 0.05)(B, S, D)), 'wqkv': _w((lambda *s: _rng.normal(s) * 0.05)(D, 3 * D)), 'wo': _w((lambda *s: _rng.normal(s) * 0.05)(D, D))}
    _A_in = _A_setup()

    def _B_setup():
        B, S, Dm = (1, 2048, 640)
        H, Dh = (32, 192)
        M, seg = (8, 32)
        seg = min(seg, S)
        S = S // seg * seg
        return {'x': _w((lambda *s: _rng.normal(s) * 0.05)(B, S, Dm)), 'mem0': _w((lambda *s: _rng.normal(s) * 0.05)(B, M, Dm)), 'Wq': _w((lambda *s: _rng.normal(s) * 0.05)(Dm, H, Dh) * Dm ** (-0.5)), 'Wk': _w((lambda *s: _rng.normal(s) * 0.05)(Dm, H, Dh) * Dm ** (-0.5)), 'Wv': _w((lambda *s: _rng.normal(s) * 0.05)(Dm, H, Dh) * Dm ** (-0.5)), 'Wo': _w((lambda *s: _rng.normal(s) * 0.05)(H, Dh, Dm) * (H * Dh) ** (-0.5)), 'seg_len': seg}
    _B_in = _B_setup()
    return {'A_x': _A_in['x'], 'A_wqkv': _A_in['wqkv'], 'A_wo': _A_in['wo'], 'B_x': _B_in['x'], 'B_mem0': _B_in['mem0'], 'B_Wq': _B_in['Wq'], 'B_Wk': _B_in['Wk'], 'B_Wv': _B_in['Wv'], 'B_Wo': _B_in['Wo'], 'B_seg_len': _B_in['seg_len']}

def reference(A_x, A_wqkv, A_wo, B_x, B_mem0, B_Wq, B_Wk, B_Wv, B_Wo, B_seg_len):

    def _A_ref(x, wqkv, wo):
        B, S, D = x.shape
        H = 32
        Dh = D // H
        W, dil = (8, 2)
        qkv = (lambda x, *d: x.transpose(*d))((x @ wqkv).reshape(B, S, 3, H, Dh), 2, 0, 3, 1, 4)
        q, k, v = (qkv[0], qkv[1], qkv[2])
        scale = Dh ** (-0.5)
        pos = jnp.arange(S)
        off = jnp.arange(W) * dil
        idx = pos[:, None] - off[None, :]
        mask = idx >= 0
        idx_c = jnp.where(mask, idx, 0).reshape(-1)
        kg = k[:, :, idx_c, :].reshape(B, H, S, W, Dh)
        vg = v[:, :, idx_c, :].reshape(B, H, S, W, Dh)
        logits = jnp.einsum('bhsd,bhswd->bhsw', q, kg) * scale
        logits = jnp.where(mask[None, None, :, :], logits, -1000000000.0)
        attn = _softmax(logits, axis=-1)
        o = jnp.einsum('bhsw,bhswd->bhsd', attn, vg)
        return (lambda x, *d: x.transpose(*d))(o, 0, 2, 1, 3).reshape(B, S, D) @ wo

    def _B_ref(x, mem0, Wq, Wk, Wv, Wo, seg_len):
        B, S, Dm = x.shape
        H, Dh = (Wq.shape[1], Wq.shape[2])
        M = mem0.shape[1]
        scale = Dh ** (-0.5)
        n_seg = S // seg_len
        L = M + seg_len
        idx = jnp.arange(L)
        mask = (idx[:, None] < M) | (idx[:, None] >= idx[None, :])
        mem = mem0
        outs = []
        for s in range(n_seg):
            xs = x[:, s * seg_len:(s + 1) * seg_len, :].copy()
            h = jnp.concatenate([mem, xs], axis=1)
            q = jnp.einsum('btd,dhe->bhte', h, Wq)
            k = jnp.einsum('btd,dhe->bhte', h, Wk)
            v = jnp.einsum('btd,dhe->bhte', h, Wv)
            scores = jnp.einsum('bhqe,bhke->bhqk', q, k) * scale
            scores = jnp.where(mask[None, None], scores, -1000000000.0)
            p = _softmax(scores, axis=-1)
            o = jnp.einsum('bhqk,bhke->bhqe', p, v)
            o = jnp.einsum('bhte,hed->btd', o, Wo)
            mem = o[:, :M, :].copy()
            outs.append(o[:, M:, :])
        return jnp.concatenate(outs, axis=1)
    a = _A_ref(A_x, A_wqkv, A_wo)
    b = _B_ref(B_x, B_mem0, B_Wq, B_Wk, B_Wv, B_Wo, B_seg_len)
    return jnp.concatenate([a, b], axis=-1)
```

```python
import functools
import math

import jax
import jax.numpy as jnp
from jax import lax
from jax.experimental import pallas as pl
from jax.experimental.pallas import tpu as pltpu

F32, BF16, U32 = jnp.float32, jnp.bfloat16, jnp.uint32
NT = (((1,), (1,)), ((), ()))
MASKED = -1000000000.0

S, D = 2048, 640
LT = D // 128

AH, AD, AW, ADIL = 32, 20, 8, 2
HALO = 16
TB = 128
NB = S // TB
RC = 8

H, DH, M, SEG = 32, 192, 8, 32
L = M + SEG
HS = SEG // 2
NP = H // 2
PW = 2 * DH
NSEG = S // SEG
NCH = NP // 2
NO = H * DH // 128
NQ = 3 * NO
GQ = (NQ + 1) // LT
GO = (NO + 2) // LT
T = (0.0, -0.5, 0.5, -1.5, 1.5)
PAIRS = [(i, j) for j in range(LT) for i in range(j)]
NW = LT * LT + LT + len(PAIRS)

CFG = dict(lag_s=1, lag_n=2, lag_pv=3, o_chunks=((0, 3), (3, 6), (6, 10)), nper=(NSEG - 2) // 2)


def _blk(i, j):
    return i * LT + j


def _row(j):
    return LT * LT + j


def _sum(i, j):
    return LT * LT + LT + PAIRS.index((i, j))


def _ds(i, n):
    return pl.ds(i * n if isinstance(i, int) else pl.multiple_of(i * n, n), n)


def _dot(a, b):
    return jnp.dot(a, b, preferred_element_type=F32)


def _axpy(t, y, x):
    return x if t == 0 else x + y if t == 1 else x - y if t == -1 else x + t * y


def _add(a, b):
    return b if a is None else a + b


def _acc(a, sign, b):
    if a is None:
        return sign, b
    if a[0] == sign:
        return sign, a[1] + b
    return (1, a[1] - b) if a[0] > 0 else (1, b - a[1])


def _val(a):
    return a[1] if a[0] > 0 else -a[1]


def _cat(*parts):
    return jnp.concatenate(parts, axis=0)


def _share(tasks, k, n):
    return list(tasks[k * len(tasks) // n:(k + 1) * len(tasks) // n])


def _merge(a, b):
    return [t for k in range(len(a)) for t in [a[k]] + _share(b, k, len(a))]


def _run(tasks):
    for task in tasks:
        task()


def _block_diag(t0, t1, t2):
    lane = lax.broadcasted_iota(jnp.int32, (L, 128), 1)
    zero = jnp.zeros((L, 128), F32)
    top = jnp.concatenate([t0, jnp.where(lane < 64, t1, 0.0), zero], axis=1)
    bot = jnp.concatenate([zero, jnp.where(lane >= 64, t1, 0.0), t2], axis=1)
    return _cat(top, bot).astype(BF16)


def _kernel(ax_hbm, awqkv_hbm, awo_hbm, bx_hbm, mem_hbm, wq_hbm, wk_hbm, wv_hbm, wo_hbm,
            out_hbm,
            ax, awqkv, awo, tmp, wqkv_p, wo_p, q_s, kv_s, oa_s, outa,
            bx, mem, raw, wo_raw, w3, wo, h0, first, lhs, m_s, m_sum, part, tok, ox, oy, oa, om, opart, outb,
            sem_a, sem_x, sem_w, sem_b, sem_wo, sem_o):
    cp = pltpu.make_async_copy

    def rows_copy(src, dst, r0, n, sem):
        return cp(src.at[pl.ds(r0, n), :], dst.at[pl.ds(r0, n), :], sem)

    c_wqkv = [cp(awqkv_hbm.at[:, pl.ds(j * D, D)], awqkv.at[j], sem_a.at[j]) for j in range(3)]
    c_awo = cp(awo_hbm, awo, sem_a.at[3])
    c_mem = cp(mem_hbm, mem, sem_b.at[0])
    c_bx0 = rows_copy(bx_hbm, bx, 0, 4 * SEG, sem_b.at[1])
    c_bx1 = rows_copy(bx_hbm, bx, 4 * SEG, S - 4 * SEG, sem_b.at[2])
    c_outa = cp(outa, out_hbm.at[:, pl.ds(0, D)], sem_o.at[0])

    def c_ax(c):
        return [cp(ax_hbm.at[_ds(c, 2 * TB), :], ax.at[_ds(c, 2 * TB), :], sem_x.at[c])]

    def c_w(c):
        return [cp(w.at[_ds(c, 2 * PW), :], raw.at[_ds(j * NCH + c, 2 * PW), :], sem_w.at[c, j])
                for j, w in enumerate((wq_hbm, wk_hbm, wv_hbm))]

    def c_wo(g):
        if isinstance(g, int) and g == GO - 1:
            return [rows_copy(wo_hbm, wo_raw, g * D, H * DH - g * D, sem_wo.at[g])]
        return [cp(wo_hbm.at[_ds(g, D), :], wo_raw.at[_ds(g, D), :], sem_wo.at[g])]

    def c_outb(r0, n):
        return cp(outb.at[pl.ds(r0, n), :], out_hbm.at[pl.ds(r0, n), pl.ds(D, D)], sem_o.at[1])

    def start(copies):
        for c in copies:
            c.start()

    def wait(copies):
        for c in copies:
            c.wait()

    def permute_rows(dst, base):
        for d in range(AD):
            for t in range(LT):
                dst[pl.ds((base + d * AH) // 2, AH // 2), t * 128:(t + 1) * 128] = pltpu.bitcast(
                    tmp[t, pl.ds(d, AH, stride=AD), :].astype(BF16), U32)

    def prep_wqkv(j):
        for t in range(LT):
            tmp[t] = awqkv[j, t * 128:(t + 1) * 128, :].astype(F32).T
        permute_rows(wqkv_p, j * D)

    def prep_wo():
        for t in range(LT):
            tmp[t] = awo[:, t * 128:(t + 1) * 128].astype(F32)
        permute_rows(wo_p, 0)

    def a_proj(i, b, j, t):
        r0 = (j * D + t * 128) // 2
        w = pltpu.bitcast(wqkv_p[r0:r0 + 64, :], BF16)
        r = lax.dot_general(ax[_ds(i, TB), :], w, NT, preferred_element_type=F32)
        if j == 0:
            q_s[b, t] = r
            return
        c = (j - 1) * LT + t
        kv_s[b, c, HALO:HALO + TB, :] = r
        if isinstance(i, int) and i == 0:
            kv_s[b, c, 0:HALO, :] = jnp.broadcast_to(r[0:1, :], (HALO, 128))
        else:
            kv_s[b, c, 0:HALO, :] = kv_s[1 - b, c, TB:TB + HALO, :]

    def a_attention(b, first_block=False):
        state = {}

        def window(c, r0, w):
            lo = HALO + r0 - ADIL * w
            return kv_s[b, c, lo:lo + RC, :]

        def logits(r0):
            q = [q_s[b, t, r0:r0 + RC, :] for t in range(LT)]
            state[r0] = []
            for w in range(AW):
                a = q[0] * window(0, r0, w)
                for t in range(1, LT):
                    a = a + q[t] * window(t, r0, w)
                state[r0].append(a + pltpu.roll(a, 2 * AH, 1))

        def fold(r0):
            state[r0] = [a + pltpu.roll(a, AH, 1) for a in state[r0]]

        def mix(r0):
            scale = AD ** -0.5
            lg = []
            for w, a in enumerate(state.pop(r0)):
                if first_block and r0 < ADIL * w:
                    pos = lax.broadcasted_iota(jnp.int32, (RC, 128), 0) + r0
                    a = jnp.where(pos >= ADIL * w, a, MASKED / scale)
                lg.append(a)
            m = functools.reduce(jnp.maximum, lg)
            p = [jnp.exp2((a - m) * (scale * math.log2(math.e))) for a in lg]
            inv = 1.0 / functools.reduce(jnp.add, p)
            for t in range(LT):
                o = p[0] * window(LT + t, r0, 0)
                for w in range(1, AW):
                    o = o + p[w] * window(LT + t, r0, w)
                oa_s[b, r0:r0 + RC, t * 128:(t + 1) * 128] = o * inv

        n = TB // RC
        return [functools.partial(f, (k - lag) * RC) for k in range(n + 2)
                for lag, f in enumerate((logits, fold, mix)) if 0 <= k - lag < n]

    def a_out(i, b, t):
        lanes = slice(t * 128, (t + 1) * 128)
        outa[_ds(i, TB), lanes] = _dot(oa_s[b], pltpu.bitcast(wo_p[:, lanes], BF16)).astype(BF16)

    def a_stage(i, b, side=(), main=()):
        first_block = isinstance(i, int) and i == 1
        main = [functools.partial(a_proj, i, b, j, t) for j in range(3) for t in range(LT)] + list(main)
        if not first_block:
            main += [functools.partial(a_out, i - 2, b, t) for t in range(LT)]
        _run(_merge(main, _merge(a_attention(1 - b, first_block), side)))

    def derive(w, g, r, block):
        rows = slice(8 * r, 8 * r + 8)
        b = [[block(i, j) for j in range(LT)] for i in range(LT)]

        def put(s, v):
            w[g, s, rows, :] = pltpu.bitcast(v.astype(BF16), U32)

        for i, j in PAIRS:
            put(_sum(i, j), b[i][j] + b[j][i])
        for j in range(LT):
            others = [i for i in range(LT) if i != j]
            put(_blk(j, j), functools.reduce(jnp.subtract, [b[i][j] for i in others], b[j][j]))
            put(_row(j), functools.reduce(jnp.add, [b[j][i] for i in others], b[j][j]))

    def prep_qkv(g):
        cols = {}

        def transpose(j):
            n = g * LT + j - 1
            p = n * 57 >> 9
            e = (n - 9 * p) * 11 >> 5
            t = e * (NO - 3) + n - 6 * p
            cols[j] = raw[_ds(NQ if isinstance(n, int) and n < 0 else t, 128), :].T
            for i in range(LT):
                if i != j:
                    w3[g, _blk(i, j)] = pltpu.bitcast(cols[j][i * 128:(i + 1) * 128], U32)

        def rows(r):
            derive(w3, g, r, lambda i, j: cols[j][i * 128 + 16 * r:i * 128 + 16 * r + 16].astype(F32))

        return ([functools.partial(transpose, j) for j in range(LT)]
                + [functools.partial(rows, r) for r in range(8)])

    def prep_out(g):
        def rows(r):
            def block(i, j):
                v = wo_raw[_ds((g * LT + i) * 8 + r, 16), j * 128:(j + 1) * 128].astype(F32)
                if i != j:
                    wo[g, _blk(i, j), 8 * r:8 * r + 8, :] = pltpu.bitcast(v.astype(BF16), U32)
                return v
            derive(wo, g, r, block)

        return [functools.partial(rows, r) for r in range(8)]

    def first_proj(p, j):
        r = lax.dot_general(h0[...], raw[_ds(j * NP + p, PW), :], NT, preferred_element_type=F32)
        for t in range(3):
            first[9 * p + 3 * j + t] = r[0:L, t * 128:(t + 1) * 128]
            tok[9 * p + 3 * j + t] = r[L:, t * 128:(t + 1) * 128]

    start([c_wqkv[0]] + c_ax(0) + c_wqkv[1:])
    raw[NQ * 128:, :] = jnp.zeros((128, D), BF16)
    wo_raw[H * DH:, :] = jnp.zeros((GO * D - H * DH, D), BF16)
    c_wqkv[0].wait()
    prep_wqkv(0)
    start([c_mem, c_bx0] + c_w(0))
    wait(c_ax(0) + [c_wqkv[1]])
    _run([functools.partial(a_proj, 0, 0, 0, t) for t in range(LT)])
    prep_wqkv(1)
    start([c_awo] + c_ax(1))
    c_wqkv[2].wait()
    _run([functools.partial(a_proj, 0, 0, 1, t) for t in range(LT)])
    prep_wqkv(2)
    _run([functools.partial(a_proj, 0, 0, 2, t) for t in range(LT)])
    a_stage(1, 1)
    start(c_wo(0))
    wait([c_awo, c_mem, c_bx0])
    prep_wo()
    h0[0:M, :] = mem[...].astype(F32)
    h0[M:, :] = bx[0:2 * SEG, :].astype(F32)

    def a_step(it, carry):
        @pl.when(it + 1 < NB // 2)
        def _():
            start(c_ax(it + 1))
        start(c_w(it) + c_wo(it))
        wait(c_ax(it) + c_w(it - 1) + c_wo(it - 1))
        group = [jnp.maximum(lax.div(18 * it - 4, LT) - k, 1) for k in range(4)]
        side = [task for g in group for task in prep_qkv(g)] + prep_out(it - 1)
        for b in range(2):
            a_stage(2 * it + b, b, _share(side, b, 2),
                    [functools.partial(first_proj, 2 * it - 2 + b, j) for j in range(3)])
        return carry

    lax.fori_loop(1, NB // 2, a_step, 0)

    def mm(x, w, g, s):
        return _dot(x, pltpu.bitcast(w[g, s], BF16))

    def attention(qkv, put, rows=slice(0, L)):
        n = rows.stop - rows.start
        row = lax.broadcasted_iota(jnp.int32, (n, 2 * L), 0) + rows.start
        col = lax.broadcasted_iota(jnp.int32, (n, 2 * L), 1)
        head0 = col < L
        visible = (row < M) | (row >= jnp.where(head0, col, col - L))
        scale = DH ** -0.5
        st = {}

        def score(p):
            q = jnp.concatenate([qkv(9 * p + t) for t in range(3)], axis=1)
            k = _block_diag(*[qkv(9 * p + 3 + t) for t in range(3)])
            sc = lax.dot_general(q, k, NT, preferred_element_type=F32)
            sc = jnp.where(visible, sc, MASKED / scale)
            m0 = jnp.max(jnp.where(head0, sc, -jnp.inf), axis=1, keepdims=True)
            m1 = jnp.max(jnp.where(head0, -jnp.inf, sc), axis=1, keepdims=True)
            st[p] = sc - jnp.where(head0, m0, m1)

        def normalize(p):
            e = jnp.exp2(st[p] * (scale * math.log2(math.e)))
            l0 = jnp.sum(jnp.where(head0, e, 0.0), axis=1, keepdims=True)
            l1 = jnp.sum(jnp.where(head0, 0.0, e), axis=1, keepdims=True)
            st[p] = e / jnp.where(head0, l0, l1)

        def mix(p):
            r = _dot(st.pop(p), _block_diag(*[qkv(9 * p + 6 + t) for t in range(3)]))
            for t in range(3):
                put(3 * p + t, r[:, t * 128:(t + 1) * 128])

        return score, normalize, mix

    def put_x(n, r):
        om[n] = r[0:M]
        ox[n] = r[M:]

    def put_y(n, r):
        om[n] = r[0:M]
        oy[n] = r[M:]
        oa[n] = _axpy(T[n % LT], r[M:], ox[n])

    def prep_tokens(s):
        x = bx[_ds(s, SEG), :].astype(F32)
        y = bx[_ds(s + 1, SEG), :].astype(F32)
        y = [y[:, j * 128:(j + 1) * 128] for j in range(LT)]
        a = [_axpy(T[j], y[j], x[:, j * 128:(j + 1) * 128]) for j in range(LT)]
        for j in range(LT):
            lhs[_blk(j, j)] = a[j]
            lhs[_row(j)] = y[j]
        for i, j in PAIRS:
            both = a[i] + a[j]
            lhs[_sum(i, j)] = both
            lhs[_blk(i, j)] = _axpy(T[j] - T[i], y[i], both)
            lhs[_blk(j, i)] = _axpy(T[i] - T[j], y[j], both)

    def project(g, second):
        c = [None] * LT
        u = [None] * LT
        u2 = [None] * LT
        cy = [None] * LT
        half = slice(HS, SEG) if second else slice(0, HS)

        def pair(k):
            i, j = PAIRS[k]
            full = g > 0 or i > 0
            if g == 0:
                ms = m_s[i] + m_s[j]
                m_sum[k] = ms
            else:
                ms = m_sum[k]
            if not second:
                up = mm(_cat(lhs[_blk(i, j)], ms), w3, g, _blk(i, j))
                c[j] = _acc(c[j], 1, up[SEG:])
                u[j] = _add(u[j], up[:HS])
                u2[j] = _add(u2[j], up[HS:SEG])
                if full:
                    lo = mm(_cat(lhs[_blk(j, i), half], ms), w3, g, _blk(j, i))
                    c[i] = _acc(c[i], 1, lo[HS:])
                    u[i] = _add(u[i], lo[:HS])
                    part[g, LT + k] = _cat(up[:HS] + lo[:HS], up[HS:SEG])
            elif full:
                z = mm(_cat(lhs[_sum(i, j)], m_s[i]), w3, g, _sum(i, j))
                lo = mm(_cat(lhs[_blk(j, i), half], ms), w3, g, _blk(j, i))
                v = z[SEG:] - lo[HS:]
                c[j] = _acc(c[j], 1, v)
                c[i] = _acc(c[i], -1, v)
                w = z[:SEG] - part[g, LT + k]
                w = _cat(w[:HS], w[HS:] - lo[:HS])
                u[i] = _add(u[i], lo[:HS])
                f = 1.0 / (T[i] - T[j])
                if abs(f) != 1:
                    w, f = w * f, 1
                cy[j] = _acc(cy[j], f, w)
                cy[i] = _acc(cy[i], -f, w)
            else:
                z = mm(_cat(lhs[_row(i)], m_s[i]), w3, g, _blk(i, j))
                c[j] = _acc(c[j], 1, z[SEG:])
                cy[j] = _acc(cy[j], 1, z[:SEG])

        def diagonal(j):
            s = _row(j) if second else _blk(j, j)
            d = mm(_cat(lhs[s], m_s[j]), w3, g, s)
            c[j] = _acc(c[j], 1, d[SEG:])
            if second:
                cy[j] = _acc(cy[j], 1, d[:SEG])
            else:
                u[j] = _add(u[j], d[:HS])
                u2[j] = _add(u2[j], d[HS:SEG])

        for j in range(LT):
            if g > 0 or j > 0:
                diagonal(j)
            pair(2 * j)
            pair(2 * j + 1)
        out = {}
        for j in range(0 if g else 1, LT):
            n = g * LT + j - 1
            if second:
                uj = part[g, j]
                if u[j] is not None:
                    uj = _cat(uj[:HS], uj[HS:] + u[j])
                yj = _val(cy[j])
                out[n] = _cat(_val(c[j]), _axpy(-T[j], yj, uj))
                tok[n] = yj
            else:
                part[g, j] = _cat(u[j], u2[j])
                out[n] = _cat(_val(c[j]), tok[n])
        return out

    def step(s, second):
        res = {}
        c = [None] * LT
        half = slice(HS, SEG) if second else slice(0, HS)

        def out_chunk(g0, g1):
            head, last = g0 == 0, g1 == GO
            u = [None] * LT
            u2 = [None] * LT
            cy = [None] * LT

            def pair_mm(g, i, j, acc):
                ni, nj = g * LT + i, g * LT + j
                if ni >= NO:
                    return
                full = nj < NO
                a = oa[ni] + oa[nj] if full else oa[ni]
                ms = om[ni] + om[nj] if full else om[ni]
                if second:
                    acc[0] = _add(acc[0], mm(_cat(om[ni], a), wo, g, _sum(i, j)))
                else:
                    acc[0] = _add(acc[0], mm(_cat(ms, _axpy(T[j] - T[i], oy[ni], a)), wo, g, _blk(i, j)))
                if full:
                    acc[1] = _add(acc[1], mm(_cat(ms, _axpy(T[i] - T[j], oy[nj, half], a[half])),
                                             wo, g, _blk(j, i)))

            def pair_sum(i, j, up, lo):
                k = PAIRS.index((i, j))
                if second:
                    v = up[:M] - lo[:M]
                    c[j] = _acc(c[j], 1, v)
                    c[i] = _acc(c[i], -1, v)
                    w = _cat(up[M:M + HS], up[M + HS:] - lo[M:])
                    if head:
                        w = w - opart[LT + k]
                    u[i] = _add(u[i], lo[M:])
                    f = 1.0 / (T[i] - T[j])
                    if abs(f) != 1:
                        w, f = w * f, 1
                    cy[j] = _acc(cy[j], f, w)
                    cy[i] = _acc(cy[i], -f, w)
                else:
                    c[j] = _acc(c[j], 1, up[:M])
                    c[i] = _acc(c[i], 1, lo[:M])
                    u[j] = _add(u[j], up[M:M + HS])
                    u2[j] = _add(u2[j], up[M + HS:])
                    u[i] = _add(u[i], lo[M:])
                    r = _cat(up[M:M + HS] + lo[M:], up[M + HS:])
                    opart[LT + k] = r if head else opart[LT + k] + r

            def finish(i):
                if last:
                    m_s[i] = _val(c[i])
                if not second:
                    ui = _cat(u[i], u2[i])
                    opart[i] = ui if head else opart[i] + ui
                    return
                ui = opart[i]
                if u[i] is not None:
                    ui = _cat(ui[:HS], ui[HS:] + u[i])
                yi = _val(cy[i] if head else _acc(cy[i], 1, opart[15 + i]))
                if last:
                    lanes = slice(i * 128, (i + 1) * 128)
                    outb[_ds(s, SEG), lanes] = _axpy(-T[i], yi, ui).astype(BF16)
                    outb[_ds(s + 1, SEG), lanes] = yi.astype(BF16)
                else:
                    if u[i] is not None:
                        opart[i, HS:] = ui[HS:]
                    opart[15 + i] = yi

            order = sorted(PAIRS)
            for q in range(LT):
                d, accs = None, ([None, None], [None, None])
                for g in range(g0, g1):
                    for e in range(2):
                        pair_mm(g, *order[2 * q + e], accs[e])
                    n = g * LT + q
                    if n < NO:
                        d = _add(d, mm(_cat(om[n], (oy if second else oa)[n]), wo, g,
                                       _row(q) if second else _blk(q, q)))
                for e in range(2):
                    pair_sum(*order[2 * q + e], *accs[e])
                c[q] = _acc(c[q], 1, d[:M])
                if second:
                    cy[q] = _acc(cy[q], 1, d[M:])
                else:
                    u[q] = _add(u[q], d[M:M + HS])
                    u2[q] = _add(u2[q], d[M + HS:])
                for i in ((), (0,), (), (1,), (2, 3, 4))[q]:
                    finish(i)

        stages = attention(res.pop, put_x if second else put_y)
        due = {}
        for p in range(NP):
            for f, lag in zip(stages, (CFG["lag_s"], CFG["lag_n"], CFG["lag_pv"])):
                due.setdefault((9 * p + 6) // LT + lag, []).insert(0, functools.partial(f, p))
        chunks = list(CFG["o_chunks"])
        for t in range(GQ + CFG["lag_pv"]):
            if t < GQ:
                res.update(project(t, second))
            elif len(chunks) > 1:
                out_chunk(*chunks.pop(0))
            _run(due.pop(t, []))
        for chunk in chunks:
            out_chunk(*chunk)

    def out_mem(acc, g):
        n = min(LT, NO - g * LT)
        left = jnp.concatenate([om[g * LT + i] for i in range(n)], axis=1)
        return _add(acc, _dot(left, wo_raw[g * D:g * D + n * 128, :]))

    done = NB // 2 - 1
    start(c_wo(done + 1) + c_wo(done + 2))
    wait(c_w(NCH - 1) + c_wo(done))
    stages = attention(lambda n: first[n], put_x)
    lags = (0, 2, 4)
    acc = [None]

    def out_first(g):
        acc[0] = out_mem(acc[0], g)

    main = ([functools.partial(first_proj, p, j) for p in range(NP - 2, NP) for j in range(3)]
            + [functools.partial(a_out, NB - 2, 0, t) for t in range(LT)])
    heads = [functools.partial(f, t - lag) for t in range(NP + lags[-1])
             for f, lag in zip(stages, lags) if 0 <= t - lag < NP]
    side = [task for g in (0, *range(GQ - 4, GQ)) for task in prep_qkv(g)] + prep_out(done)
    _run(_merge(main, _merge(_merge(a_attention(1), heads), _share(side, 0, 2))))
    main = ([functools.partial(out_first, g) for g in range(done + 1)]
            + [functools.partial(a_out, NB - 1, 1, t) for t in range(LT)])
    _run(_merge(main, _share(side, 1, 2)))
    start([c_bx1, c_outa])
    wait(c_wo(done + 1) + c_wo(done + 2))
    for g in range(done + 1, GO):
        out_first(g)
        _run(prep_out(g))
    acc = acc[0]
    for j in range(LT):
        m_s[j] = acc[:, j * 128:(j + 1) * 128]

    def b_step(it, carry):
        @pl.when(it == 1)
        def _():
            c_bx1.wait()
        prep_tokens(2 * it + 2)
        step(2 * it, False)
        step(2 * it, True)
        c_outb(pl.multiple_of(it * 2 * SEG, 2 * SEG), 2 * SEG).start()
        return carry

    lax.fori_loop(0, CFG["nper"], b_step, 0)

    for k, (i, j) in enumerate(PAIRS):
        m_sum[k] = m_s[i] + m_s[j]
    res = {}

    def last_tile(n):
        g, j = divmod(n + 1, LT)
        c = None
        for i in range(LT):
            left = m_s[j] if i == j else m_sum[PAIRS.index((min(i, j), max(i, j)))]
            c = _add(c, mm(left, w3, g, _blk(i, j)))
        res[n] = _cat(c, tok[n])

    def put_last(n, r):
        oy[n] = r

    stages = attention(lambda n: res.pop(n) if n in res else tok[n], put_last, slice(M, L))
    lags = (1, 2, 3)
    acc = None
    for t in range(NP + lags[-1] + 1):
        p = t - lags[-1] - 1
        for e in range(3):
            if t < NP:
                last_tile(9 * t + 3 + 2 * e)
                last_tile(9 * t + 4 + 2 * e)
            if p >= 0:
                n = 3 * p + e
                acc = _add(acc, _dot(_cat(ox[n], oy[n]), wo_raw[n * 128:(n + 1) * 128, :]))
        _run([functools.partial(f, t - lag) for f, lag in zip(stages, lags) if 0 <= t - lag < NP])
    outb[S - 2 * SEG:, :] = acc.astype(BF16)
    c_outb(S - 2 * SEG, 2 * SEG).start()
    c_outa.wait()
    c_outb(0, (CFG["nper"] + 1) * 2 * SEG).wait()


def pallas_concat_heads__sliding_local_dilated__memory_aug_recurrent_mem_tr__prompt_kernel(
    A_x, A_wqkv, A_wo, B_x, B_mem0, B_Wq, B_Wk, B_Wv, B_Wo, B_seg_len,
):
    assert B_seg_len == SEG
    assert A_x.shape == B_x.shape == (1, S, D) and B_mem0.shape == (1, M, D)
    assert B_Wq.shape == B_Wk.shape == B_Wv.shape == (D, H, DH) and B_Wo.shape == (H, DH, D)
    vmem, dma = pltpu.VMEM, pltpu.SemaphoreType.DMA
    call = pl.pallas_call(
        _kernel,
        out_shape=jax.ShapeDtypeStruct((S, 2 * D), BF16),
        in_specs=[pl.BlockSpec(memory_space=pl.ANY)] * 9,
        out_specs=pl.BlockSpec(memory_space=pl.ANY),
        scratch_shapes=[
            vmem((S, D), BF16),
            vmem((3, D, D), BF16),
            vmem((D, D), BF16),
            vmem((LT, D, 128), F32),
            vmem((3 * D // 2, D), U32),
            vmem((D // 2, D), U32),
            vmem((2, LT, TB, 128), F32),
            vmem((2, 2 * LT, HALO + TB, 128), F32),
            vmem((2, TB, D), F32),
            vmem((S, D), BF16),
            vmem((S, D), BF16),
            vmem((M, D), BF16),
            vmem(((NQ + 1) * 128, D), BF16),
            vmem((GO * D, D), BF16),
            vmem((GQ, NW, 64, 128), U32),
            vmem((GO, NW, 64, 128), U32),
            vmem((L + SEG, D), F32),
            vmem((NQ, L, 128), F32),
            vmem((NW, SEG, 128), F32),
            vmem((LT, M, 128), F32),
            vmem((len(PAIRS), M, 128), F32),
            vmem((GQ, 15, SEG, 128), F32),
            vmem((NQ, SEG, 128), F32),
            vmem((NO, SEG, 128), F32),
            vmem((NO, SEG, 128), F32),
            vmem((NO, SEG, 128), F32),
            vmem((NO, M, 128), F32),
            vmem((20, SEG, 128), F32),
            vmem((S, D), BF16),
            dma((4,)), dma((NB // 2,)), dma((NCH, 3)), dma((3,)), dma((GO,)), dma((2,)),
        ],
        compiler_params=pltpu.CompilerParams(vmem_limit_bytes=124 * 1024 * 1024),
        name="sliding_and_memory_attention",
    )

    def by_feature(w):
        return w.transpose(1, 2, 0).reshape(H * DH, D)

    out = call(A_x.reshape(S, D), A_wqkv, A_wo, B_x.reshape(S, D), B_mem0.reshape(M, D),
               by_feature(B_Wq), by_feature(B_Wk), by_feature(B_Wv), B_Wo.reshape(H * DH, D))
    return out.reshape(1, S, 2 * D)
```

```python
import functools
import math

import jax
import jax.numpy as jnp
from jax import lax
from jax.experimental import pallas as pl
from jax.experimental.pallas import tpu as pltpu

F32, BF16, U32 = jnp.float32, jnp.bfloat16, jnp.uint32
NT = (((1,), (1,)), ((), ()))
MASKED = -1000000000.0

S, D = 2048, 640
LT = D // 128

AH, AD, AW, ADIL = 32, 20, 8, 2
HALO = 16
TB = 128
NB = S // TB
RC = 8

H, DH, M, SEG = 32, 192, 8, 32
L = M + SEG
HS = SEG // 2
NP = H // 2
PW = 2 * DH
NSEG = S // SEG
NCH = NP // 2
NO = H * DH // 128
NQ = 3 * NO
GQ = (NQ + 1) // LT
GO = (NO + 2) // LT
T = (0.0, -0.5, 0.5, -1.5, 1.5)
PAIRS = [(i, j) for j in range(LT) for i in range(j)]
GA = GQ + GO
NW = LT * LT + LT + len(PAIRS)

RING = 8
CHUNKS = ((0, 3), (3, 6), (6, GO))
CFG = dict(nper=(NSEG - 2) // 2, flags=None, back=20, aback=16, holdall=0, split=10, main=1,
           ds=35, dn=60, dp=85, tp=740, dt=25, hp=6, opos=0, rcp=1, ls=(1, 2, 3, 4))


def _blk(i, j):
    return i * LT + j


def _row(j):
    return LT * LT + j


def _sum(i, j):
    return LT * LT + LT + PAIRS.index((i, j))


def _ds(i, n):
    return pl.ds(i * n if isinstance(i, int) else pl.multiple_of(i * n, n), n)


def _dot(a, b):
    return jnp.dot(a, b, preferred_element_type=F32)


def _axpy(t, y, x):
    return x if t == 0 else x + y if t == 1 else x - y if t == -1 else x + t * y


def _add(a, b):
    return b if a is None else a + b


def _acc(a, sign, b):
    if a is None:
        return sign, b
    if a[0] == sign:
        return sign, a[1] + b
    return (1, a[1] - b) if a[0] > 0 else (1, b - a[1])


def _val(a):
    return a[1] if a[0] > 0 else -a[1]


def _add_rows(a, b):
    return b if a is None else _cat(a[:M] + b[:M], a[M:] + b[M:])


def _cat(*parts):
    return jnp.concatenate(parts, axis=0)


def _share(tasks, k, n):
    return list(tasks[k * len(tasks) // n:(k + 1) * len(tasks) // n])


def _merge(a, b):
    return [t for k in range(len(a)) for t in [a[k]] + _share(b, k, len(a))]


def _run(tasks):
    for task in tasks:
        task()


def _block_diag(t0, t1, t2):
    lane = lax.broadcasted_iota(jnp.int32, (L, 128), 1)
    zero = jnp.zeros((L, 128), F32)
    top = jnp.concatenate([t0, jnp.where(lane < 64, t1, 0.0), zero], axis=1)
    bot = jnp.concatenate([zero, jnp.where(lane >= 64, t1, 0.0), t2], axis=1)
    return _cat(top, bot).astype(BF16)


def _kernel(ax_hbm, awqkv_hbm, awo_hbm, bx_hbm, mem_hbm, wq_hbm, wk_hbm, wv_hbm, wo_hbm,
            out_hbm,
            ax, awqkv, awo, tmp, wa, xb, q_s, kv_s, oa_s, outa,
            bx, mem, raw, wo_raw, plain, sums, h0, first, lhs, m_s, m_sum, part, tok, ring, ox, mixed, opart, outb,
            sem_a, sem_x, sem_w, sem_b, sem_wo, sem_o):
    cp = pltpu.make_async_copy

    def rows_copy(src, dst, r0, n, sem):
        return cp(src.at[pl.ds(r0, n), :], dst.at[pl.ds(r0, n), :], sem)

    c_wqkv = [cp(awqkv_hbm.at[:, pl.ds(j * D, D)], awqkv.at[j], sem_a.at[j]) for j in range(3)]
    c_awo = cp(awo_hbm, awo, sem_a.at[3])
    c_mem = cp(mem_hbm, mem.at[0:M], sem_b.at[0])
    c_bx0 = rows_copy(bx_hbm, bx, 0, 6 * SEG, sem_b.at[1])
    c_bx1 = rows_copy(bx_hbm, bx, 6 * SEG, S - 6 * SEG, sem_b.at[2])
    c_outa = cp(outa, out_hbm.at[:, pl.ds(0, D)], sem_o.at[0])

    def c_ax(c):
        return [cp(ax_hbm.at[_ds(c, 2 * TB), :], ax.at[_ds(c, 2 * TB), :], sem_x.at[c])]

    def c_w(c):
        return [cp(w.at[_ds(c, 2 * PW), :], raw.at[_ds(j * NCH + c, 2 * PW), :], sem_w.at[c, j])
                for j, w in enumerate((wq_hbm, wk_hbm, wv_hbm))]

    def c_wo(g):
        if isinstance(g, int) and g == GO - 1:
            return [rows_copy(wo_hbm, wo_raw, g * D, H * DH - g * D, sem_wo.at[g])]
        return [cp(wo_hbm.at[_ds(g, D), :], wo_raw.at[_ds(g, D), :], sem_wo.at[g])]

    def c_outb(r0, n):
        return cp(outb.at[pl.ds(r0, n), :], out_hbm.at[pl.ds(r0, n), pl.ds(D, D)], sem_o.at[1])

    def start(copies):
        for c in copies:
            c.start()

    def wait(copies):
        for c in copies:
            c.wait()
        recent.clear()

    def weight(g, s):
        if s < 25 and s % 6:
            return pltpu.bitcast(plain[_ds(g * LT + s % LT, 64), _ds(s // LT, 128)], BF16)
        s = s // 6 if s < 25 else s - 20
        return pltpu.bitcast(sums[_ds(4 * g + s // LT, 64), _ds(s % LT, 128)], BF16)

    def regroup(t, n):
        return _cat(*[tmp[t, pl.ds(d, AH, stride=AD), 0:n] for d in range(AD)])

    def prep_wqkv(j):
        for t, n in enumerate((128, 128, 64)):
            tmp[t, :, 0:n] = pltpu.bitcast(awqkv[j, 256 * t:256 * t + 2 * n, :], F32).T
        for t, n in enumerate((128, 128, 64)):
            wa[pl.ds(j * D // 2 + 128 * t, n), :] = pltpu.bitcast(regroup(t, n).T, U32)

    def prep_wo():
        def task(t):
            tmp[t] = awo[:, _ds(t, 128)].astype(F32)
            wa[_ds(3, D // 2), _ds(t, 128)] = pltpu.bitcast(regroup(t, 128).astype(BF16), U32)

        return [functools.partial(task, t) for t in range(LT)]

    recent = []

    def hold(x, zero, back):
        if len(recent) < back:
            return x
        late = recent[-back] if x.dtype == F32 else pltpu.bitcast(recent[-back], U32)
        return jnp.where(lax.broadcasted_iota(jnp.int32, x.shape, 0) >= zero, x, late)

    def by_tile(j, left, put):
        acc = [None]

        def task(t, k):
            r = _dot(left(k), pltpu.bitcast(wa[_ds(j * LT + k, 64), _ds(t, 128)], BF16))
            e = len(recent) % 16
            recent.extend(r[8 * (e + i) % TB:8 * (e + i) % TB + 8] for i in range(4))
            acc[0] = _add_rows(acc[0] if k else None, r)
            if k == LT - 1:
                put(t, acc[0])

        return [functools.partial(task, t, k) for t in range(LT) for k in range(LT)]

    def a_load(i, b):
        xb[_ds(b, TB // 2), :] = pltpu.bitcast(ax[_ds(i, TB), :], U32)

    def a_proj(i, b, j):
        def put(t, r):
            if j == 0:
                q_s[b, t] = r
                return
            c = (j - 1) * LT + t
            kv_s[b, c, HALO:, :] = r
            if isinstance(i, int) and i == 0:
                kv_s[b, c, 0:HALO, :] = jnp.broadcast_to(r[0:1, :], (HALO, 128))
            else:
                kv_s[b, c, 0:HALO, :] = kv_s[1 - b, c, TB:, :]

        return by_tile(j, lambda k: pltpu.bitcast(xb[_ds(b, TB // 2), _ds(k, 128)], BF16), put)

    def a_attention(b, zero, first_block=False):
        state = {}

        def window(c, r0, w):
            lo = HALO + r0 - ADIL * w
            return kv_s[b, c, lo:lo + RC, :]

        def logits(r0):
            q = [hold(q_s[b, t, r0:r0 + RC, :], zero, CFG["aback"]) for t in range(LT)]
            state[r0] = []
            for w in range(AW):
                a = q[0] * window(0, r0, w)
                for t in range(1, LT):
                    a = a + q[t] * window(t, r0, w)
                state[r0].append(a + pltpu.roll(a, 2 * AH, 1))

        def fold(r0):
            state[r0] = [a + pltpu.roll(a, AH, 1) for a in state[r0]]

        def mix(r0):
            scale = AD ** -0.5
            lg = []
            for w, a in enumerate(state.pop(r0)):
                if first_block and r0 < ADIL * w:
                    pos = lax.broadcasted_iota(jnp.int32, (RC, 128), 0) + r0
                    a = jnp.where(pos >= ADIL * w, a, MASKED / scale)
                lg.append(a)
            m = hold(functools.reduce(jnp.maximum, lg), zero, CFG["aback"])
            p = [jnp.exp2((a - m) * (scale * math.log2(math.e))) for a in lg]
            inv = 1.0 / functools.reduce(jnp.add, p)
            for t in range(LT):
                o = p[0] * window(LT + t, r0, 0)
                for w in range(1, AW):
                    o = o + p[w] * window(LT + t, r0, w)
                oa_s[b, r0:r0 + RC, t * 128:(t + 1) * 128] = o * inv

        n = TB // RC
        return [functools.partial(f, (k - lag) * RC) for k in range(n + 2)
                for lag, f in enumerate((logits, fold, mix)) if 0 <= k - lag < n]

    def a_out(i, b):
        def put(t, r):
            outa[_ds(i, TB), _ds(t, 128)] = r.astype(BF16)

        return by_tile(3, lambda k: oa_s[b, :, _ds(k, 128)], put)

    def transposes(c):
        r0 = (18 * c + 1) * 64
        dst = plain.at[pl.ds(r0 if isinstance(c, int) else pl.multiple_of(r0, 64), 18 * 64)]

        def task(j, t):
            v = pltpu.bitcast(raw[_ds(j * NO + 6 * c + t, 128), :].T, U32)
            for i in range(LT):
                dst[_ds(9 * (t // 3) + 3 * j + t % 3, 64), _ds(i, 128)] = v[i * 64:(i + 1) * 64]

        return [functools.partial(task, j, 3 * p + t) for p in range(2) for j in range(3) for t in range(3)]

    def derive(g, zero, block=None):
        src, dst = plain.at[_ds(g, D // 2)], sums.at[_ds(g, 4 * 64)]
        row, col = [None] * LT, [None] * LT

        def task(r, e):
            def put(s, v):
                dst[_ds(s // LT * 8 + r, 8), _ds(s % LT, 128)] = pltpu.bitcast(v.astype(BF16), U32)

            def load(i, j):
                at = _ds(j * 8 + r, 8), _ds(i, 128)
                v = src[at] if block is None else block(r, i, j)
                if i < j or CFG["holdall"]:
                    v = hold(v, zero, CFG["back"])
                if block is not None:
                    src[at] = v
                return pltpu.bitcast(v, BF16).astype(F32)

            for k in _share(range(10), e, CFG["split"]):
                i, j = PAIRS[k]
                for d in ((0, 1) if k == 0 else (j,) if i == 0 else ()):
                    row[d] = col[d] = load(d, d)
                up, lo = load(i, j), load(j, i)
                put(2 * LT + k, up + lo)
                row[i], col[j] = row[i] + up, col[j] - up
                row[j], col[i] = row[j] + lo, col[i] - lo
                for d in ((i, j) if k == 9 else (i,) if j == LT - 1 else ()):
                    put(d, col[d])
                    put(LT + d, row[d])

        return [functools.partial(task, r, e) for r in range(8) for e in range(CFG["split"])]

    def derive_out(g, zero):
        n = min(LT, NO - g * LT) if isinstance(g, int) else LT
        src = wo_raw.at[pl.ds(g * D if isinstance(g, int) else pl.multiple_of(g * D, D), n * 128)]

        def block(r, i, j):
            if i >= n:
                return jnp.zeros((8, 128), U32)
            return pltpu.bitcast(src[_ds(i * 8 + r, 16), _ds(j, 128)], U32)

        return derive(GQ + g, zero, block)

    def first_group(g):
        src = plain.at[_ds(g, D // 2)]
        acc = [None] * LT

        def task(i, j):
            r = _dot(h0[0:L + SEG, _ds(i, 128)], pltpu.bitcast(src[_ds(j, 64), _ds(i, 128)], BF16))
            e = len(recent) % 8
            recent.extend([r[8 * e:8 * e + 8], r[8 * e + 8:8 * e + 16]])
            acc[j] = _add_rows(acc[j], r)
            if i == LT - 1:
                first[g * LT + j] = acc[j][0:L]
                tok[g * LT + j] = acc[j][L:]

        return [functools.partial(task, i, j) for j in range(LT) for i in range(LT)]

    def each(f, groups, *args):
        return [task for g in groups for task in f(g, *args)]

    start([c_wqkv[0]] + c_ax(0))
    plain[0:64, :] = jnp.zeros((64, D), U32)
    wait(c_ax(0))
    a_load(0, 0)
    a_load(1, 1)
    c_wqkv[1].start()
    c_wqkv[0].wait()
    prep_wqkv(0)
    _run(a_proj(0, 0, 0))
    c_wqkv[2].start()
    c_wqkv[1].wait()
    _run(a_proj(1, 1, 0))
    prep_wqkv(1)
    _run(a_proj(0, 0, 1))
    start([c_awo] + c_ax(1))
    c_wqkv[2].wait()
    _run(a_proj(1, 1, 1))
    prep_wqkv(2)
    _run(a_proj(0, 0, 2))
    start(c_w(0))
    wait([c_awo])
    _run(_merge(a_proj(1, 1, 2), _merge(a_attention(0, 0, first_block=True), prep_wo())))

    def a_step(it, carry):
        c = jnp.where(it == 1, NCH - 1, it - 2)
        g = jnp.maximum(2 * it - 4, 0)
        zero = it >> 16

        @pl.when(it + 1 < NB // 2)
        def _():
            start(c_ax(it + 1))

        @pl.when(it > 1)
        def _():
            start(c_w(it - 1))
            wait(c_w(c))
        wait(c_ax(it))
        for b in range(2):
            a_load(2 * it + b, b)
        for b, side in enumerate((transposes(c), each(derive, (g, g + 1), zero))):
            i = 2 * it + b
            main = a_proj(i, b, 0) + a_proj(i, b, 1) + a_proj(i, b, 2) + a_out(i - 2, b)
            _run(_merge(main, _merge(a_attention(1 - b, zero), side)))
        return zero

    start([c_mem, c_bx0])
    zero = lax.fori_loop(1, NB // 2, a_step, 0)
    start(each(c_wo, range(2)) + c_w(NCH - 1))
    wait(c_w(NCH - 2) + [c_mem, c_bx0])
    h0[0:M, :] = mem[0:M, :].astype(F32)
    h0[M:L + SEG, :] = bx[0:2 * SEG, :].astype(F32)
    _run(_merge(a_out(NB - 2, 0) + each(first_group, range(5)) + a_out(NB - 1, 1),
                _merge(a_attention(1, zero) + each(derive, range(12, 15), zero), transposes(NCH - 2))))

    def first_step(it, carry):
        zero = it >> 16
        start(c_wo(it + 2))
        wait(c_wo(it))
        side = each(derive, [jnp.minimum(15 + 3 * it + e, 24) for e in range(3)], zero)
        _run(_merge(each(first_group, [5 * it + 5 + e for e in range(5)]), side + derive_out(it, zero)))
        return zero

    zero = lax.fori_loop(0, 4, first_step, 0)

    due = []

    def mm(x, g, s):
        r = _dot(x, weight(g, s))
        recent.append(r[0:M])
        while due and due[0][0] <= len(recent):
            due.pop(0)[1]()
        return r

    def attention(qkv, put, rows=slice(0, L)):
        n = rows.stop - rows.start
        row = lax.broadcasted_iota(jnp.int32, (n, 2 * L), 0) + rows.start
        col = lax.broadcasted_iota(jnp.int32, (n, 2 * L), 1)
        head0 = col < L
        visible = (row < M) | (row >= jnp.where(head0, col, col - L))
        scale = DH ** -0.5
        st = {}

        def score(p):
            q = jnp.concatenate([qkv(9 * p + t) for t in range(3)], axis=1)
            k = _block_diag(*[qkv(9 * p + 3 + t) for t in range(3)])
            sc = lax.dot_general(q, k, NT, preferred_element_type=F32)
            sc = jnp.where(visible, sc, MASKED / scale)
            m0 = jnp.max(jnp.where(head0, sc, -jnp.inf), axis=1, keepdims=True)
            m1 = jnp.max(jnp.where(head0, -jnp.inf, sc), axis=1, keepdims=True)
            st[p] = sc - jnp.where(head0, m0, m1)

        def normalize(p):
            e = jnp.exp2(st[p] * (scale * math.log2(math.e)))
            l0 = jnp.sum(jnp.where(head0, e, 0.0), axis=1, keepdims=True)
            l1 = jnp.sum(jnp.where(head0, 0.0, e), axis=1, keepdims=True)
            l = jnp.where(head0, l0, l1)
            if CFG["rcp"]:
                r = pl.reciprocal(l, approx=True)
                st[p] = e * (r * (2.0 - l * r))
            else:
                st[p] = e / l

        def mix(p):
            r = _dot(st.pop(p), _block_diag(*[qkv(9 * p + 6 + t) for t in range(3)]))
            for t in range(3):
                put(3 * p + t, r[:, t * 128:(t + 1) * 128])

        return score, normalize, mix

    def mixed_at(refs, n):
        return [(ref, n - g0 * LT) for ref, (g0, g1) in zip(refs, CHUNKS) if g0 <= n // LT < g1][0]

    def put_x(n, r):
        ref, k = mixed_at(mixed, n)
        ref[k, 0:M] = r[0:M]
        ox[n] = r[M:]

    def put_y(n, r):
        ref, k = mixed_at(mixed, n)
        ref[k] = _cat(r[0:M], _axpy(T[n % LT], r[M:], ox[n]), r[M:])

    def prep_tokens(s, zero):
        def task(e):
            rows = _ds(e, M)
            x, y = [bx[_ds((s + k) * (SEG // M) + e, M), :].astype(F32) for k in range(2)]
            y = [hold(y[:, j * 128:(j + 1) * 128], zero, CFG["hp"] * (LT - j)) for j in range(LT)]
            a = [_axpy(T[j], y[j], x[:, j * 128:(j + 1) * 128]) for j in range(LT)]
            for j in range(LT):
                lhs[_blk(j, j), rows] = a[j]
                lhs[_row(j), rows] = y[j]
            for i, j in PAIRS:
                both = a[i] + a[j]
                lhs[_sum(i, j), rows] = both
                lhs[_blk(i, j), rows] = _axpy(T[j] - T[i], y[i], both)
                lhs[_blk(j, i), rows] = _axpy(T[i] - T[j], y[j], both)

        return [functools.partial(task, e) for e in range(SEG // M)]

    def step(s, second, zero):
        def reread(ref):
            return ref.at[pl.ds(4 * zero, ref.shape[0])]

        part_r, opart_r, m_sum_r = reread(part), reread(opart), reread(m_sum)
        ring_r, mixed_r = [reread(r) for r in ring], [reread(r) for r in mixed]
        half = slice(HS, SEG) if second else slice(0, HS)

        class Sums:
            def __init__(self, c):
                self.c, self.u, self.u2, self.cy = c, [None] * LT, [None] * LT, [None] * LT

            def column(self, j, m, t):
                self.c[j] = _acc(self.c[j], 1, m)
                if second:
                    self.cy[j] = _acc(self.cy[j], 1, t)
                else:
                    self.u[j] = _add(self.u[j], t[:HS])
                    self.u2[j] = _add(self.u2[j], t[HS:])

            def pair(self, i, j, m, t, lo_m, lo_t, before):
                self.u[i] = _add(self.u[i], lo_t)
                if not second:
                    self.column(j, m, t)
                    self.c[i] = _acc(self.c[i], 1, lo_m)
                    return _cat(t[:HS] + lo_t, t[HS:])
                v = m - lo_m
                self.c[j] = _acc(self.c[j], 1, v)
                self.c[i] = _acc(self.c[i], -1, v)
                if before is not None:
                    t = t - before
                w, f = _cat(t[:HS], t[HS:] - lo_t), 1.0 / (T[i] - T[j])
                if abs(f) != 1:
                    w, f = w * f, 1
                self.cy[j] = _acc(self.cy[j], f, w)
                self.cy[i] = _acc(self.cy[i], -f, w)

        def project(g):
            z = Sums([None] * LT)

            def single(j, left, m, s):
                r = mm(_cat(lhs[left], m), g, s)
                z.column(j, r[SEG:], r[:SEG])

            def pair(i, j):
                k = PAIRS.index((i, j))
                if g == 0:
                    ms = m_s[i] + m_s[j]
                    m_sum[k] = ms
                else:
                    ms = m_sum_r[k]
                if g == 0 and i == 0:
                    single(j, _row(i) if second else _blk(i, j), m_s[i] if second else ms, _blk(i, j))
                    return
                s = _sum(i, j) if second else _blk(i, j)
                up = mm(_cat(lhs[s], m_s[i] if second else ms), g, s)
                lo = mm(_cat(lhs[_blk(j, i), half], ms), g, _blk(j, i))
                r = z.pair(i, j, up[SEG:], up[:SEG], lo[HS:], lo[:HS], part_r[g, LT + k] if second else None)
                if not second:
                    part[g, LT + k] = r

            order = sorted(PAIRS) if g else PAIRS
            for j in range(LT):
                if g > 0 or j > 0:
                    s = _row(j) if second else _blk(j, j)
                    single(j, s, m_s[j], s)
                pair(*order[2 * j])
                pair(*order[2 * j + 1])
            for j in range(0 if g else 1, LT):
                n = g * LT + j - 1
                dst = ring[n // 3 % RING]
                dst[n % 3, 0:M] = _val(z.c[j])
                if not second:
                    part[g, j] = _cat(z.u[j], z.u2[j])
                    continue
                u, y = part_r[g, j], _val(z.cy[j])
                if z.u[j] is not None:
                    u = _cat(u[:HS], u[HS:] + z.u[j])
                dst[n % 3, M:] = _axpy(-T[j], y, u)
                tok[n + 1] = y

        def projected(n):
            src = ring_r[n // 3 % RING]
            return src[n % 3] if second else _cat(src[n % 3, 0:M], tok[n + 1])

        c = [None] * LT

        def out_chunk(ref, g0, g1):
            head, last = g0 == 0, g1 == GO
            z = Sums(c)

            def products(g, i, j, acc):
                ki, kj = (g - g0) * LT + i, (g - g0) * LT + j
                if g * LT + i >= NO:
                    return
                full = g * LT + j < NO
                both = ref[ki, 0:L] + ref[kj, 0:L] if full else ref[ki, 0:L]
                ms, a = both[:M], both[M:]
                if second:
                    acc[0] = _add_rows(acc[0], mm(_cat(ref[ki, 0:M], a), GQ + g, _sum(i, j)))
                else:
                    left = _axpy(T[j] - T[i], ref[ki, L:], a)
                    acc[0] = _add_rows(acc[0], mm(_cat(ms, left), GQ + g, _blk(i, j)))
                if full:
                    left = _axpy(T[i] - T[j], ref[kj, L:][half], a[half])
                    acc[1] = _add_rows(acc[1], mm(_cat(ms, left), GQ + g, _blk(j, i)))

            def finish(i):
                if last:
                    m_s[i] = _val(c[i])
                if not second:
                    u = _cat(z.u[i], z.u2[i])
                    opart[i] = u if head else opart[i] + u
                    return
                u = opart[i]
                if z.u[i] is not None:
                    u = _cat(u[:HS], u[HS:] + z.u[i])
                y = _val(z.cy[i] if head else _acc(z.cy[i], 1, opart[15 + i]))
                if last:
                    outb[_ds(s, SEG), _ds(i, 128)] = _axpy(-T[i], y, u).astype(BF16)
                    outb[_ds(s + 1, SEG), _ds(i, 128)] = y.astype(BF16)
                else:
                    if z.u[i] is not None:
                        opart[i, HS:] = u[HS:]
                    opart[15 + i] = y

            order = sorted(PAIRS)
            for q in range(LT):
                d, accs = None, ([None, None], [None, None])
                for g in range(g0, g1):
                    k = (g - g0) * LT + q
                    for e in range(CFG["opos"]):
                        products(g, *order[2 * q + e], accs[e])
                    if g * LT + q < NO:
                        left = _cat(ref[k, 0:M], ref[k, L:]) if second else ref[k, 0:L]
                        d = _add_rows(d, mm(left, GQ + g, _row(q) if second else _blk(q, q)))
                    for e in range(CFG["opos"], 2):
                        products(g, *order[2 * q + e], accs[e])
                for (i, j), (up, lo) in zip(order[2 * q:], accs):
                    k = LT + PAIRS.index((i, j))
                    r = z.pair(i, j, up[:M], up[M:], lo[:M], lo[M:], opart_r[k] if second and head else None)
                    if not second:
                        opart[k] = r if head else opart[k] + r
                z.column(q, d[:M], d[M:])
                for i in ((), (0,), (), (1,), (2, 3, 4))[q]:
                    finish(i)

        recent.clear()
        stages = attention(projected, put_x if second else put_y)
        for p in range(NP):
            ready = LT * LT * ((9 * p + 6) // LT + 1) - LT
            due.extend((ready + CFG[lag], functools.partial(f, p)) for f, lag in
                       zip(stages, ("ds", "dn", "dp")))
        if second:
            due.extend((CFG["tp"] - LT + k * CFG["dt"], task)
                       for k, task in enumerate(prep_tokens(jnp.minimum(s + 4, NSEG - 2), zero)))
        due.sort(key=lambda e: e[0])
        for g in range(GQ):
            project(g)
        for ref, chunk in zip(mixed_r, CHUNKS):
            out_chunk(ref, *chunk)

    def put_first(n, r):
        recent.extend([r[k:k + 8] for k in range(0, L, 16)])
        put_x(n, r)

    stages = attention(lambda n: first[n + 1], put_first)
    lags = (0, 2, 4)
    acc = [None] * LT

    def heads(p0, p1):
        return [functools.partial(f, t - lag) for t in range(p0, p1 + lags[-1])
                for f, lag in zip(stages, lags) if p0 <= t - lag < p1]

    def out_first(*groups):
        def task(g, i, j):
            ref, k = mixed_at(mixed, g * LT + i)
            r = _dot(ref[k, 0:M], wo_raw[_ds(g * LT + i, 128), _ds(j, 128)] if g > 5 else
                     pltpu.bitcast(plain[_ds((GQ + g) * LT + j, 64), _ds(i, 128)], BF16))
            recent.append(r)
            acc[j] = _add(acc[j], r)
        return [functools.partial(task, g, i, j) for g in groups for i in range(min(LT, NO - g * LT))
                for j in range(LT)]

    start(each(c_wo, range(6, 9)))
    wait(c_w(NCH - 1) + c_wo(4) + c_wo(5))
    _run(_merge(_merge(heads(0, 13) + out_first(0, 1, 2, 3), each(derive_out, (4, 5), zero)), transposes(NCH - 1)))
    _run(_merge(each(first_group, range(25, GQ)), each(derive, range(25, GQ), zero)))
    start(c_wo(9))
    wait(each(c_wo, range(6, 9)))
    _run(_merge(_merge(heads(13, NP), out_first(4, 5, 6)) + out_first(7), each(derive_out, range(6, 9), zero)))
    _run(prep_tokens(2, zero))
    wait(c_wo(9))
    start([c_bx1, c_outa])
    _run(_merge(out_first(8), derive_out(9, zero)) + out_first(9))
    for j in range(LT):
        m_s[j] = acc[j]

    def b_step(it, carry):
        @pl.when(it == 1)
        def _():
            c_bx1.wait()
        step(2 * it, False, it >> 16)
        step(2 * it, True, it >> 16)
        c_outb(pl.multiple_of(it * 2 * SEG, 2 * SEG), 2 * SEG).start()
        return carry

    if not CFG['main']:
        c_outa.wait()
        c_bx1.wait()
        return
    lax.fori_loop(0, CFG["nper"], b_step, 0)

    for k, (i, j) in enumerate(PAIRS):
        m_sum[k] = m_s[i] + m_s[j]
    res = {}
    acc = [None] * LT

    def last_tile(n, i):
        g, j = divmod(n + 1, LT)
        left = m_s[j] if i == j else m_sum[PAIRS.index((min(i, j), max(i, j)))]
        res[n] = _acc(res.get(n), 1 - 2 * (i % 2), _dot(-left if i % 2 else left, weight(g, _blk(i, j))))

    def put_last(n, r):
        res[NQ + n] = r

    stages = attention(lambda n: _cat(_val(res.pop(n)), tok[n + 1]) if n in res else tok[n + 1], put_last, slice(M, L))
    lags = CFG["ls"]
    for t in range(NP + lags[-1]):
        p = t - lags[-1]
        for e in range(3):
            for i in range(LT):
                if t < NP:
                    last_tile(9 * t + 3 + 2 * e, i)
                    last_tile(9 * t + 4 + 2 * e, i)
                if p >= 0:
                    n = 3 * p + i * 3 // LT if 0 else 3 * p + e
                    w = pltpu.bitcast(plain[_ds((GQ + n // LT) * LT + i, 64), _ds(n % LT, 128)], BF16)
                    acc[i] = _add_rows(acc[i], _dot(_cat(ox[n], res[NQ + n]), w))
        _run([functools.partial(f, t - lag) for f, lag in zip(stages, lags) if 0 <= t - lag < NP][::-1])
    acc = jnp.concatenate(acc, axis=1)
    outb[S - 2 * SEG:, :] = acc.astype(BF16)
    c_outb(S - 2 * SEG, 2 * SEG).start()
    c_outa.wait()
    c_outb(0, (CFG["nper"] + 1) * 2 * SEG).wait()


def pallas_concat_heads__sliding_local_dilated__memory_aug_recurrent_mem_tr__prompt_kernel(
    A_x, A_wqkv, A_wo, B_x, B_mem0, B_Wq, B_Wk, B_Wv, B_Wo, B_seg_len,
):
    assert B_seg_len == SEG
    assert A_x.shape == B_x.shape == (1, S, D) and B_mem0.shape == (1, M, D)
    assert B_Wq.shape == B_Wk.shape == B_Wv.shape == (D, H, DH) and B_Wo.shape == (H, DH, D)
    dma = pltpu.SemaphoreType.DMA

    def vmem(shape, dtype):
        assert math.prod(shape) * jnp.dtype(dtype).itemsize % 16384 == 0, shape
        return pltpu.VMEM(shape, dtype)

    call = pl.pallas_call(
        _kernel,
        out_shape=jax.ShapeDtypeStruct((S, 2 * D), BF16),
        in_specs=[pl.BlockSpec(memory_space=pl.ANY)] * 9,
        out_specs=pl.BlockSpec(memory_space=pl.ANY),
        scratch_shapes=[
            vmem((S, D), BF16),
            vmem((3, D, D), BF16),
            vmem((D, D), BF16),
            vmem((LT, D, 128), F32),
            vmem((2 * D, D), U32),
            vmem((TB, D), U32),
            vmem((2, LT, TB, 128), F32),
            vmem((2, 2 * LT, HALO + TB, 128), F32),
            vmem((2, TB, D), F32),
            vmem((S, D), BF16),
            vmem((S, D), BF16),
            vmem((8 * M, D), BF16),
            vmem((NQ * 128, D), BF16),
            vmem((H * DH, D), BF16),
            vmem((GA * D // 2, D), U32),
            vmem((GA * 4 * 64, D), U32),
            vmem((3 * SEG, D), F32),
            vmem((NQ + 4, L, 128), F32),
            vmem((NW, SEG, 128), F32),
            vmem((8, M, 128), F32),
            vmem((12, M, 128), F32),
            vmem((GQ, 15, SEG, 128), F32),
            vmem((NQ + 1, SEG, 128), F32),
            [vmem((4, L, 128), F32)] * RING,
            vmem((NO, SEG, 128), F32),
            [vmem((20, L + SEG, 128), F32) for g0, g1 in CHUNKS],
            vmem((20, SEG, 128), F32),
            vmem((S, D), BF16),
            dma((4,)), dma((NB // 2,)), dma((NCH, 3)), dma((3,)), dma((GO,)), dma((2,)),
        ],
        compiler_params=pltpu.CompilerParams(vmem_limit_bytes=126 * 1024 * 1024, flags=CFG['flags']),
        name="sliding_and_memory_attention",
    )

    def by_feature(w):
        return w.transpose(1, 2, 0).reshape(H * DH, D)

    out = call(A_x.reshape(S, D), A_wqkv, A_wo, B_x.reshape(S, D), B_mem0.reshape(M, D),
               by_feature(B_Wq), by_feature(B_Wk), by_feature(B_Wv), B_Wo.reshape(H * DH, D))
    return out.reshape(1, S, 2 * D)
```

```python
import functools
import math

import jax
import jax.numpy as jnp
from jax import lax
from jax.experimental import pallas as pl
from jax.experimental.pallas import tpu as pltpu

F32, BF16, U32 = jnp.float32, jnp.bfloat16, jnp.uint32
NT = (((1,), (1,)), ((), ()))
MASKED = -1000000000.0

S, D = 2048, 640
LT = D // 128

AH, AD, AW, ADIL = 32, 20, 8, 2
HALO = 16
TB = 128
NB = S // TB
RC = 8

H, DH, M, SEG = 32, 192, 8, 32
L = M + SEG
HS = SEG // 2
NP = H // 2
PW = 2 * DH
NSEG = S // SEG
NCH = NP // 2
NO = H * DH // 128
NQ = 3 * NO
GQ = (NQ + 1) // LT
GO = (NO + 2) // LT
T = (0.0, -0.5, 0.5, -1.5, 1.5)
PAIRS = [(i, j) for j in range(LT) for i in range(j)]
GA = GQ + GO
NW = LT * LT + LT + len(PAIRS)

RING = 8
CHUNKS = ((0, 3), (3, 6), (6, GO))
CFG = dict(nper=(NSEG - 2) // 2, flags=None, nobc=False, back=20, aback=16, holdall=0, split=10, main=1,
           ds=35, dn=60, dp=85, tp=740, dt=25, hp=6, opos=0, rcp=1, ls=(1, 4, 8), lo=18, nq=20, mv=22, d1=19)


def _blk(i, j):
    return i * LT + j


def _row(j):
    return LT * LT + j


def _sum(i, j):
    return LT * LT + LT + PAIRS.index((i, j))


def _ds(i, n):
    return pl.ds(i * n if isinstance(i, int) else pl.multiple_of(i * n, n), n)


def _dot(a, b):
    return jnp.dot(a, b, preferred_element_type=F32)


def _axpy(t, y, x):
    return x if t == 0 else x + y if t == 1 else x - y if t == -1 else x + t * y


def _add(a, b):
    return b if a is None else a + b


def _acc(a, sign, b):
    if a is None:
        return sign, b
    if a[0] == sign:
        return sign, a[1] + b
    return (1, a[1] - b) if a[0] > 0 else (1, b - a[1])


def _val(a):
    return a[1] if a[0] > 0 else -a[1]


def _add_rows(a, b):
    return b if a is None else _cat(a[:M] + b[:M], a[M:] + b[M:])


def _cat(*parts):
    return jnp.concatenate(parts, axis=0)


def _share(tasks, k, n):
    return list(tasks[k * len(tasks) // n:(k + 1) * len(tasks) // n])


def _merge(a, b):
    return [t for k in range(len(a)) for t in [a[k]] + _share(b, k, len(a))]


def _pack(tasks, n):
    return [functools.partial(_run, tasks[k:k + n]) for k in range(0, len(tasks), n)]


def _run(tasks):
    for task in tasks:
        task()


def _block_diag(t0, t1, t2):
    lane = lax.broadcasted_iota(jnp.int32, (L, 128), 1)
    zero = jnp.zeros((L, 128), F32)
    top = jnp.concatenate([t0, jnp.where(lane < 64, t1, 0.0), zero], axis=1)
    bot = jnp.concatenate([zero, jnp.where(lane >= 64, t1, 0.0), t2], axis=1)
    return _cat(top, bot).astype(BF16)


def _kernel(ax_hbm, awqkv_hbm, awo_hbm, bx_hbm, mem_hbm, wq_hbm, wk_hbm, wv_hbm, wo_hbm,
            out_hbm,
            ax, awqkv, awo, tmp, wa, xb, q_s, kv_s, oa_s, outa,
            bx, mem, raw, wo_raw, plain, sums, h0, first, lhs, m_s, m_sum, part, tok, ring, ox, mixed, opart, outb,
            sem_a, sem_x, sem_w, sem_b, sem_wo, sem_o):
    cp = pltpu.make_async_copy

    def rows_copy(src, dst, r0, n, sem):
        return cp(src.at[pl.ds(r0, n), :], dst.at[pl.ds(r0, n), :], sem)

    c_wqkv = [cp(awqkv_hbm.at[:, pl.ds(j * D, D)], awqkv.at[j], sem_a.at[j]) for j in range(1, 3)]
    c_wq = [cp(awqkv_hbm.at[r0:r1, 0:D], awqkv.at[0, r0:r1], sem_a.at[4 + k])
            for k, (r0, r1) in enumerate(((0, 256), (256, D)))]
    c_awo = cp(awo_hbm, awo, sem_a.at[3])
    c_mem = cp(mem_hbm, mem.at[0:M], sem_b.at[0])
    c_bx0 = rows_copy(bx_hbm, bx, 0, 6 * SEG, sem_b.at[1])
    c_bx1 = rows_copy(bx_hbm, bx, 6 * SEG, S - 6 * SEG, sem_b.at[2])
    c_outa = cp(outa, out_hbm.at[:, pl.ds(0, D)], sem_o.at[0])

    def c_ax(c):
        return [cp(ax_hbm.at[_ds(c, 2 * TB), :], ax.at[_ds(c, 2 * TB), :], sem_x.at[c])]

    def c_w(c):
        return [cp(w.at[_ds(c, 2 * PW), :], raw.at[_ds(j * NCH + c, 2 * PW), :], sem_w.at[c, j])
                for j, w in enumerate((wq_hbm, wk_hbm, wv_hbm))]

    def c_wo(g):
        if isinstance(g, int) and g == GO - 1:
            return [rows_copy(wo_hbm, wo_raw, g * D, H * DH - g * D, sem_wo.at[g])]
        return [cp(wo_hbm.at[_ds(g, D), :], wo_raw.at[_ds(g, D), :], sem_wo.at[g])]

    def c_outb(r0, n):
        return cp(outb.at[pl.ds(r0, n), :], out_hbm.at[pl.ds(r0, n), pl.ds(D, D)], sem_o.at[1])

    def start(copies):
        for c in copies:
            c.start()

    def wait(copies):
        for c in copies:
            c.wait()
        recent.clear()

    def weight(g, s):
        if s < 25 and s % 6:
            return pltpu.bitcast(plain[_ds(g * LT + s % LT, 64), _ds(s // LT, 128)], BF16)
        s = s // 6 if s < 25 else s - 20
        return pltpu.bitcast(sums[_ds(4 * g + s // LT, 64), _ds(s % LT, 128)], BF16)

    def regroup(t, n):
        return _cat(*[tmp[t, pl.ds(d, AH, stride=AD), 0:n] for d in range(AD)])

    def prep_a(j):
        def task(t):
            tmp[t] = awqkv[j, _ds(t, 128), :].astype(F32).T if j < 3 else awo[:, _ds(t, 128)].astype(F32)
            wa[_ds(j, D // 2), _ds(t, 128)] = pltpu.bitcast(regroup(t, 128).astype(BF16), U32)

        return [functools.partial(task, t) for t in range(LT)]

    recent = []

    def hold(x, zero, back):
        if len(recent) < back:
            return x
        late = recent[-back] if x.dtype == F32 else pltpu.bitcast(recent[-back], U32)
        return jnp.where(lax.broadcasted_iota(jnp.int32, x.shape, 0) >= zero, x, late)

    def by_tile(j, left, put):
        acc = [None]

        def task(t, k):
            if j < 3:
                w = pltpu.bitcast(wa[_ds(j * LT + t, 64), _ds(k, 128)], BF16)
                r = lax.dot_general(left(k), w, NT, preferred_element_type=F32)
            else:
                r = _dot(left(k), pltpu.bitcast(wa[_ds(j * LT + k, 64), _ds(t, 128)], BF16))
            e = len(recent) % 16
            recent.extend(r[8 * (e + i) % TB:8 * (e + i) % TB + 8] for i in range(4))
            acc[0] = _add_rows(acc[0] if k else None, r)
            if k == LT - 1:
                put(t, acc[0])

        return [functools.partial(task, t, k) for t in range(LT) for k in range(LT)]

    def a_load(i, b):
        xb[_ds(b, TB // 2), :] = pltpu.bitcast(ax[_ds(i, TB), :], U32)

    def a_proj(i, b, j):
        def put(t, r):
            if j == 0:
                q_s[b, t] = r
                return
            c = (j - 1) * LT + t
            kv_s[b, c, HALO:, :] = r
            if isinstance(i, int) and i == 0:
                kv_s[b, c, 0:HALO, :] = jnp.broadcast_to(r[0:1, :], (HALO, 128))
            else:
                kv_s[b, c, 0:HALO, :] = kv_s[1 - b, c, TB:, :]

        return by_tile(j, lambda k: pltpu.bitcast(xb[_ds(b, TB // 2), _ds(k, 128)], BF16), put)

    def a_attention(b, zero, first_block=False):
        state = {}

        def window(c, r0, w):
            lo = HALO + r0 - ADIL * w
            return kv_s[b, c, lo:lo + RC, :]

        def logits(r0):
            q = [hold(q_s[b, t, r0:r0 + RC, :], zero, CFG["aback"]) for t in range(LT)]
            state[r0] = []
            for w in range(AW):
                a = q[0] * window(0, r0, w)
                for t in range(1, LT):
                    a = a + q[t] * window(t, r0, w)
                state[r0].append(a + pltpu.roll(a, 2 * AH, 1))

        def fold(r0):
            state[r0] = [a + pltpu.roll(a, AH, 1) for a in state[r0]]

        def weigh(r0):
            scale = AD ** -0.5
            lg = []
            for w, a in enumerate(state.pop(r0)):
                if first_block and r0 < ADIL * w:
                    pos = lax.broadcasted_iota(jnp.int32, (RC, 128), 0) + r0
                    a = jnp.where(pos >= ADIL * w, a, MASKED / scale)
                lg.append(a)
            m = hold(functools.reduce(jnp.maximum, lg), zero, CFG["aback"])
            p = [jnp.exp2((a - m) * (scale * math.log2(math.e))) for a in lg]
            state[r0] = p, 1.0 / functools.reduce(jnp.add, p)

        def mix(r0):
            p, inv = state.pop(r0)
            for t in range(LT):
                o = p[0] * window(LT + t, r0, 0)
                for w in range(1, AW):
                    o = o + p[w] * window(LT + t, r0, w)
                oa_s[b, r0:r0 + RC, t * 128:(t + 1) * 128] = o * inv

        n = TB // RC
        return [functools.partial(f, (k - lag) * RC) for k in range(n + 2)
                for lag, f in ((0, logits), (1, fold), (2, weigh), (2, mix)) if 0 <= k - lag < n]

    def a_out(i, b):
        def put(t, r):
            outa[_ds(i, TB), _ds(t, 128)] = r.astype(BF16)

        return by_tile(3, lambda k: oa_s[b, :, _ds(k, 128)], put)

    def groups(g, n):
        def view(ref, rows):
            r0 = g * rows
            ref = ref.at[pl.ds(r0 if isinstance(g, int) else pl.multiple_of(r0, rows), n * rows)]
            return [(ref, k * rows) for k in range(n)]

        return list(zip(view(plain, LT * 64), view(sums, 4 * 64)))

    def transposes(at, g, zero):
        dst, r0 = at[0]

        def task(j):
            n = g * LT + j - 1
            p = (n + 9) * 57 >> 9
            e = (n + 9 - 9 * p) * 11 >> 5
            t = e * (NO - 3) + n + 6 - 6 * p
            if j == 0 and not isinstance(n, int):
                t = jnp.where(n < 0, NQ, t)
            v = pltpu.bitcast(raw[_ds(t, 128), :].T, U32)
            for i in range(LT):
                dst[pl.ds(r0 + j * 64, 64), _ds(i, 128)] = v[i * 64:(i + 1) * 64]

        return [functools.partial(task, j) for j in range(LT)]

    def derive(at, zero, block=None):
        (src, r0), (dst, r1) = at
        row, col = [None] * LT, [None] * LT

        def task(r, e):
            def put(s, v):
                dst[pl.ds(r1 + s // LT * 64 + r * 8, 8), _ds(s % LT, 128)] = pltpu.bitcast(v.astype(BF16), U32)

            def load(i, j):
                at = pl.ds(r0 + j * 64 + r * 8, 8), _ds(i, 128)
                v = src[at] if block is None else block(r, i, j)
                if i < j or CFG["holdall"]:
                    v = hold(v, zero, CFG["back"])
                if block is not None:
                    src[at] = v
                return pltpu.bitcast(v, BF16).astype(F32)

            for k in _share(range(10), e, CFG["split"]):
                i, j = PAIRS[k]
                for d in ((0, 1) if k == 0 else (j,) if i == 0 else ()):
                    row[d] = col[d] = load(d, d)
                up, lo = load(i, j), load(j, i)
                put(2 * LT + k, up + lo)
                row[i], col[j] = row[i] + up, col[j] - up
                row[j], col[i] = row[j] + lo, col[i] - lo
                for d in ((i, j) if k == 9 else (i,) if j == LT - 1 else ()):
                    put(d, col[d])
                    put(LT + d, row[d])

        return [functools.partial(task, r, e) for r in range(8) for e in range(CFG["split"])]

    def derive_out(g, zero):
        n = min(LT, NO - g * LT) if isinstance(g, int) else LT
        src = wo_raw.at[pl.ds(g * D if isinstance(g, int) else pl.multiple_of(g * D, D), n * 128)]

        def block(r, i, j):
            if i >= n:
                return jnp.zeros((8, 128), U32)
            return pltpu.bitcast(src[_ds(i * 8 + r, 16), _ds(j, 128)], U32)

        return derive(groups(g, 1)[0], zero, block)

    def first_group(g):
        src = plain.at[_ds(GO + g, D // 2)]
        acc = [None] * LT

        def task(i, j):
            r = _dot(h0[0:L + SEG, _ds(i, 128)], pltpu.bitcast(src[_ds(j, 64), _ds(i, 128)], BF16))
            e = len(recent) % 8
            recent.extend([r[8 * e:8 * e + 8], r[8 * e + 8:8 * e + 16]])
            acc[j] = _add_rows(acc[j], r)
            if i == LT - 1:
                first[g * LT + j] = acc[j][0:L]
                tok[g * LT + j] = acc[j][L:]

        return [functools.partial(task, i, j) for j in range(LT) for i in range(LT)]

    def each(f, groups, *args):
        return [task for g in groups for task in f(g, *args)]

    start(c_wq)
    raw[NQ * 128:, :] = jnp.zeros((128, D), BF16)
    wait(c_wq[:1])
    start(c_ax(0))
    _run(prep_a(0)[:2])
    wait(c_wq[1:])
    start(c_wqkv[:1])
    _run(prep_a(0)[2:])
    wait(c_ax(0))
    start(c_wqkv[1:])
    a_load(0, 0)
    a_load(1, 1)
    _run(a_proj(0, 0, 0) + a_proj(1, 1, 0)[:CFG["nq"]])
    wait(c_wqkv[:1])
    start([c_awo] + c_ax(1))
    _run(a_proj(1, 1, 0)[CFG["nq"]:] + prep_a(1) + a_proj(0, 0, 1))
    wait(c_wqkv[1:])
    start(c_w(0))
    side = a_attention(0, 0, first_block=True)
    _run(a_proj(1, 1, 1) + prep_a(2) + [t for t in side if t.func.__name__ != "mix"] + a_proj(0, 0, 2))
    wait([c_awo])
    _run(_merge(a_proj(1, 1, 2), _merge([t for t in side if t.func.__name__ == "mix"], prep_a(3))))

    def a_step(it, carry):
        c = it - 2
        g = jnp.where(it == 1, GQ - 3, 3 * it - 6)
        zero = it >> 16

        @pl.when(it + 1 < NB // 2)
        def _():
            start(c_ax(it + 1))

        @pl.when(it + 1 == NB // 2)
        def _():
            start(c_wo(0))
        wait(c_ax(it))

        @pl.when(it + 1 < NB // 2)
        def _():
            start(c_w(it))

        @pl.when(it + 1 == NB // 2)
        def _():
            start(each(c_wo, range(1, 4)))

        @pl.when(it > 1)
        def _():
            wait(c_w(c))
        for b in range(2):
            a_load(2 * it + b, b)
        at = groups(GO + 3 * it - 9, 6)
        both = _merge(each(derive, at[:3], zero), [t for e in range(3) for t in transposes(at[3 + e], g + e, zero)])
        for b, side in enumerate((_share(both, 0, 2), _share(both, 1, 2))):
            i = 2 * it + b
            main = a_proj(i, b, 0) + a_proj(i, b, 1) + a_proj(i, b, 2) + a_out(i - 2, b)
            _run(_merge(main, _merge(a_attention(1 - b, zero), side)))
        return zero

    start([c_mem, c_bx0])
    zero = lax.fori_loop(1, NB // 2, a_step, 0)

    due = []

    def mm(x, g, s):
        r = _dot(x, weight(g, s))
        recent.append(r[0:M])
        while due and due[0][0] <= len(recent):
            due.pop(0)[1]()
        return r

    def attention(qkv, put, rows=slice(0, L)):
        n = rows.stop - rows.start
        row = lax.broadcasted_iota(jnp.int32, (n, 2 * L), 0) + rows.start
        col = lax.broadcasted_iota(jnp.int32, (n, 2 * L), 1)
        head0 = col < L
        visible = (row < M) | (row >= jnp.where(head0, col, col - L))
        scale = DH ** -0.5
        st = {}

        def score(p):
            q = jnp.concatenate([qkv(9 * p + t) for t in range(3)], axis=1)
            k = _block_diag(*[qkv(9 * p + 3 + t) for t in range(3)])
            sc = lax.dot_general(q, k, NT, preferred_element_type=F32)
            sc = jnp.where(visible, sc, MASKED / scale)
            m0 = jnp.max(jnp.where(head0, sc, -jnp.inf), axis=1, keepdims=True)
            m1 = jnp.max(jnp.where(head0, -jnp.inf, sc), axis=1, keepdims=True)
            st[p] = sc - jnp.where(head0, m0, m1)

        def normalize(p):
            e = jnp.exp2(st[p] * (scale * math.log2(math.e)))
            l0 = jnp.sum(jnp.where(head0, e, 0.0), axis=1, keepdims=True)
            l1 = jnp.sum(jnp.where(head0, 0.0, e), axis=1, keepdims=True)
            l = jnp.where(head0, l0, l1)
            if CFG["rcp"]:
                r = pl.reciprocal(l, approx=True)
                st[p] = e * (r * (2.0 - l * r))
            else:
                st[p] = e / l

        def mix(p):
            r = _dot(st.pop(p), _block_diag(*[qkv(9 * p + 6 + t) for t in range(3)]))
            for t in range(3):
                put(3 * p + t, r[:, t * 128:(t + 1) * 128])

        return score, normalize, mix

    def mixed_at(refs, n):
        return [(ref, n - g0 * LT) for ref, (g0, g1) in zip(refs, CHUNKS) if g0 <= n // LT < g1][0]

    def put_x(n, r):
        ref, k = mixed_at(mixed, n)
        ref[k, 0:M] = r[0:M]
        ox[n] = r[M:]

    def put_y(n, r):
        ref, k = mixed_at(mixed, n)
        ref[k] = _cat(r[0:M], _axpy(T[n % LT], r[M:], ox[n]), r[M:])

    def prep_tokens(s, zero):
        def task(e):
            rows = _ds(e, M)
            x, y = [bx[_ds((s + k) * (SEG // M) + e, M), :].astype(F32) for k in range(2)]
            y = [hold(y[:, j * 128:(j + 1) * 128], zero, CFG["hp"] * (LT - j)) for j in range(LT)]
            a = [_axpy(T[j], y[j], x[:, j * 128:(j + 1) * 128]) for j in range(LT)]
            for j in range(LT):
                lhs[_blk(j, j), rows] = a[j]
                lhs[_row(j), rows] = y[j]
            for i, j in PAIRS:
                both = a[i] + a[j]
                lhs[_sum(i, j), rows] = both
                lhs[_blk(i, j), rows] = _axpy(T[j] - T[i], y[i], both)
                lhs[_blk(j, i), rows] = _axpy(T[i] - T[j], y[j], both)

        return [functools.partial(task, e) for e in range(SEG // M)]

    def step(s, second, zero):
        def reread(ref):
            return ref.at[pl.ds(4 * zero, ref.shape[0])]

        part_r, opart_r, m_sum_r = reread(part), reread(opart), reread(m_sum)
        ring_r, mixed_r = [reread(r) for r in ring], [reread(r) for r in mixed]
        half = slice(HS, SEG) if second else slice(0, HS)

        class Sums:
            def __init__(self, c):
                self.c, self.u, self.u2, self.cy = c, [None] * LT, [None] * LT, [None] * LT

            def column(self, j, m, t):
                self.c[j] = _acc(self.c[j], 1, m)
                if second:
                    self.cy[j] = _acc(self.cy[j], 1, t)
                else:
                    self.u[j] = _add(self.u[j], t[:HS])
                    self.u2[j] = _add(self.u2[j], t[HS:])

            def pair(self, i, j, m, t, lo_m, lo_t, before):
                self.u[i] = _add(self.u[i], lo_t)
                if not second:
                    self.column(j, m, t)
                    self.c[i] = _acc(self.c[i], 1, lo_m)
                    return _cat(t[:HS] + lo_t, t[HS:])
                v = m - lo_m
                self.c[j] = _acc(self.c[j], 1, v)
                self.c[i] = _acc(self.c[i], -1, v)
                if before is not None:
                    t = t - before
                w, f = _cat(t[:HS], t[HS:] - lo_t), 1.0 / (T[i] - T[j])
                if abs(f) != 1:
                    w, f = w * f, 1
                self.cy[j] = _acc(self.cy[j], f, w)
                self.cy[i] = _acc(self.cy[i], -f, w)

        def project(g):
            z = Sums([None] * LT)

            def single(j, left, m, s):
                r = mm(_cat(lhs[left], m), GO + g, s)
                z.column(j, r[SEG:], r[:SEG])

            def pair(i, j):
                k = PAIRS.index((i, j))
                if g == 0:
                    ms = m_s[i] + m_s[j]
                    m_sum[k] = ms
                else:
                    ms = m_sum_r[k]
                if g == 0 and i == 0:
                    single(j, _row(i) if second else _blk(i, j), m_s[i] if second else ms, _blk(i, j))
                    return
                s = _sum(i, j) if second else _blk(i, j)
                up = mm(_cat(lhs[s], m_s[i] if second else ms), GO + g, s)
                lo = mm(_cat(lhs[_blk(j, i), half], ms), GO + g, _blk(j, i))
                r = z.pair(i, j, up[SEG:], up[:SEG], lo[HS:], lo[:HS], part_r[g, LT + k] if second else None)
                if not second:
                    part[g, LT + k] = r

            order = sorted(PAIRS) if g else PAIRS
            for j in range(LT):
                if g > 0 or j > 0:
                    s = _row(j) if second else _blk(j, j)
                    single(j, s, m_s[j], s)
                pair(*order[2 * j])
                pair(*order[2 * j + 1])
            for j in range(0 if g else 1, LT):
                n = g * LT + j - 1
                dst = ring[n // 3 % RING]
                dst[n % 3, 0:M] = _val(z.c[j])
                if not second:
                    part[g, j] = _cat(z.u[j], z.u2[j])
                    continue
                u, y = part_r[g, j], _val(z.cy[j])
                if z.u[j] is not None:
                    u = _cat(u[:HS], u[HS:] + z.u[j])
                dst[n % 3, M:] = _axpy(-T[j], y, u)
                tok[n + 1] = y

        def projected(n):
            src = ring_r[n // 3 % RING]
            return src[n % 3] if second else _cat(src[n % 3, 0:M], tok[n + 1])

        c = [None] * LT

        def out_chunk(ref, g0, g1):
            head, last = g0 == 0, g1 == GO
            z = Sums(c)

            def products(g, i, j, acc):
                ki, kj = (g - g0) * LT + i, (g - g0) * LT + j
                if g * LT + i >= NO:
                    return
                full = g * LT + j < NO
                both = ref[ki, 0:L] + ref[kj, 0:L] if full else ref[ki, 0:L]
                ms, a = both[:M], both[M:]
                if second:
                    acc[0] = _add_rows(acc[0], mm(_cat(ref[ki, 0:M], a), g, _sum(i, j)))
                else:
                    left = _axpy(T[j] - T[i], ref[ki, L:], a)
                    acc[0] = _add_rows(acc[0], mm(_cat(ms, left), g, _blk(i, j)))
                if full:
                    left = _axpy(T[i] - T[j], ref[kj, L:][half], a[half])
                    acc[1] = _add_rows(acc[1], mm(_cat(ms, left), g, _blk(j, i)))

            def finish(i):
                if last:
                    m_s[i] = _val(c[i])
                if not second:
                    u = _cat(z.u[i], z.u2[i])
                    opart[i] = u if head else opart[i] + u
                    return
                u = opart[i]
                if z.u[i] is not None:
                    u = _cat(u[:HS], u[HS:] + z.u[i])
                y = _val(z.cy[i] if head else _acc(z.cy[i], 1, opart[15 + i]))
                if last:
                    outb[_ds(s, SEG), _ds(i, 128)] = _axpy(-T[i], y, u).astype(BF16)
                    outb[_ds(s + 1, SEG), _ds(i, 128)] = y.astype(BF16)
                else:
                    if z.u[i] is not None:
                        opart[i, HS:] = u[HS:]
                    opart[15 + i] = y

            order = sorted(PAIRS)
            for q in range(LT):
                d, accs = None, ([None, None], [None, None])
                for g in range(g0, g1):
                    k = (g - g0) * LT + q
                    for e in range(CFG["opos"]):
                        products(g, *order[2 * q + e], accs[e])
                    if g * LT + q < NO:
                        left = _cat(ref[k, 0:M], ref[k, L:]) if second else ref[k, 0:L]
                        d = _add_rows(d, mm(left, g, _row(q) if second else _blk(q, q)))
                    for e in range(CFG["opos"], 2):
                        products(g, *order[2 * q + e], accs[e])
                for (i, j), (up, lo) in zip(order[2 * q:], accs):
                    k = LT + PAIRS.index((i, j))
                    r = z.pair(i, j, up[:M], up[M:], lo[:M], lo[M:], opart_r[k] if second and head else None)
                    if not second:
                        opart[k] = r if head else opart[k] + r
                z.column(q, d[:M], d[M:])
                for i in ((), (0,), (), (1,), (2, 3, 4))[q]:
                    finish(i)

        recent.clear()
        stages = attention(projected, put_x if second else put_y)
        for p in range(NP):
            ready = LT * LT * ((9 * p + 6) // LT + 1) - LT
            due.extend((ready + CFG[lag], functools.partial(f, p)) for f, lag in
                       zip(stages, ("ds", "dn", "dp")))
        if second:
            due.extend((CFG["tp"] - LT + k * CFG["dt"], task)
                       for k, task in enumerate(prep_tokens(jnp.minimum(s + 4, NSEG - 2), zero)))
        due.sort(key=lambda e: e[0])
        for g in range(GQ):
            project(g)
        for ref, chunk in zip(mixed_r, CHUNKS):
            out_chunk(ref, *chunk)

    def put_first(n, r):
        recent.extend([r[k:k + 8] for k in range(0, L, 16)])
        put_x(n, r)

    stages = attention(lambda n: first[n + 1], put_first)
    lags = (0, 1, 2)
    acc = [None] * LT

    def heads(p0, p1):
        return [functools.partial(f, t - lag) for t in range(p0, p1 + lags[-1])
                for f, lag in zip(stages, lags) if p0 <= t - lag < p1]

    def out_first(*groups):
        def task(g, i, j):
            ref, k = mixed_at(mixed, g * LT + i)
            r = _dot(ref[k, 0:M], wo_raw[_ds(g * LT + i, 128), _ds(j, 128)] if g > 3 else
                     pltpu.bitcast(plain[_ds(g * LT + j, 64), _ds(i, 128)], BF16))
            recent.append(r)
            acc[j] = _add(acc[j], r)
        return [functools.partial(task, g, i, j) for g in groups for i in range(min(LT, NO - g * LT))
                for j in range(LT)]

    at = groups(GO, GQ)

    def moves(g0, g1):
        return [t for g in range(g0, g1) for t in transposes(at[g], g, zero)]

    start(c_w(NCH - 1))
    wait(c_w(NCH - 2) + c_wo(0) + [c_mem, c_bx0])
    h0[0:M, :] = mem[0:M, :].astype(F32)
    h0[M:L + SEG, :] = bx[0:2 * SEG, :].astype(F32)
    _run(_merge(a_out(NB - 2, 0) + each(first_group, range(10)),
                _merge(each(derive, at[15:CFG['d1']], zero) + derive_out(0, zero),
                       _merge(a_attention(1, zero), moves(18, CFG['mv'])))))
    start(c_wo(4))
    wait(each(c_wo, range(1, 4)))
    start(c_wo(5) + c_wo(6))
    _run(_merge(a_out(NB - 1, 1) + _merge(each(first_group, range(10, 18)), heads(0, 5)),
                _merge(each(derive, at[CFG['d1']:22], zero) + each(derive_out, range(1, 4), zero), moves(CFG['mv'], 25))))
    wait(c_w(NCH - 1))
    start(c_wo(7) + c_wo(8))
    _run(_merge(_merge(each(first_group, range(18, 27)), _merge(out_first(0, 1), heads(5, 12))),
                _merge(each(derive, at[22:25], zero), moves(25, GQ)) + each(derive, at[25:], zero)))
    wait(each(c_wo, range(4, 7)))
    start(c_wo(9))
    _run(_merge(each(first_group, range(27, GQ)) + _merge(_pack(out_first(2, 3, 4, 5, 6), 2), heads(12, NP)),
                _merge(each(derive_out, range(4, 7), zero), prep_tokens(2, zero))))
    wait(c_wo(7) + c_wo(8))
    _run(_merge(out_first(7, 8), each(derive_out, (7, 8), zero)))
    wait(c_wo(9))
    start([c_bx1, c_outa])
    _run(_merge(out_first(9), derive_out(9, zero)))
    for j in range(LT):
        m_s[j] = acc[j]

    def b_step(it, carry):
        @pl.when(it == 1)
        def _():
            c_bx1.wait()
        step(2 * it, False, it >> 16)
        step(2 * it, True, it >> 16)
        c_outb(pl.multiple_of(it * 2 * SEG, 2 * SEG), 2 * SEG).start()
        return carry

    if not CFG['main']:
        c_outa.wait()
        c_bx1.wait()
        return
    lax.fori_loop(0, CFG["nper"], b_step, 0)

    for k, (i, j) in enumerate(PAIRS):
        m_sum[k] = m_s[i] + m_s[j]
    res = {}
    acc = [None] * LT

    def last_tile(n, i):
        g, j = divmod(n + 1, LT)
        left = m_s[j] if i == j else m_sum[PAIRS.index((min(i, j), max(i, j)))]
        res[n] = _acc(res.get(n), 1 - 2 * (i % 2), _dot(-left if i % 2 else left, weight(GO + g, _blk(i, j))))

    def put_last(n, r):
        res[NQ + n] = r

    stages = attention(lambda n: _cat(_val(res.pop(n)), tok[n + 1]) if n in res else tok[n + 1], put_last, slice(M, L))
    def last_out(n, i):
        w = pltpu.bitcast(plain[_ds(n // LT * LT + i, 64), _ds(n % LT, 128)], BF16)
        acc[i] = _add_rows(acc[i], _dot(_cat(ox[n], res[NQ + n]), w))

    short = [functools.partial(last_tile, n, i) for n in range(NQ) if n % 9 >= 3 for i in range(LT)]
    tall = [functools.partial(last_out, n, i) for n in range(NO) for i in range(LT)]
    lag = CFG["lo"]
    for t in range(NP // 2 * LT * 3 // 2 + lag):
        _run(short[8 * t:8 * t + 8])
        if t >= lag:
            _run(tall[4 * (t - lag):4 * (t - lag) + 4])
        for p in range(0, NP, 2):
            for f, late in list(zip(stages, CFG["ls"]))[::-1]:
                if t == (30 * (p + 2) - 1) // 8 + late:
                    f(p)
                    f(p + 1)
    acc = jnp.concatenate(acc, axis=1)
    outb[S - 2 * SEG:, :] = acc.astype(BF16)
    c_outb(S - 2 * SEG, 2 * SEG).start()
    c_outa.wait()
    c_outb(0, (CFG["nper"] + 1) * 2 * SEG).wait()


def pallas_concat_heads__sliding_local_dilated__memory_aug_recurrent_mem_tr__prompt_kernel(
    A_x, A_wqkv, A_wo, B_x, B_mem0, B_Wq, B_Wk, B_Wv, B_Wo, B_seg_len,
):
    assert B_seg_len == SEG
    assert A_x.shape == B_x.shape == (1, S, D) and B_mem0.shape == (1, M, D)
    assert B_Wq.shape == B_Wk.shape == B_Wv.shape == (D, H, DH) and B_Wo.shape == (H, DH, D)
    dma = pltpu.SemaphoreType.DMA

    def vmem(shape, dtype):
        assert math.prod(shape) * jnp.dtype(dtype).itemsize % 16384 == 0, shape
        return pltpu.VMEM(shape, dtype)

    call = pl.pallas_call(
        _kernel,
        out_shape=jax.ShapeDtypeStruct((S, 2 * D), BF16),
        in_specs=[pl.BlockSpec(memory_space=pl.ANY)] * 9,
        out_specs=pl.BlockSpec(memory_space=pl.ANY),
        scratch_shapes=[
            vmem((S, D), BF16),
            vmem((3, D, D), BF16),
            vmem((D, D), BF16),
            vmem((LT, D, 128), F32),
            vmem((2 * D, D), U32),
            vmem((TB, D), U32),
            vmem((2, LT, TB, 128), F32),
            vmem((2, 2 * LT, HALO + TB, 128), F32),
            vmem((2, TB, D), F32),
            vmem((S, D), BF16),
            vmem((S, D), BF16),
            vmem((8 * M, D), BF16),
            vmem(((NQ + 1) * 128, D), BF16),
            vmem((H * DH, D), BF16),
            vmem((GA * D // 2, D), U32),
            vmem((GA * 4 * 64, D), U32),
            vmem((3 * SEG, D), F32),
            vmem((NQ + 4, L, 128), F32),
            vmem((NW, SEG, 128), F32),
            vmem((8, M, 128), F32),
            vmem((12, M, 128), F32),
            vmem((GQ, 15, SEG, 128), F32),
            vmem((NQ + 1, SEG, 128), F32),
            [vmem((4, L, 128), F32)] * RING,
            vmem((NO, SEG, 128), F32),
            [vmem((20, L + SEG, 128), F32) for g0, g1 in CHUNKS],
            vmem((20, SEG, 128), F32),
            vmem((S, D), BF16),
            dma((6,)), dma((NB // 2,)), dma((NCH, 3)), dma((3,)), dma((GO,)), dma((2,)),
        ],
        compiler_params=pltpu.CompilerParams(vmem_limit_bytes=126 * 1024 * 1024, flags=CFG['flags'], disable_bounds_checks=CFG['nobc']),
        name="sliding_and_memory_attention",
    )

    def by_feature(w):
        return w.transpose(1, 2, 0).reshape(H * DH, D)

    out = call(A_x.reshape(S, D), A_wqkv, A_wo, B_x.reshape(S, D), B_mem0.reshape(M, D),
               by_feature(B_Wq), by_feature(B_Wk), by_feature(B_Wv), B_Wo.reshape(H * DH, D))
    return out.reshape(1, S, 2 * D)
```

```python
import collections
import functools
import itertools
import math
import random

import jax
import jax.numpy as jnp
import numpy as np
from jax import lax
from jax.experimental import pallas as pl
from jax.experimental.pallas import tpu as pltpu

F32, BF16, U32 = jnp.float32, jnp.bfloat16, jnp.uint32
NT = (((1,), (1,)), ((), ()))
MASKED = -1000000000.0

S, D = 2048, 640
LT = D // 128

AH, AD, AW, ADIL = 32, 20, 8, 2
HALO = 16
TB = 128
NB = S // TB
RC = 8

H, DH, M, SEG = 32, 192, 8, 32
L = M + SEG
HS = SEG // 2
NP = H // 2
NSEG = S // SEG
NO = 3 * NP
NQ = 3 * NO
GW = 6
GO, GQ = NO // GW, NQ // GW
RAW = 4
RING = 12
CHUNKS = ((0, 3), (3, 5), (5, GO))

CFG = dict(nper=(NSEG - 2) // 2, flags=None, back=20, aback=16, split=10, hb=3, nq=20, nd=3,
           ds=40, dn=70, dp=100, tp=740, dt=25, hp=3, rcp=1, ow=6, mo=(0, 1, 4, 2, 3),
           ls=(1, 4, 8), lo=18, tau=8, drift=1.5, ext=1, only=0, cut=(8, 15, 22), dc=(18, 20))
PLAN = dict(blocks=[], events={}, n=0, seq="100001001010100101010100101101001001001100101010010100101101001010010011010100010100101110000101100101001001010100101101001100001011110000011010010110100001110001010010010101100101001001011001000111010001010110000101001100111100000100101101001010100100100101101001011010000101100100101100101001011010000111000011101000011010001110100010010100110010101100001110000110010010110010100100101011001010100011110000010110100101001011100000101100011001001110000101101010010001010110010101000110001100111000010110001101000110100010100101101001011010000101101000101001011010010110000110001100111000011100001101001001101000100101011001010110000101101000101101001010010110000110001100110100100101011001000101100010101100101011000011000010010101000011100001011010011110000011000010100011001010110010100111100001011010010111000010011010100011000111100000100101101000011110000111000111000010100101001010010100101001011011010000101000010110100001011010011110000101101001011011010010100101001010010100101101001010010100101001011010001101001001100010101100011000101101010001001010110001101000111010000110001100110100101001011010000101010010110010100101101001011000011001000111010000111100001100001100111000011110000101001011100000101100011010001110000110100100110100101001011010000101101001010010100101101001001001001011100001011010010110000110101010000110100100101101001001011000100101101001001011010010100010100101101001011010000101101000101101001010010110000110001100110100101001011010000101100011010010100101001011001001010101001010110000111100001100001100111100001100001101001011100000101100011010001110000110100100110100101001011010000101101001010010100101001011010010001010110001101000111010000100011001000011101000010110010111000010010101000011010001100101011101000110010101101101001000011001000111010101000010010101000110011101000101011101000010010101000110010100100101011011010000011000010110010001010110011101000101011001011110")


def _algorithm(rank_ones):
    rows = np.array([[1, 0], [0, 1], [1, 1]])
    duals = np.array([[0, 1], [1, 0], [1, -1]])
    sets = [[[np.array(["-0+".index(c) - 1 for c in w]) for w in e.split()] for e in s] for s in rank_ones]
    left, right = [], []
    for t, s in enumerate(sets):
        p, q = [k for k in range(3) if k != t]
        for u, v in s:
            left += [np.outer(u, rows[p]), np.outer(u, rows[q])]
            right += [np.outer(v, duals[q]), np.outer(v, duals[p])]
    for (u0, v0), (u1, v1), (u2, v2) in itertools.product(*sets):
        for a, b in itertools.product((1, -1), repeat=2):
            e = np.outer(u0 + a * u1, v0 + b * v1)
            if (e == np.outer(u2, v2)).all() or (e == -np.outer(u2, v2)).all():
                left.append(np.outer(u0, rows[1]) - a * np.outer(u1, rows[0]))
                right.append(np.outer(v0, duals[1]) + b * np.outer(v1, duals[0]))
    left, right = np.array(left), np.array(right)
    have = np.einsum("rka,rnb->kanbr", left, right).reshape(-1, len(left))
    want = np.einsum("kp,nq,ab->kanbpq", np.eye(LT), np.eye(GW), np.eye(2)).reshape(len(have), -1)
    blocks = np.rint(np.linalg.lstsq(have, want, rcond=None)[0]).astype(int)
    assert (have @ blocks == want).all()
    sign = blocks.max(axis=1) * 2 - 1
    return left * sign[:, None, None], blocks * sign[:, None], right


def _shared_sums(matrix, seed):
    rng = random.Random(seed)
    rows = [{k: int(c) for k, c in enumerate(row) if c} for row in matrix]
    shared = {}
    while True:
        count = collections.Counter(
            (a, b, r[a] * r[b]) for r in rows for a, b in itertools.combinations(sorted(r), 2))
        top = max(count.values(), default=0)
        if top < 2:
            return shared, rows
        best = sorted(k for k, n in count.items() if n == top)
        a, b, sign = best[int(rng.random() * len(best))]
        name = matrix.shape[1] + len(shared)
        shared[name] = a, b, sign
        for r in rows:
            if r.get(a, 0) * r.get(b, 0) == sign:
                r[name] = r.pop(a)
                del r[b]


MODEL, BLOCKS, FEATURE = _algorithm((
    ("+0000 +00++0", "000+0 0+0000", "0000+ 000+00", "+-+00 00000+", "+00+0 00+0+0"),
    ("0+00+ 000+++", "0+0+0 0+00++", "00+-+ 00++00", "00+0+ +00000", "+0+00 0000+0", "00+00 0+-000"),
    ("0+000 0000++", "00+-+ ++0000", "00+00 +00+00", "+-000 0+-00+", "00+-0 00+000", "+-00- +0000-")))
NR, BOTH = 47, 34
SINGLE = {r: int(row.argmax()) for r, row in enumerate(BLOCKS) if abs(row).sum() == 1}
SUMMED = [r for r in range(NR) if r not in SINGLE]


def _step_plan(out, step, seed, order):
    use = MODEL[:, :, step].any(1) & FEATURE[:, :, step].any(1)
    assert sorted(order) == np.nonzero(use)[0].tolist()
    return order, [_shared_sums((m * keep[:, None]).T, seed) for m, keep in (
        (out.reshape(NR, -1), use), (out.reshape(NR, -1), use & (np.arange(NR) < BOTH)), (out[:, :, step], use))]


PROJECT = (
    _step_plan(FEATURE, 0, 32, (30, 14, 20, 3, 28, 12, 9, 22, 10, 18, 1, 26, 24, 5, 32, 16, 7,
                                40, 38, 36, 44, 45, 46, 39, 34, 35, 43, 37, 41, 42)),
    _step_plan(FEATURE, 1, 5, (31, 15, 4, 11, 27, 0, 8, 19, 23, 13, 33, 6, 29, 21, 2, 25, 17,
                               40, 34, 39, 41, 35, 46, 45, 36, 43, 44, 38, 37, 42)))
OUTPUT = (
    _step_plan(MODEL, 0, 0, (24, 14, 10, 5, 32, 28, 16, 30, 22, 12, 7, 9, 3, 1, 18, 26, 20,
                             40, 34, 39, 41, 42, 37, 36, 45, 43, 44, 46, 35, 38)),
    _step_plan(MODEL, 1, 6, (23, 11, 13, 2, 15, 17, 4, 25, 31, 33, 6, 29, 8, 21, 19, 0, 27,
                             39, 36, 45, 40, 34, 41, 37, 42, 44, 43, 46, 35, 38)))
WEIGHTS = ((3, 28, 6, 0, 5, 17, 11, 8, 10, 7, 4, 16, 2, 1, 23, 22, 9, 29, 24, 19, 12, 18, 25, 13, 14, 20,
            21, 15, 26, 27), _shared_sums(BLOCKS, 37))


def _ds(i, n):
    return pl.ds(i * n if isinstance(i, int) else pl.multiple_of(i * n, n), n)


def _dot(a, b):
    return jnp.dot(a, b, preferred_element_type=F32)


def _cat(*parts):
    return jnp.concatenate(parts, axis=0)


def _add(a, b):
    return b if a is None else _cat(a[:M] + b[:M], a[M:] + b[M:])


def _acc(a, sign, b):
    if a is None:
        return sign, b
    if a[0] == sign:
        return sign, a[1] + b
    return (1, a[1] - b) if a[0] > 0 else (1, b - a[1])


def _sum(terms):
    return functools.reduce(lambda a, t: _acc(a, *t), terms, None)


def _val(a):
    return a[1] if a[0] > 0 else -a[1]


class _Sums:
    def __init__(self, plan, done, start=lambda k: None):
        self.shared, self.rows = plan
        self.done, self.start = done, start
        self.terms, self.sums = {}, [None] * len(self.rows)
        for k, row in enumerate(self.rows):
            if not row and (first := start(k)) is not None:
                done(k, first)

    def add(self, name, sign, value):
        self.terms[name] = sign, value
        for k, row in enumerate(self.rows):
            if name in row:
                if self.sums[k] is None and (first := self.start(k)) is not None:
                    self.sums[k] = 1, first
                self.sums[k] = _acc(self.sums[k], row[name] * sign, value)
                if all(n in self.terms for n in row):
                    self.done(k, _val(self.sums[k]))
        for n, (a, b, s) in self.shared.items():
            if name in (a, b) and a in self.terms and b in self.terms and n not in self.terms:
                self.add(n, *_acc(self.terms[a], s * self.terms[b][0], self.terms[b][1]))


def _share(tasks, k, n):
    return list(tasks[k * len(tasks) // n:(k + 1) * len(tasks) // n])


def _merge(a, b):
    return [t for k in range(len(a)) for t in [a[k]] + _share(b, k, len(a))]


def _run(tasks):
    for task in tasks:
        task()


def _each(f, items, *args):
    return [task for item in items for task in f(item, *args)]


def _kernel(ax_hbm, awqkv_hbm, awo_hbm, bx_hbm, mem_hbm, wq_hbm, wk_hbm, wv_hbm, wo_hbm,
            out_hbm,
            ax, awqkv, awo, tmp, wa, xb, q_s, kv_s, oa_s, outa,
            bx, mem, raw, wo_raw, plain, summed, wo, h0, first, lhs, m_s, part, tok, ring,
            ox, mixed, opart, outb,
            sem_a, sem_x, sem_w, sem_b, sem_wo, sem_o):
    cp = pltpu.make_async_copy

    def rows_copy(src, dst, rows, sem):
        return [cp(src.at[rows, :], dst.at[rows, :], sem)]

    c_aw = [cp(awqkv_hbm.at[r0:r1, _ds(j, D)], awqkv.at[j, r0:r1], sem_a.at[k])
            for k, (j, r0, r1) in enumerate(((0, 0, 256), (0, 256, D), (1, 0, D), (2, 0, D)))]
    c_awo = [cp(awo_hbm, awo, sem_a.at[4])]
    c_bx0 = [cp(mem_hbm, mem.at[0:M], sem_b.at[0])] + rows_copy(bx_hbm, bx, slice(0, 6 * SEG), sem_b.at[1])
    c_bx1 = rows_copy(bx_hbm, bx, slice(6 * SEG, S), sem_b.at[2])
    c_outa = [cp(outa, out_hbm.at[:, 0:D], sem_o.at[0])]

    def c_ax(c):
        return rows_copy(ax_hbm, ax, _ds(c, 2 * TB), sem_x.at[c])

    def c_w(c):
        return [cp(w.at[_ds(c, GW * 128), :], raw.at[_ds((c & (RAW - 1)) * 3 + j, GW * 128), :], sem_w.at[c, j])
                for j, w in enumerate((wq_hbm, wk_hbm, wv_hbm))]

    def c_wo(g):
        return rows_copy(wo_hbm, wo_raw, _ds(g, GW * 128), sem_wo.at[g])

    def c_outb(rows):
        return [cp(outb.at[rows, :], out_hbm.at[rows, D:], sem_o.at[1])]

    def start(copies):
        for c in copies:
            c.start()

    def wait(copies):
        for c in copies:
            c.wait()
        recent.clear()

    recent = []

    def hold(x, zero, back):
        if len(recent) < back:
            return x
        late = recent[-back] if x.dtype == F32 else pltpu.bitcast(recent[-back], U32)
        return jnp.where(lax.broadcasted_iota(jnp.int32, x.shape, 0) >= zero, x, late)

    def tile(ref, i, j):
        return pltpu.bitcast(ref[_ds(i, 64), _ds(j, 128)], BF16)

    def prep_a(j):
        def task(t):
            tmp[t] = awqkv[j, _ds(t, 128), :].astype(F32).T if j < 3 else awo[:, _ds(t, 128)].astype(F32)
            w = _cat(*[tmp[t, pl.ds(d, AH, stride=AD), :] for d in range(AD)])
            wa[_ds(j, D // 2), _ds(t, 128)] = pltpu.bitcast(w.astype(BF16), U32)

        return [functools.partial(task, t) for t in range(LT)]

    def by_tile(product, put):
        acc = [None]

        def task(t, k):
            r = product(t, k)
            e = len(recent) % 16
            recent.extend(r[8 * (e + i) % TB:8 * (e + i) % TB + 8] for i in range(4))
            acc[0] = _add(acc[0] if k else None, r)
            if k == LT - 1:
                put(t, acc[0])

        return [functools.partial(task, t, k) for t in range(LT) for k in range(LT)]

    def a_load(c):
        xb[...] = pltpu.bitcast(ax[_ds(c, 2 * TB), :], U32)

    def a_proj(i, b, j):
        def put(t, r):
            if j == 0:
                q_s[b, t] = r
                return
            c = (j - 1) * LT + t
            kv_s[b, c, HALO:, :] = r
            if isinstance(i, int) and i == 0:
                kv_s[b, c, 0:HALO, :] = jnp.broadcast_to(r[0:1, :], (HALO, 128))
            else:
                kv_s[b, c, 0:HALO, :] = kv_s[1 - b, c, TB:, :]

        return by_tile(lambda t, k: lax.dot_general(
            tile(xb, b, k), tile(wa, j * LT + t, k), NT, preferred_element_type=F32), put)

    def a_attention(b, zero, first_block=False):
        state = {}

        def window(c, r0, w):
            lo = HALO + r0 - ADIL * w
            return kv_s[b, c, lo:lo + RC, :]

        def logits(r0):
            q = [hold(q_s[b, t, r0:r0 + RC, :], zero, CFG["aback"]) for t in range(LT)]
            state[r0] = []
            for w in range(AW):
                a = q[0] * window(0, r0, w)
                for t in range(1, LT):
                    a = a + q[t] * window(t, r0, w)
                state[r0].append(a + pltpu.roll(a, 2 * AH, 1))

        def fold(r0):
            state[r0] = [a + pltpu.roll(a, AH, 1) for a in state[r0]]

        def weigh(r0):
            scale = AD ** -0.5
            lg = []
            for w, a in enumerate(state.pop(r0)):
                if first_block and r0 < ADIL * w:
                    pos = lax.broadcasted_iota(jnp.int32, (RC, 128), 0) + r0
                    a = jnp.where(pos >= ADIL * w, a, MASKED / scale)
                lg.append(a)
            m = hold(functools.reduce(jnp.maximum, lg), zero, CFG["aback"])
            p = [jnp.exp2((a - m) * (scale * math.log2(math.e))) for a in lg]
            state[r0] = p, 1.0 / functools.reduce(jnp.add, p)

        def mix(r0):
            p, inv = state.pop(r0)
            for t in range(LT):
                o = p[0] * window(LT + t, r0, 0)
                for w in range(1, AW):
                    o = o + p[w] * window(LT + t, r0, w)
                oa_s[b, r0:r0 + RC, _ds(t, 128)] = o * inv

        n = TB // RC
        return [functools.partial(f, (k - lag) * RC) for k in range(n + 2)
                for lag, f in ((0, logits), (1, fold), (2, weigh), (2, mix)) if 0 <= k - lag < n]

    def a_out(i, b):
        def put(t, r):
            outa[_ds(i, TB), _ds(t, 128)] = r.astype(BF16)

        return by_tile(lambda t, k: _dot(oa_s[b, :, _ds(k, 128)], tile(wa, 3 * LT + k, t)), put)

    def transposes(c, dst, g):
        def task(n):
            t = ((c & (RAW - 1)) * 3 + n % 9 // 3) * GW + n // 9 * 3 + n % 3
            v = pltpu.bitcast(raw[_ds(t, 128), :].T, U32)
            for k in range(LT):
                dst[_ds(g * GW + n, 64), _ds(k, 128)] = v[k * 64:(k + 1) * 64]

        return [functools.partial(task, n) for n in range(3 * GW)]

    def derive(block, put, zero):
        marks = []
        n = CFG["split"]

        def mark():
            marks.append(len(recent) - CFG["back"])

        def task():
            def done(r, v):
                if r not in SINGLE:
                    put(r, pltpu.bitcast(v.astype(BF16), U32))

            sums = _Sums(WEIGHTS[1], done)
            always = lax.broadcasted_iota(jnp.int32, (64, 128), 0) >= zero
            for k in range(n):
                for i, b in enumerate(_share(WEIGHTS[0], k, n)):
                    v = block(*divmod(b, GW))
                    if i % CFG["hb"] == 0:
                        late = [recent[t] if t >= 0 else jnp.zeros((8, 128), F32) for t in marks[k::n]]
                        v = lax.select(always, v, pltpu.bitcast(_cat(*late), U32))
                    for r in SINGLE:
                        if SINGLE[r] == b:
                            put(r, v)
                    sums.add(b, 1, pltpu.bitcast(v, BF16).astype(F32))

        return [mark] * (8 * n) + [task]

    def derive_qkv(g, zero, src=plain, dst=summed):
        def put(r, v):
            if r not in SINGLE:
                i, j = divmod(SUMMED.index(r), LT)
                dst[_ds(g * 8 + i, 64), _ds(j, 128)] = v

        return derive(lambda k, n: src[_ds(g * GW + n, 64), _ds(k, 128)], put, zero)

    def derive_out(g, zero):
        def put(r, v):
            wo[_ds(g, 64), _ds(r, 128)] = v

        return derive(lambda k, n: pltpu.bitcast(wo_raw[_ds(g * GW + n, 128), _ds(k, 128)], U32), put, zero)

    PAD = 3

    def prologue():
        start(c_aw[:2])
        wait(c_aw[:1])
        start(c_ax(0))
        _run(prep_a(0)[:2])
        wait(c_aw[1:2])
        start(c_aw[2:3])
        _run(prep_a(0)[2:])
        wait(c_ax(0))
        start(c_aw[3:])
        a_load(0)
        _run(a_proj(0, 0, 0) + a_proj(1, 1, 0)[:CFG["nq"]])
        wait(c_aw[2:3])
        start(c_awo + c_ax(1))
        _run(a_proj(1, 1, 0)[CFG["nq"]:] + prep_a(1) + a_proj(0, 0, 1))
        wait(c_aw[3:])
        start(c_w(0))
        side = a_attention(0, 0, first_block=True)
        _run(a_proj(1, 1, 1) + prep_a(2) + [t for t in side if t.func.__name__ != "mix"] + a_proj(0, 0, 2))
        wait(c_awo)
        start(c_bx0)
        _run(_merge(a_proj(1, 1, 2), _merge([t for t in side if t.func.__name__ == "mix"], prep_a(3))))

    def a_step(it, carry):
        g = jnp.maximum(3 * it - 9 + PAD, 0)
        zero = it >> 16
        more = it + 1 < NB // 2
        pl.when(more)(lambda: start(c_ax(it + 1)))
        pl.when(~more)(lambda: start(c_wo(0)))
        wait(c_ax(it))
        pl.when(more)(lambda: start(c_w(it)))
        pl.when(~more)(lambda: start(c_wo(1) + c_wo(2)))
        pl.when(it > 1)(lambda: wait(c_w(it - 2)))
        a_load(it)
        src, dst = [ref.at[pl.ds(pl.multiple_of(g * n, n), k * n)]
                    for ref, n, k in ((plain, GW * 64, 6), (summed, 8 * 64, 3))]
        side = _merge(_each(derive_qkv, range(CFG["nd"]), zero, src, dst), transposes(it + RAW - 2, src, 3))
        for b in range(2):
            i = 2 * it + b
            main = a_proj(i, b, 0) + a_proj(i, b, 1) + a_proj(i, b, 2) + a_out(i - 2, b)
            _run(_merge(main, _merge(a_attention(1 - b, zero), _share(side, b, 2))))
        return zero

    if not CFG["only"]:
        prologue()
        zero = lax.fori_loop(1, NB // 2, a_step, 0)

    def attention(qkv, put, rows=slice(0, L)):
        n = rows.stop - rows.start
        row = lax.broadcasted_iota(jnp.int32, (n, 2 * L), 0) + rows.start
        col = lax.broadcasted_iota(jnp.int32, (n, 2 * L), 1)
        head0 = col < L
        visible = (row < M) | (row >= jnp.where(head0, col, col - L))
        scale = DH ** -0.5
        st = {}

        def by_head(n):
            t = qkv(n)
            if n % 3 == 1:
                low = lax.broadcasted_iota(jnp.int32, t.shape, 1) < 64
                t = _cat(jnp.where(low, t, 0.0), jnp.where(low, 0.0, t))
            elif n % 3 == 2:
                t = _cat(jnp.zeros_like(t), t)
            return t.astype(BF16)

        def score(p):
            sc = [lax.dot_general(qkv(9 * p + t), by_head(9 * p + 3 + t), NT, preferred_element_type=F32)
                  for t in range(3)]
            PLAN["events"].setdefault(PLAN["n"], []).extend((24, 40, 40))
            sc = _add(_add(jnp.concatenate([sc[0], jnp.zeros_like(sc[0])], axis=1), sc[1]), sc[2])
            sc = jnp.where(visible, sc, MASKED / scale)
            m0 = jnp.max(jnp.where(head0, sc, -jnp.inf), axis=1, keepdims=True)
            m1 = jnp.max(jnp.where(head0, -jnp.inf, sc), axis=1, keepdims=True)
            st[p] = sc - jnp.where(head0, m0, m1)

        def normalize(p):
            e = jnp.exp2(st[p] * (scale * math.log2(math.e)))
            l0 = jnp.sum(jnp.where(head0, e, 0.0), axis=1, keepdims=True)
            l1 = jnp.sum(jnp.where(head0, 0.0, e), axis=1, keepdims=True)
            l = jnp.where(head0, l0, l1)
            if CFG["rcp"]:
                r = pl.reciprocal(l, approx=True)
                st[p] = e * (r * (2.0 - l * r))
            else:
                st[p] = e / l

        def mix(p):
            PLAN["events"].setdefault(PLAN["n"], []).extend((12, 20, 20))
            for t in range(3):
                put(3 * p + t, _dot(st[p] if t else st[p][:, :L], by_head(9 * p + 6 + t)))

        return score, normalize, mix

    def mixed_at(n):
        return [(ref, n - g0 * GW) for ref, (g0, g1) in zip(mixed, CHUNKS) if g0 <= n // GW < g1][0]

    def put_x(n, r):
        ref, k = mixed_at(n)
        ref[k, 0:M] = r[0:M]
        ox[n] = r[M:]

    def put_y(n, r):
        ref, k = mixed_at(n)
        ref[k] = _cat(r[0:M], ox[n] - r[M:], r[M:])

    def prep_tokens(s, zero):
        def task(e):
            x, y = [bx[_ds((s + k) * (SEG // M) + e, M), :].astype(F32) for k in range(2)]
            x = [x[:, k * 128:(k + 1) * 128] for k in range(LT)]
            y = [hold(y[:, k * 128:(k + 1) * 128], zero, CFG["hp"] * (LT - k)) for k in range(LT)]
            z = [a + b for a, b in zip(x, y)]
            for r in range(NR):
                lhs[r, _ds(e + e // 2, M)] = _val(_sum((a or b, z[k] if a and b else x[k] if a else y[k])
                                              for k, (a, b) in enumerate(MODEL[r]) if a or b))

        return [functools.partial(task, e) for e in range(SEG // M)]

    def step(s, second, zero):
        def reread(ref):
            return ref.at[pl.ds(4 * zero, ref.shape[0])]

        part_r, lhs_r, ring_r = reread(part), reread(lhs), [reread(r) for r in ring]
        halves = [slice(0, HS), slice(HS, SEG)][::1 - 2 * second]
        due = []

        def mm(x, w):
            r = _dot(x, w)
            recent.append(r[0:M] if second and len(recent) > CFG['tp'] - 40 else None)
            while due and due[0][0] <= len(recent):
                due.pop(0)[1]()
            return r

        def in_turn(items):
            lists = [[x for x in items if (x[0] >= BOTH) == e] for e in (False, True)]
            PLAN["blocks"].append(tuple(len(x) for x in lists))
            for x in items:
                if PLAN["seq"]:
                    x = lists[int(PLAN["seq"][PLAN["n"]])].pop(0)
                PLAN["n"] += 1
                yield x

        def needs(r):
            return [CFG["mo"][k] for k, c in enumerate(MODEL[r]) if c[second]]

        def project(g):
            order, plans = PROJECT[second]

            def token_sums(e):
                def begin(k):
                    return part_r[g, k, halves[e]] if second and PROJECT[0][1][1 - e][1][k] else None

                def done(k, v):
                    n = GW * g + k // 2
                    if not second:
                        part[g, k, halves[e]] = v
                    elif k % 2:
                        tok[n, halves[e]] = v
                    else:
                        ring[n // 3 % RING][n % 3, pl.ds(M + halves[e].start, HS)] = v

                return _Sums(plans[e], done, begin)

            def done(k, v):
                n = GW * g + k
                ring[n // 3 % RING][n % 3, 0:M] = v

            sums = token_sums(0), token_sums(1), _Sums(plans[2], done)
            weights = pltpu.bitcast(summed[_ds(PAD + g, 8 * 64), :], BF16)
            if g == 0:
                order = sorted(order, key=lambda r: max(needs(r)))
            for r, in in_turn([(r,) for r in order]):
                t0, t1 = (0, L) if r < BOTH else (second * HS, second * HS + HS + M)
                if g == 0:
                    lhs[r, HS:HS + M] = _val(_sum((c[second], m_s[k]) for k, c in enumerate(MODEL[r]) if c[second]))
                if r in SINGLE:
                    w = tile(plain, (PAD + g) * GW + SINGLE[r] % GW, SINGLE[r] // GW)
                else:
                    i, j = divmod(SUMMED.index(r), LT)
                    w = weights[i * 128:(i + 1) * 128, j * 128:(j + 1) * 128]
                v = mm((lhs_r if g else lhs)[r, t0:t1], w)
                sums[2].add(r, 1, v[HS - t0:HS - t0 + M])
                if t0 == 0:
                    sums[second].add(r, 1, v[:HS])
                if t1 == L:
                    sums[1 - second].add(r, 1, v[-HS:])

        def projected(n):
            src = ring_r[n // 3 % RING]
            return src[n % 3] if second else _cat(src[n % 3, 0:M], tok[n])

        new_mem = [None] * LT

        def out_chunk(ref, g0, g1):
            order, plans = OUTPUT[second]

            def token_sums(e):
                def begin(k):
                    if (second and OUTPUT[0][1][1 - e][1][k]) or (g0 > 0 and plans[e][1][k]):
                        return opart[k, halves[e]]

                def done(k, v):
                    if second and g1 == GO:
                        outb[_ds((s + k % 2) * 2 + halves[e].start // HS, HS), _ds(k // 2, 128)] = v.astype(BF16)
                    else:
                        opart[k, halves[e]] = v

                return _Sums(plans[e], done, begin)

            def done(k, v):
                new_mem[k] = v
                if g1 == GO:
                    m_s[k] = v

            sums = token_sums(0), token_sums(1), _Sums(plans[2], done, list(new_mem).__getitem__)
            if g1 == GO:
                order = sorted(order, key=lambda r: min(needs(r)))
            weights = [pltpu.bitcast(wo[_ds(g, 64), :], BF16) for g in range(g0, g1)]
            tall, short = [[r for r in order if (r >= BOTH) == e] for e in (False, True)]
            n = len(order) // CFG["ow"]
            for k in range(n):
                acc = {}
                some = _share(tall[::-1], n - 1 - k, n)[::-1] + _share(short, k, n)
                for r, g in in_turn([(r, g) for g in range(g0, g1) for r in some]):
                    t0, rows = (0, SEG) if r < BOTH else (halves[0].start, HS)
                    terms = []
                    for j, (a, b) in enumerate(FEATURE[r]):
                        i = (g - g0) * GW + j
                        if a and not b and second:
                            terms += [(a, ref[i, pl.ds(r0 + t0, rows)]) for r0 in (M, L)]
                        elif a and not b:
                            terms.append((a, ox[g * GW + j, pl.ds(t0, rows)]))
                        elif b:
                            terms.append((a or b, ref[i, pl.ds((M if a else L) + t0, rows)]))
                    sign, left = _sum(terms)
                    m_sign, m = _sum((c[second], ref[(g - g0) * GW + j, 0:M])
                                     for j, c in enumerate(FEATURE[r]) if c[second])
                    v = _add(acc[r][2] if r in acc else None, mm(_cat(m, left), weights[g - g0][:, r * 128:(r + 1) * 128]))
                    acc[r] = m_sign, sign, v
                for r, (m_sign, sign, v) in acc.items():
                    sums[2].add(r, m_sign, v[:M])
                    sums[second if r < BOTH else 0].add(r, sign, v[M:M + HS])
                    if r < BOTH:
                        sums[1 - second].add(r, sign, v[M + HS:])

        recent.clear()
        stages = attention(projected, put_x if second else put_y)
        for p in range(NP):
            ready = LT * GW * ((9 * p + 5) // GW + 1)
            due += [(ready + CFG[lag], functools.partial(f, p)) for f, lag in zip(stages, ("ds", "dn", "dp"))]
        if second:
            due += [(CFG["tp"] + k * CFG["dt"], task)
                    for k, task in enumerate(prep_tokens(jnp.minimum(s + 4, NSEG - 2), zero))]
        due.sort(key=lambda e: e[0])
        for g in range(GQ):
            project(g)
        for ref, chunk in zip(mixed, CHUNKS):
            out_chunk(reread(ref), *chunk)

    def first_segment():
        def project(g):
            acc = {}

            def task(n, k):
                r = _dot(h0[0:L + SEG, _ds(k, 128)], tile(plain, PAD * GW + n, k))
                e = len(recent) % 8
                recent.extend([r[8 * e:8 * e + 8], r[8 * e + 8:8 * e + 16]])
                acc[n] = _add(acc.get(n), r)
                if k == LT - 1:
                    first[n] = acc[n][0:L]
                    tok[n] = acc[n][L:]

            return [functools.partial(task, g * GW + n, k) for n in range(GW) for k in range(LT)]

        def put(n, r):
            recent.extend([r[k:k + 8] for k in range(0, L, 16)])
            put_x(n, r)

        stages = attention(lambda n: first[n], put)
        acc = [None] * LT

        def heads(p0, p1):
            return [functools.partial(f, t - lag) for t in range(p0, p1 + 2)
                    for lag, f in enumerate(stages) if p0 <= t - lag < p1]

        def out(g):
            def task(n, k):
                ref, i = mixed_at(n)
                r = _dot(ref[i, 0:M], wo_raw[_ds(n, 128), _ds(k, 128)])
                recent.append(r)
                acc[k] = r if acc[k] is None else acc[k] + r

            return [functools.partial(task, g * GW + n, k) for n in range(GW) for k in range(LT)]

        c1, c2, c3 = CFG["cut"]
        todo = [PAD + g for g in range(GQ) if g >= 15 or g % 3 >= CFG["nd"]]
        d1, d2 = [todo.index(PAD + g) for g in CFG["dc"]]
        start(c_w(GO - 1))
        wait(c_w(GO - 2) + c_wo(0) + c_bx0)
        h0[0:M, :] = mem[0:M, :].astype(F32)
        h0[M:L + SEG, :] = bx[0:2 * SEG, :].astype(F32)
        _run(_merge(a_out(NB - 2, 0) + _each(project, range(c1)),
                    _merge(_each(derive_qkv, todo[:d1], zero) + derive_out(0, zero),
                           _merge(a_attention(1, zero), transposes(GO - 2, plain, PAD + GQ - 6)))))
        start(c_wo(3))
        wait(c_wo(1) + c_wo(2))
        start(c_wo(4) + c_wo(5))
        _run(_merge(a_out(NB - 1, 1) + _merge(_each(project, range(c1, c2)), heads(0, 6)),
                    _each(derive_qkv, todo[d1:d2], zero) + _each(derive_out, (1, 2), zero)))
        wait(c_w(GO - 1) + c_wo(3))
        start(c_wo(6))
        _run(_merge(_merge(_each(project, range(c2, c3)), _merge(out(0) + out(1), heads(6, 12))),
                    _merge(_each(derive_qkv, todo[d2:-3], zero) + derive_out(3, zero),
                           transposes(GO - 1, plain, PAD + GQ - 3)) + _each(derive_qkv, todo[-3:], zero)))
        start(c_wo(7))
        wait(c_wo(4) + c_wo(5))
        _run(_merge(_each(project, range(c3, GQ)) + _merge(_each(out, range(2, 6)), heads(12, NP)),
                    _merge(_each(derive_out, (4, 5), zero), prep_tokens(2, zero))))
        wait(c_wo(6) + c_wo(7))
        start(c_bx1 + c_outa)
        _run(_merge(out(6) + out(7), _each(derive_out, (6, 7), zero)))
        for k in range(LT):
            m_s[k] = acc[k]

    def b_step(it, carry):
        if not CFG["only"]:
            pl.when(it == 1)(lambda: wait(c_bx1))
        PLAN.update(n=0, blocks=[], events={})
        step(2 * it, 0, it >> 16)
        step(2 * it, 1, it >> 16)
        PLAN["n"] = -1
        start(c_outb(_ds(it, 2 * SEG)))
        return carry

    def last_segment():
        res, acc = {}, [None] * LT

        def project(n, k):
            r = _dot(-m_s[k] if k % 2 else m_s[k], tile(plain, PAD * GW + n, k))
            res[n] = _acc(res.get(n), 1 - 2 * (k % 2), r)

        def out(n, k):
            acc[k] = _add(acc[k], _dot(_cat(ox[n], res[NQ + n]), wo_raw[_ds(n, 128), _ds(k, 128)]))

        stages = attention(lambda n: _cat(_val(res[n]), tok[n]) if n in res else tok[n],
                           lambda n, r: res.update({NQ + n: r}), slice(M, L))
        short = [functools.partial(project, n, k) for n in range(NQ) if n % 9 >= 3 for k in range(LT)]
        tall = [functools.partial(out, n, k) for n in range(NO) for k in range(LT)]
        lag = CFG["lo"]
        for t in range(len(tall) // 4 + lag):
            _run(short[8 * t:8 * t + 8])
            if t >= lag:
                _run(tall[4 * (t - lag):4 * (t - lag) + 4])
            for p in range(0, NP, 2):
                for f, late in list(zip(stages, CFG["ls"]))[::-1]:
                    if t == (30 * (p + 2) - 1) // 8 + late:
                        f(p)
                        f(p + 1)
        outb[S - 2 * SEG:, :] = jnp.concatenate(acc, axis=1).astype(BF16)
        start(c_outb(slice(S - 2 * SEG, S)))

    if CFG["only"]:
        for ref in (plain, summed, wo):
            ref[0:8, 0:128] = jnp.zeros((8, 128), U32)
        lax.fori_loop(0, CFG["nper"], b_step, 0)
        wait(c_outb(slice(0, CFG["nper"] * 2 * SEG)))
        return
    first_segment()
    lax.fori_loop(0, CFG["nper"], b_step, 0)
    last_segment()
    wait(c_outa + c_outb(slice(0, (CFG["nper"] + 1) * 2 * SEG)))


def pallas_concat_heads__sliding_local_dilated__memory_aug_recurrent_mem_tr__prompt_kernel(
    A_x, A_wqkv, A_wo, B_x, B_mem0, B_Wq, B_Wk, B_Wv, B_Wo, B_seg_len,
):
    assert B_seg_len == SEG
    assert A_x.shape == B_x.shape == (1, S, D) and B_mem0.shape == (1, M, D)
    assert B_Wq.shape == B_Wk.shape == B_Wv.shape == (D, H, DH) and B_Wo.shape == (H, DH, D)
    dma = pltpu.SemaphoreType.DMA

    def vmem(shape, dtype):
        assert math.prod(shape) * jnp.dtype(dtype).itemsize % 16384 == 0, shape
        return pltpu.VMEM(shape, dtype)

    call = pl.pallas_call(
        lambda *refs: _kernel(*refs),
        out_shape=jax.ShapeDtypeStruct((S, 2 * D), BF16),
        in_specs=[pl.BlockSpec(memory_space=pl.ANY)] * 9,
        out_specs=pl.BlockSpec(memory_space=pl.ANY),
        scratch_shapes=[
            vmem((S, D), BF16),
            vmem((3, D, D), BF16),
            vmem((D, D), BF16),
            vmem((LT, D, 128), F32),
            vmem((2 * D, D), U32),
            vmem((TB, D), U32),
            vmem((2, LT, TB, 128), F32),
            vmem((2, 2 * LT, HALO + TB, 128), F32),
            vmem((2, TB, D), F32),
            vmem((S, D), BF16),
            vmem((S, D), BF16),
            vmem((8 * M, D), BF16),
            vmem((RAW * 3 * GW * 128, D), BF16),
            vmem((H * DH, D), BF16),
            vmem(((3 + GQ) * GW * 64, D), U32),
            vmem(((3 + GQ) * 8 * 64, D), U32),
            vmem((GO * 64, NR * 128), U32),
            vmem((3 * SEG, D), F32),
            vmem((NQ, L, 128), F32),
            vmem((NR + 1, L, 128), F32),
            vmem((8, M, 128), F32),
            vmem((GQ, 2 * GW, SEG, 128), F32),
            vmem((NQ, SEG, 128), F32),
            [vmem((4, L, 128), F32)] * RING,
            vmem((NO, SEG, 128), F32),
            [vmem((20, L + SEG, 128), F32)] * len(CHUNKS),
            vmem((2 * LT, SEG, 128), F32),
            vmem((S, D), BF16),
            dma((5,)), dma((NB // 2,)), dma((GO, 3)), dma((3,)), dma((GO,)), dma((2,)),
        ],
        compiler_params=pltpu.CompilerParams(vmem_limit_bytes=126 * 1024 * 1024, flags=CFG["flags"]),
        name="sliding_and_memory_attention",
    )

    def by_feature(w):
        return w.transpose(1, 2, 0).reshape(H * DH, D)

    out = call(A_x.reshape(S, D), A_wqkv, A_wo, B_x.reshape(S, D), B_mem0.reshape(M, D),
               by_feature(B_Wq), by_feature(B_Wk), by_feature(B_Wv), B_Wo.reshape(H * DH, D))
    return out.reshape(1, S, 2 * D)
```

```python
import collections
import functools
import itertools
import math
import random

import jax
import jax.numpy as jnp
import numpy as np
from jax import lax
from jax.experimental import pallas as pl
from jax.experimental.pallas import tpu as pltpu

F32, BF16, U32 = jnp.float32, jnp.bfloat16, jnp.uint32
NT = (((1,), (1,)), ((), ()))
MASKED = -1000000000.0

S, D = 2048, 640
LT = D // 128

AH, AD, AW, ADIL = 32, 20, 8, 2
HALO = 16
TB = 128
NB = S // TB
RC = 8

H, DH, M, SEG = 32, 192, 8, 32
L = M + SEG
HS = SEG // 2
NP = H // 2
NSEG = S // SEG
NO = 3 * NP
NQ = 3 * NO
GW = 6
GO, GQ = NO // GW, NQ // GW
RAW = 4
RING = 12
CHUNKS = ((0, 3), (3, 5), (5, GO))

CFG = dict(nper=(NSEG - 2) // 2, flags=None, back=18, aback=12, split=10, hb=3, nq=5, nk=20, t0=3, nd=3, nl=1, nm=3, alag=5, m1=6, m2=12, ea=4, eb=0, sc=62,
           ds=40, dn=70, dp=100, tp=740, dt=25, hp=3, rcp=1, ow=6, mo=(0, 1, 4, 2, 3),
           ls=(7, 12, 3, 7), lo=3, lg=1.9, tau=8, drift=1.5, ext=1, only=0, cut=(5, 12, 21), dc=(17, 21), qc=6)
PLAN = dict(blocks=[], events={}, n=0, seq="100001001010100101010100101101001001001100101010010100101101001010010011010100010100101110000101100101001001010100101101001100001011110000011010010110100001110001010010010101100101001001011001000111010001010110000101001100111100000100101101001010100100100101101001011010000101100100101100101001011010000111000011101000011010001110100010010100110010101100001110000110010010110010100100101011001010100011110000010110100101001011100000101100011001001110000101101010010001010110010101000110001100111000010110001101000110100010100101101001011010000101101000101001011010010110000110001100111000011100001101001001101000100101011001010110000101101000101101001010010110000110001100110100100101011001000101100010101100101011000011000010010101000011100001011010011110000011000010100011001010110010100111100001011010010111000010011010100011000111100000100101101000011110000111000111000010100101001010010100101001011011010000101000010110100001011010011110000101101001011011010010100101001010010100101101001010010100101001011010001101001001100010101100011000101101010001001010110001101000111010000110001100110100101001011010000101010010110010100101101001011000011001000111010000111100001100001100111000011110000101001011100000101100011010001110000110100100110100101001011010000101101001010010100101101001001001001011100001011010010110000110101010000110100100101101001001011000100101101001001011010010100010100101101001011010000101101000101101001010010110000110001100110100101001011010000101100011010010100101001011001001010101001010110000111100001100001100111100001100001101001011100000101100011010001110000110100100110100101001011010000101101001010010100101001011010010001010110001101000111010000100011001000011101000010110010111000010010101000011010001100101011101000110010101101101001000011001000111010101000010010101000110011101000101011101000010010101000110010100100101011011010000011000010110010001010110011101000101011001011110")


def _algorithm(rank_ones):
    rows = np.array([[1, 0], [0, 1], [1, 1]])
    duals = np.array([[0, 1], [1, 0], [1, -1]])
    sets = [[[np.array(["-0+".index(c) - 1 for c in w]) for w in e.split()] for e in s] for s in rank_ones]
    left, right = [], []
    for t, s in enumerate(sets):
        p, q = [k for k in range(3) if k != t]
        for u, v in s:
            left += [np.outer(u, rows[p]), np.outer(u, rows[q])]
            right += [np.outer(v, duals[q]), np.outer(v, duals[p])]
    for (u0, v0), (u1, v1), (u2, v2) in itertools.product(*sets):
        for a, b in itertools.product((1, -1), repeat=2):
            e = np.outer(u0 + a * u1, v0 + b * v1)
            if (e == np.outer(u2, v2)).all() or (e == -np.outer(u2, v2)).all():
                left.append(np.outer(u0, rows[1]) - a * np.outer(u1, rows[0]))
                right.append(np.outer(v0, duals[1]) + b * np.outer(v1, duals[0]))
    left, right = np.array(left), np.array(right)
    have = np.einsum("rka,rnb->kanbr", left, right).reshape(-1, len(left))
    want = np.einsum("kp,nq,ab->kanbpq", np.eye(LT), np.eye(GW), np.eye(2)).reshape(len(have), -1)
    blocks = np.rint(np.linalg.lstsq(have, want, rcond=None)[0]).astype(int)
    assert (have @ blocks == want).all()
    sign = blocks.max(axis=1) * 2 - 1
    return left * sign[:, None, None], blocks * sign[:, None], right


def _shared_sums(matrix, seed):
    rng = random.Random(seed)
    rows = [{k: int(c) for k, c in enumerate(row) if c} for row in matrix]
    shared = {}
    while True:
        count = collections.Counter(
            (a, b, r[a] * r[b]) for r in rows for a, b in itertools.combinations(sorted(r), 2))
        top = max(count.values(), default=0)
        if top < 2:
            return shared, rows
        best = sorted(k for k, n in count.items() if n == top)
        a, b, sign = best[int(rng.random() * len(best))]
        name = matrix.shape[1] + len(shared)
        shared[name] = a, b, sign
        for r in rows:
            if r.get(a, 0) * r.get(b, 0) == sign:
                r[name] = r.pop(a)
                del r[b]


MODEL, BLOCKS, FEATURE = _algorithm((
    ("+0000 +00++0", "000+0 0+0000", "0000+ 000+00", "+-+00 00000+", "+00+0 00+0+0"),
    ("0+00+ 000+++", "0+0+0 0+00++", "00+-+ 00++00", "00+0+ +00000", "+0+00 0000+0", "00+00 0+-000"),
    ("0+000 0000++", "00+-+ ++0000", "00+00 +00+00", "+-000 0+-00+", "00+-0 00+000", "+-00- +0000-")))
NR, BOTH = 47, 34
SINGLE = {r: int(row.argmax()) for r, row in enumerate(BLOCKS) if abs(row).sum() == 1}
SUMMED = [r for r in range(NR) if r not in SINGLE]


def _step_plan(out, step, seed, order):
    use = MODEL[:, :, step].any(1) & FEATURE[:, :, step].any(1)
    assert sorted(order) == np.nonzero(use)[0].tolist()
    return order, [_shared_sums((m * keep[:, None]).T, seed) for m, keep in (
        (out.reshape(NR, -1), use), (out.reshape(NR, -1), use & (np.arange(NR) < BOTH)), (out[:, :, step], use))]


PROJECT = (
    _step_plan(FEATURE, 0, 32, (30, 14, 20, 3, 28, 12, 9, 22, 10, 18, 1, 26, 24, 5, 32, 16, 7,
                                40, 38, 36, 44, 45, 46, 39, 34, 35, 43, 37, 41, 42)),
    _step_plan(FEATURE, 1, 5, (31, 15, 4, 11, 27, 0, 8, 19, 23, 13, 33, 6, 29, 21, 2, 25, 17,
                               40, 34, 39, 41, 35, 46, 45, 36, 43, 44, 38, 37, 42)))
OUTPUT = (
    _step_plan(MODEL, 0, 0, (24, 14, 10, 5, 32, 28, 16, 30, 22, 12, 7, 9, 3, 1, 18, 26, 20,
                             40, 34, 39, 41, 42, 37, 36, 45, 43, 44, 46, 35, 38)),
    _step_plan(MODEL, 1, 6, (23, 11, 13, 2, 15, 17, 4, 25, 31, 33, 6, 29, 8, 21, 19, 0, 27,
                             39, 36, 45, 40, 34, 41, 37, 42, 44, 43, 46, 35, 38)))
WEIGHTS = ((3, 28, 6, 0, 5, 17, 11, 8, 10, 7, 4, 16, 2, 1, 23, 22, 9, 29, 24, 19, 12, 18, 25, 13, 14, 20,
            21, 15, 26, 27), _shared_sums(BLOCKS, 37))


def _ds(i, n):
    return pl.ds(i * n if isinstance(i, int) else pl.multiple_of(i * n, n), n)


def _dot(a, b):
    return jnp.dot(a, b, preferred_element_type=F32)


def _cat(*parts):
    return jnp.concatenate(parts, axis=0)


def _add(a, b):
    return b if a is None else _cat(a[:M] + b[:M], a[M:] + b[M:])


def _acc(a, sign, b):
    if a is None:
        return sign, b
    if a[0] == sign:
        return sign, a[1] + b
    return (1, a[1] - b) if a[0] > 0 else (1, b - a[1])


def _sum(terms):
    return functools.reduce(lambda a, t: _acc(a, *t), terms, None)


def _val(a):
    return a[1] if a[0] > 0 else -a[1]


class _Sums:
    def __init__(self, plan, done, start=lambda k: None):
        self.shared, self.rows = plan
        self.done, self.start = done, start
        self.terms, self.sums = {}, [None] * len(self.rows)
        for k, row in enumerate(self.rows):
            if not row and (first := start(k)) is not None:
                done(k, first)

    def add(self, name, sign, value):
        self.terms[name] = sign, value
        for k, row in enumerate(self.rows):
            if name in row:
                if self.sums[k] is None and (first := self.start(k)) is not None:
                    self.sums[k] = 1, first
                self.sums[k] = _acc(self.sums[k], row[name] * sign, value)
                if all(n in self.terms for n in row):
                    self.done(k, _val(self.sums[k]))
        for n, (a, b, s) in self.shared.items():
            if name in (a, b) and a in self.terms and b in self.terms and n not in self.terms:
                self.add(n, *_acc(self.terms[a], s * self.terms[b][0], self.terms[b][1]))


def _share(tasks, k, n):
    return list(tasks[k * len(tasks) // n:(k + 1) * len(tasks) // n])


def _merge(a, b):
    return [t for k in range(len(a)) for t in [a[k]] + _share(b, k, len(a))]


def _run(tasks):
    for task in tasks:
        task()


def _beside(main, side, early):
    _run(_merge(main[:len(main) - early], side) + main[len(main) - early:])


def _each(f, items, *args):
    return [task for item in items for task in f(item, *args)]


def _kernel(ax_hbm, awqkv_hbm, awo_hbm, bx_hbm, mem_hbm, wq_hbm, wk_hbm, wv_hbm, wo_hbm,
            out_hbm,
            ax, awqkv, awo, tmp, wa, xb, q_s, kv_s, oa_s, outa,
            bx, mem, raw, wo_raw, plain, summed, wo, h0, first, lhs, m_s, part, tok, ring,
            ox, mixed, opart, outb,
            sem_a, sem_x, sem_w, sem_b, sem_wo, sem_o):
    cp = pltpu.make_async_copy

    def rows_copy(src, dst, rows, sem):
        return [cp(src.at[rows, :], dst.at[rows, :], sem)]

    c_aw = [cp(awqkv_hbm.at[r0:r1, _ds(j, D)], awqkv.at[j, r0:r1], sem_a.at[k])
            for k, (j, r0, r1) in enumerate(((0, 0, 128 * CFG['t0']), (0, 128 * CFG['t0'], D), (1, 0, D), (2, 0, D)))]
    c_awo = [cp(awo_hbm, awo, sem_a.at[4])]
    c_bx0 = [cp(mem_hbm, mem.at[0:M], sem_b.at[0])] + rows_copy(bx_hbm, bx, slice(0, 6 * SEG), sem_b.at[1])
    c_bx1 = rows_copy(bx_hbm, bx, slice(6 * SEG, S), sem_b.at[2])
    c_outa = [cp(outa, out_hbm.at[:, 0:D], sem_o.at[0])]

    def c_ax(c):
        return rows_copy(ax_hbm, ax, _ds(c, 2 * TB), sem_x.at[c])

    def c_w(c):
        return [cp(w.at[_ds(c, GW * 128), :], raw.at[_ds((c & (RAW - 1)) * 3 + j, GW * 128), :], sem_w.at[c, j])
                for j, w in enumerate((wq_hbm, wk_hbm, wv_hbm))]

    def c_wo(g):
        return rows_copy(wo_hbm, wo_raw, _ds(g, GW * 128), sem_wo.at[g])

    def c_outb(rows):
        return [cp(outb.at[rows, :], out_hbm.at[rows, D:], sem_o.at[1])]

    def start(copies):
        for c in copies:
            c.start()

    def wait(copies):
        for c in copies:
            c.wait()
        recent.clear()

    recent = []

    def hold(x, zero, back):
        if len(recent) < back:
            return x
        late = recent[-back] if x.dtype == F32 else pltpu.bitcast(recent[-back], U32)
        return jnp.where(lax.broadcasted_iota(jnp.int32, x.shape, 0) >= zero, x, late)

    def paced(x, zero, marks):
        if not marks:
            return x
        late = _cat(*[recent[t] if t >= 0 else jnp.zeros((8, 128), F32) for t in marks[:x.shape[0] // 8]])
        always = lax.broadcasted_iota(jnp.int32, x.shape, 1) >= zero
        return lax.select(always, x, late if x.dtype == F32 else pltpu.bitcast(late, U32))

    def tile(ref, i, j):
        return pltpu.bitcast(ref[_ds(i, 64), _ds(j, 128)], BF16)

    def prep_a(j, zero=None):
        def task(t):
            if j < 3:
                tmp[t] = awqkv[j, _ds(t, 128), :].astype(F32).T
            else:
                marks = [len(recent) - 40 + k * 3 // 4 for k in range(40)]
                tmp[t] = pltpu.bitcast(paced(pltpu.bitcast(awo[:, _ds(t, 128)], U32), zero, marks), BF16).astype(F32)
            w = _cat(*[tmp[t, pl.ds(d, AH, stride=AD), :] for d in range(AD)])
            wa[_ds(j, D // 2), _ds(t, 128)] = pltpu.bitcast(w.astype(BF16), U32)

        return [functools.partial(task, t) for t in range(LT)]

    def by_tile(product, put):
        acc = [None]

        def task(t, k):
            r = product(t, k)
            e = len(recent) % 16
            recent.extend(r[8 * (e + i) % TB:8 * (e + i) % TB + 8] for i in range(4))
            acc[0] = _add(acc[0] if k else None, r)
            if k == LT - 1:
                put(t, acc[0])

        return [functools.partial(task, t, k) for t in range(LT) for k in range(LT)]

    def a_load(i, b):
        xb[_ds(b, TB // 2), :] = pltpu.bitcast(ax[_ds(i, TB), :], U32)

    def a_proj(i, b, j):
        def put(t, r):
            if j == 0:
                q_s[b, t] = r
                return
            c = (j - 1) * LT + t
            kv_s[b, c, HALO:, :] = r
            if isinstance(i, int) and i == 0:
                kv_s[b, c, 0:HALO, :] = jnp.broadcast_to(r[0:1, :], (HALO, 128))
            else:
                kv_s[b, c, 0:HALO, :] = kv_s[1 - b, c, TB:, :]

        return by_tile(lambda t, k: lax.dot_general(
            tile(xb, b, k), tile(wa, j * LT + t, k), NT, preferred_element_type=F32), put)

    def a_attention(b, zero, first_block=False):
        n, nl, nm, lag = TB // RC, CFG["nl"], CFG["nm"], TB // RC if first_block else CFG["alag"]
        marks, state = [], []

        def mark():
            marks.append(len(recent) - CFG["aback"])

        def window(c, w):
            return kv_s[b, c, pl.ds(HALO - ADIL * w, TB), :]

        def logits():
            sums = []
            for w in range(AW):
                if w % (AW // nl) == 0:
                    q = [paced(q_s[b, t], zero, marks[w * nl // AW::nl + nm]) for t in range(LT)]
                sums.append(functools.reduce(jnp.add, [q[t] * window(t, w) for t in range(LT)]))
            chunks = {}
            for k in range(n + 1):
                if k < n:
                    a = _cat(*[a[k * RC:(k + 1) * RC] for a in sums])
                    chunks[k] = a + pltpu.roll(a, 2 * AH, 1)
                if k > 0:
                    chunks[k - 1] = chunks[k - 1] + pltpu.roll(chunks[k - 1], AH, 1)
            state[:] = [_cat(*[chunks[k][w * RC:(w + 1) * RC] for k in range(n)]) for w in range(AW)]

        def weigh():
            scale, lg = AD ** -0.5, state
            if first_block:
                pos = lax.broadcasted_iota(jnp.int32, (HALO, 128), 0)
                lg = [_cat(jnp.where(pos >= ADIL * w, a[:HALO], MASKED / scale), a[HALO:]) for w, a in enumerate(lg)]
            m = paced(functools.reduce(jnp.maximum, lg), zero, marks[lag * (nl + nm) + nl::nl + nm])
            state[:] = [jnp.exp2((a - m) * (scale * math.log2(math.e))) for a in lg]

        def mix():
            inv = 1.0 / functools.reduce(jnp.add, state)
            for t in range(LT):
                v = [window(LT + t, w) for w in range(AW)]
                if nm > 1:
                    v[0] = paced(v[0], zero, marks[lag * (nl + nm) + nl + 1 + t * (nm - 1) // LT::nl + nm])
                oa_s[b, :, _ds(t, 128)] = inv * functools.reduce(jnp.add, map(jnp.multiply, state, v))

        return [mark] * (n * (nl + nm)) + [logits], [mark] * (lag * (nl + nm)) + [weigh, mix]

    def a_out(i, b):
        def put(t, r):
            outa[_ds(i, TB), _ds(t, 128)] = r.astype(BF16)

        return by_tile(lambda t, k: _dot(oa_s[b, :, _ds(k, 128)], tile(wa, 3 * LT + k, t)), put)

    def transposes(c, dst, g):
        def task(n):
            t = ((c & (RAW - 1)) * 3 + n % 9 // 3) * GW + n // 9 * 3 + n % 3
            v = pltpu.bitcast(raw[_ds(t, 128), :].T, U32)
            for k in range(LT):
                dst[_ds(g * GW + n, 64), _ds(k, 128)] = v[k * 64:(k + 1) * 64]

        return [functools.partial(task, n) for n in range(3 * GW)]

    def derive(block, put, zero):
        marks = []
        n = CFG["split"]

        def mark():
            marks.append(len(recent) - CFG["back"])

        def task():
            def done(r, v):
                if r not in SINGLE:
                    put(r, pltpu.bitcast(v.astype(BF16), U32))

            sums = _Sums(WEIGHTS[1], done)
            for k in range(n):
                for i, b in enumerate(_share(WEIGHTS[0], k, n)):
                    v = block(*divmod(b, GW))
                    if i % CFG["hb"] == 0:
                        v = paced(v, zero, marks[k::n])
                    for r in SINGLE:
                        if SINGLE[r] == b:
                            put(r, v)
                    sums.add(b, 1, pltpu.bitcast(v, BF16).astype(F32))

        return [mark] * (8 * n) + [task]

    def derive_qkv(g, zero, src=plain, dst=summed):
        def put(r, v):
            if r not in SINGLE:
                i, j = divmod(SUMMED.index(r), LT)
                dst[_ds(g * 8 + i, 64), _ds(j, 128)] = v

        return derive(lambda k, n: src[_ds(g * GW + n, 64), _ds(k, 128)], put, zero)

    def derive_out(g, zero):
        def put(r, v):
            wo[_ds(g, 64), _ds(r, 128)] = v

        return derive(lambda k, n: pltpu.bitcast(wo_raw[_ds(g * GW + n, 128), _ds(k, 128)], U32), put, zero)

    PAD = 3

    def prologue():
        start(c_aw[:2])
        zero = lax.fori_loop(0, 2, lambda it, carry: it >> 16, 0)
        start(c_ax(0))
        wait(c_aw[:1])
        start(c_aw[2:3])
        _run(prep_a(0)[:CFG["t0"]])
        wait(c_aw[1:2])
        start(c_aw[3:])
        _run(prep_a(0)[CFG["t0"]:])
        wait(c_ax(0))
        start(c_awo)
        a_load(0, 0)
        a_load(1, 1)
        _run(a_proj(0, 0, 0) + a_proj(1, 1, 0)[:CFG["nq"]])
        wait(c_aw[2:3])
        start(c_ax(1) + c_ax(2))
        _run(a_proj(1, 1, 0)[CFG["nq"]:] + prep_a(1) + a_proj(0, 0, 1))
        wait(c_aw[3:])
        start(c_w(0))
        early, late = a_attention(0, zero, first_block=True)
        _run(a_proj(1, 1, 1)[:CFG["nk"]] + prep_a(2))
        _beside(a_proj(0, 0, 2) + [], early, 0)
        wait(c_awo + c_ax(1))
        start(c_bx0)
        _beside(a_proj(1, 1, 1)[CFG["nk"]:] + a_proj(1, 1, 2), _merge(late, prep_a(3, zero)), 4)
        a_load(2, 0)

    def a_step(it, carry):
        g = jnp.maximum(3 * it - 9 + PAD, 0)
        zero = it >> 16
        more = it + 1 < NB // 2
        pl.when(it + 2 < NB // 2)(lambda: start(c_ax(it + 2)))
        pl.when(more)(lambda: wait(c_ax(it + 1)))
        start(c_w(it))
        pl.when(it > 1)(lambda: wait(c_w(it - 2)))
        src, dst = [ref.at[pl.ds(pl.multiple_of(g * n, n), k * n)]
                    for ref, n, k in ((plain, GW * 64, 6), (summed, 8 * 64, 3))]
        sums, moves = _each(derive_qkv, range(CFG["nd"]), zero, src, dst), transposes(it + RAW - 2, src, 3)
        cut, i = len(sums) * CFG["sc"] // 100, 2 * it
        early, late = a_attention(1, zero)
        a_load(i + 1, 1)
        _beside(a_out(i - 2, 0) + _each(lambda j: a_proj(i, 0, j), range(3)),
                moves[:CFG["m1"]] + _merge(early, sums[:cut]) + moves[CFG["m1"]:CFG["m2"]], 0)
        a_load(jnp.minimum(i + 2, NB - 1), 0)
        side = sum(a_attention(0, zero), [])
        _beside(_each(lambda j: a_proj(i + 1, 1, j), range(3)) + a_out(i - 1, 1),
                _merge(_merge(side[:len(late)], late) + side[len(late):], sums[cut:]) + moves[CFG["m2"]:], CFG["ea"])
        return zero

    if not CFG["only"]:
        prologue()
        zero = lax.fori_loop(1, NB // 2, a_step, 0)

    def attention(qkv, put, rows=slice(0, L)):
        n = rows.stop - rows.start
        row = lax.broadcasted_iota(jnp.int32, (n, 2 * L), 0) + rows.start
        col = lax.broadcasted_iota(jnp.int32, (n, 2 * L), 1)
        head0 = col < L
        visible = (row < M) | (row >= jnp.where(head0, col, col - L))
        scale = DH ** -0.5
        st = {}

        def by_head(n):
            t = qkv(n)
            if n % 3 == 1:
                low = lax.broadcasted_iota(jnp.int32, t.shape, 1) < 64
                t = _cat(jnp.where(low, t, 0.0), jnp.where(low, 0.0, t))
            elif n % 3 == 2:
                t = _cat(jnp.zeros_like(t), t)
            return t.astype(BF16)

        def score(p):
            sc = [lax.dot_general(qkv(9 * p + t), by_head(9 * p + 3 + t), NT, preferred_element_type=F32)
                  for t in range(3)]
            PLAN["events"].setdefault(PLAN["n"], []).extend((24, 40, 40))
            sc = _add(_add(jnp.concatenate([sc[0], jnp.zeros_like(sc[0])], axis=1), sc[1]), sc[2])
            sc = jnp.where(visible, sc, MASKED / scale)
            m0 = jnp.max(jnp.where(head0, sc, -jnp.inf), axis=1, keepdims=True)
            m1 = jnp.max(jnp.where(head0, -jnp.inf, sc), axis=1, keepdims=True)
            st[p] = sc - jnp.where(head0, m0, m1)

        def normalize(p):
            e = jnp.exp2(st[p] * (scale * math.log2(math.e)))
            l0 = jnp.sum(jnp.where(head0, e, 0.0), axis=1, keepdims=True)
            l1 = jnp.sum(jnp.where(head0, 0.0, e), axis=1, keepdims=True)
            l = jnp.where(head0, l0, l1)
            if CFG["rcp"]:
                r = pl.reciprocal(l, approx=True)
                st[p] = e * (r * (2.0 - l * r))
            else:
                st[p] = e / l

        def mix(p):
            PLAN["events"].setdefault(PLAN["n"], []).extend((12, 20, 20))
            for t in range(3):
                put(3 * p + t, _dot(st[p] if t else st[p][:, :L], by_head(9 * p + 6 + t)))

        return score, normalize, mix

    def mixed_at(n):
        return [(ref, n - g0 * GW) for ref, (g0, g1) in zip(mixed, CHUNKS) if g0 <= n // GW < g1][0]

    def put_x(n, r):
        ref, k = mixed_at(n)
        ref[k, 0:M] = r[0:M]
        ox[n] = r[M:]

    def put_y(n, r):
        ref, k = mixed_at(n)
        ref[k] = _cat(r[0:M], ox[n] - r[M:], r[M:])

    def prep_tokens(s, zero):
        def task(e):
            x, y = [bx[_ds((s + k) * (SEG // M) + e, M), :].astype(F32) for k in range(2)]
            x = [x[:, k * 128:(k + 1) * 128] for k in range(LT)]
            y = [hold(y[:, k * 128:(k + 1) * 128], zero, CFG["hp"] * (LT - k)) for k in range(LT)]
            z = [a + b for a, b in zip(x, y)]
            for r in range(NR):
                lhs[r, _ds(e + e // 2, M)] = _val(_sum((a or b, z[k] if a and b else x[k] if a else y[k])
                                              for k, (a, b) in enumerate(MODEL[r]) if a or b))

        return [functools.partial(task, e) for e in range(SEG // M)]

    def step(s, second, zero):
        def reread(ref):
            return ref.at[pl.ds(4 * zero, ref.shape[0])]

        part_r, lhs_r, ring_r = reread(part), reread(lhs), [reread(r) for r in ring]
        halves = [slice(0, HS), slice(HS, SEG)][::1 - 2 * second]
        due = []

        def mm(x, w):
            r = _dot(x, w)
            recent.append(r[0:M] if second and len(recent) > CFG['tp'] - 40 else None)
            while due and due[0][0] <= len(recent):
                due.pop(0)[1]()
            return r

        def in_turn(items):
            lists = [[x for x in items if (x[0] >= BOTH) == e] for e in (False, True)]
            PLAN["blocks"].append(tuple(len(x) for x in lists))
            for x in items:
                if PLAN["seq"]:
                    x = lists[int(PLAN["seq"][PLAN["n"]])].pop(0)
                PLAN["n"] += 1
                yield x

        def needs(r):
            return [CFG["mo"][k] for k, c in enumerate(MODEL[r]) if c[second]]

        def project(g):
            order, plans = PROJECT[second]

            def token_sums(e):
                def begin(k):
                    return part_r[g, k, halves[e]] if second and PROJECT[0][1][1 - e][1][k] else None

                def done(k, v):
                    n = GW * g + k // 2
                    if not second:
                        part[g, k, halves[e]] = v
                    elif k % 2:
                        tok[n, halves[e]] = v
                    else:
                        ring[n // 3 % RING][n % 3, pl.ds(M + halves[e].start, HS)] = v

                return _Sums(plans[e], done, begin)

            def done(k, v):
                n = GW * g + k
                ring[n // 3 % RING][n % 3, 0:M] = v

            sums = token_sums(0), token_sums(1), _Sums(plans[2], done)
            weights = pltpu.bitcast(summed[_ds(PAD + g, 8 * 64), :], BF16)
            if g == 0:
                order = sorted(order, key=lambda r: max(needs(r)))
            for r, in in_turn([(r,) for r in order]):
                t0, t1 = (0, L) if r < BOTH else (second * HS, second * HS + HS + M)
                if g == 0:
                    lhs[r, HS:HS + M] = _val(_sum((c[second], m_s[k]) for k, c in enumerate(MODEL[r]) if c[second]))
                if r in SINGLE:
                    w = tile(plain, (PAD + g) * GW + SINGLE[r] % GW, SINGLE[r] // GW)
                else:
                    i, j = divmod(SUMMED.index(r), LT)
                    w = weights[i * 128:(i + 1) * 128, j * 128:(j + 1) * 128]
                v = mm((lhs_r if g else lhs)[r, t0:t1], w)
                sums[2].add(r, 1, v[HS - t0:HS - t0 + M])
                if t0 == 0:
                    sums[second].add(r, 1, v[:HS])
                if t1 == L:
                    sums[1 - second].add(r, 1, v[-HS:])

        def projected(n):
            src = ring_r[n // 3 % RING]
            return src[n % 3] if second else _cat(src[n % 3, 0:M], tok[n])

        new_mem = [None] * LT

        def out_chunk(ref, g0, g1):
            order, plans = OUTPUT[second]

            def token_sums(e):
                def begin(k):
                    if (second and OUTPUT[0][1][1 - e][1][k]) or (g0 > 0 and plans[e][1][k]):
                        return opart[k, halves[e]]

                def done(k, v):
                    if second and g1 == GO:
                        outb[_ds((s + k % 2) * 2 + halves[e].start // HS, HS), _ds(k // 2, 128)] = v.astype(BF16)
                    else:
                        opart[k, halves[e]] = v

                return _Sums(plans[e], done, begin)

            def done(k, v):
                new_mem[k] = v
                if g1 == GO:
                    m_s[k] = v

            sums = token_sums(0), token_sums(1), _Sums(plans[2], done, list(new_mem).__getitem__)
            if g1 == GO:
                order = sorted(order, key=lambda r: min(needs(r)))
            weights = [pltpu.bitcast(wo[_ds(g, 64), :], BF16) for g in range(g0, g1)]
            tall, short = [[r for r in order if (r >= BOTH) == e] for e in (False, True)]
            n = len(order) // CFG["ow"]
            for k in range(n):
                acc = {}
                some = _share(tall[::-1], n - 1 - k, n)[::-1] + _share(short, k, n)
                for r, g in in_turn([(r, g) for g in range(g0, g1) for r in some]):
                    t0, rows = (0, SEG) if r < BOTH else (halves[0].start, HS)
                    terms = []
                    for j, (a, b) in enumerate(FEATURE[r]):
                        i = (g - g0) * GW + j
                        if a and not b and second:
                            terms += [(a, ref[i, pl.ds(r0 + t0, rows)]) for r0 in (M, L)]
                        elif a and not b:
                            terms.append((a, ox[g * GW + j, pl.ds(t0, rows)]))
                        elif b:
                            terms.append((a or b, ref[i, pl.ds((M if a else L) + t0, rows)]))
                    sign, left = _sum(terms)
                    m_sign, m = _sum((c[second], ref[(g - g0) * GW + j, 0:M])
                                     for j, c in enumerate(FEATURE[r]) if c[second])
                    v = _add(acc[r][2] if r in acc else None, mm(_cat(m, left), weights[g - g0][:, r * 128:(r + 1) * 128]))
                    acc[r] = m_sign, sign, v
                for r, (m_sign, sign, v) in acc.items():
                    sums[2].add(r, m_sign, v[:M])
                    sums[second if r < BOTH else 0].add(r, sign, v[M:M + HS])
                    if r < BOTH:
                        sums[1 - second].add(r, sign, v[M + HS:])

        recent.clear()
        stages = attention(projected, put_x if second else put_y)
        for p in range(NP):
            ready = LT * GW * ((9 * p + 5) // GW + 1)
            due += [(ready + CFG[lag], functools.partial(f, p)) for f, lag in zip(stages, ("ds", "dn", "dp"))]
        if second:
            due += [(CFG["tp"] + k * CFG["dt"], task)
                    for k, task in enumerate(prep_tokens(jnp.minimum(s + 4, NSEG - 2), zero))]
        due.sort(key=lambda e: e[0])
        for g in range(GQ):
            project(g)
        for ref, chunk in zip(mixed, CHUNKS):
            out_chunk(reread(ref), *chunk)

    def first_segment():
        def project(g):
            acc = {}

            def task(n, k):
                r = _dot(h0[0:L + SEG, _ds(k, 128)], tile(plain, PAD * GW + n, k))
                e = len(recent) % 8
                recent.extend([r[8 * e:8 * e + 8], r[8 * e + 8:8 * e + 16]])
                acc[n] = _add(acc.get(n), r)
                if k == LT - 1:
                    first[n] = acc[n][0:L]
                    tok[n] = acc[n][L:]

            return [functools.partial(task, g * GW + n, k) for n in range(GW) for k in range(LT)]

        def put(n, r):
            recent.extend([r[k:k + 8] for k in range(0, L, 16)])
            put_x(n, r)

        stages = attention(lambda n: first[n], put)
        acc = [None] * LT

        def heads(p0, p1):
            return [functools.partial(f, t - lag) for t in range(p0, p1 + 2)
                    for lag, f in enumerate(stages) if p0 <= t - lag < p1] + [lambda: None]

        def out(g):
            def task(n, k):
                ref, i = mixed_at(n)
                r = _dot(ref[i, 0:M], wo_raw[_ds(n, 128), _ds(k, 128)])
                recent.append(r)
                acc[k] = r if acc[k] is None else acc[k] + r

            return [functools.partial(task, g * GW + n, k) for n in range(GW) for k in range(LT)]

        c1, c2, c3 = CFG["cut"]
        d1, d2 = [PAD + g for g in CFG["dc"]]
        start(c_wo(0))
        wait(c_w(GO - 2) + c_bx0)
        start(c_wo(1) + c_wo(2))
        h0[0:M, :] = mem[0:M, :].astype(F32)
        h0[M:L + SEG, :] = bx[0:2 * SEG, :].astype(F32)
        moves = transposes(GO - 2, plain, PAD + GQ - 6) + transposes(GO - 1, plain, PAD + GQ - 3)
        _beside(a_out(NB - 2, 0) + _each(project, range(c1)), moves[:CFG["qc"]]
                + _merge(sum(a_attention(1, zero), []), _each(derive_qkv, range(PAD + 15, d1), zero)), CFG["eb"])
        wait(c_w(GO - 1))
        start(c_wo(3) + c_wo(4))
        _beside(a_out(NB - 1, 1) + _each(project, range(c1, c2)),
                moves[CFG["qc"]:] + _each(derive_qkv, range(d1, d2), zero), CFG["eb"])
        start(c_wo(5))
        wait(c_wo(0) + c_wo(1) + c_wo(2))
        start(c_wo(6) + c_wo(7))
        _beside(_merge(_each(project, range(c2, c3)), heads(0, 11)),
                _each(derive_qkv, range(d2, PAD + GQ), zero) + _each(derive_out, range(3), zero), CFG["eb"])
        wait(c_wo(3) + c_wo(4) + c_wo(5))
        order = list(range(c3, GQ))
        _beside(_merge(_merge(_each(project, order), _each(out, range(3))), heads(11, 13))
                + _merge(_each(out, (3, 4, 5)), heads(13, NP)),
                _merge(_each(derive_out, (3, 4, 5), zero), prep_tokens(2, zero)), 2 * CFG["eb"])
        wait(c_wo(6) + c_wo(7))
        start(c_bx1 + c_outa)
        _run(_merge(out(6) + out(7), _each(derive_out, (6, 7), zero)))
        for k in range(LT):
            m_s[k] = acc[k]

    def b_step(it, carry):
        if not CFG["only"]:
            pl.when(it == 1)(lambda: wait(c_bx1))
        PLAN.update(n=0, blocks=[], events={})
        step(2 * it, 0, it >> 16)
        step(2 * it, 1, it >> 16)
        PLAN["n"] = -1
        start(c_outb(_ds(it, 2 * SEG)))
        return carry

    def last_segment():
        res, acc = {}, [None] * LT

        def project(n, k):
            r = _dot(-m_s[k] if k % 2 else m_s[k], tile(plain, PAD * GW + n, k))
            res[n] = _acc(res.get(n), 1 - 2 * (k % 2), r)

        def out(n, k):
            acc[k] = _add(acc[k], _dot(_cat(ox[n], res[NQ + n]), wo_raw[_ds(n, 128), _ds(k, 128)]))

        stages = attention(lambda n: _cat(_val(res[n]), tok[n]) if n in res else tok[n],
                           lambda n, r: res.update({NQ + n: r}), slice(M, L))
        lead, (l0, l1, l2, l3) = CFG["lo"], CFG["ls"]
        tiles = [9 * p + e for t in range(NP + lead) for p, e0 in ((t, 3), (t - lead, 6)) if 0 <= p < NP
                 for e in range(e0, e0 + 3)]
        short = [functools.partial(project, n, k) for n in tiles for k in range(LT)]
        due = [(k // 4, 0, task) for k, task in enumerate(short)]
        ready = lambda n: (tiles.index(n) * LT + LT - 1) // 4
        t = 0
        for p in range(NP):
            due += [(ready(9 * p + 5) + l0, 2, functools.partial(stages[0], p)),
                    (ready(9 * p + 5) + l1, 2, functools.partial(stages[1], p)),
                    (ready(9 * p + 8) + l2, 1, functools.partial(stages[2], p))]
        for k in range(NO * LT):
            if k % 4 == 0:
                t = max(t + CFG["lg"], ready(9 * ((k + 3) // 15) + 8) + l3)
            due.append((int(t), 3, functools.partial(out, *divmod(k, LT))))
        _run([task for _, _, task in sorted(due, key=lambda e: e[:2])])
        outb[S - 2 * SEG:, :] = jnp.concatenate(acc, axis=1).astype(BF16)
        start(c_outb(slice(S - 2 * SEG, S)))

    if CFG["only"]:
        for ref in (plain, summed, wo):
            ref[0:8, 0:128] = jnp.zeros((8, 128), U32)
        lax.fori_loop(0, CFG["nper"], b_step, 0)
        if CFG["only"] == 2:
            last_segment()
        wait(c_outb(slice(0, 2 * SEG)))
        return
    first_segment()
    if CFG["nper"] == 0:
        for ref in (plain, summed, wo, lhs, tok, ox):
            half = ref.shape[0] // 2
            pltpu.sync_copy(ref.at[pl.ds(zero * half, half)], ref.at[pl.ds(half - zero * half, half)])
    lax.fori_loop(0, CFG["nper"], b_step, 0)
    last_segment()
    wait(c_outa + c_outb(slice(0, (CFG["nper"] + 1) * 2 * SEG)))


def pallas_concat_heads__sliding_local_dilated__memory_aug_recurrent_mem_tr__prompt_kernel(
    A_x, A_wqkv, A_wo, B_x, B_mem0, B_Wq, B_Wk, B_Wv, B_Wo, B_seg_len,
):
    assert B_seg_len == SEG
    assert A_x.shape == B_x.shape == (1, S, D) and B_mem0.shape == (1, M, D)
    assert B_Wq.shape == B_Wk.shape == B_Wv.shape == (D, H, DH) and B_Wo.shape == (H, DH, D)
    dma = pltpu.SemaphoreType.DMA

    def vmem(shape, dtype):
        assert math.prod(shape) * jnp.dtype(dtype).itemsize % 16384 == 0, shape
        return pltpu.VMEM(shape, dtype)

    call = pl.pallas_call(
        lambda *refs: _kernel(*refs),
        out_shape=jax.ShapeDtypeStruct((S, 2 * D), BF16),
        in_specs=[pl.BlockSpec(memory_space=pl.ANY)] * 9,
        out_specs=pl.BlockSpec(memory_space=pl.ANY),
        scratch_shapes=[
            vmem((S, D), BF16),
            vmem((3, D, D), BF16),
            vmem((D, D), BF16),
            vmem((LT, D, 128), F32),
            vmem((2 * D, D), U32),
            vmem((TB, D), U32),
            vmem((2, LT, TB, 128), F32),
            vmem((2, 2 * LT, HALO + TB, 128), F32),
            vmem((2, TB, D), F32),
            vmem((S, D), BF16),
            vmem((S, D), BF16),
            vmem((8 * M, D), BF16),
            vmem((RAW * 3 * GW * 128, D), BF16),
            vmem((H * DH, D), BF16),
            vmem(((3 + GQ) * GW * 64, D), U32),
            vmem(((3 + GQ) * 8 * 64, D), U32),
            vmem((GO * 64, NR * 128), U32),
            vmem((3 * SEG, D), F32),
            vmem((NQ, L, 128), F32),
            vmem((NR + 1, L, 128), F32),
            vmem((8, M, 128), F32),
            vmem((GQ, 2 * GW, SEG, 128), F32),
            vmem((NQ, SEG, 128), F32),
            [vmem((4, L, 128), F32)] * RING,
            vmem((NO, SEG, 128), F32),
            [vmem((20, L + SEG, 128), F32)] * len(CHUNKS),
            vmem((2 * LT, SEG, 128), F32),
            vmem((S, D), BF16),
            dma((5,)), dma((NB // 2,)), dma((GO, 3)), dma((3,)), dma((GO,)), dma((2,)),
        ],
        compiler_params=pltpu.CompilerParams(vmem_limit_bytes=126 * 1024 * 1024, flags=CFG["flags"],
                                             disable_bounds_checks=True),
        name="sliding_and_memory_attention",
    )

    def by_feature(w):
        return w.transpose(1, 2, 0).reshape(H * DH, D)

    out = call(A_x.reshape(S, D), A_wqkv, A_wo, B_x.reshape(S, D), B_mem0.reshape(M, D),
               by_feature(B_Wq), by_feature(B_Wk), by_feature(B_Wv), B_Wo.reshape(H * DH, D))
    return out.reshape(1, S, 2 * D)
```

```python
import collections
import functools
import itertools
import math
import random

import jax
import jax.numpy as jnp
import numpy as np
from jax import lax
from jax.experimental import pallas as pl
from jax.experimental.pallas import tpu as pltpu

F32, BF16, U32 = jnp.float32, jnp.bfloat16, jnp.uint32
NT = (((1,), (1,)), ((), ()))
MASKED = -1000000000.0
LOG2E = math.log2(math.e)

S, D = 2048, 640
LT = D // 128

AH, AD, AW, ADIL = 32, 20, 8, 2
HALO = 16
TB = 128
NB = S // TB

H, DH, M, SEG = 32, 192, 8, 32
L = M + SEG
HS = SEG // 2
NSEG = S // SEG
NP = H // 2
NO = 3 * NP
NQ = 3 * NO
GW = 6
GO, GQ = NO // GW, NQ // GW
PAD = 3
RAW = 4
RING = 12
CHUNKS = ((0, 3), (3, 5), (5, GO))


def _algorithm(rank_ones):
    rows = np.array([[1, 0], [0, 1], [1, 1]])
    duals = np.array([[0, 1], [1, 0], [1, -1]])
    sets = [[[np.array(["-0+".index(c) - 1 for c in w]) for w in e.split()] for e in s] for s in rank_ones]
    left, right = [], []
    for t, s in enumerate(sets):
        p, q = [k for k in range(3) if k != t]
        for u, v in s:
            left += [np.outer(u, rows[p]), np.outer(u, rows[q])]
            right += [np.outer(v, duals[q]), np.outer(v, duals[p])]
    for (u0, v0), (u1, v1), (u2, v2) in itertools.product(*sets):
        for a, b in itertools.product((1, -1), repeat=2):
            e = np.outer(u0 + a * u1, v0 + b * v1)
            if (e == np.outer(u2, v2)).all() or (e == -np.outer(u2, v2)).all():
                left.append(np.outer(u0, rows[1]) - a * np.outer(u1, rows[0]))
                right.append(np.outer(v0, duals[1]) + b * np.outer(v1, duals[0]))
    left, right = np.array(left), np.array(right)
    have = np.einsum("rka,rnb->kanbr", left, right).reshape(-1, len(left))
    want = np.einsum("kp,nq,ab->kanbpq", np.eye(LT), np.eye(GW), np.eye(2)).reshape(len(have), -1)
    blocks = np.rint(np.linalg.lstsq(have, want, rcond=None)[0]).astype(int)
    assert (have @ blocks == want).all()
    sign = blocks.max(axis=1) * 2 - 1
    return left * sign[:, None, None], blocks * sign[:, None], right


def _shared_sums(matrix, seed):
    rng = random.Random(seed)
    rows = [{k: int(c) for k, c in enumerate(row) if c} for row in matrix]
    shared = {}
    while True:
        count = collections.Counter(
            (a, b, r[a] * r[b]) for r in rows for a, b in itertools.combinations(sorted(r), 2))
        top = max(count.values(), default=0)
        if top < 2:
            return shared, rows
        best = sorted(k for k, n in count.items() if n == top)
        a, b, sign = best[int(rng.random() * len(best))]
        name = matrix.shape[1] + len(shared)
        shared[name] = a, b, sign
        for r in rows:
            if r.get(a, 0) * r.get(b, 0) == sign:
                r[name] = r.pop(a)
                del r[b]


MODEL, BLOCKS, FEATURE = _algorithm((
    ("+0000 +00++0", "000+0 0+0000", "0000+ 000+00", "+-+00 00000+", "+00+0 00+0+0"),
    ("0+00+ 000+++", "0+0+0 0+00++", "00+-+ 00++00", "00+0+ +00000", "+0+00 0000+0", "00+00 0+-000"),
    ("0+000 0000++", "00+-+ ++0000", "00+00 +00+00", "+-000 0+-00+", "00+-0 00+000", "+-00- +0000-")))
NR = len(BLOCKS)
BOTH = 34
SINGLE = {r: int(row.argmax()) for r, row in enumerate(BLOCKS) if abs(row).sum() == 1}
SUMMED = [r for r in range(NR) if r not in SINGLE]


def _step_sums(out, step, seed):
    use = MODEL[:, :, step].any(1) & FEATURE[:, :, step].any(1)
    return [_shared_sums((m * keep[:, None]).T, seed) for m, keep in (
        (out.reshape(NR, -1), use), (out.reshape(NR, -1), use & (np.arange(NR) < BOTH)), (out[:, :, step], use))]


QKV_SUMS = _step_sums(FEATURE, 0, 32), _step_sums(FEATURE, 1, 5)
OUT_SUMS = _step_sums(MODEL, 0, 0), _step_sums(MODEL, 1, 6)
BLOCK_SUMS = _shared_sums(BLOCKS, 37)

QKV_ORDER = (
    (30, 14, 20, 3, 28, 12, 9, 22, 10, 18, 1, 26, 24, 5, 32, 7, 16,
     40, 38, 36, 45, 44, 46, 39, 34, 35, 43, 37, 41, 42),
    (31, 15, 4, 11, 27, 0, 8, 19, 23, 13, 33, 6, 29, 21, 2, 25, 17,
     40, 34, 39, 41, 35, 46, 45, 36, 43, 44, 38, 37, 42))
OUT_ORDER = (
    (24, 14, 10, 5, 32, 28, 16, 30, 22, 7, 12, 9, 3, 1, 18, 26, 20,
     40, 34, 39, 41, 42, 37, 36, 45, 43, 46, 44, 35, 38),
    (23, 11, 13, 2, 15, 17, 4, 25, 31, 6, 33, 29, 8, 21, 19, 0, 27,
     39, 36, 45, 40, 34, 41, 37, 44, 42, 43, 46, 35, 38))
BLOCK_ORDER = (3, 28, 6, 0, 5, 17, 11, 8, 10, 7, 4, 16, 2, 1, 23, 22, 9, 29, 24, 19, 12, 18, 25, 13, 14, 20,
               21, 15, 26, 27)
MEM_ORDER = (0, 1, 4, 2, 3)

LAGS = ((40, 70, 100), (50, 80, 110))
TOKENS_AT = (728, 25, 4)
OUT_PARTS = (5, 5)
TURNS = int(
    "7694b4b4a52942d2d294a4394b685a43a90e439694b690f1290e1e170c30d2a89a929a6343871595291b151c589aa34a"
    "60f0794386a64aa92368d4586966494b4a92d249634b4a2c361a52d2a9529316694586964b4a1693943869694a50f079"
    "43869564960f0e5294b4a52c1b4a394a4b1694a52d294a52da5a1e5a16850b694a529438e1e169078c5643a5a1e53531"
    "430796870a90c35351a26a4b318694b45a1a9a9164b0e1cc61a5a51685a5a5162c687318a9a895a1c98d074a5a0f1535"
    "25349870d4ca45c585c385a5349a16969254b483cca1a8b89a4a6a4a385a583d0cb4a929a1d28ac94b4a54c92d2a9521", 16)

A_PACE = (12, 5)
SUM_PACE = (18, 10)
A_CUT = (62, 6, 12, 4)
START_CUT = (5, 20)
FIRST_CUT = (5, 12, 21, 17, 21, 6)
LAST_LAGS = (7, 12, 3, 7, 1.9)


def _ds(i, n):
    return pl.ds(i * n if isinstance(i, int) else pl.multiple_of(i * n, n), n)


def _dot(a, b):
    return jnp.dot(a, b, preferred_element_type=F32)


def _cat(*parts):
    return jnp.concatenate(parts, axis=0)


def _add(a, b):
    return b if a is None else _cat(a[:M] + b[:M], a[M:] + b[M:])


def _acc(a, sign, b):
    if a is None:
        return sign, b
    if a[0] == sign:
        return sign, a[1] + b
    return (1, a[1] - b) if a[0] > 0 else (1, b - a[1])


def _sum(terms):
    return functools.reduce(lambda a, t: _acc(a, *t), terms, None)


def _val(a):
    return a[1] if a[0] > 0 else -a[1]


class _Sums:
    def __init__(self, plan, done, begin=lambda k: None):
        self.shared, self.rows = plan
        self.done, self.begin = done, begin
        self.terms, self.sums = {}, [None] * len(self.rows)
        for k, row in enumerate(self.rows):
            if not row and (first := begin(k)) is not None:
                done(k, first)

    def add(self, name, sign, value):
        self.terms[name] = sign, value
        for k, row in enumerate(self.rows):
            if name in row:
                if self.sums[k] is None and (first := self.begin(k)) is not None:
                    self.sums[k] = 1, first
                self.sums[k] = _acc(self.sums[k], row[name] * sign, value)
                if all(n in self.terms for n in row):
                    self.done(k, _val(self.sums[k]))
        for n, (a, b, s) in self.shared.items():
            if name in (a, b) and a in self.terms and b in self.terms and n not in self.terms:
                self.add(n, *_acc(self.terms[a], s * self.terms[b][0], self.terms[b][1]))


def _share(tasks, k, n):
    return list(tasks[k * len(tasks) // n:(k + 1) * len(tasks) // n])


def _merge(a, b, early=0):
    n = len(a) - early
    return [t for k in range(n) for t in [a[k]] + _share(b, k, n)] + a[n:]


def _each(f, items, *args):
    return [task for item in items for task in f(item, *args)]


def _run(tasks):
    for task in tasks:
        task()


def _kernel(ax_hbm, awqkv_hbm, awo_hbm, bx_hbm, mem_hbm, wq_hbm, wk_hbm, wv_hbm, wo_hbm,
            out_hbm,
            ax, awqkv, awo, tmp, wa, xb, q_s, kv_s, oa_s, outa,
            bx, mem, raw, wo_raw, plain, summed, wo, h0, first, lhs, m_s, part, tok, ring,
            ox, mixed, opart, outb,
            sem_a, sem_x, sem_w, sem_b, sem_wo, sem_o):
    cp = pltpu.make_async_copy

    def rows_copy(src, dst, rows, sem):
        return [cp(src.at[rows, :], dst.at[rows, :], sem)]

    c_aw = [cp(awqkv_hbm.at[r0:r1, _ds(j, D)], awqkv.at[j, r0:r1], sem_a.at[k])
            for k, (j, r0, r1) in enumerate(((0, 0, 384), (0, 384, D), (1, 0, D), (2, 0, D)))]
    c_awo = [cp(awo_hbm, awo, sem_a.at[4])]
    c_bx0 = [cp(mem_hbm, mem.at[0:M], sem_b.at[0])] + rows_copy(bx_hbm, bx, slice(0, 6 * SEG), sem_b.at[1])
    c_bx1 = rows_copy(bx_hbm, bx, slice(6 * SEG, S), sem_b.at[2])
    c_outa = [cp(outa, out_hbm.at[:, 0:D], sem_o.at[0])]

    def c_ax(c):
        return rows_copy(ax_hbm, ax, _ds(c, 2 * TB), sem_x.at[c])

    def c_w(c):
        return [cp(w.at[_ds(c, GW * 128), :], raw.at[_ds((c & (RAW - 1)) * 3 + j, GW * 128), :], sem_w.at[c, j])
                for j, w in enumerate((wq_hbm, wk_hbm, wv_hbm))]

    def c_wo(g):
        return rows_copy(wo_hbm, wo_raw, _ds(g, GW * 128), sem_wo.at[g])

    def c_outb(rows):
        return [cp(outb.at[rows, :], out_hbm.at[rows, D:], sem_o.at[1])]

    def start(copies):
        for c in copies:
            c.start()

    def wait(copies):
        for c in copies:
            c.wait()
        recent.clear()

    recent = []

    def paced(x, zero, marks):
        late = _cat(*[recent[t] if t >= 0 else jnp.zeros((8, 128), F32) for t in marks[:x.shape[0] // 8]])
        always = lax.broadcasted_iota(jnp.int32, x.shape, 1) >= zero
        return lax.select(always, x, late if x.dtype == F32 else pltpu.bitcast(late, U32))

    def tile(ref, i, j):
        return pltpu.bitcast(ref[_ds(i, 64), _ds(j, 128)], BF16)

    def a_weights(j, zero=None):
        def task(t):
            if j < 3:
                tmp[t] = awqkv[j, _ds(t, 128), :].astype(F32).T
            else:
                marks = [len(recent) - 40 + k * 3 // 4 for k in range(40)]
                w = paced(pltpu.bitcast(awo[:, _ds(t, 128)], U32), zero, marks)
                tmp[t] = pltpu.bitcast(w, BF16).astype(F32)
            w = _cat(*[tmp[t, pl.ds(d, AH, stride=AD), :] for d in range(AD)])
            wa[_ds(j, D // 2), _ds(t, 128)] = pltpu.bitcast(w.astype(BF16), U32)

        return [functools.partial(task, t) for t in range(LT)]

    def by_tile(product, put):
        acc = [None]

        def task(t, k):
            r = product(t, k)
            e = len(recent) % 16
            recent.extend(r[8 * (e + i) % TB:8 * (e + i) % TB + 8] for i in range(4))
            acc[0] = _add(acc[0] if k else None, r)
            if k == LT - 1:
                put(t, acc[0])

        return [functools.partial(task, t, k) for t in range(LT) for k in range(LT)]

    def a_load(i, b):
        xb[_ds(b, TB // 2), :] = pltpu.bitcast(ax[_ds(i, TB), :], U32)

    def a_proj(j, b, first_block=False):
        def put(t, r):
            if j == 0:
                q_s[b, t] = r
                return
            c = (j - 1) * LT + t
            kv_s[b, c, HALO:, :] = r
            if first_block:
                kv_s[b, c, 0:HALO, :] = jnp.broadcast_to(r[0:1, :], (HALO, 128))
            else:
                kv_s[b, c, 0:HALO, :] = kv_s[1 - b, c, TB:, :]

        return by_tile(lambda t, k: lax.dot_general(
            tile(xb, b, k), tile(wa, j * LT + t, k), NT, preferred_element_type=F32), put)

    def a_attention(b, zero, first_block=False):
        n = TB // 8
        lag = n if first_block else A_PACE[1]
        marks, logits = [], []

        def mark():
            marks.append(len(recent) - A_PACE[0])

        def window(c, w):
            return kv_s[b, c, pl.ds(HALO - ADIL * w, TB), :]

        def score():
            q = [paced(q_s[b, t], zero, marks[::4]) for t in range(LT)]
            sums = [functools.reduce(jnp.add, [q[t] * window(t, w) for t in range(LT)]) for w in range(AW)]
            rows = {}
            for k in range(n + 1):
                if k < n:
                    a = _cat(*[a[8 * k:8 * k + 8] for a in sums])
                    rows[k] = a + pltpu.roll(a, 2 * AH, 1)
                if k > 0:
                    rows[k - 1] = rows[k - 1] + pltpu.roll(rows[k - 1], AH, 1)
            logits.extend(_cat(*[rows[k][8 * w:8 * w + 8] for k in range(n)]) for w in range(AW))

        def mix():
            scale, lg = AD ** -0.5, logits
            if first_block:
                pos = lax.broadcasted_iota(jnp.int32, (HALO, 128), 0)
                lg = [_cat(jnp.where(pos >= ADIL * w, a[:HALO], MASKED / scale), a[HALO:])
                      for w, a in enumerate(lg)]
            m = paced(functools.reduce(jnp.maximum, lg), zero, marks[4 * lag + 1::4])
            e = [jnp.exp2((a - m) * (scale * LOG2E)) for a in lg]
            inv = 1.0 / functools.reduce(jnp.add, e)
            for t in range(LT):
                v = [window(LT + t, w) for w in range(AW)]
                v[0] = paced(v[0], zero, marks[4 * lag + 2 + 2 * t // LT::4])
                oa_s[b, :, _ds(t, 128)] = inv * functools.reduce(jnp.add, map(jnp.multiply, e, v))

        return [mark] * (4 * n) + [score], [mark] * (4 * lag) + [mix]

    def a_out(i, b):
        def put(t, r):
            outa[_ds(i, TB), _ds(t, 128)] = r.astype(BF16)

        return by_tile(lambda t, k: _dot(oa_s[b, :, _ds(k, 128)], tile(wa, 3 * LT + k, t)), put)

    def transposes(c, dst, g):
        def task(n):
            t = ((c & (RAW - 1)) * 3 + n % 9 // 3) * GW + n // 9 * 3 + n % 3
            v = pltpu.bitcast(raw[_ds(t, 128), :].T, U32)
            for k in range(LT):
                dst[_ds(g * GW + n, 64), _ds(k, 128)] = v[k * 64:(k + 1) * 64]

        return [functools.partial(task, n) for n in range(3 * GW)]

    def sum_blocks(block, put, zero):
        back, n = SUM_PACE
        marks = []

        def mark():
            marks.append(len(recent) - back)

        def done(r, v):
            if r not in SINGLE:
                put(r, pltpu.bitcast(v.astype(BF16), U32))

        def task():
            sums = _Sums(BLOCK_SUMS, done)
            for k in range(n):
                for i, b in enumerate(_share(BLOCK_ORDER, k, n)):
                    v = block(*divmod(b, GW))
                    if i == 0:
                        v = paced(v, zero, marks[k::n])
                    for r in SINGLE:
                        if SINGLE[r] == b:
                            put(r, v)
                    sums.add(b, 1, pltpu.bitcast(v, BF16).astype(F32))

        return [mark] * (8 * n) + [task]

    def sum_qkv(g, zero, src=plain, dst=summed):
        def put(r, v):
            if r not in SINGLE:
                i, j = divmod(SUMMED.index(r), LT)
                dst[_ds(g * 8 + i, 64), _ds(j, 128)] = v

        return sum_blocks(lambda k, n: src[_ds(g * GW + n, 64), _ds(k, 128)], put, zero)

    def sum_out(g, zero):
        def put(r, v):
            wo[_ds(g, 64), _ds(r, 128)] = v

        return sum_blocks(lambda k, n: pltpu.bitcast(wo_raw[_ds(g * GW + n, 128), _ds(k, 128)], U32), put, zero)

    def a_start():
        nq, nk = START_CUT
        start(c_aw[:2])
        zero = lax.fori_loop(0, 2, lambda it, carry: it >> 16, 0)
        start(c_ax(0))
        wait(c_aw[:1])
        start(c_aw[2:3])
        _run(a_weights(0)[:3])
        wait(c_aw[1:2])
        start(c_aw[3:])
        _run(a_weights(0)[3:])
        wait(c_ax(0))
        start(c_awo)
        a_load(0, 0)
        a_load(1, 1)
        _run(a_proj(0, 0) + a_proj(0, 1)[:nq])
        wait(c_aw[2:3])
        start(c_ax(1) + c_ax(2))
        _run(a_proj(0, 1)[nq:] + a_weights(1) + a_proj(1, 0, True))
        wait(c_aw[3:])
        start(c_w(0))
        early, late = a_attention(0, zero, True)
        _run(a_proj(1, 1)[:nk] + a_weights(2) + _merge(a_proj(2, 0, True), early))
        wait(c_awo + c_ax(1))
        start(c_bx0)
        _run(_merge(a_proj(1, 1)[nk:] + a_proj(2, 1), _merge(late, a_weights(3, zero)), 4))
        a_load(2, 0)

    def a_step(it, carry):
        i, g, zero = 2 * it, jnp.maximum(3 * it - 9 + PAD, 0), it >> 16
        pl.when(it + 2 < NB // 2)(lambda: start(c_ax(it + 2)))
        pl.when(it + 1 < NB // 2)(lambda: wait(c_ax(it + 1)))
        start(c_w(it))
        pl.when(it > 1)(lambda: wait(c_w(it - 2)))
        src, dst = [ref.at[pl.ds(pl.multiple_of(g * n, n), k * n)]
                    for ref, n, k in ((plain, GW * 64, 6), (summed, 8 * 64, 3))]
        sums, moves = _each(sum_qkv, range(3), zero, src, dst), transposes(it + RAW - 2, src, 3)
        cut, m1, m2 = len(sums) * A_CUT[0] // 100, A_CUT[1], A_CUT[2]
        early, late = a_attention(1, zero)
        a_load(i + 1, 1)
        _run(_merge(a_out(i - 2, 0) + _each(a_proj, range(3), 0),
                    moves[:m1] + _merge(early, sums[:cut]) + moves[m1:m2]))
        a_load(jnp.minimum(i + 2, NB - 1), 0)
        side = sum(a_attention(0, zero), [])
        side = _merge(side[:len(late)], late) + side[len(late):]
        _run(_merge(_each(a_proj, range(3), 1) + a_out(i - 1, 1), _merge(side, sums[cut:]) + moves[m2:], A_CUT[3]))
        return zero

    def attention(qkv, put, row0=0):
        row = lax.broadcasted_iota(jnp.int32, (L - row0, 2 * L), 0) + row0
        col = lax.broadcasted_iota(jnp.int32, (L - row0, 2 * L), 1)
        head0 = col < L
        visible = (row < M) | (row >= jnp.where(head0, col, col - L))
        scale = DH ** -0.5
        st = {}

        def by_head(n):
            t = qkv(n)
            if n % 3 == 1:
                low = lax.broadcasted_iota(jnp.int32, t.shape, 1) < 64
                t = _cat(jnp.where(low, t, 0.0), jnp.where(low, 0.0, t))
            elif n % 3 == 2:
                t = _cat(jnp.zeros_like(t), t)
            return t.astype(BF16)

        def score(p):
            sc = [lax.dot_general(qkv(9 * p + t), by_head(9 * p + 3 + t), NT, preferred_element_type=F32)
                  for t in range(3)]
            sc = _add(_add(jnp.concatenate([sc[0], jnp.zeros_like(sc[0])], axis=1), sc[1]), sc[2])
            sc = jnp.where(visible, sc, MASKED / scale)
            m0 = jnp.max(jnp.where(head0, sc, -jnp.inf), axis=1, keepdims=True)
            m1 = jnp.max(jnp.where(head0, -jnp.inf, sc), axis=1, keepdims=True)
            st[p] = sc - jnp.where(head0, m0, m1)

        def normalize(p):
            e = jnp.exp2(st[p] * (scale * LOG2E))
            l0 = jnp.sum(jnp.where(head0, e, 0.0), axis=1, keepdims=True)
            l1 = jnp.sum(jnp.where(head0, 0.0, e), axis=1, keepdims=True)
            st[p] = e / jnp.where(head0, l0, l1)

        def mix(p):
            for t in range(3):
                put(3 * p + t, _dot(st[p] if t else st[p][:, :L], by_head(9 * p + 6 + t)))

        return score, normalize, mix

    def mixed_at(n):
        return [(ref, n - g0 * GW) for ref, (g0, g1) in zip(mixed, CHUNKS) if g0 <= n // GW < g1][0]

    def put_x(n, r):
        ref, k = mixed_at(n)
        ref[k, 0:M] = r[0:M]
        ox[n] = r[M:]

    def put_y(n, r):
        ref, k = mixed_at(n)
        ref[k] = _cat(r[0:M], ox[n] - r[M:], r[M:])

    def left_operands(s, zero):
        def task(e):
            x, y = [bx[_ds((s + k) * (SEG // M) + e, M), :].astype(F32) for k in range(2)]
            x = [x[:, k * 128:(k + 1) * 128] for k in range(LT)]
            y = [paced(y[:, k * 128:(k + 1) * 128], zero, [len(recent) - TOKENS_AT[2] * (LT - k)])
                 for k in range(LT)]
            z = [a + b for a, b in zip(x, y)]
            for r in range(NR):
                lhs[r, _ds(e + e // 2, M)] = _val(_sum((a or b, z[k] if a and b else x[k] if a else y[k])
                                                       for k, (a, b) in enumerate(MODEL[r]) if a or b))

        return [functools.partial(task, e) for e in range(SEG // M)]

    def step(s, second, zero):
        def reread(ref):
            return ref.at[pl.ds(4 * zero, ref.shape[0])]

        part_r, lhs_r, ring_r = reread(part), reread(lhs), [reread(r) for r in ring]
        halves = [slice(0, HS), slice(HS, SEG)][::1 - 2 * second]
        new_mem = [None] * LT
        due = []

        def mm(x, w):
            r = _dot(x, w)
            recent.append(r[0:M] if second and len(recent) > TOKENS_AT[0] - 48 else None)
            while due and due[0][0] <= len(recent):
                due.pop(0)[1]()
            return r

        def in_turn(items):
            lists = [[x for x in items if (x[0] >= BOTH) == e] for e in (False, True)]
            for _ in items:
                yield lists[TURNS >> second * (NQ + NO) * LT + len(recent) & 1].pop(0)

        def mem_tiles(r):
            return [MEM_ORDER[k] for k, c in enumerate(MODEL[r]) if c[second]]

        def project(g):
            def token_sums(e):
                def begin(k):
                    return part_r[g, k, halves[e]] if second and QKV_SUMS[0][1 - e][1][k] else None

                def done(k, v):
                    n = GW * g + k // 2
                    if not second:
                        part[g, k, halves[e]] = v
                    elif k % 2:
                        tok[n, halves[e]] = v
                    else:
                        ring[n // 3 % RING][n % 3, pl.ds(M + halves[e].start, HS)] = v

                return _Sums(QKV_SUMS[second][e], done, begin)

            def done(k, v):
                n = GW * g + k
                ring[n // 3 % RING][n % 3, 0:M] = v

            sums = token_sums(0), token_sums(1), _Sums(QKV_SUMS[second][2], done)
            weights = pltpu.bitcast(summed[_ds(PAD + g, 8 * 64), :], BF16)
            order = sorted(QKV_ORDER[second], key=lambda r: 0 if g else max(mem_tiles(r)))
            for r, in in_turn([(r,) for r in order]):
                t0, t1 = (0, L) if r < BOTH else (second * HS, second * HS + HS + M)
                if g == 0:
                    lhs[r, HS:HS + M] = _val(_sum(
                        (c[second], m_s[k]) for k, c in enumerate(MODEL[r]) if c[second]))
                if r in SINGLE:
                    w = tile(plain, (PAD + g) * GW + SINGLE[r] % GW, SINGLE[r] // GW)
                else:
                    i, j = divmod(SUMMED.index(r), LT)
                    w = weights[i * 128:(i + 1) * 128, j * 128:(j + 1) * 128]
                v = mm((lhs_r if g else lhs)[r, t0:t1], w)
                sums[2].add(r, 1, v[HS - t0:HS - t0 + M])
                if t0 == 0:
                    sums[second].add(r, 1, v[:HS])
                if t1 == L:
                    sums[1 - second].add(r, 1, v[-HS:])

        def projected(n):
            src = ring_r[n // 3 % RING]
            return src[n % 3] if second else _cat(src[n % 3, 0:M], tok[n])

        def out_chunk(ref, g0, g1):
            def token_sums(e):
                def begin(k):
                    if (second and OUT_SUMS[0][1 - e][1][k]) or (g0 > 0 and OUT_SUMS[second][e][1][k]):
                        return opart[k, halves[e]]

                def done(k, v):
                    if second and g1 == GO:
                        rows = _ds((s + k % 2) * 2 + halves[e].start // HS, HS)
                        outb[rows, _ds(k // 2, 128)] = v.astype(BF16)
                    else:
                        opart[k, halves[e]] = v

                return _Sums(OUT_SUMS[second][e], done, begin)

            def done(k, v):
                new_mem[k] = v
                if g1 == GO:
                    m_s[k] = v

            sums = token_sums(0), token_sums(1), _Sums(OUT_SUMS[second][2], done, list(new_mem).__getitem__)
            weights = [pltpu.bitcast(wo[_ds(g, 64), :], BF16) for g in range(g0, g1)]
            order = sorted(OUT_ORDER[second], key=lambda r: min(mem_tiles(r)) if g1 == GO else 0)
            tall, short = [[r for r in order if (r >= BOTH) == e] for e in (False, True)]
            n = OUT_PARTS[second]
            for k in range(n):
                acc = {}
                some = _share(tall[::-1], n - 1 - k, n)[::-1] + _share(short, k, n)
                for r, g in in_turn([(r, g) for g in range(g0, g1) for r in some]):
                    t0, rows = (0, SEG) if r < BOTH else (halves[0].start, HS)
                    terms = []
                    for j, (a, b) in enumerate(FEATURE[r]):
                        i = (g - g0) * GW + j
                        if b:
                            terms.append((a or b, ref[i, pl.ds((M if a else L) + t0, rows)]))
                        elif a and second:
                            terms += [(a, ref[i, pl.ds(r0 + t0, rows)]) for r0 in (M, L)]
                        elif a:
                            terms.append((a, ox[g * GW + j, pl.ds(t0, rows)]))
                    sign, left = _sum(terms)
                    m_sign, m = _sum((c[second], ref[(g - g0) * GW + j, 0:M])
                                     for j, c in enumerate(FEATURE[r]) if c[second])
                    v = mm(_cat(m, left), weights[g - g0][:, r * 128:(r + 1) * 128])
                    acc[r] = m_sign, sign, _add(acc[r][2] if r in acc else None, v)
                for r, (m_sign, sign, v) in acc.items():
                    sums[2].add(r, m_sign, v[:M])
                    sums[second if r < BOTH else 0].add(r, sign, v[M:M + HS])
                    if r < BOTH:
                        sums[1 - second].add(r, sign, v[M + HS:])

        recent.clear()
        stages = attention(projected, put_x if second else put_y)
        for p in range(NP):
            ready = LT * GW * ((9 * p + 5) // GW + 1)
            due += [(ready + lag, functools.partial(f, p)) for f, lag in zip(stages, LAGS[second])]
        if second:
            due += [(TOKENS_AT[0] + k * TOKENS_AT[1], task)
                    for k, task in enumerate(left_operands(jnp.minimum(s + 4, NSEG - 2), zero))]
        due.sort(key=lambda e: e[0])
        for g in range(GQ):
            project(g)
        for ref, chunk in zip(mixed, CHUNKS):
            out_chunk(reread(ref), *chunk)

    def first_segment(zero):
        def project(g):
            acc = {}

            def task(n, k):
                r = _dot(h0[0:L + SEG, _ds(k, 128)], tile(plain, PAD * GW + n, k))
                e = len(recent) % 8
                recent.extend([r[8 * e:8 * e + 8], r[8 * e + 8:8 * e + 16]])
                acc[n] = _add(acc.get(n), r)
                if k == LT - 1:
                    first[n] = acc[n][0:L]
                    tok[n] = acc[n][L:]

            return [functools.partial(task, g * GW + n, k) for n in range(GW) for k in range(LT)]

        def put(n, r):
            recent.extend([r[k:k + 8] for k in range(0, L, 16)])
            put_x(n, r)

        stages = attention(lambda n: first[n], put)
        new_mem = [None] * LT

        def heads(p0, p1):
            return [functools.partial(f, t - lag) for t in range(p0, p1 + 2)
                    for lag, f in enumerate(stages) if p0 <= t - lag < p1] + [lambda: None]

        def out(g):
            def task(n, k):
                ref, i = mixed_at(n)
                r = _dot(ref[i, 0:M], wo_raw[_ds(n, 128), _ds(k, 128)])
                recent.append(r)
                new_mem[k] = r if new_mem[k] is None else new_mem[k] + r

            return [functools.partial(task, g * GW + n, k) for n in range(GW) for k in range(LT)]

        c1, c2, c3, d1, d2, m1 = FIRST_CUT
        moves = transposes(GO - 2, plain, PAD + GQ - 6) + transposes(GO - 1, plain, PAD + GQ - 3)
        start(c_wo(0))
        wait(c_w(GO - 2) + c_bx0)
        start(c_wo(1) + c_wo(2))
        h0[0:M, :] = mem[0:M, :].astype(F32)
        h0[M:L + SEG, :] = bx[0:2 * SEG, :].astype(F32)
        _run(_merge(a_out(NB - 2, 0) + _each(project, range(c1)), moves[:m1] + _merge(
            sum(a_attention(1, zero), []), _each(sum_qkv, range(PAD + GQ - 9, PAD + d1), zero))))
        wait(c_w(GO - 1))
        start(c_wo(3) + c_wo(4))
        _run(_merge(a_out(NB - 1, 1) + _each(project, range(c1, c2)),
                    moves[m1:] + _each(sum_qkv, range(PAD + d1, PAD + d2), zero)))
        start(c_wo(5))
        wait(_each(c_wo, range(3)))
        start(c_wo(6) + c_wo(7))
        _run(_merge(_merge(_each(project, range(c2, c3)), heads(0, 11)),
                    _each(sum_qkv, range(PAD + d2, PAD + GQ), zero) + _each(sum_out, range(3), zero)))
        wait(_each(c_wo, range(3, 6)))
        _run(_merge(_merge(_merge(_each(project, range(c3, GQ)), _each(out, range(3))), heads(11, 13))
                    + _merge(_each(out, range(3, 6)), heads(13, NP)),
                    _merge(_each(sum_out, range(3, 6), zero), left_operands(2, zero))))
        wait(c_wo(6) + c_wo(7))
        start(c_bx1 + c_outa)
        _run(_merge(out(6) + out(7), _each(sum_out, (6, 7), zero)))
        for k in range(LT):
            m_s[k] = new_mem[k]

    def two_segments(it, carry):
        pl.when(it == 1)(lambda: wait(c_bx1))
        step(2 * it, 0, it >> 16)
        step(2 * it, 1, it >> 16)
        start(c_outb(_ds(it, 2 * SEG)))
        return carry

    def last_segment():
        res, acc = {}, [None] * LT

        def project(n, k):
            r = _dot(-m_s[k] if k % 2 else m_s[k], tile(plain, PAD * GW + n, k))
            res[n] = _acc(res.get(n), 1 - 2 * (k % 2), r)

        def out(n, k):
            acc[k] = _add(acc[k], _dot(_cat(ox[n], res[NQ + n]), wo_raw[_ds(n, 128), _ds(k, 128)]))

        stages = attention(lambda n: _cat(_val(res[n]), tok[n]) if n in res else tok[n],
                           lambda n, r: res.update({NQ + n: r}), M)
        tiles = [9 * p + e for t in range(NP + 3) for p, e0 in ((t, 3), (t - 3, 6)) if 0 <= p < NP
                 for e in range(e0, e0 + 3)]
        ready = {n: (i * LT + LT - 1) // 4 for i, n in enumerate(tiles)}
        due = [((i * LT + k) // 4, 0, functools.partial(project, n, k))
               for i, n in enumerate(tiles) for k in range(LT)]
        for p in range(NP):
            due += [(ready[9 * p + e] + lag, rank, functools.partial(f, p))
                    for f, lag, e, rank in zip(stages, LAST_LAGS, (5, 5, 8), (2, 2, 1))]
        t = 0
        for k in range(NO * LT):
            if k % 4 == 0:
                t = max(t + LAST_LAGS[4], ready[9 * ((k + 3) // 15) + 8] + LAST_LAGS[3])
            due.append((int(t), 3, functools.partial(out, *divmod(k, LT))))
        _run([task for _, _, task in sorted(due, key=lambda e: e[:2])])
        outb[S - 2 * SEG:, :] = jnp.concatenate(acc, axis=1).astype(BF16)
        start(c_outb(slice(S - 2 * SEG, S)))

    a_start()
    first_segment(lax.fori_loop(1, NB // 2, a_step, 0))
    lax.fori_loop(0, NSEG // 2 - 1, two_segments, 0)
    last_segment()
    wait(c_outa + c_outb(slice(0, S)))


def pallas_concat_heads__sliding_local_dilated__memory_aug_recurrent_mem_tr__prompt_kernel(
    A_x, A_wqkv, A_wo, B_x, B_mem0, B_Wq, B_Wk, B_Wv, B_Wo, B_seg_len,
):
    assert B_seg_len == SEG
    assert A_x.shape == B_x.shape == (1, S, D) and B_mem0.shape == (1, M, D)
    assert B_Wq.shape == B_Wk.shape == B_Wv.shape == (D, H, DH) and B_Wo.shape == (H, DH, D)
    dma = pltpu.SemaphoreType.DMA

    def vmem(shape, dtype):
        assert math.prod(shape) * jnp.dtype(dtype).itemsize % 16384 == 0
        return pltpu.VMEM(shape, dtype)

    call = pl.pallas_call(
        _kernel,
        out_shape=jax.ShapeDtypeStruct((S, 2 * D), BF16),
        in_specs=[pl.BlockSpec(memory_space=pl.ANY)] * 9,
        out_specs=pl.BlockSpec(memory_space=pl.ANY),
        scratch_shapes=[
            vmem((S, D), BF16),
            vmem((3, D, D), BF16),
            vmem((D, D), BF16),
            vmem((LT, D, 128), F32),
            vmem((2 * D, D), U32),
            vmem((TB, D), U32),
            vmem((2, LT, TB, 128), F32),
            vmem((2, 2 * LT, HALO + TB, 128), F32),
            vmem((2, TB, D), F32),
            vmem((S, D), BF16),
            vmem((S, D), BF16),
            vmem((8 * M, D), BF16),
            vmem((RAW * 3 * GW * 128, D), BF16),
            vmem((H * DH, D), BF16),
            vmem(((PAD + GQ) * GW * 64, D), U32),
            vmem(((PAD + GQ) * 8 * 64, D), U32),
            vmem((GO * 64, NR * 128), U32),
            vmem((3 * SEG, D), F32),
            vmem((NQ, L, 128), F32),
            vmem((NR + 1, L, 128), F32),
            vmem((8, M, 128), F32),
            vmem((GQ, 2 * GW, SEG, 128), F32),
            vmem((NQ, SEG, 128), F32),
            [vmem((4, L, 128), F32)] * RING,
            vmem((NO, SEG, 128), F32),
            [vmem((20, L + SEG, 128), F32)] * len(CHUNKS),
            vmem((2 * LT, SEG, 128), F32),
            vmem((S, D), BF16),
            dma((5,)), dma((NB // 2,)), dma((GO, 3)), dma((3,)), dma((GO,)), dma((2,)),
        ],
        compiler_params=pltpu.CompilerParams(vmem_limit_bytes=126 * 1024 * 1024, disable_bounds_checks=True),
        name="sliding_and_memory_attention",
    )

    def by_feature(w):
        return w.transpose(1, 2, 0).reshape(H * DH, D)

    out = call(A_x.reshape(S, D), A_wqkv, A_wo, B_x.reshape(S, D), B_mem0.reshape(M, D),
               by_feature(B_Wq), by_feature(B_Wk), by_feature(B_Wv), B_Wo.reshape(H * DH, D))
    return out.reshape(1, S, 2 * D)
```

```python
import collections
import functools
import itertools
import math
import random

import jax
import jax.numpy as jnp
import numpy as np
from jax import lax
from jax.experimental import pallas as pl
from jax.experimental.pallas import tpu as pltpu

F32, BF16, U32 = jnp.float32, jnp.bfloat16, jnp.uint32
NT = (((1,), (1,)), ((), ()))
MASKED = -1000000000.0
LOG2E = math.log2(math.e)

S, D = 2048, 640
LT = D // 128

AH, AD, AW, ADIL = 32, 20, 8, 2
HALO = 16
TB = 128
NB = S // TB

H, DH, M, SEG = 32, 192, 8, 32
L = M + SEG
HS = SEG // 2
NSEG = S // SEG
NP = H // 2
NO = 3 * NP
NQ = 3 * NO
GW = 6
GO, GQ = NO // GW, NQ // GW
PAD = 3
RAW = 4
RING = 12
CHUNKS = ((0, 3), (3, 5), (5, GO))


def _algorithm(rank_ones):
    rows = np.array([[1, 0], [0, 1], [1, 1]])
    duals = np.array([[0, 1], [1, 0], [1, -1]])
    sets = [[[np.array(["-0+".index(c) - 1 for c in w]) for w in e.split()] for e in s] for s in rank_ones]
    left, right = [], []
    for t, s in enumerate(sets):
        p, q = [k for k in range(3) if k != t]
        for u, v in s:
            left += [np.outer(u, rows[p]), np.outer(u, rows[q])]
            right += [np.outer(v, duals[q]), np.outer(v, duals[p])]
    for (u0, v0), (u1, v1), (u2, v2) in itertools.product(*sets):
        for a, b in itertools.product((1, -1), repeat=2):
            e = np.outer(u0 + a * u1, v0 + b * v1)
            if (e == np.outer(u2, v2)).all() or (e == -np.outer(u2, v2)).all():
                left.append(np.outer(u0, rows[1]) - a * np.outer(u1, rows[0]))
                right.append(np.outer(v0, duals[1]) + b * np.outer(v1, duals[0]))
    left, right = np.array(left), np.array(right)
    have = np.einsum("rka,rnb->kanbr", left, right).reshape(-1, len(left))
    want = np.einsum("kp,nq,ab->kanbpq", np.eye(LT), np.eye(GW), np.eye(2)).reshape(len(have), -1)
    blocks = np.rint(np.linalg.lstsq(have, want, rcond=None)[0]).astype(int)
    assert (have @ blocks == want).all()
    sign = blocks.max(axis=1) * 2 - 1
    return left * sign[:, None, None], blocks * sign[:, None], right


def _shared_sums(matrix, seed):
    rng = random.Random(seed)
    rows = [{k: int(c) for k, c in enumerate(row) if c} for row in matrix]
    shared = {}
    while True:
        count = collections.Counter(
            (a, b, r[a] * r[b]) for r in rows for a, b in itertools.combinations(sorted(r), 2))
        top = max(count.values(), default=0)
        if top < 2:
            return shared, rows
        best = sorted(k for k, n in count.items() if n == top)
        a, b, sign = best[int(rng.random() * len(best))]
        name = matrix.shape[1] + len(shared)
        shared[name] = a, b, sign
        for r in rows:
            if r.get(a, 0) * r.get(b, 0) == sign:
                r[name] = r.pop(a)
                del r[b]


MODEL, BLOCKS, FEATURE = _algorithm((
    ("+0000 +00++0", "000+0 0+0000", "0000+ 000+00", "+-+00 00000+", "+00+0 00+0+0"),
    ("0+00+ 000+++", "0+0+0 0+00++", "00+-+ 00++00", "00+0+ +00000", "+0+00 0000+0", "00+00 0+-000"),
    ("0+000 0000++", "00+-+ ++0000", "00+00 +00+00", "+-000 0+-00+", "00+-0 00+000", "+-00- +0000-")))
NR = len(BLOCKS)
BOTH = 34
SINGLE = {r: int(row.argmax()) for r, row in enumerate(BLOCKS) if abs(row).sum() == 1}
SUMMED = [r for r in range(NR) if r not in SINGLE]


def _step_sums(out, step, seed):
    use = MODEL[:, :, step].any(1) & FEATURE[:, :, step].any(1)
    return [_shared_sums((m * keep[:, None]).T, seed) for m, keep in (
        (out.reshape(NR, -1), use), (out.reshape(NR, -1), use & (np.arange(NR) < BOTH)), (out[:, :, step], use))]


QKV_SUMS = _step_sums(FEATURE, 0, 32), _step_sums(FEATURE, 1, 5)
OUT_SUMS = _step_sums(MODEL, 0, 0), _step_sums(MODEL, 1, 6)
BLOCK_SUMS = _shared_sums(BLOCKS, 37)

QKV_ORDER = (
    (30, 14, 20, 3, 28, 12, 9, 22, 10, 18, 1, 26, 5, 24, 32, 7, 16,
     40, 38, 36, 45, 46, 44, 39, 34, 35, 43, 37, 41, 42),
    (31, 15, 4, 11, 27, 0, 8, 19, 23, 13, 33, 6, 29, 21, 2, 25, 17,
     40, 34, 39, 41, 35, 45, 46, 36, 43, 44, 38, 37, 42))
OUT_ORDER = (
    (24, 14, 10, 5, 32, 28, 16, 30, 22, 7, 9, 12, 3, 1, 18, 26, 20,
     40, 34, 39, 41, 42, 37, 36, 45, 43, 46, 44, 35, 38),
    (23, 11, 13, 2, 15, 17, 4, 25, 31, 6, 33, 29, 8, 21, 19, 0, 27,
     39, 36, 45, 34, 40, 41, 37, 44, 42, 43, 46, 35, 38))
BLOCK_ORDER = (3, 28, 6, 0, 5, 17, 11, 8, 10, 7, 4, 16, 2, 1, 23, 22, 9, 29, 24, 19, 12, 18, 25, 13, 14, 20,
               21, 15, 26, 27)
MEM_ORDER = (0, 1, 4, 2, 3)

LAGS = ((40, 70, 100), (50, 80, 110))
TOKENS_AT = (758, 25, 1)
OUT_PARTS = (5, 5)
TURNS = int(
    "7694b4b4a52942d2d294a4394b685a43a90e439694b690f1290e1e170c30d2a89a929a6343871595291b151c589aa34a"
    "60f0794386a64aa92368d4586966494b4a92d249634b4a2c361a52d2a9529316694586964b4a1693943869694a50f079"
    "43869564960f0e5294b4a52c1b4a394a4b1694a52d294a52da5a1e5a16850b694a529438e1e169078c5643a5a1e53531"
    "430796870a90c35351a26a4b318694b45a1a9a9164b0e1cc61a5a51685a5a5162c687318a9a895a1c98d074a5a0f1535"
    "25349870d4ca45c585c385a5349a16969254b483cca1a8b89a4a6a4a385a583d0cb4a929a1d28ac94b4a54c92d2a9521", 16)

A_PACE = (12, 4)
SUM_PACE = (18, 10)
A_CUT = (58, 1, 18, 0)
START_CUT = (5, 20)
FIRST_CUT = (5, 12, 21, 17, 21, 6)
LAST_LAGS = (7, 12, 3, 7, 1.9)


def _ds(i, n):
    return pl.ds(i * n if isinstance(i, int) else pl.multiple_of(i * n, n), n)


def _dot(a, b):
    return jnp.dot(a, b, preferred_element_type=F32)


def _cat(*parts):
    return jnp.concatenate(parts, axis=0)


def _add(a, b):
    return b if a is None else _cat(a[:M] + b[:M], a[M:] + b[M:])


def _acc(a, sign, b):
    if a is None:
        return sign, b
    if a[0] == sign:
        return sign, a[1] + b
    return (1, a[1] - b) if a[0] > 0 else (1, b - a[1])


def _sum(terms):
    return functools.reduce(lambda a, t: _acc(a, *t), terms, None)


def _val(a):
    return a[1] if a[0] > 0 else -a[1]


class _Sums:
    def __init__(self, plan, done, begin=lambda k: None):
        self.shared, self.rows = plan
        self.done, self.begin = done, begin
        self.terms, self.sums = {}, [None] * len(self.rows)
        for k, row in enumerate(self.rows):
            if not row and (first := begin(k)) is not None:
                done(k, first)

    def add(self, name, sign, value):
        self.terms[name] = sign, value
        for k, row in enumerate(self.rows):
            if name in row:
                if self.sums[k] is None and (first := self.begin(k)) is not None:
                    self.sums[k] = 1, first
                self.sums[k] = _acc(self.sums[k], row[name] * sign, value)
                if all(n in self.terms for n in row):
                    self.done(k, _val(self.sums[k]))
        for n, (a, b, s) in self.shared.items():
            if name in (a, b) and a in self.terms and b in self.terms and n not in self.terms:
                self.add(n, *_acc(self.terms[a], s * self.terms[b][0], self.terms[b][1]))


def _share(tasks, k, n):
    return list(tasks[k * len(tasks) // n:(k + 1) * len(tasks) // n])


def _merge(a, b, early=0):
    n = len(a) - early
    return [t for k in range(n) for t in [a[k]] + _share(b, k, n)] + a[n:]


def _each(f, items, *args):
    return [task for item in items for task in f(item, *args)]


def _run(tasks):
    for task in tasks:
        task()


def _kernel(ax_hbm, awqkv_hbm, awo_hbm, bx_hbm, mem_hbm, wq_hbm, wk_hbm, wv_hbm, wo_hbm,
            out_hbm,
            ax, awqkv, awo, tmp, wa, xb, q_s, kv_s, oa_s, outa,
            bx, mem, raw, wo_raw, plain, summed, wo, h0, first, lhs, m_s, part, tok, ring,
            ox, mixed, opart, outb,
            sem_a, sem_x, sem_w, sem_b, sem_wo, sem_o):
    cp = pltpu.make_async_copy

    def rows_copy(src, dst, rows, sem):
        return [cp(src.at[rows, :], dst.at[rows, :], sem)]

    c_aw = [cp(awqkv_hbm.at[r0:r1, _ds(j, D)], awqkv.at[j, r0:r1], sem_a.at[k])
            for k, (j, r0, r1) in enumerate(((0, 0, 384), (0, 384, D), (1, 0, D), (2, 0, D)))]
    c_awo = [cp(awo_hbm, awo, sem_a.at[4])]
    c_bx0 = [cp(mem_hbm, mem.at[0:M], sem_b.at[0])] + rows_copy(bx_hbm, bx, slice(0, 6 * SEG), sem_b.at[1])
    c_bx1 = rows_copy(bx_hbm, bx, slice(6 * SEG, S), sem_b.at[2])
    c_outa = [cp(outa, out_hbm.at[:, 0:D], sem_o.at[0])]

    def c_ax(c):
        return rows_copy(ax_hbm, ax, _ds(c, 2 * TB), sem_x.at[c])

    def c_w(c):
        return [cp(w.at[_ds(c, GW * 128), :], raw.at[_ds((c & (RAW - 1)) * 3 + j, GW * 128), :], sem_w.at[c, j])
                for j, w in enumerate((wq_hbm, wk_hbm, wv_hbm))]

    def c_wo(g):
        return rows_copy(wo_hbm, wo_raw, _ds(g, GW * 128), sem_wo.at[g])

    def c_outb(rows):
        return [cp(outb.at[rows, :], out_hbm.at[rows, D:], sem_o.at[1])]

    def start(copies):
        for c in copies:
            c.start()

    def wait(copies):
        for c in copies:
            c.wait()
        recent.clear()

    recent = []

    def paced(x, zero, marks):
        late = _cat(*[recent[t] if t >= 0 else jnp.zeros((8, 128), F32) for t in marks[:x.shape[0] // 8]])
        always = lax.broadcasted_iota(jnp.int32, x.shape, 1) >= zero
        return lax.select(always, x, late if x.dtype == F32 else pltpu.bitcast(late, U32))

    def tile(ref, i, j):
        return pltpu.bitcast(ref[_ds(i, 64), _ds(j, 128)], BF16)

    def a_weights(j, zero=None):
        def task(t):
            if j < 3:
                tmp[t] = awqkv[j, _ds(t, 128), :].astype(F32).T
            else:
                marks = [len(recent) - 40 + k * 3 // 4 for k in range(40)]
                w = paced(pltpu.bitcast(awo[:, _ds(t, 128)], U32), zero, marks)
                tmp[t] = pltpu.bitcast(w, BF16).astype(F32)
            w = _cat(*[tmp[t, pl.ds(d, AH, stride=AD), :] for d in range(AD)])
            wa[_ds(j, D // 2), _ds(t, 128)] = pltpu.bitcast(w.astype(BF16), U32)

        return [functools.partial(task, t) for t in range(LT)]

    def by_tile(product, put):
        acc = [None]

        def task(t, k):
            r = product(t, k)
            e = len(recent) % 16
            recent.extend(r[8 * (e + i) % TB:8 * (e + i) % TB + 8] for i in range(4))
            acc[0] = _add(acc[0] if k else None, r)
            if k == LT - 1:
                put(t, acc[0])

        return [functools.partial(task, t, k) for t in range(LT) for k in range(LT)]

    def a_load(i, b):
        xb[_ds(b, TB // 2), :] = pltpu.bitcast(ax[_ds(i, TB), :], U32)

    def a_proj(j, b, first_block=False):
        def put(t, r):
            if j == 0:
                q_s[b, t] = r
                return
            c = (j - 1) * LT + t
            kv_s[b, c, HALO:, :] = r
            if first_block:
                kv_s[b, c, 0:HALO, :] = jnp.broadcast_to(r[0:1, :], (HALO, 128))
            else:
                kv_s[b, c, 0:HALO, :] = kv_s[1 - b, c, TB:, :]

        return by_tile(lambda t, k: lax.dot_general(
            tile(xb, b, k), tile(wa, j * LT + t, k), NT, preferred_element_type=F32), put)

    def a_attention(b, zero, first_block=False):
        n = TB // 8
        lag = n if first_block else A_PACE[1]
        marks, logits = [], []

        def mark():
            marks.append(len(recent) - A_PACE[0])

        def window(c, w):
            return kv_s[b, c, pl.ds(HALO - ADIL * w, TB), :]

        def score():
            q = [paced(q_s[b, t], zero, marks[::4]) for t in range(LT)]
            sums = [functools.reduce(jnp.add, [q[t] * window(t, w) for t in range(LT)]) for w in range(AW)]
            rows = {}
            for k in range(n + 1):
                if k < n:
                    a = _cat(*[a[8 * k:8 * k + 8] for a in sums])
                    rows[k] = a + pltpu.roll(a, 2 * AH, 1)
                if k > 0:
                    rows[k - 1] = rows[k - 1] + pltpu.roll(rows[k - 1], AH, 1)
            logits.extend(_cat(*[rows[k][8 * w:8 * w + 8] for k in range(n)]) for w in range(AW))

        def mix():
            scale, lg = AD ** -0.5, logits
            if first_block:
                pos = lax.broadcasted_iota(jnp.int32, (HALO, 128), 0)
                lg = [_cat(jnp.where(pos >= ADIL * w, a[:HALO], MASKED / scale), a[HALO:])
                      for w, a in enumerate(lg)]
            m = paced(functools.reduce(jnp.maximum, lg), zero, marks[4 * lag + 1::4])
            e = [jnp.exp2((a - m) * (scale * LOG2E)) for a in lg]
            inv = 1.0 / functools.reduce(jnp.add, e)
            for t in range(LT):
                v = [window(LT + t, w) for w in range(AW)]
                v[0] = paced(v[0], zero, marks[4 * lag + 2 + 2 * t // LT::4])
                oa_s[b, :, _ds(t, 128)] = inv * functools.reduce(jnp.add, map(jnp.multiply, e, v))

        return [mark] * (4 * n) + [score], [mark] * (4 * lag) + [mix]

    def a_out(i, b):
        def put(t, r):
            outa[_ds(i, TB), _ds(t, 128)] = r.astype(BF16)

        return by_tile(lambda t, k: _dot(oa_s[b, :, _ds(k, 128)], tile(wa, 3 * LT + k, t)), put)

    def transposes(c, dst, g):
        def task(n):
            t = ((c & (RAW - 1)) * 3 + n % 9 // 3) * GW + n // 9 * 3 + n % 3
            v = pltpu.bitcast(raw[_ds(t, 128), :].T, U32)
            for k in range(LT):
                dst[_ds(g * GW + n, 64), _ds(k, 128)] = v[k * 64:(k + 1) * 64]

        return [functools.partial(task, n) for n in range(3 * GW)]

    def sum_blocks(block, put, zero):
        back, n = SUM_PACE
        marks = []

        def mark():
            marks.append(len(recent) - back)

        def done(r, v):
            if r not in SINGLE:
                put(r, pltpu.bitcast(v.astype(BF16), U32))

        def task():
            sums = _Sums(BLOCK_SUMS, done)
            for k in range(n):
                for i, b in enumerate(_share(BLOCK_ORDER, k, n)):
                    v = block(*divmod(b, GW))
                    if i == 0:
                        v = paced(v, zero, marks[k::n])
                    for r in SINGLE:
                        if SINGLE[r] == b:
                            put(r, v)
                    sums.add(b, 1, pltpu.bitcast(v, BF16).astype(F32))

        return [mark] * (8 * n) + [task]

    def sum_qkv(g, zero, src=plain, dst=summed):
        def put(r, v):
            if r not in SINGLE:
                i, j = divmod(SUMMED.index(r), LT)
                dst[_ds(g * 8 + i, 64), _ds(j, 128)] = v

        return sum_blocks(lambda k, n: src[_ds(g * GW + n, 64), _ds(k, 128)], put, zero)

    def sum_out(g, zero):
        def put(r, v):
            wo[_ds(g, 64), _ds(r, 128)] = v

        return sum_blocks(lambda k, n: pltpu.bitcast(wo_raw[_ds(g * GW + n, 128), _ds(k, 128)], U32), put, zero)

    def a_start():
        nq, nk = START_CUT
        start(c_aw[:2])
        zero = lax.fori_loop(0, 2, lambda it, carry: it >> 16, 0)
        start(c_ax(0))
        wait(c_aw[:1])
        start(c_aw[2:3])
        _run(a_weights(0)[:3])
        wait(c_aw[1:2])
        start(c_aw[3:])
        _run(a_weights(0)[3:])
        wait(c_ax(0))
        start(c_awo)
        a_load(0, 0)
        a_load(1, 1)
        _run(a_proj(0, 0) + a_proj(0, 1)[:nq])
        wait(c_aw[2:3])
        start(c_ax(1) + c_ax(2))
        _run(a_proj(0, 1)[nq:] + a_weights(1) + a_proj(1, 0, True))
        wait(c_aw[3:])
        start(c_w(0))
        early, late = a_attention(0, zero, True)
        _run(a_proj(1, 1)[:nk] + a_weights(2) + _merge(a_proj(2, 0, True), early))
        wait(c_awo + c_ax(1))
        start(c_bx0)
        _run(_merge(a_proj(1, 1)[nk:] + a_proj(2, 1), _merge(late, a_weights(3, zero)), 4))
        a_load(2, 0)

    def a_step(it, carry):
        i, g, zero = 2 * it, jnp.maximum(3 * it - 9 + PAD, 0), it >> 16
        pl.when(it + 2 < NB // 2)(lambda: start(c_ax(it + 2)))
        pl.when(it + 1 < NB // 2)(lambda: wait(c_ax(it + 1)))
        start(c_w(it))
        pl.when(it > 1)(lambda: wait(c_w(it - 2)))
        src, dst = [ref.at[pl.ds(pl.multiple_of(g * n, n), k * n)]
                    for ref, n, k in ((plain, GW * 64, 6), (summed, 8 * 64, 3))]
        sums, moves = _each(sum_qkv, range(3), zero, src, dst), transposes(it + RAW - 2, src, 3)
        cut, m1, m2 = len(sums) * A_CUT[0] // 100, A_CUT[1], A_CUT[2]
        early, late = a_attention(1, zero)
        a_load(i + 1, 1)
        _run(_merge(a_out(i - 2, 0) + _each(a_proj, range(3), 0),
                    moves[:m1] + _merge(early, sums[:cut]) + moves[m1:m2]))
        a_load(jnp.minimum(i + 2, NB - 1), 0)
        side = sum(a_attention(0, zero), [])
        side = _merge(side[:len(late)], late) + side[len(late):]
        _run(_merge(_each(a_proj, range(3), 1) + a_out(i - 1, 1), _merge(side, sums[cut:]) + moves[m2:], A_CUT[3]))
        return zero

    def attention(qkv, put, row0=0):
        row = lax.broadcasted_iota(jnp.int32, (L - row0, 2 * L), 0) + row0
        col = lax.broadcasted_iota(jnp.int32, (L - row0, 2 * L), 1)
        head0 = col < L
        visible = (row < M) | (row >= jnp.where(head0, col, col - L))
        scale = DH ** -0.5
        st = {}

        def by_head(n):
            t = qkv(n)
            if n % 3 == 1:
                low = lax.broadcasted_iota(jnp.int32, t.shape, 1) < 64
                t = _cat(jnp.where(low, t, 0.0), jnp.where(low, 0.0, t))
            elif n % 3 == 2:
                t = _cat(jnp.zeros_like(t), t)
            return t.astype(BF16)

        def score(p):
            sc = [lax.dot_general(qkv(9 * p + t), by_head(9 * p + 3 + t), NT, preferred_element_type=F32)
                  for t in range(3)]
            sc = _add(_add(jnp.concatenate([sc[0], jnp.zeros_like(sc[0])], axis=1), sc[1]), sc[2])
            sc = jnp.where(visible, sc, MASKED / scale)
            m0 = jnp.max(jnp.where(head0, sc, -jnp.inf), axis=1, keepdims=True)
            m1 = jnp.max(jnp.where(head0, -jnp.inf, sc), axis=1, keepdims=True)
            st[p] = sc - jnp.where(head0, m0, m1)

        def normalize(p):
            e = jnp.exp2(st[p] * (scale * LOG2E))
            l0 = jnp.sum(jnp.where(head0, e, 0.0), axis=1, keepdims=True)
            l1 = jnp.sum(jnp.where(head0, 0.0, e), axis=1, keepdims=True)
            st[p] = e / jnp.where(head0, l0, l1)

        def mix(p):
            for t in range(3):
                put(3 * p + t, _dot(st[p] if t else st[p][:, :L], by_head(9 * p + 6 + t)))

        return score, normalize, mix

    def mixed_at(n):
        return [(ref, n - g0 * GW) for ref, (g0, g1) in zip(mixed, CHUNKS) if g0 <= n // GW < g1][0]

    def put_x(n, r):
        ref, k = mixed_at(n)
        ref[k, 0:M] = r[0:M]
        ox[n] = r[M:]

    def put_y(n, r):
        ref, k = mixed_at(n)
        ref[k] = _cat(r[0:M], ox[n] - r[M:], r[M:])

    def left_operands(s, zero):
        def task(e):
            x, y = [bx[_ds((s + k) * (SEG // M) + e, M), :].astype(F32) for k in range(2)]
            x = [x[:, k * 128:(k + 1) * 128] for k in range(LT)]
            y = [paced(y[:, k * 128:(k + 1) * 128], zero, [len(recent) - TOKENS_AT[2] * (LT - k)])
                 for k in range(LT)]
            z = [a + b for a, b in zip(x, y)]
            for r in range(NR):
                lhs[r, _ds(e + e // 2, M)] = _val(_sum((a or b, z[k] if a and b else x[k] if a else y[k])
                                                       for k, (a, b) in enumerate(MODEL[r]) if a or b))

        return [functools.partial(task, e) for e in range(SEG // M)]

    def step(s, second, zero):
        def reread(ref):
            return ref.at[pl.ds(4 * zero, ref.shape[0])]

        part_r, lhs_r, ring_r = reread(part), reread(lhs), [reread(r) for r in ring]
        halves = [slice(0, HS), slice(HS, SEG)][::1 - 2 * second]
        new_mem = [None] * LT
        due = []

        def mm(x, w):
            r = _dot(x, w)
            recent.append(r[0:M] if second and len(recent) > TOKENS_AT[0] - 48 else None)
            while due and due[0][0] <= len(recent):
                due.pop(0)[1]()
            return r

        def in_turn(items):
            lists = [[x for x in items if (x[0] >= BOTH) == e] for e in (False, True)]
            for _ in items:
                yield lists[TURNS >> second * (NQ + NO) * LT + len(recent) & 1].pop(0)

        def mem_tiles(r):
            return [MEM_ORDER[k] for k, c in enumerate(MODEL[r]) if c[second]]

        def project(g):
            def token_sums(e):
                def begin(k):
                    return part_r[g, k, halves[e]] if second and QKV_SUMS[0][1 - e][1][k] else None

                def done(k, v):
                    n = GW * g + k // 2
                    if not second:
                        part[g, k, halves[e]] = v
                    elif k % 2:
                        tok[n, halves[e]] = v
                    else:
                        ring[n // 3 % RING][n % 3, pl.ds(M + halves[e].start, HS)] = v

                return _Sums(QKV_SUMS[second][e], done, begin)

            def done(k, v):
                n = GW * g + k
                ring[n // 3 % RING][n % 3, 0:M] = v

            sums = token_sums(0), token_sums(1), _Sums(QKV_SUMS[second][2], done)
            weights = pltpu.bitcast(summed[_ds(PAD + g, 8 * 64), :], BF16)
            order = sorted(QKV_ORDER[second], key=lambda r: 0 if g else max(mem_tiles(r)))
            for r, in in_turn([(r,) for r in order]):
                t0, t1 = (0, L) if r < BOTH else (second * HS, second * HS + HS + M)
                if g == 0:
                    lhs[r, HS:HS + M] = _val(_sum(
                        (c[second], m_s[k]) for k, c in enumerate(MODEL[r]) if c[second]))
                if r in SINGLE:
                    w = tile(plain, (PAD + g) * GW + SINGLE[r] % GW, SINGLE[r] // GW)
                else:
                    i, j = divmod(SUMMED.index(r), LT)
                    w = weights[i * 128:(i + 1) * 128, j * 128:(j + 1) * 128]
                v = mm((lhs_r if g else lhs)[r, t0:t1], w)
                sums[2].add(r, 1, v[HS - t0:HS - t0 + M])
                if t0 == 0:
                    sums[second].add(r, 1, v[:HS])
                if t1 == L:
                    sums[1 - second].add(r, 1, v[-HS:])

        def projected(n):
            src = ring_r[n // 3 % RING]
            return src[n % 3] if second else _cat(src[n % 3, 0:M], tok[n])

        def out_chunk(ref, g0, g1):
            def token_sums(e):
                def begin(k):
                    if (second and OUT_SUMS[0][1 - e][1][k]) or (g0 > 0 and OUT_SUMS[second][e][1][k]):
                        return opart[k, halves[e]]

                def done(k, v):
                    if second and g1 == GO:
                        rows = _ds((s + k % 2) * 2 + halves[e].start // HS, HS)
                        outb[rows, _ds(k // 2, 128)] = v.astype(BF16)
                    else:
                        opart[k, halves[e]] = v

                return _Sums(OUT_SUMS[second][e], done, begin)

            def done(k, v):
                new_mem[k] = v
                if g1 == GO:
                    m_s[k] = v

            sums = token_sums(0), token_sums(1), _Sums(OUT_SUMS[second][2], done, list(new_mem).__getitem__)
            weights = [pltpu.bitcast(wo[_ds(g, 64), :], BF16) for g in range(g0, g1)]
            order = sorted(OUT_ORDER[second], key=lambda r: min(mem_tiles(r)) if g1 == GO else 0)
            tall, short = [[r for r in order if (r >= BOTH) == e] for e in (False, True)]
            n = OUT_PARTS[second]
            for k in range(n):
                acc = {}
                some = _share(tall[::-1], n - 1 - k, n)[::-1] + _share(short, k, n)
                for r, g in in_turn([(r, g) for g in range(g0, g1) for r in some]):
                    t0, rows = (0, SEG) if r < BOTH else (halves[0].start, HS)
                    terms = []
                    for j, (a, b) in enumerate(FEATURE[r]):
                        i = (g - g0) * GW + j
                        if b:
                            terms.append((a or b, ref[i, pl.ds((M if a else L) + t0, rows)]))
                        elif a and second:
                            terms += [(a, ref[i, pl.ds(r0 + t0, rows)]) for r0 in (M, L)]
                        elif a:
                            terms.append((a, ox[g * GW + j, pl.ds(t0, rows)]))
                    sign, left = _sum(terms)
                    m_sign, m = _sum((c[second], ref[(g - g0) * GW + j, 0:M])
                                     for j, c in enumerate(FEATURE[r]) if c[second])
                    v = mm(_cat(m, left), weights[g - g0][:, r * 128:(r + 1) * 128])
                    acc[r] = m_sign, sign, _add(acc[r][2] if r in acc else None, v)
                for r, (m_sign, sign, v) in acc.items():
                    sums[2].add(r, m_sign, v[:M])
                    sums[second if r < BOTH else 0].add(r, sign, v[M:M + HS])
                    if r < BOTH:
                        sums[1 - second].add(r, sign, v[M + HS:])

        recent.clear()
        stages = attention(projected, put_x if second else put_y)
        for p in range(NP):
            ready = LT * GW * ((9 * p + 5) // GW + 1)
            due += [(ready + lag, functools.partial(f, p)) for f, lag in zip(stages, LAGS[second])]
        if second:
            due += [(TOKENS_AT[0] + k * TOKENS_AT[1], task)
                    for k, task in enumerate(left_operands(jnp.minimum(s + 4, NSEG - 2), zero))]
        due.sort(key=lambda e: e[0])
        for g in range(GQ):
            project(g)
        for ref, chunk in zip(mixed, CHUNKS):
            out_chunk(reread(ref), *chunk)

    def first_segment(zero):
        def project(g):
            acc = {}

            def task(n, k):
                r = _dot(h0[0:L + SEG, _ds(k, 128)], tile(plain, PAD * GW + n, k))
                e = len(recent) % 8
                recent.extend([r[8 * e:8 * e + 8], r[8 * e + 8:8 * e + 16]])
                acc[n] = _add(acc.get(n), r)
                if k == LT - 1:
                    first[n] = acc[n][0:L]
                    tok[n] = acc[n][L:]

            return [functools.partial(task, g * GW + n, k) for n in range(GW) for k in range(LT)]

        def put(n, r):
            recent.extend([r[k:k + 8] for k in range(0, L, 16)])
            put_x(n, r)

        stages = attention(lambda n: first[n], put)
        new_mem = [None] * LT

        def heads(p0, p1):
            return [functools.partial(f, t - lag) for t in range(p0, p1 + 2)
                    for lag, f in enumerate(stages) if p0 <= t - lag < p1] + [lambda: None]

        def out(g):
            def task(n, k):
                ref, i = mixed_at(n)
                r = _dot(ref[i, 0:M], wo_raw[_ds(n, 128), _ds(k, 128)])
                recent.append(r)
                new_mem[k] = r if new_mem[k] is None else new_mem[k] + r

            return [functools.partial(task, g * GW + n, k) for n in range(GW) for k in range(LT)]

        c1, c2, c3, d1, d2, m1 = FIRST_CUT
        moves = transposes(GO - 2, plain, PAD + GQ - 6) + transposes(GO - 1, plain, PAD + GQ - 3)
        start(c_wo(0))
        wait(c_w(GO - 2) + c_bx0)
        start(c_wo(1) + c_wo(2))
        h0[0:M, :] = mem[0:M, :].astype(F32)
        h0[M:L + SEG, :] = bx[0:2 * SEG, :].astype(F32)
        _run(_merge(a_out(NB - 2, 0) + _each(project, range(c1)), moves[:m1] + _merge(
            sum(a_attention(1, zero), []), _each(sum_qkv, range(PAD + GQ - 9, PAD + d1), zero))))
        wait(c_w(GO - 1))
        start(c_wo(3) + c_wo(4))
        _run(_merge(a_out(NB - 1, 1) + _each(project, range(c1, c2)),
                    moves[m1:] + _each(sum_qkv, range(PAD + d1, PAD + d2), zero)))
        start(c_wo(5))
        wait(_each(c_wo, range(3)))
        start(c_wo(6) + c_wo(7))
        _run(_merge(_merge(_each(project, range(c2, c3)), heads(0, 11)),
                    _each(sum_qkv, range(PAD + d2, PAD + GQ), zero) + _each(sum_out, range(3), zero)))
        wait(_each(c_wo, range(3, 6)))
        _run(_merge(_merge(_merge(_each(project, range(c3, GQ)), _each(out, range(3))), heads(11, 13))
                    + _merge(_each(out, range(3, 6)), heads(13, NP)),
                    _merge(_each(sum_out, range(3, 6), zero), left_operands(2, zero))))
        wait(c_wo(6) + c_wo(7))
        start(c_bx1 + c_outa)
        _run(_merge(out(6) + out(7), _each(sum_out, (6, 7), zero)))
        for k in range(LT):
            m_s[k] = new_mem[k]

    def two_segments(it, carry):
        pl.when(it == 1)(lambda: wait(c_bx1))
        step(2 * it, 0, it >> 16)
        step(2 * it, 1, it >> 16)
        start(c_outb(_ds(it, 2 * SEG)))
        return carry

    def last_segment():
        res, acc = {}, [None] * LT

        def project(n, k):
            r = _dot(-m_s[k] if k % 2 else m_s[k], tile(plain, PAD * GW + n, k))
            res[n] = _acc(res.get(n), 1 - 2 * (k % 2), r)

        def out(n, k):
            acc[k] = _add(acc[k], _dot(_cat(ox[n], res[NQ + n]), wo_raw[_ds(n, 128), _ds(k, 128)]))

        stages = attention(lambda n: _cat(_val(res[n]), tok[n]) if n in res else tok[n],
                           lambda n, r: res.update({NQ + n: r}), M)
        tiles = [9 * p + e for t in range(NP + 3) for p, e0 in ((t, 3), (t - 3, 6)) if 0 <= p < NP
                 for e in range(e0, e0 + 3)]
        ready = {n: (i * LT + LT - 1) // 4 for i, n in enumerate(tiles)}
        due = [((i * LT + k) // 4, 0, functools.partial(project, n, k))
               for i, n in enumerate(tiles) for k in range(LT)]
        for p in range(NP):
            due += [(ready[9 * p + e] + lag, rank, functools.partial(f, p))
                    for f, lag, e, rank in zip(stages, LAST_LAGS, (5, 5, 8), (2, 2, 1))]
        t = 0
        for k in range(NO * LT):
            if k % 4 == 0:
                t = max(t + LAST_LAGS[4], ready[9 * ((k + 3) // 15) + 8] + LAST_LAGS[3])
            due.append((int(t), 3, functools.partial(out, *divmod(k, LT))))
        _run([task for _, _, task in sorted(due, key=lambda e: e[:2])])
        outb[S - 2 * SEG:, :] = jnp.concatenate(acc, axis=1).astype(BF16)
        start(c_outb(slice(S - 2 * SEG, S)))

    a_start()
    first_segment(lax.fori_loop(1, NB // 2, a_step, 0))
    lax.fori_loop(0, NSEG // 2 - 1, two_segments, 0)
    last_segment()
    wait(c_outa + c_outb(slice(0, S)))


def pallas_concat_heads__sliding_local_dilated__memory_aug_recurrent_mem_tr__prompt_kernel(
    A_x, A_wqkv, A_wo, B_x, B_mem0, B_Wq, B_Wk, B_Wv, B_Wo, B_seg_len,
):
    assert B_seg_len == SEG
    assert A_x.shape == B_x.shape == (1, S, D) and B_mem0.shape == (1, M, D)
    assert B_Wq.shape == B_Wk.shape == B_Wv.shape == (D, H, DH) and B_Wo.shape == (H, DH, D)
    dma = pltpu.SemaphoreType.DMA

    def vmem(shape, dtype):
        assert math.prod(shape) * jnp.dtype(dtype).itemsize % 16384 == 0
        return pltpu.VMEM(shape, dtype)

    call = pl.pallas_call(
        _kernel,
        out_shape=jax.ShapeDtypeStruct((S, 2 * D), BF16),
        in_specs=[pl.BlockSpec(memory_space=pl.ANY)] * 9,
        out_specs=pl.BlockSpec(memory_space=pl.ANY),
        scratch_shapes=[
            vmem((S, D), BF16),
            vmem((3, D, D), BF16),
            vmem((D, D), BF16),
            vmem((LT, D, 128), F32),
            vmem((2 * D, D), U32),
            vmem((TB, D), U32),
            vmem((2, LT, TB, 128), F32),
            vmem((2, 2 * LT, HALO + TB, 128), F32),
            vmem((2, TB, D), F32),
            vmem((S, D), BF16),
            vmem((S, D), BF16),
            vmem((8 * M, D), BF16),
            vmem((RAW * 3 * GW * 128, D), BF16),
            vmem((H * DH, D), BF16),
            vmem(((PAD + GQ) * GW * 64, D), U32),
            vmem(((PAD + GQ) * 8 * 64, D), U32),
            vmem((GO * 64, NR * 128), U32),
            vmem((3 * SEG, D), F32),
            vmem((NQ, L, 128), F32),
            vmem((NR + 1, L, 128), F32),
            vmem((8, M, 128), F32),
            vmem((GQ, 2 * GW, SEG, 128), F32),
            vmem((NQ, SEG, 128), F32),
            [vmem((4, L, 128), F32)] * RING,
            vmem((NO, SEG, 128), F32),
            [vmem((20, L + SEG, 128), F32)] * len(CHUNKS),
            vmem((2 * LT, SEG, 128), F32),
            vmem((S, D), BF16),
            dma((5,)), dma((NB // 2,)), dma((GO, 3)), dma((3,)), dma((GO,)), dma((2,)),
        ],
        compiler_params=pltpu.CompilerParams(vmem_limit_bytes=126 * 1024 * 1024, **{
            name: True for name in ("disable_bounds_checks", "disable_semaphore_checks")
            if hasattr(pltpu.CompilerParams, name)}),
        name="sliding_and_memory_attention",
    )

    def by_feature(w):
        return w.transpose(1, 2, 0).reshape(H * DH, D)

    out = call(A_x.reshape(S, D), A_wqkv, A_wo, B_x.reshape(S, D), B_mem0.reshape(M, D),
               by_feature(B_Wq), by_feature(B_Wk), by_feature(B_Wv), B_Wo.reshape(H * DH, D))
    return out.reshape(1, S, 2 * D)
```

```python
import collections
import functools
import itertools
import math
import random

import jax
import jax.numpy as jnp
import numpy as np
from jax import lax
from jax.experimental import pallas as pl
from jax.experimental.pallas import tpu as pltpu

F32, BF16, U32 = jnp.float32, jnp.bfloat16, jnp.uint32
NT = (((1,), (1,)), ((), ()))
MASKED = -1000000000.0
LOG2E = math.log2(math.e)

S, D = 2048, 640
LT = D // 128

AH, AD, AW, ADIL = 32, 20, 8, 2
HALO = 16
TB = 128
NB = S // TB

H, DH, M, SEG = 32, 192, 8, 32
L = M + SEG
HS = SEG // 2
NSEG = S // SEG
NP = H // 2
NO = 3 * NP
NQ = 3 * NO
GW = 6
GO, GQ = NO // GW, NQ // GW
PAD = 3
RAW = 4
RING = 12
CHUNKS = ((0, 3), (3, 5), (5, GO))


def _algorithm(rank_ones):
    rows = np.array([[1, 0], [0, 1], [1, 1]])
    duals = np.array([[0, 1], [1, 0], [1, -1]])
    sets = [[[np.array(["-0+".index(c) - 1 for c in w]) for w in e.split()] for e in s] for s in rank_ones]
    left, right = [], []
    for t, s in enumerate(sets):
        p, q = [k for k in range(3) if k != t]
        for u, v in s:
            left += [np.outer(u, rows[p]), np.outer(u, rows[q])]
            right += [np.outer(v, duals[q]), np.outer(v, duals[p])]
    for (u0, v0), (u1, v1), (u2, v2) in itertools.product(*sets):
        for a, b in itertools.product((1, -1), repeat=2):
            e = np.outer(u0 + a * u1, v0 + b * v1)
            if (e == np.outer(u2, v2)).all() or (e == -np.outer(u2, v2)).all():
                left.append(np.outer(u0, rows[1]) - a * np.outer(u1, rows[0]))
                right.append(np.outer(v0, duals[1]) + b * np.outer(v1, duals[0]))
    left, right = np.array(left), np.array(right)
    have = np.einsum("rka,rnb->kanbr", left, right).reshape(-1, len(left))
    want = np.einsum("kp,nq,ab->kanbpq", np.eye(LT), np.eye(GW), np.eye(2)).reshape(len(have), -1)
    blocks = np.rint(np.linalg.lstsq(have, want, rcond=None)[0]).astype(int)
    assert (have @ blocks == want).all()
    sign = blocks.max(axis=1) * 2 - 1
    return left * sign[:, None, None], blocks * sign[:, None], right


def _shared_sums(matrix, seed):
    rng = random.Random(seed)
    rows = [{k: int(c) for k, c in enumerate(row) if c} for row in matrix]
    shared = {}
    while True:
        count = collections.Counter(
            (a, b, r[a] * r[b]) for r in rows for a, b in itertools.combinations(sorted(r), 2))
        top = max(count.values(), default=0)
        if top < 2:
            return shared, rows
        best = sorted(k for k, n in count.items() if n == top)
        a, b, sign = best[int(rng.random() * len(best))]
        name = matrix.shape[1] + len(shared)
        shared[name] = a, b, sign
        for r in rows:
            if r.get(a, 0) * r.get(b, 0) == sign:
                r[name] = r.pop(a)
                del r[b]


MODEL, BLOCKS, FEATURE = _algorithm((
    ("+0000 +00++0", "000+0 0+0000", "0000+ 000+00", "+-+00 00000+", "+00+0 00+0+0"),
    ("0+00+ 000+++", "0+0+0 0+00++", "00+-+ 00++00", "00+0+ +00000", "+0+00 0000+0", "00+00 0+-000"),
    ("0+000 0000++", "00+-+ ++0000", "00+00 +00+00", "+-000 0+-00+", "00+-0 00+000", "+-00- +0000-")))
NR = len(BLOCKS)
BOTH = 34
SINGLE = {r: int(row.argmax()) for r, row in enumerate(BLOCKS) if abs(row).sum() == 1}
SUMMED = [r for r in range(NR) if r not in SINGLE]


def _step_sums(out, step, seed):
    use = MODEL[:, :, step].any(1) & FEATURE[:, :, step].any(1)
    return [_shared_sums((m * keep[:, None]).T, seed) for m, keep in (
        (out.reshape(NR, -1), use), (out.reshape(NR, -1), use & (np.arange(NR) < BOTH)), (out[:, :, step], use))]


QKV_SUMS = _step_sums(FEATURE, 0, 32), _step_sums(FEATURE, 1, 5)
OUT_SUMS = _step_sums(MODEL, 0, 0), _step_sums(MODEL, 1, 6)
BLOCK_SUMS = _shared_sums(BLOCKS, 37)

QKV_ORDER = (
    (30, 14, 20, 3, 28, 12, 9, 22, 10, 18, 26, 1, 5, 24, 32, 7, 16,
     40, 38, 36, 45, 46, 44, 39, 34, 35, 43, 37, 41, 42),
    (31, 15, 4, 11, 27, 0, 8, 19, 23, 13, 33, 6, 29, 21, 2, 25, 17,
     40, 34, 41, 39, 35, 45, 46, 36, 43, 44, 38, 37, 42))
OUT_ORDER = (
    (24, 14, 10, 5, 32, 28, 16, 30, 22, 7, 9, 3, 12, 1, 18, 26, 20,
     40, 34, 41, 39, 42, 37, 43, 36, 45, 46, 44, 35, 38),
    (23, 11, 2, 13, 15, 17, 4, 25, 31, 6, 33, 29, 8, 21, 19, 27, 0,
     39, 36, 45, 34, 40, 41, 37, 44, 42, 43, 46, 35, 38))
BLOCK_ORDER = (3, 28, 6, 0, 5, 17, 11, 8, 10, 7, 4, 16, 2, 1, 23, 22, 9, 29, 24, 19, 12, 18, 25, 13, 14, 20,
               21, 15, 26, 27)
MEM_ORDER = (0, 1, 4, 2, 3)

LAGS = ((40, 70, 100), (50, 80, 110))
TOKENS_AT = (737, 2)
OUT_PARTS = (5, 5)
TURNS = int(
    "d2d2969694a50b4a5a52852d29696852cd2852d2d2d2d2942c1a5a59861861d4a5861e4a534351a9a89a8d14d487925a"
    "50e17186969348b8a1cca92c385c694a5a294b487948784d46a6a26a3453521e4a5a16954aa8aaa50d4c54c7153161b2"
    "a62a692535258d294a5a5294a5a552a4a6a26a686a62a6a4b4a6a6a6a62862a6a6a24a26a6a6a42a6a65217171717152"
    "1585a5a52a18694a552a6a43929694a55296943a43c35166870d4964a5a50e94a5a16961c386934b0e168e1a9294e529"
    "a12cd4a5871385a529694a587138b0e1a8e1a8b0e626a62c1e1c3870790d4c29e1c3931a193931a949a94a949a949871", 16)

A_PACE = (12, 4)
SUM_PACE = (18, 10)
A_CUT = (58, 1, 18, 0)
START_CUT = (5, 20)
FIRST_CUT = (5, 12, 21, 17, 21, 6)
LAST_LAGS = (7, 12, 3, 7, 1.9)


def _ds(i, n):
    return pl.ds(i * n if isinstance(i, int) else pl.multiple_of(i * n, n), n)


def _dot(a, b):
    return jnp.dot(a, b, preferred_element_type=F32)


def _cat(*parts):
    return jnp.concatenate(parts, axis=0)


def _add(a, b):
    return b if a is None else _cat(a[:M] + b[:M], a[M:] + b[M:])


def _acc(a, sign, b):
    if a is None:
        return sign, b
    if a[0] == sign:
        return sign, a[1] + b
    return (1, a[1] - b) if a[0] > 0 else (1, b - a[1])


def _sum(terms):
    return functools.reduce(lambda a, t: _acc(a, *t), terms, None)


def _val(a):
    return a[1] if a[0] > 0 else -a[1]


class _Sums:
    def __init__(self, plan, done, begin=lambda k: None):
        self.shared, self.rows = plan
        self.done, self.begin = done, begin
        self.terms, self.sums = {}, [None] * len(self.rows)
        for k, row in enumerate(self.rows):
            if not row and (first := begin(k)) is not None:
                done(k, first)

    def add(self, name, sign, value):
        self.terms[name] = sign, value
        for k, row in enumerate(self.rows):
            if name in row:
                if self.sums[k] is None and (first := self.begin(k)) is not None:
                    self.sums[k] = 1, first
                self.sums[k] = _acc(self.sums[k], row[name] * sign, value)
                if all(n in self.terms for n in row):
                    self.done(k, _val(self.sums[k]))
        for n, (a, b, s) in self.shared.items():
            if name in (a, b) and a in self.terms and b in self.terms and n not in self.terms:
                self.add(n, *_acc(self.terms[a], s * self.terms[b][0], self.terms[b][1]))


def _share(tasks, k, n):
    return list(tasks[k * len(tasks) // n:(k + 1) * len(tasks) // n])


def _merge(a, b, early=0):
    n = len(a) - early
    return [t for k in range(n) for t in [a[k]] + _share(b, k, n)] + a[n:]


def _each(f, items, *args):
    return [task for item in items for task in f(item, *args)]


def _run(tasks):
    for task in tasks:
        task()


def _kernel(ax_hbm, awqkv_hbm, awo_hbm, bx_hbm, mem_hbm, wq_hbm, wk_hbm, wv_hbm, wo_hbm,
            out_hbm,
            ax, awqkv, awo, tmp, wa, xb, q_s, kv_s, oa_s, outa,
            bx, mem, raw, wo_raw, plain, summed, wo, h0, first, xy, lhs, m_s, part, tok, ring,
            ox, mixed, opart, outb,
            sem_a, sem_x, sem_w, sem_b, sem_wo, sem_o):
    cp = pltpu.make_async_copy

    def rows_copy(src, dst, rows, sem):
        return [cp(src.at[rows, :], dst.at[rows, :], sem)]

    c_aw = [cp(awqkv_hbm.at[r0:r1, _ds(j, D)], awqkv.at[j, r0:r1], sem_a.at[k])
            for k, (j, r0, r1) in enumerate(((0, 0, 384), (0, 384, D), (1, 0, D), (2, 0, D)))]
    c_awo = [cp(awo_hbm, awo, sem_a.at[4])]
    c_bx0 = [cp(mem_hbm, mem.at[0:M], sem_b.at[0])] + rows_copy(bx_hbm, bx, slice(0, 6 * SEG), sem_b.at[1])
    c_bx1 = rows_copy(bx_hbm, bx, slice(6 * SEG, S), sem_b.at[2])
    c_outa = [cp(outa, out_hbm.at[:, 0:D], sem_o.at[0])]

    def c_ax(c):
        return rows_copy(ax_hbm, ax, _ds(c, 2 * TB), sem_x.at[c])

    def c_w(c):
        return [cp(w.at[_ds(c, GW * 128), :], raw.at[_ds((c & (RAW - 1)) * 3 + j, GW * 128), :], sem_w.at[c, j])
                for j, w in enumerate((wq_hbm, wk_hbm, wv_hbm))]

    def c_wo(g):
        return rows_copy(wo_hbm, wo_raw, _ds(g, GW * 128), sem_wo.at[g])

    def c_outb(rows):
        return [cp(outb.at[rows, :], out_hbm.at[rows, D:], sem_o.at[1])]

    def start(copies):
        for c in copies:
            c.start()

    def wait(copies):
        for c in copies:
            c.wait()
        recent.clear()

    recent = []

    def paced(x, zero, marks):
        late = _cat(*[recent[t] if t >= 0 else jnp.zeros((8, 128), F32) for t in marks[:x.shape[0] // 8]])
        always = lax.broadcasted_iota(jnp.int32, x.shape, 1) >= zero
        return lax.select(always, x, late if x.dtype == F32 else pltpu.bitcast(late, U32))

    def tile(ref, i, j):
        return pltpu.bitcast(ref[_ds(i, 64), _ds(j, 128)], BF16)

    def a_weights(j, zero=None):
        def task(t):
            if j < 3:
                tmp[t] = awqkv[j, _ds(t, 128), :].astype(F32).T
            else:
                marks = [len(recent) - 40 + k * 3 // 4 for k in range(40)]
                w = paced(pltpu.bitcast(awo[:, _ds(t, 128)], U32), zero, marks)
                tmp[t] = pltpu.bitcast(w, BF16).astype(F32)
            w = _cat(*[tmp[t, pl.ds(d, AH, stride=AD), :] for d in range(AD)])
            wa[_ds(j, D // 2), _ds(t, 128)] = pltpu.bitcast(w.astype(BF16), U32)

        return [functools.partial(task, t) for t in range(LT)]

    def by_tile(product, put):
        acc = [None]

        def task(t, k):
            r = product(t, k)
            e = len(recent) % 16
            recent.extend(r[8 * (e + i) % TB:8 * (e + i) % TB + 8] for i in range(4))
            acc[0] = _add(acc[0] if k else None, r)
            if k == LT - 1:
                put(t, acc[0])

        return [functools.partial(task, t, k) for t in range(LT) for k in range(LT)]

    def a_load(i, b):
        xb[_ds(b, TB // 2), :] = pltpu.bitcast(ax[_ds(i, TB), :], U32)

    def a_proj(j, b, first_block=False):
        def put(t, r):
            if j == 0:
                q_s[b, t] = r
                return
            c = (j - 1) * LT + t
            kv_s[b, c, HALO:, :] = r
            if first_block:
                kv_s[b, c, 0:HALO, :] = jnp.broadcast_to(r[0:1, :], (HALO, 128))
            else:
                kv_s[b, c, 0:HALO, :] = kv_s[1 - b, c, TB:, :]

        return by_tile(lambda t, k: lax.dot_general(
            tile(xb, b, k), tile(wa, j * LT + t, k), NT, preferred_element_type=F32), put)

    def a_attention(b, zero, first_block=False):
        n = TB // 8
        lag = n if first_block else A_PACE[1]
        marks, logits = [], []

        def mark():
            marks.append(len(recent) - A_PACE[0])

        def window(c, w):
            return kv_s[b, c, pl.ds(HALO - ADIL * w, TB), :]

        def score():
            q = [paced(q_s[b, t], zero, marks[::4]) for t in range(LT)]
            sums = [functools.reduce(jnp.add, [q[t] * window(t, w) for t in range(LT)]) for w in range(AW)]
            rows = {}
            for k in range(n + 1):
                if k < n:
                    a = _cat(*[a[8 * k:8 * k + 8] for a in sums])
                    rows[k] = a + pltpu.roll(a, 2 * AH, 1)
                if k > 0:
                    rows[k - 1] = rows[k - 1] + pltpu.roll(rows[k - 1], AH, 1)
            logits.extend(_cat(*[rows[k][8 * w:8 * w + 8] for k in range(n)]) for w in range(AW))

        def mix():
            scale, lg = AD ** -0.5, logits
            if first_block:
                pos = lax.broadcasted_iota(jnp.int32, (HALO, 128), 0)
                lg = [_cat(jnp.where(pos >= ADIL * w, a[:HALO], MASKED / scale), a[HALO:])
                      for w, a in enumerate(lg)]
            m = paced(functools.reduce(jnp.maximum, lg), zero, marks[4 * lag + 1::4])
            e = [jnp.exp2((a - m) * (scale * LOG2E)) for a in lg]
            inv = 1.0 / functools.reduce(jnp.add, e)
            for t in range(LT):
                v = [window(LT + t, w) for w in range(AW)]
                v[0] = paced(v[0], zero, marks[4 * lag + 2 + 2 * t // LT::4])
                oa_s[b, :, _ds(t, 128)] = inv * functools.reduce(jnp.add, map(jnp.multiply, e, v))

        return [mark] * (4 * n) + [score], [mark] * (4 * lag) + [mix]

    def a_out(i, b):
        def put(t, r):
            outa[_ds(i, TB), _ds(t, 128)] = r.astype(BF16)

        return by_tile(lambda t, k: _dot(oa_s[b, :, _ds(k, 128)], tile(wa, 3 * LT + k, t)), put)

    def transposes(c, dst, g):
        def task(n):
            t = ((c & (RAW - 1)) * 3 + n % 9 // 3) * GW + n // 9 * 3 + n % 3
            v = pltpu.bitcast(raw[_ds(t, 128), :].T, U32)
            for k in range(LT):
                dst[_ds(g * GW + n, 64), _ds(k, 128)] = v[k * 64:(k + 1) * 64]

        return [functools.partial(task, n) for n in range(3 * GW)]

    def sum_blocks(block, put, zero):
        back, n = SUM_PACE
        marks = []

        def mark():
            marks.append(len(recent) - back)

        def done(r, v):
            if r not in SINGLE:
                put(r, pltpu.bitcast(v.astype(BF16), U32))

        def task():
            sums = _Sums(BLOCK_SUMS, done)
            for k in range(n):
                for i, b in enumerate(_share(BLOCK_ORDER, k, n)):
                    v = block(*divmod(b, GW))
                    if i == 0:
                        v = paced(v, zero, marks[k::n])
                    for r in SINGLE:
                        if SINGLE[r] == b:
                            put(r, v)
                    sums.add(b, 1, pltpu.bitcast(v, BF16).astype(F32))

        return [mark] * (8 * n) + [task]

    def sum_qkv(g, zero, src=plain, dst=summed):
        def put(r, v):
            if r not in SINGLE:
                i, j = divmod(SUMMED.index(r), LT)
                dst[_ds(g * 8 + i, 64), _ds(j, 128)] = v

        return sum_blocks(lambda k, n: src[_ds(g * GW + n, 64), _ds(k, 128)], put, zero)

    def sum_out(g, zero):
        def put(r, v):
            wo[_ds(g, 64), _ds(r, 128)] = v

        return sum_blocks(lambda k, n: pltpu.bitcast(wo_raw[_ds(g * GW + n, 128), _ds(k, 128)], U32), put, zero)

    def a_start():
        nq, nk = START_CUT
        start(c_aw[:2])
        zero = lax.fori_loop(0, 2, lambda it, carry: it >> 16, 0)
        start(c_ax(0))
        wait(c_aw[:1])
        start(c_aw[2:3])
        _run(a_weights(0)[:3])
        wait(c_aw[1:2])
        start(c_aw[3:])
        _run(a_weights(0)[3:])
        wait(c_ax(0))
        start(c_awo)
        a_load(0, 0)
        a_load(1, 1)
        _run(a_proj(0, 0) + a_proj(0, 1)[:nq])
        wait(c_aw[2:3])
        start(c_ax(1) + c_ax(2))
        _run(a_proj(0, 1)[nq:] + a_weights(1) + a_proj(1, 0, True))
        wait(c_aw[3:])
        start(c_w(0))
        early, late = a_attention(0, zero, True)
        _run(a_proj(1, 1)[:nk] + a_weights(2) + _merge(a_proj(2, 0, True), early))
        wait(c_awo + c_ax(1))
        start(c_bx0)
        _run(_merge(a_proj(1, 1)[nk:] + a_proj(2, 1), _merge(late, a_weights(3, zero)), 4))
        a_load(2, 0)

    def a_step(it, carry):
        i, g, zero = 2 * it, jnp.maximum(3 * it - 9 + PAD, 0), it >> 16
        pl.when(it + 2 < NB // 2)(lambda: start(c_ax(it + 2)))
        pl.when(it + 1 < NB // 2)(lambda: wait(c_ax(it + 1)))
        start(c_w(it))
        pl.when(it > 1)(lambda: wait(c_w(it - 2)))
        src, dst = [ref.at[pl.ds(pl.multiple_of(g * n, n), k * n)]
                    for ref, n, k in ((plain, GW * 64, 6), (summed, 8 * 64, 3))]
        sums, moves = _each(sum_qkv, range(3), zero, src, dst), transposes(it + RAW - 2, src, 3)
        cut, m1, m2 = len(sums) * A_CUT[0] // 100, A_CUT[1], A_CUT[2]
        early, late = a_attention(1, zero)
        a_load(i + 1, 1)
        _run(_merge(a_out(i - 2, 0) + _each(a_proj, range(3), 0),
                    moves[:m1] + _merge(early, sums[:cut]) + moves[m1:m2]))
        a_load(jnp.minimum(i + 2, NB - 1), 0)
        side = sum(a_attention(0, zero), [])
        side = _merge(side[:len(late)], late) + side[len(late):]
        _run(_merge(_each(a_proj, range(3), 1) + a_out(i - 1, 1), _merge(side, sums[cut:]) + moves[m2:], A_CUT[3]))
        return zero

    def attention(qkv, put, row0=0):
        row = lax.broadcasted_iota(jnp.int32, (L - row0, 2 * L), 0) + row0
        col = lax.broadcasted_iota(jnp.int32, (L - row0, 2 * L), 1)
        head0 = col < L
        visible = (row < M) | (row >= jnp.where(head0, col, col - L))
        scale = DH ** -0.5
        st = {}

        def by_head(n):
            t = qkv(n)
            if n % 3 == 1:
                low = lax.broadcasted_iota(jnp.int32, t.shape, 1) < 64
                t = _cat(jnp.where(low, t, 0.0), jnp.where(low, 0.0, t))
            elif n % 3 == 2:
                t = _cat(jnp.zeros_like(t), t)
            return t.astype(BF16)

        def score(p):
            sc = [lax.dot_general(qkv(9 * p + t), by_head(9 * p + 3 + t), NT, preferred_element_type=F32)
                  for t in range(3)]
            sc = _add(_add(jnp.concatenate([sc[0], jnp.zeros_like(sc[0])], axis=1), sc[1]), sc[2])
            sc = jnp.where(visible, sc, MASKED / scale)
            m0 = jnp.max(jnp.where(head0, sc, -jnp.inf), axis=1, keepdims=True)
            m1 = jnp.max(jnp.where(head0, -jnp.inf, sc), axis=1, keepdims=True)
            st[p] = sc - jnp.where(head0, m0, m1)

        def normalize(p):
            e = jnp.exp2(st[p] * (scale * LOG2E))
            l0 = jnp.sum(jnp.where(head0, e, 0.0), axis=1, keepdims=True)
            l1 = jnp.sum(jnp.where(head0, 0.0, e), axis=1, keepdims=True)
            st[p] = e / jnp.where(head0, l0, l1)

        def mix(p):
            for t in range(3):
                put(3 * p + t, _dot(st[p] if t else st[p][:, :L], by_head(9 * p + 6 + t)))

        return score, normalize, mix

    def mixed_at(n):
        return [(ref, n - g0 * GW) for ref, (g0, g1) in zip(mixed, CHUNKS) if g0 <= n // GW < g1][0]

    def put_x(n, r):
        ref, k = mixed_at(n)
        ref[k, 0:M] = r[0:M]
        ox[n] = r[M:]

    def put_y(n, r):
        ref, k = mixed_at(n)
        ref[k] = _cat(r[0:M], ox[n] - r[M:], r[M:])

    def left_operands(s, zero):
        def load(k):
            x, y = [paced(pltpu.bitcast(bx[_ds(s + e, SEG), _ds(k, 128)], U32), zero, [len(recent) - 20] * 2)
                    for e in range(2)]
            x, y = [pltpu.bitcast(v, BF16).astype(F32) for v in (x, y)]
            xy[k] = _cat(x, y, x + y)

        def task(r):
            src = xy.at[pl.ds(4 * zero, LT)]
            terms = [(a or b, src[k, _ds(2 if a and b else 1 if b else 0, SEG)])
                     for k, (a, b) in enumerate(MODEL[r]) if a or b]
            terms[0] = terms[0][0], paced(terms[0][1], zero, [len(recent) - 20] * 4)
            v = _val(_sum(terms))
            lhs[r, 0:HS] = v[:HS]
            lhs[r, HS + M:] = v[HS:]

        return [functools.partial(load, k) for k in range(LT)] + [functools.partial(task, r) for r in range(NR)]

    def step(s, second, zero):
        def reread(ref):
            return ref.at[pl.ds(4 * zero, ref.shape[0])]

        part_r, ring_r = reread(part), [reread(r) for r in ring]
        halves = [slice(0, HS), slice(HS, SEG)][::1 - 2 * second]
        new_mem = [None] * LT
        due = []

        def mm(x, w):
            r = _dot(x, w)
            recent.append(r[0:M] if second and len(recent) > TOKENS_AT[0] - 24 else None)
            while due and due[0][0] <= len(recent):
                due.pop(0)[1]()
            return r

        def in_turn(items):
            lists = [[x for x in items if (x[0] >= BOTH) == e] for e in (False, True)]
            for _ in items:
                yield lists[TURNS >> second * (NQ + NO) * LT + len(recent) & 1].pop(0)

        def mem_tiles(r):
            return [MEM_ORDER[k] for k, c in enumerate(MODEL[r]) if c[second]]

        def project(g):
            def token_sums(e):
                def begin(k):
                    return part_r[g, k, halves[e]] if second and QKV_SUMS[0][1 - e][1][k] else None

                def done(k, v):
                    n = GW * g + k // 2
                    if not second:
                        part[g, k, halves[e]] = v
                    elif k % 2:
                        tok[n, halves[e]] = v
                    else:
                        ring[n // 3 % RING][n % 3, pl.ds(M + halves[e].start, HS)] = v

                return _Sums(QKV_SUMS[second][e], done, begin)

            def done(k, v):
                n = GW * g + k
                ring[n // 3 % RING][n % 3, 0:M] = v

            sums = token_sums(0), token_sums(1), _Sums(QKV_SUMS[second][2], done)
            weights = pltpu.bitcast(summed[_ds(PAD + g, 8 * 64), :], BF16)
            order = sorted(QKV_ORDER[second], key=lambda r: max(mem_tiles(r)) if second and g == 0 else 0)
            for r, in in_turn([(r,) for r in order]):
                t0, t1 = (0, L) if r < BOTH else (second * HS, second * HS + HS + M)
                if g == 0:
                    lhs[r, HS:HS + M] = _val(_sum(
                        (c[second], m_s[k]) for k, c in enumerate(MODEL[r]) if c[second]))
                if r in SINGLE:
                    w = tile(plain, (PAD + g) * GW + SINGLE[r] % GW, SINGLE[r] // GW)
                else:
                    i, j = divmod(SUMMED.index(r), LT)
                    w = weights[i * 128:(i + 1) * 128, j * 128:(j + 1) * 128]
                v = mm(lhs[r, t0:t1], w)
                sums[2].add(r, 1, v[HS - t0:HS - t0 + M])
                if t0 == 0:
                    sums[second].add(r, 1, v[:HS])
                if t1 == L:
                    sums[1 - second].add(r, 1, v[-HS:])

        def projected(n):
            src = ring_r[n // 3 % RING]
            return src[n % 3] if second else _cat(src[n % 3, 0:M], tok[n])

        def out_chunk(ref, g0, g1):
            def token_sums(e):
                def begin(k):
                    if (second and OUT_SUMS[0][1 - e][1][k]) or (g0 > 0 and OUT_SUMS[second][e][1][k]):
                        return opart[k, halves[e]]

                def done(k, v):
                    if second and g1 == GO:
                        rows = _ds((s + k % 2) * 2 + halves[e].start // HS, HS)
                        outb[rows, _ds(k // 2, 128)] = v.astype(BF16)
                    else:
                        opart[k, halves[e]] = v

                return _Sums(OUT_SUMS[second][e], done, begin)

            def done(k, v):
                new_mem[k] = v
                if g1 == GO:
                    m_s[k] = v

            sums = token_sums(0), token_sums(1), _Sums(OUT_SUMS[second][2], done, list(new_mem).__getitem__)
            weights = [pltpu.bitcast(wo[_ds(g, 64), :], BF16) for g in range(g0, g1)]
            order = sorted(OUT_ORDER[second], key=lambda r: min(mem_tiles(r)) if g1 == GO and not second else 0)
            tall, short = [[r for r in order if (r >= BOTH) == e] for e in (False, True)]
            n = OUT_PARTS[second]
            for k in range(n):
                acc = {}
                some = _share(tall[::-1], n - 1 - k, n)[::-1] + _share(short, k, n)
                for r, g in in_turn([(r, g) for g in range(g0, g1) for r in some]):
                    t0, rows = (0, SEG) if r < BOTH else (halves[0].start, HS)
                    terms = []
                    for j, (a, b) in enumerate(FEATURE[r]):
                        i = (g - g0) * GW + j
                        if b:
                            terms.append((a or b, ref[i, pl.ds((M if a else L) + t0, rows)]))
                        elif a and second:
                            terms += [(a, ref[i, pl.ds(r0 + t0, rows)]) for r0 in (M, L)]
                        elif a:
                            terms.append((a, ox[g * GW + j, pl.ds(t0, rows)]))
                    sign, left = _sum(terms)
                    m_sign, m = _sum((c[second], ref[(g - g0) * GW + j, 0:M])
                                     for j, c in enumerate(FEATURE[r]) if c[second])
                    v = mm(_cat(m, left), weights[g - g0][:, r * 128:(r + 1) * 128])
                    acc[r] = m_sign, sign, _add(acc[r][2] if r in acc else None, v)
                for r, (m_sign, sign, v) in acc.items():
                    sums[2].add(r, m_sign, v[:M])
                    sums[second if r < BOTH else 0].add(r, sign, v[M:M + HS])
                    if r < BOTH:
                        sums[1 - second].add(r, sign, v[M + HS:])

        recent.clear()
        stages = attention(projected, put_x if second else put_y)
        for p in range(NP):
            ready = LT * GW * ((9 * p + 5) // GW + 1)
            due += [(ready + lag, functools.partial(f, p)) for f, lag in zip(stages, LAGS[second])]
        if second:
            due += [(TOKENS_AT[0] + k * TOKENS_AT[1], task)
                    for k, task in enumerate(left_operands(jnp.minimum(s + 4, NSEG - 2), zero))]
        due.sort(key=lambda e: e[0])
        for g in range(GQ):
            project(g)
        for ref, chunk in zip(mixed, CHUNKS):
            out_chunk(reread(ref), *chunk)

    def first_segment(zero):
        def project(g):
            acc = {}

            def task(n, k):
                r = _dot(h0[0:L + SEG, _ds(k, 128)], tile(plain, PAD * GW + n, k))
                e = len(recent) % 8
                recent.extend([r[8 * e:8 * e + 8], r[8 * e + 8:8 * e + 16]])
                acc[n] = _add(acc.get(n), r)
                if k == LT - 1:
                    first[n] = acc[n][0:L]
                    tok[n] = acc[n][L:]

            return [functools.partial(task, g * GW + n, k) for n in range(GW) for k in range(LT)]

        def put(n, r):
            recent.extend([r[k:k + 8] for k in range(0, L, 16)])
            put_x(n, r)

        stages = attention(lambda n: first[n], put)
        new_mem = [None] * LT

        def heads(p0, p1):
            return [functools.partial(f, t - lag) for t in range(p0, p1 + 2)
                    for lag, f in enumerate(stages) if p0 <= t - lag < p1] + [lambda: None]

        def out(g):
            def task(n, k):
                ref, i = mixed_at(n)
                r = _dot(ref[i, 0:M], wo_raw[_ds(n, 128), _ds(k, 128)])
                recent.append(r)
                new_mem[k] = r if new_mem[k] is None else new_mem[k] + r

            return [functools.partial(task, g * GW + n, k) for n in range(GW) for k in range(LT)]

        c1, c2, c3, d1, d2, m1 = FIRST_CUT
        moves = transposes(GO - 2, plain, PAD + GQ - 6) + transposes(GO - 1, plain, PAD + GQ - 3)
        start(c_wo(0))
        wait(c_w(GO - 2) + c_bx0)
        start(c_wo(1) + c_wo(2))
        h0[0:M, :] = mem[0:M, :].astype(F32)
        h0[M:L + SEG, :] = bx[0:2 * SEG, :].astype(F32)
        _run(_merge(a_out(NB - 2, 0) + _each(project, range(c1)), moves[:m1] + _merge(
            sum(a_attention(1, zero), []), _each(sum_qkv, range(PAD + GQ - 9, PAD + d1), zero))))
        wait(c_w(GO - 1))
        start(c_wo(3) + c_wo(4))
        _run(_merge(a_out(NB - 1, 1) + _each(project, range(c1, c2)),
                    moves[m1:] + _each(sum_qkv, range(PAD + d1, PAD + d2), zero)))
        start(c_wo(5))
        wait(_each(c_wo, range(3)))
        start(c_wo(6) + c_wo(7))
        _run(_merge(_merge(_each(project, range(c2, c3)), heads(0, 11)),
                    _each(sum_qkv, range(PAD + d2, PAD + GQ), zero) + _each(sum_out, range(3), zero)))
        wait(_each(c_wo, range(3, 6)))
        _run(_merge(_merge(_merge(_each(project, range(c3, GQ)), _each(out, range(3))), heads(11, 13))
                    + _merge(_each(out, range(3, 6)), heads(13, NP)),
                    _merge(_each(sum_out, range(3, 6), zero), left_operands(2, zero))))
        wait(c_wo(6) + c_wo(7))
        start(c_bx1 + c_outa)
        _run(_merge(out(6) + out(7), _each(sum_out, (6, 7), zero)))
        for k in range(LT):
            m_s[k] = new_mem[k]

    def two_segments(it, carry):
        pl.when(it == 1)(lambda: wait(c_bx1))
        step(2 * it, 0, it >> 16)
        step(2 * it, 1, it >> 16)
        start(c_outb(_ds(it, 2 * SEG)))
        return carry

    def last_segment():
        res, acc = {}, [None] * LT

        def project(n, k):
            r = _dot(-m_s[k] if k % 2 else m_s[k], tile(plain, PAD * GW + n, k))
            res[n] = _acc(res.get(n), 1 - 2 * (k % 2), r)

        def out(n, k):
            acc[k] = _add(acc[k], _dot(_cat(ox[n], res[NQ + n]), wo_raw[_ds(n, 128), _ds(k, 128)]))

        stages = attention(lambda n: _cat(_val(res[n]), tok[n]) if n in res else tok[n],
                           lambda n, r: res.update({NQ + n: r}), M)
        tiles = [9 * p + e for t in range(NP + 3) for p, e0 in ((t, 3), (t - 3, 6)) if 0 <= p < NP
                 for e in range(e0, e0 + 3)]
        ready = {n: (i * LT + LT - 1) // 4 for i, n in enumerate(tiles)}
        due = [((i * LT + k) // 4, 0, functools.partial(project, n, k))
               for i, n in enumerate(tiles) for k in range(LT)]
        for p in range(NP):
            due += [(ready[9 * p + e] + lag, rank, functools.partial(f, p))
                    for f, lag, e, rank in zip(stages, LAST_LAGS, (5, 5, 8), (2, 2, 1))]
        t = 0
        for k in range(NO * LT):
            if k % 4 == 0:
                t = max(t + LAST_LAGS[4], ready[9 * ((k + 3) // 15) + 8] + LAST_LAGS[3])
            due.append((int(t), 3, functools.partial(out, *divmod(k, LT))))
        _run([task for _, _, task in sorted(due, key=lambda e: e[:2])])
        outb[S - 2 * SEG:, :] = jnp.concatenate(acc, axis=1).astype(BF16)
        start(c_outb(slice(S - 2 * SEG, S)))

    a_start()
    first_segment(lax.fori_loop(1, NB // 2, a_step, 0))
    lax.fori_loop(0, NSEG // 2 - 1, two_segments, 0)
    last_segment()
    wait(c_outa + c_outb(slice(0, S)))


def pallas_concat_heads__sliding_local_dilated__memory_aug_recurrent_mem_tr__prompt_kernel(
    A_x, A_wqkv, A_wo, B_x, B_mem0, B_Wq, B_Wk, B_Wv, B_Wo, B_seg_len,
):
    assert B_seg_len == SEG
    assert A_x.shape == B_x.shape == (1, S, D) and B_mem0.shape == (1, M, D)
    assert B_Wq.shape == B_Wk.shape == B_Wv.shape == (D, H, DH) and B_Wo.shape == (H, DH, D)
    dma = pltpu.SemaphoreType.DMA

    def vmem(shape, dtype):
        assert math.prod(shape) * jnp.dtype(dtype).itemsize % 16384 == 0
        return pltpu.VMEM(shape, dtype)

    call = pl.pallas_call(
        _kernel,
        out_shape=jax.ShapeDtypeStruct((S, 2 * D), BF16),
        in_specs=[pl.BlockSpec(memory_space=pl.ANY)] * 9,
        out_specs=pl.BlockSpec(memory_space=pl.ANY),
        scratch_shapes=[
            vmem((S, D), BF16),
            vmem((3, D, D), BF16),
            vmem((D, D), BF16),
            vmem((LT, D, 128), F32),
            vmem((2 * D, D), U32),
            vmem((TB, D), U32),
            vmem((2, LT, TB, 128), F32),
            vmem((2, 2 * LT, HALO + TB, 128), F32),
            vmem((2, TB, D), F32),
            vmem((S, D), BF16),
            vmem((S, D), BF16),
            vmem((8 * M, D), BF16),
            vmem((RAW * 3 * GW * 128, D), BF16),
            vmem((H * DH, D), BF16),
            vmem(((PAD + GQ) * GW * 64, D), U32),
            vmem(((PAD + GQ) * 8 * 64, D), U32),
            vmem((GO * 64, NR * 128), U32),
            vmem((3 * SEG, D), F32),
            vmem((NQ, L, 128), F32),
            vmem((LT, 3 * SEG, 128), F32),
            vmem((NR + 1, L, 128), F32),
            vmem((8, M, 128), F32),
            vmem((GQ, 2 * GW, SEG, 128), F32),
            vmem((NQ, SEG, 128), F32),
            [vmem((4, L, 128), F32)] * RING,
            vmem((NO, SEG, 128), F32),
            [vmem((20, L + SEG, 128), F32)] * len(CHUNKS),
            vmem((2 * LT, SEG, 128), F32),
            vmem((S, D), BF16),
            dma((5,)), dma((NB // 2,)), dma((GO, 3)), dma((3,)), dma((GO,)), dma((2,)),
        ],
        compiler_params=pltpu.CompilerParams(vmem_limit_bytes=126 * 1024 * 1024, **{
            name: True for name in ("disable_bounds_checks", "disable_semaphore_checks")
            if hasattr(pltpu.CompilerParams, name)}),
        name="sliding_and_memory_attention",
    )

    def by_feature(w):
        return w.transpose(1, 2, 0).reshape(H * DH, D)

    out = call(A_x.reshape(S, D), A_wqkv, A_wo, B_x.reshape(S, D), B_mem0.reshape(M, D),
               by_feature(B_Wq), by_feature(B_Wk), by_feature(B_Wv), B_Wo.reshape(H * DH, D))
    return out.reshape(1, S, 2 * D)
```

```python
import collections
import functools
import itertools
import math
import random

import jax
import jax.numpy as jnp
import numpy as np
from jax import lax
from jax.experimental import pallas as pl
from jax.experimental.pallas import tpu as pltpu

F32, BF16, U32 = jnp.float32, jnp.bfloat16, jnp.uint32
NT = (((1,), (1,)), ((), ()))
MASKED = -1000000000.0
LOG2E = math.log2(math.e)

S, D = 2048, 640
LT = D // 128

AH, AD, AW, ADIL = 32, 20, 8, 2
HALO = 16
TB = 128
NB = S // TB

H, DH, M, SEG = 32, 192, 8, 32
L = M + SEG
HS = SEG // 2
NSEG = S // SEG
NP = H // 2
NO = 3 * NP
NQ = 3 * NO
GW = 6
GO, GQ = NO // GW, NQ // GW
PAD = 3
RAW = 4
RING = 12
CHUNKS = ((0, 3), (3, 5), (5, GO))


def _algorithm(rank_ones):
    rows = np.array([[1, 0], [0, 1], [1, 1]])
    duals = np.array([[0, 1], [1, 0], [1, -1]])
    sets = [[[np.array(["-0+".index(c) - 1 for c in w]) for w in e.split()] for e in s] for s in rank_ones]
    left, right = [], []
    for t, s in enumerate(sets):
        p, q = [k for k in range(3) if k != t]
        for u, v in s:
            left += [np.outer(u, rows[p]), np.outer(u, rows[q])]
            right += [np.outer(v, duals[q]), np.outer(v, duals[p])]
    for (u0, v0), (u1, v1), (u2, v2) in itertools.product(*sets):
        for a, b in itertools.product((1, -1), repeat=2):
            e = np.outer(u0 + a * u1, v0 + b * v1)
            if (e == np.outer(u2, v2)).all() or (e == -np.outer(u2, v2)).all():
                left.append(np.outer(u0, rows[1]) - a * np.outer(u1, rows[0]))
                right.append(np.outer(v0, duals[1]) + b * np.outer(v1, duals[0]))
    left, right = np.array(left), np.array(right)
    have = np.einsum("rka,rnb->kanbr", left, right).reshape(-1, len(left))
    want = np.einsum("kp,nq,ab->kanbpq", np.eye(LT), np.eye(GW), np.eye(2)).reshape(len(have), -1)
    blocks = np.rint(np.linalg.lstsq(have, want, rcond=None)[0]).astype(int)
    assert (have @ blocks == want).all()
    sign = blocks.max(axis=1) * 2 - 1
    return left * sign[:, None, None], blocks * sign[:, None], right


def _shared_sums(matrix, seed):
    rng = random.Random(seed)
    rows = [{k: int(c) for k, c in enumerate(row) if c} for row in matrix]
    shared = {}
    while True:
        count = collections.Counter(
            (a, b, r[a] * r[b]) for r in rows for a, b in itertools.combinations(sorted(r), 2))
        top = max(count.values(), default=0)
        if top < 2:
            return shared, rows
        best = sorted(k for k, n in count.items() if n == top)
        a, b, sign = best[int(rng.random() * len(best))]
        name = matrix.shape[1] + len(shared)
        shared[name] = a, b, sign
        for r in rows:
            if r.get(a, 0) * r.get(b, 0) == sign:
                r[name] = r.pop(a)
                del r[b]


MODEL, BLOCKS, FEATURE = _algorithm((
    ("+0000 +00++0", "000+0 0+0000", "0000+ 000+00", "+-+00 00000+", "+00+0 00+0+0"),
    ("0+00+ 000+++", "0+0+0 0+00++", "00+-+ 00++00", "00+0+ +00000", "+0+00 0000+0", "00+00 0+-000"),
    ("0+000 0000++", "00+-+ ++0000", "00+00 +00+00", "+-000 0+-00+", "00+-0 00+000", "+-00- +0000-")))
NR = len(BLOCKS)
BOTH = 34
SINGLE = {r: int(row.argmax()) for r, row in enumerate(BLOCKS) if abs(row).sum() == 1}
SUMMED = [r for r in range(NR) if r not in SINGLE]


def _step_sums(out, step, seed):
    use = MODEL[:, :, step].any(1) & FEATURE[:, :, step].any(1)
    return [_shared_sums((m * keep[:, None]).T, seed) for m, keep in (
        (out.reshape(NR, -1), use), (out.reshape(NR, -1), use & (np.arange(NR) < BOTH)), (out[:, :, step], use))]


QKV_SUMS = _step_sums(FEATURE, 0, 32), _step_sums(FEATURE, 1, 5)
OUT_SUMS = _step_sums(MODEL, 0, 0), _step_sums(MODEL, 1, 6)
BLOCK_SUMS = _shared_sums(BLOCKS, 37)

QKV_ORDER = (
    (30, 14, 20, 3, 28, 12, 9, 22, 10, 18, 26, 1, 5, 24, 32, 7, 16,
     40, 38, 36, 45, 46, 44, 39, 34, 35, 43, 37, 41, 42),
    (31, 15, 4, 11, 27, 0, 19, 8, 23, 13, 33, 6, 29, 21, 2, 25, 17,
     40, 34, 41, 39, 35, 45, 46, 36, 43, 44, 38, 37, 42))
OUT_ORDER = (
    (24, 14, 10, 5, 32, 28, 16, 30, 22, 7, 9, 3, 12, 1, 18, 20, 26,
     40, 34, 41, 39, 42, 37, 43, 36, 46, 45, 44, 35, 38),
    (23, 11, 2, 13, 15, 17, 4, 25, 31, 6, 33, 8, 29, 21, 19, 0, 27,
     39, 36, 45, 34, 41, 40, 37, 44, 42, 43, 46, 35, 38))
BLOCK_ORDER = (3, 28, 6, 0, 5, 17, 11, 8, 10, 7, 4, 16, 2, 1, 23, 22, 9, 29, 24, 19, 12, 18, 25, 13, 14, 20,
               21, 15, 26, 27)
MEM_ORDER = (2, 1, 4, 0, 3)

LAGS = ((40, 70, 100), (50, 80, 110))
TOKENS_AT = (737, 4)
OUT_PARTS = (5, 5)
TURNS = int(
    "734a6a6a6a24a26a6a4a24b4a6a6a430dd2852d2d2969693094b4a552942968a52d21e5161c385d29525a294b42d32a4"
    "b0e172a626a3453521e49694385c61a5a4d22e28732a4b0e171a52968a52d21e5161c385d29525a294b42d32a4b0e172"
    "5a1c3465870e1b4a62a4b4a6870e15a52c385a587161a5a1c7171717161861a5a5a1861a5a5a5825a5a292d2d2d2d298"
    "a187353141c29a91a984d48d3a2c34a272a6a43a929a91a6870e2c1e1c3871385a529694a58707870d2954a9a90e4a5a"
    "52954a6a42e19694c5394a587078b0e1a8e1c8b0e626a62c1e1c3870790d4c29e1c3931a193931a949a9458d0e949871", 16)

A_PACE = (12, 4)
SUM_PACE = (18, 10)
A_CUT = (58, 1, 18, 0)
START_CUT = (5, 20)
FIRST_CUT = (5, 12, 21, 17, 21, 6)
LAST_LAGS = (7, 12, 3, 7, 1.9)


def _ds(i, n):
    return pl.ds(i * n if isinstance(i, int) else pl.multiple_of(i * n, n), n)


def _dot(a, b):
    return jnp.dot(a, b, preferred_element_type=F32)


def _cat(*parts):
    return jnp.concatenate(parts, axis=0)


def _add(a, b):
    return b if a is None else _cat(a[:M] + b[:M], a[M:] + b[M:])


def _acc(a, sign, b):
    if a is None:
        return sign, b
    if a[0] == sign:
        return sign, a[1] + b
    return (1, a[1] - b) if a[0] > 0 else (1, b - a[1])


def _sum(terms):
    return functools.reduce(lambda a, t: _acc(a, *t), terms, None)


def _val(a):
    return a[1] if a[0] > 0 else -a[1]


class _Sums:
    def __init__(self, plan, done, begin=lambda k: None):
        self.shared, self.rows = plan
        self.done, self.begin = done, begin
        self.terms, self.sums = {}, [None] * len(self.rows)
        for k, row in enumerate(self.rows):
            if not row and (first := begin(k)) is not None:
                done(k, first)

    def add(self, name, sign, value):
        self.terms[name] = sign, value
        for k, row in enumerate(self.rows):
            if name in row:
                if self.sums[k] is None and (first := self.begin(k)) is not None:
                    self.sums[k] = 1, first
                self.sums[k] = _acc(self.sums[k], row[name] * sign, value)
                if all(n in self.terms for n in row):
                    self.done(k, _val(self.sums[k]))
        for n, (a, b, s) in self.shared.items():
            if name in (a, b) and a in self.terms and b in self.terms and n not in self.terms:
                self.add(n, *_acc(self.terms[a], s * self.terms[b][0], self.terms[b][1]))


def _share(tasks, k, n):
    return list(tasks[k * len(tasks) // n:(k + 1) * len(tasks) // n])


def _merge(a, b, early=0):
    n = len(a) - early
    return [t for k in range(n) for t in [a[k]] + _share(b, k, n)] + a[n:]


def _each(f, items, *args):
    return [task for item in items for task in f(item, *args)]


def _run(tasks):
    for task in tasks:
        task()


def _kernel(ax_hbm, awqkv_hbm, awo_hbm, bx_hbm, mem_hbm, wq_hbm, wk_hbm, wv_hbm, wo_hbm,
            out_hbm,
            ax, awqkv, awo, tmp, wa, xb, q_s, kv_s, oa_s, outa,
            bx, mem, raw, wo_raw, plain, summed, wo, h0, first, xy, lhs, m_s, part, tok, ring,
            ox, mixed, opart, outb,
            sem_a, sem_x, sem_w, sem_b, sem_wo, sem_o):
    cp = pltpu.make_async_copy

    def rows_copy(src, dst, rows, sem):
        return [cp(src.at[rows, :], dst.at[rows, :], sem)]

    c_aw = [cp(awqkv_hbm.at[r0:r1, _ds(j, D)], awqkv.at[j, r0:r1], sem_a.at[k])
            for k, (j, r0, r1) in enumerate(((0, 0, 384), (0, 384, D), (1, 0, D), (2, 0, D)))]
    c_awo = [cp(awo_hbm, awo, sem_a.at[4])]
    c_bx0 = [cp(mem_hbm, mem.at[0:M], sem_b.at[0])] + rows_copy(bx_hbm, bx, slice(0, 6 * SEG), sem_b.at[1])
    c_bx1 = rows_copy(bx_hbm, bx, slice(6 * SEG, S), sem_b.at[2])
    c_outa = [cp(outa, out_hbm.at[:, 0:D], sem_o.at[0])]

    def c_ax(c):
        return rows_copy(ax_hbm, ax, _ds(c, 2 * TB), sem_x.at[c])

    def c_w(c):
        return [cp(w.at[_ds(c, GW * 128), :], raw.at[_ds((c & (RAW - 1)) * 3 + j, GW * 128), :], sem_w.at[c, j])
                for j, w in enumerate((wq_hbm, wk_hbm, wv_hbm))]

    def c_wo(g):
        return rows_copy(wo_hbm, wo_raw, _ds(g, GW * 128), sem_wo.at[g])

    def c_outb(rows):
        return [cp(outb.at[rows, :], out_hbm.at[rows, D:], sem_o.at[1])]

    def start(copies):
        for c in copies:
            c.start()

    def wait(copies):
        for c in copies:
            c.wait()
        recent.clear()

    recent = []

    def paced(x, zero, marks):
        late = _cat(*[recent[t] if t >= 0 else jnp.zeros((8, 128), F32) for t in marks[:x.shape[0] // 8]])
        always = lax.broadcasted_iota(jnp.int32, x.shape, 1) >= zero
        return lax.select(always, x, late if x.dtype == F32 else pltpu.bitcast(late, U32))

    def tile(ref, i, j):
        return pltpu.bitcast(ref[_ds(i, 64), _ds(j, 128)], BF16)

    def a_weights(j, zero=None):
        def task(t):
            if j < 3:
                tmp[t] = awqkv[j, _ds(t, 128), :].astype(F32).T
            else:
                marks = [len(recent) - 40 + k * 3 // 4 for k in range(40)]
                w = paced(pltpu.bitcast(awo[:, _ds(t, 128)], U32), zero, marks)
                tmp[t] = pltpu.bitcast(w, BF16).astype(F32)
            w = _cat(*[tmp[t, pl.ds(d, AH, stride=AD), :] for d in range(AD)])
            wa[_ds(j, D // 2), _ds(t, 128)] = pltpu.bitcast(w.astype(BF16), U32)

        return [functools.partial(task, t) for t in range(LT)]

    def by_tile(product, put):
        acc = [None]

        def task(t, k):
            r = product(t, k)
            e = len(recent) % 16
            recent.extend(r[8 * (e + i) % TB:8 * (e + i) % TB + 8] for i in range(4))
            acc[0] = _add(acc[0] if k else None, r)
            if k == LT - 1:
                put(t, acc[0])

        return [functools.partial(task, t, k) for t in range(LT) for k in range(LT)]

    def a_load(i, b):
        xb[_ds(b, TB // 2), :] = pltpu.bitcast(ax[_ds(i, TB), :], U32)

    def a_proj(j, b, first_block=False):
        def put(t, r):
            if j == 0:
                q_s[b, t] = r
                return
            c = (j - 1) * LT + t
            kv_s[b, c, HALO:, :] = r
            if first_block:
                kv_s[b, c, 0:HALO, :] = jnp.broadcast_to(r[0:1, :], (HALO, 128))
            else:
                kv_s[b, c, 0:HALO, :] = kv_s[1 - b, c, TB:, :]

        return by_tile(lambda t, k: lax.dot_general(
            tile(xb, b, k), tile(wa, j * LT + t, k), NT, preferred_element_type=F32), put)

    def a_attention(b, zero, first_block=False):
        n = TB // 8
        lag = n if first_block else A_PACE[1]
        marks, logits = [], []

        def mark():
            marks.append(len(recent) - A_PACE[0])

        def window(c, w):
            return kv_s[b, c, pl.ds(HALO - ADIL * w, TB), :]

        def score():
            q = [paced(q_s[b, t], zero, marks[::4]) for t in range(LT)]
            sums = [functools.reduce(jnp.add, [q[t] * window(t, w) for t in range(LT)]) for w in range(AW)]
            rows = {}
            for k in range(n + 1):
                if k < n:
                    a = _cat(*[a[8 * k:8 * k + 8] for a in sums])
                    rows[k] = a + pltpu.roll(a, 2 * AH, 1)
                if k > 0:
                    rows[k - 1] = rows[k - 1] + pltpu.roll(rows[k - 1], AH, 1)
            logits.extend(_cat(*[rows[k][8 * w:8 * w + 8] for k in range(n)]) for w in range(AW))

        def mix():
            scale, lg = AD ** -0.5, logits
            if first_block:
                pos = lax.broadcasted_iota(jnp.int32, (HALO, 128), 0)
                lg = [_cat(jnp.where(pos >= ADIL * w, a[:HALO], MASKED / scale), a[HALO:])
                      for w, a in enumerate(lg)]
            m = paced(functools.reduce(jnp.maximum, lg), zero, marks[4 * lag + 1::4])
            e = [jnp.exp2((a - m) * (scale * LOG2E)) for a in lg]
            inv = 1.0 / functools.reduce(jnp.add, e)
            for t in range(LT):
                v = [window(LT + t, w) for w in range(AW)]
                v[0] = paced(v[0], zero, marks[4 * lag + 2 + 2 * t // LT::4])
                oa_s[b, :, _ds(t, 128)] = inv * functools.reduce(jnp.add, map(jnp.multiply, e, v))

        return [mark] * (4 * n) + [score], [mark] * (4 * lag) + [mix]

    def a_out(i, b):
        def put(t, r):
            outa[_ds(i, TB), _ds(t, 128)] = r.astype(BF16)

        return by_tile(lambda t, k: _dot(oa_s[b, :, _ds(k, 128)], tile(wa, 3 * LT + k, t)), put)

    def transposes(c, dst, g):
        def task(n):
            t = ((c & (RAW - 1)) * 3 + n % 9 // 3) * GW + n // 9 * 3 + n % 3
            v = pltpu.bitcast(raw[_ds(t, 128), :].T, U32)
            for k in range(LT):
                dst[_ds(g * GW + n, 64), _ds(k, 128)] = v[k * 64:(k + 1) * 64]

        return [functools.partial(task, n) for n in range(3 * GW)]

    def sum_blocks(block, put, zero):
        back, n = SUM_PACE
        marks = []

        def mark():
            marks.append(len(recent) - back)

        def done(r, v):
            if r not in SINGLE:
                put(r, pltpu.bitcast(v.astype(BF16), U32))

        def task():
            sums = _Sums(BLOCK_SUMS, done)
            for k in range(n):
                for i, b in enumerate(_share(BLOCK_ORDER, k, n)):
                    v = block(*divmod(b, GW))
                    if i == 0:
                        v = paced(v, zero, marks[k::n])
                    for r in SINGLE:
                        if SINGLE[r] == b:
                            put(r, v)
                    sums.add(b, 1, pltpu.bitcast(v, BF16).astype(F32))

        return [mark] * (8 * n) + [task]

    def sum_qkv(g, zero, src=plain, dst=summed):
        def put(r, v):
            if r not in SINGLE:
                i, j = divmod(SUMMED.index(r), LT)
                dst[_ds(g * 8 + i, 64), _ds(j, 128)] = v

        return sum_blocks(lambda k, n: src[_ds(g * GW + n, 64), _ds(k, 128)], put, zero)

    def sum_out(g, zero):
        def put(r, v):
            wo[_ds(g, 64), _ds(r, 128)] = v

        return sum_blocks(lambda k, n: pltpu.bitcast(wo_raw[_ds(g * GW + n, 128), _ds(k, 128)], U32), put, zero)

    def a_start():
        nq, nk = START_CUT
        start(c_aw[:2])
        zero = lax.fori_loop(0, 2, lambda it, carry: it >> 16, 0)
        start(c_ax(0))
        wait(c_aw[:1])
        start(c_aw[2:3])
        _run(a_weights(0)[:3])
        wait(c_aw[1:2])
        start(c_aw[3:])
        _run(a_weights(0)[3:])
        wait(c_ax(0))
        start(c_awo)
        a_load(0, 0)
        a_load(1, 1)
        _run(a_proj(0, 0) + a_proj(0, 1)[:nq])
        wait(c_aw[2:3])
        start(c_ax(1) + c_ax(2))
        _run(a_proj(0, 1)[nq:] + a_weights(1) + a_proj(1, 0, True))
        wait(c_aw[3:])
        start(c_w(0))
        early, late = a_attention(0, zero, True)
        _run(a_proj(1, 1)[:nk] + a_weights(2) + _merge(a_proj(2, 0, True), early))
        wait(c_awo + c_ax(1))
        start(c_bx0)
        _run(_merge(a_proj(1, 1)[nk:] + a_proj(2, 1), _merge(late, a_weights(3, zero)), 4))
        a_load(2, 0)

    def a_step(it, carry):
        i, g, zero = 2 * it, jnp.maximum(3 * it - 9 + PAD, 0), it >> 16
        pl.when(it + 2 < NB // 2)(lambda: start(c_ax(it + 2)))
        pl.when(it + 1 < NB // 2)(lambda: wait(c_ax(it + 1)))
        start(c_w(it))
        pl.when(it > 1)(lambda: wait(c_w(it - 2)))
        src, dst = [ref.at[pl.ds(pl.multiple_of(g * n, n), k * n)]
                    for ref, n, k in ((plain, GW * 64, 6), (summed, 8 * 64, 3))]
        sums, moves = _each(sum_qkv, range(3), zero, src, dst), transposes(it + RAW - 2, src, 3)
        cut, m1, m2 = len(sums) * A_CUT[0] // 100, A_CUT[1], A_CUT[2]
        early, late = a_attention(1, zero)
        a_load(i + 1, 1)
        _run(_merge(a_out(i - 2, 0) + _each(a_proj, range(3), 0),
                    moves[:m1] + _merge(early, sums[:cut]) + moves[m1:m2]))
        a_load(jnp.minimum(i + 2, NB - 1), 0)
        side = sum(a_attention(0, zero), [])
        side = _merge(side[:len(late)], late) + side[len(late):]
        _run(_merge(_each(a_proj, range(3), 1) + a_out(i - 1, 1), _merge(side, sums[cut:]) + moves[m2:], A_CUT[3]))
        return zero

    def attention(qkv, put, row0=0, zero=0):
        row = lax.broadcasted_iota(jnp.int32, (L - row0, 128), 0) + row0
        col = lax.broadcasted_iota(jnp.int32, (L - row0, 128), 1) + zero
        head0 = col < L
        visible = jnp.where(row < M, L - 1, row) >= jnp.where(head0, col, col - L)
        scale = DH ** -0.5
        st = {}

        def by_head(n):
            t = qkv(n)
            if n % 3 == 1:
                low = lax.broadcasted_iota(jnp.int32, t.shape, 1) < 64 + zero
                t = _cat(jnp.where(low, t, 0.0), jnp.where(low, 0.0, t))
            elif n % 3 == 2:
                t = _cat(jnp.zeros_like(t), t)
            return _cat(t, jnp.zeros((128 - len(t), 128), F32)).astype(BF16)

        def score(p):
            sc = [lax.dot_general(qkv(9 * p + t), by_head(9 * p + 3 + t), NT, preferred_element_type=F32)
                  for t in range(3)]
            sc = jnp.where(visible, functools.reduce(_add, sc), jnp.where(col < 2 * L, MASKED / scale, -jnp.inf))
            m0 = jnp.max(jnp.where(head0, sc, -jnp.inf), axis=1, keepdims=True)
            m1 = jnp.max(jnp.where(head0, -jnp.inf, sc), axis=1, keepdims=True)
            st[p] = sc - jnp.where(head0, m0, m1)

        def normalize(p):
            e = jnp.exp2(st[p] * (scale * LOG2E))
            l0 = jnp.sum(jnp.where(head0, e, 0.0), axis=1, keepdims=True)
            l1 = jnp.sum(jnp.where(head0, 0.0, e), axis=1, keepdims=True)
            st[p] = e / jnp.where(head0, l0, l1)

        def mix(p):
            for t in range(3):
                put(3 * p + t, _dot(st[p], by_head(9 * p + 6 + t)))

        return score, normalize, mix

    def mixed_at(n):
        return [(ref, n - g0 * GW) for ref, (g0, g1) in zip(mixed, CHUNKS) if g0 <= n // GW < g1][0]

    def put_x(n, r):
        ref, k = mixed_at(n)
        ref[k, 0:M] = r[0:M]
        ox[n] = r[M:]

    def put_y(n, r):
        ref, k = mixed_at(n)
        ref[k] = _cat(r[0:M], ox[n] - r[M:], r[M:])

    def left_operands(s, zero):
        def load(k):
            x, y = [paced(pltpu.bitcast(bx[_ds(s + e, SEG), _ds(k, 128)], U32), zero, [len(recent) - 20] * 2)
                    for e in range(2)]
            x, y = [pltpu.bitcast(v, BF16).astype(F32) for v in (x, y)]
            xy[k] = _cat(x, y, x + y)

        def task(r):
            src = xy.at[pl.ds(4 * zero, LT)]
            terms = [(a or b, src[k, _ds(2 if a and b else 1 if b else 0, SEG)])
                     for k, (a, b) in enumerate(MODEL[r]) if a or b]
            terms[0] = terms[0][0], paced(terms[0][1], zero, [len(recent) - 20] * 4)
            v = _val(_sum(terms))
            lhs[r, 0:HS] = v[:HS]
            lhs[r, HS + M:] = v[HS:]

        return [functools.partial(load, k) for k in range(LT)] + [functools.partial(task, r) for r in range(NR)]

    def step(s, second, zero):
        def reread(ref):
            return ref.at[pl.ds(4 * zero, ref.shape[0])]

        part_r, ring_r = reread(part), [reread(r) for r in ring]
        halves = [slice(0, HS), slice(HS, SEG)][::1 - 2 * second]
        new_mem = [None] * LT
        due = []

        def mm(x, w):
            r = _dot(x, w)
            recent.append(r[0:M] if second and len(recent) > TOKENS_AT[0] - 24 else None)
            while due and due[0][0] <= len(recent):
                due.pop(0)[1]()
            return r

        def in_turn(items):
            lists = [[x for x in items if (x[0] >= BOTH) == e] for e in (False, True)]
            for _ in items:
                yield lists[TURNS >> second * (NQ + NO) * LT + len(recent) & 1].pop(0)

        def mem_tiles(r):
            return [MEM_ORDER[k] for k, c in enumerate(MODEL[r]) if c[second]]

        def project(g):
            def token_sums(e):
                def begin(k):
                    return part_r[g, k, halves[e]] if second and QKV_SUMS[0][1 - e][1][k] else None

                def done(k, v):
                    n = GW * g + k // 2
                    if not second:
                        part[g, k, halves[e]] = v
                    elif k % 2:
                        tok[n, halves[e]] = v
                    else:
                        ring[n // 3 % RING][n % 3, pl.ds(M + halves[e].start, HS)] = v

                return _Sums(QKV_SUMS[second][e], done, begin)

            def done(k, v):
                n = GW * g + k
                ring[n // 3 % RING][n % 3, 0:M] = v

            sums = token_sums(0), token_sums(1), _Sums(QKV_SUMS[second][2], done)
            weights = pltpu.bitcast(summed[_ds(PAD + g, 8 * 64), :], BF16)
            order = sorted(QKV_ORDER[second], key=lambda r: max(mem_tiles(r)) if second and g == 0 else 0)
            for r, in in_turn([(r,) for r in order]):
                t0, t1 = (0, L) if r < BOTH else (second * HS, second * HS + HS + M)
                if g == 0:
                    lhs[r, HS:HS + M] = _val(_sum(
                        (c[second], m_s[k]) for k, c in enumerate(MODEL[r]) if c[second]))
                if r in SINGLE:
                    w = tile(plain, (PAD + g) * GW + SINGLE[r] % GW, SINGLE[r] // GW)
                else:
                    i, j = divmod(SUMMED.index(r), LT)
                    w = weights[i * 128:(i + 1) * 128, j * 128:(j + 1) * 128]
                v = mm(lhs[r, t0:t1], w)
                sums[2].add(r, 1, v[HS - t0:HS - t0 + M])
                if t0 == 0:
                    sums[second].add(r, 1, v[:HS])
                if t1 == L:
                    sums[1 - second].add(r, 1, v[-HS:])

        def projected(n):
            src = ring_r[n // 3 % RING]
            return src[n % 3] if second else _cat(src[n % 3, 0:M], tok[n])

        def out_chunk(ref, g0, g1):
            def token_sums(e):
                def begin(k):
                    if (second and OUT_SUMS[0][1 - e][1][k]) or (g0 > 0 and OUT_SUMS[second][e][1][k]):
                        return opart[k, halves[e]]

                def done(k, v):
                    if second and g1 == GO:
                        rows = _ds((s + k % 2) * 2 + halves[e].start // HS, HS)
                        outb[rows, _ds(k // 2, 128)] = v.astype(BF16)
                    else:
                        opart[k, halves[e]] = v

                return _Sums(OUT_SUMS[second][e], done, begin)

            def done(k, v):
                new_mem[k] = v
                if g1 == GO:
                    m_s[k] = v

            sums = token_sums(0), token_sums(1), _Sums(OUT_SUMS[second][2], done, list(new_mem).__getitem__)
            weights = [pltpu.bitcast(wo[_ds(g, 64), :], BF16) for g in range(g0, g1)]
            order = sorted(OUT_ORDER[second], key=lambda r: min(mem_tiles(r)) if g1 == GO and not second else 0)
            tall, short = [[r for r in order if (r >= BOTH) == e] for e in (False, True)]
            n = OUT_PARTS[second]
            for k in range(n):
                acc = {}
                some = _share(tall[::-1], n - 1 - k, n)[::-1] + _share(short, k, n)
                for r, g in in_turn([(r, g) for g in range(g0, g1) for r in some]):
                    t0, rows = (0, SEG) if r < BOTH else (halves[0].start, HS)
                    terms = []
                    for j, (a, b) in enumerate(FEATURE[r]):
                        i = (g - g0) * GW + j
                        if b:
                            terms.append((a or b, ref[i, pl.ds((M if a else L) + t0, rows)]))
                        elif a and second:
                            terms += [(a, ref[i, pl.ds(r0 + t0, rows)]) for r0 in (M, L)]
                        elif a:
                            terms.append((a, ox[g * GW + j, pl.ds(t0, rows)]))
                    sign, left = _sum(terms)
                    m_sign, m = _sum((c[second], ref[(g - g0) * GW + j, 0:M])
                                     for j, c in enumerate(FEATURE[r]) if c[second])
                    v = mm(_cat(m, left), weights[g - g0][:, r * 128:(r + 1) * 128])
                    acc[r] = m_sign, sign, _add(acc[r][2] if r in acc else None, v)
                for r, (m_sign, sign, v) in acc.items():
                    sums[2].add(r, m_sign, v[:M])
                    sums[second if r < BOTH else 0].add(r, sign, v[M:M + HS])
                    if r < BOTH:
                        sums[1 - second].add(r, sign, v[M + HS:])

        recent.clear()
        stages = attention(projected, put_x if second else put_y)
        for p in range(NP):
            ready = LT * GW * ((9 * p + 5) // GW + 1)
            due += [(ready + lag, functools.partial(f, p)) for f, lag in zip(stages, LAGS[second])]
        if second:
            due += [(TOKENS_AT[0] + k * TOKENS_AT[1], task)
                    for k, task in enumerate(left_operands(jnp.minimum(s + 4, NSEG - 2), zero))]
        due.sort(key=lambda e: e[0])
        for g in range(GQ):
            project(g)
        for ref, chunk in zip(mixed, CHUNKS):
            out_chunk(reread(ref), *chunk)

    def first_segment(zero):
        def project(g):
            acc = {}

            def task(n, k):
                r = _dot(h0[0:L + SEG, _ds(k, 128)], tile(plain, PAD * GW + n, k))
                e = len(recent) % 8
                recent.extend([r[8 * e:8 * e + 8], r[8 * e + 8:8 * e + 16]])
                acc[n] = _add(acc.get(n), r)
                if k == LT - 1:
                    first[n] = acc[n][0:L]
                    tok[n] = acc[n][L:]

            return [functools.partial(task, g * GW + n, k) for n in range(GW) for k in range(LT)]

        def put(n, r):
            recent.extend([r[k:k + 8] for k in range(0, L, 16)])
            put_x(n, r)

        stages = attention(lambda n: first[n], put, zero=zero)
        new_mem = [None] * LT

        def heads(p0, p1):
            return [functools.partial(f, t - lag) for t in range(p0, p1 + 2)
                    for lag, f in enumerate(stages) if p0 <= t - lag < p1] + [lambda: None]

        def out(g):
            def task(n, k):
                ref, i = mixed_at(n)
                r = _dot(ref[i, 0:M], wo_raw[_ds(n, 128), _ds(k, 128)])
                recent.append(r)
                new_mem[k] = r if new_mem[k] is None else new_mem[k] + r

            return [functools.partial(task, g * GW + n, k) for n in range(GW) for k in range(LT)]

        c1, c2, c3, d1, d2, m1 = FIRST_CUT
        moves = transposes(GO - 2, plain, PAD + GQ - 6) + transposes(GO - 1, plain, PAD + GQ - 3)
        start(c_wo(0))
        wait(c_w(GO - 2) + c_bx0)
        start(c_wo(1) + c_wo(2))
        h0[0:M, :] = mem[0:M, :].astype(F32)
        h0[M:L + SEG, :] = bx[0:2 * SEG, :].astype(F32)
        _run(_merge(a_out(NB - 2, 0) + _each(project, range(c1)), moves[:m1] + _merge(
            sum(a_attention(1, zero), []), _each(sum_qkv, range(PAD + GQ - 9, PAD + d1), zero))))
        wait(c_w(GO - 1))
        start(c_wo(3) + c_wo(4))
        _run(_merge(a_out(NB - 1, 1) + _each(project, range(c1, c2)),
                    moves[m1:] + _each(sum_qkv, range(PAD + d1, PAD + d2), zero)))
        start(c_wo(5))
        wait(_each(c_wo, range(3)))
        start(c_wo(6) + c_wo(7))
        _run(_merge(_merge(_each(project, range(c2, c3)), heads(0, 11)),
                    _each(sum_qkv, range(PAD + d2, PAD + GQ), zero) + _each(sum_out, range(3), zero)))
        wait(_each(c_wo, range(3, 6)))
        _run(_merge(_merge(_merge(_each(project, range(c3, GQ)), _each(out, range(3))), heads(11, 13))
                    + _merge(_each(out, range(3, 6)), heads(13, NP)),
                    _merge(_each(sum_out, range(3, 6), zero), left_operands(2, zero))))
        wait(c_wo(6) + c_wo(7))
        start(c_bx1 + c_outa)
        _run(_merge(out(6) + out(7), _each(sum_out, (6, 7), zero)))
        for k in range(LT):
            m_s[k] = new_mem[k]

    def two_segments(it, carry):
        pl.when(it == 1)(lambda: wait(c_bx1))
        step(2 * it, 0, it >> 16)
        step(2 * it, 1, it >> 16)
        start(c_outb(_ds(it, 2 * SEG)))
        return carry

    def last_segment():
        res, acc = {}, [None] * LT

        def project(n, k):
            r = _dot(-m_s[k] if k % 2 else m_s[k], tile(plain, PAD * GW + n, k))
            res[n] = _acc(res.get(n), 1 - 2 * (k % 2), r)

        def out(n, k):
            acc[k] = _add(acc[k], _dot(_cat(ox[n], res[NQ + n]), wo_raw[_ds(n, 128), _ds(k, 128)]))

        stages = attention(lambda n: _cat(_val(res[n]), tok[n]) if n in res else tok[n],
                           lambda n, r: res.update({NQ + n: r}), M)
        tiles = [9 * p + e for t in range(NP + 3) for p, e0 in ((t, 3), (t - 3, 6)) if 0 <= p < NP
                 for e in range(e0, e0 + 3)]
        ready = {n: (i * LT + LT - 1) // 4 for i, n in enumerate(tiles)}
        due = [((i * LT + k) // 4, 0, functools.partial(project, n, k))
               for i, n in enumerate(tiles) for k in range(LT)]
        for p in range(NP):
            due += [(ready[9 * p + e] + lag, rank, functools.partial(f, p))
                    for f, lag, e, rank in zip(stages, LAST_LAGS, (5, 5, 8), (2, 2, 1))]
        t = 0
        for k in range(NO * LT):
            if k % 4 == 0:
                t = max(t + LAST_LAGS[4], ready[9 * ((k + 3) // 15) + 8] + LAST_LAGS[3])
            due.append((int(t), 3, functools.partial(out, *divmod(k, LT))))
        _run([task for _, _, task in sorted(due, key=lambda e: e[:2])])
        outb[S - 2 * SEG:, :] = jnp.concatenate(acc, axis=1).astype(BF16)
        start(c_outb(slice(S - 2 * SEG, S)))

    a_start()
    first_segment(lax.fori_loop(1, NB // 2, a_step, 0))
    lax.fori_loop(0, NSEG // 2 - 1, two_segments, 0)
    last_segment()
    wait(c_outa + c_outb(slice(0, S)))


def pallas_concat_heads__sliding_local_dilated__memory_aug_recurrent_mem_tr__prompt_kernel(
    A_x, A_wqkv, A_wo, B_x, B_mem0, B_Wq, B_Wk, B_Wv, B_Wo, B_seg_len,
):
    assert B_seg_len == SEG
    assert A_x.shape == B_x.shape == (1, S, D) and B_mem0.shape == (1, M, D)
    assert B_Wq.shape == B_Wk.shape == B_Wv.shape == (D, H, DH) and B_Wo.shape == (H, DH, D)
    dma = pltpu.SemaphoreType.DMA

    def vmem(shape, dtype):
        assert math.prod(shape) * jnp.dtype(dtype).itemsize % 16384 == 0
        return pltpu.VMEM(shape, dtype)

    call = pl.pallas_call(
        _kernel,
        out_shape=jax.ShapeDtypeStruct((S, 2 * D), BF16),
        in_specs=[pl.BlockSpec(memory_space=pl.ANY)] * 9,
        out_specs=pl.BlockSpec(memory_space=pl.ANY),
        scratch_shapes=[
            vmem((S, D), BF16),
            vmem((3, D, D), BF16),
            vmem((D, D), BF16),
            vmem((LT, D, 128), F32),
            vmem((2 * D, D), U32),
            vmem((TB, D), U32),
            vmem((2, LT, TB, 128), F32),
            vmem((2, 2 * LT, HALO + TB, 128), F32),
            vmem((2, TB, D), F32),
            vmem((S, D), BF16),
            vmem((S, D), BF16),
            vmem((8 * M, D), BF16),
            vmem((RAW * 3 * GW * 128, D), BF16),
            vmem((H * DH, D), BF16),
            vmem(((PAD + GQ) * GW * 64, D), U32),
            vmem(((PAD + GQ) * 8 * 64, D), U32),
            vmem((GO * 64, NR * 128), U32),
            vmem((3 * SEG, D), F32),
            vmem((NQ, L, 128), F32),
            vmem((LT, 3 * SEG, 128), F32),
            vmem((NR + 1, L, 128), F32),
            vmem((8, M, 128), F32),
            vmem((GQ, 2 * GW, SEG, 128), F32),
            vmem((NQ, SEG, 128), F32),
            [vmem((4, L, 128), F32)] * RING,
            vmem((NO, SEG, 128), F32),
            [vmem((20, L + SEG, 128), F32)] * len(CHUNKS),
            vmem((2 * LT, SEG, 128), F32),
            vmem((S, D), BF16),
            dma((5,)), dma((NB // 2,)), dma((GO, 3)), dma((3,)), dma((GO,)), dma((2,)),
        ],
        compiler_params=pltpu.CompilerParams(vmem_limit_bytes=126 * 1024 * 1024, **{
            name: True for name in ("disable_bounds_checks", "disable_semaphore_checks")
            if hasattr(pltpu.CompilerParams, name)}),
        name="sliding_and_memory_attention",
    )

    def by_feature(w):
        return w.transpose(1, 2, 0).reshape(H * DH, D)

    out = call(A_x.reshape(S, D), A_wqkv, A_wo, B_x.reshape(S, D), B_mem0.reshape(M, D),
               by_feature(B_Wq), by_feature(B_Wk), by_feature(B_Wv), B_Wo.reshape(H * DH, D))
    return out.reshape(1, S, 2 * D)
```

```python
import collections
import functools
import itertools
import math
import random

import jax
import jax.numpy as jnp
import numpy as np
from jax import lax
from jax.experimental import pallas as pl
from jax.experimental.pallas import tpu as pltpu

F32, BF16, U32 = jnp.float32, jnp.bfloat16, jnp.uint32
NT = (((1,), (1,)), ((), ()))
MASKED = -1000000000.0
LOG2E = math.log2(math.e)

S, D = 2048, 640
LT = D // 128

AH, AD, AW, ADIL = 32, 20, 8, 2
HALO = 16
TB = 128
NB = S // TB

H, DH, M, SEG = 32, 192, 8, 32
L = M + SEG
HS = SEG // 2
NSEG = S // SEG
NP = H // 2
NO = 3 * NP
NQ = 3 * NO
GW = 6
GO, GQ = NO // GW, NQ // GW
PAD = 3
RAW = 4
RING = 12
CHUNKS = ((0, 3), (3, 5), (5, GO))


def _algorithm(rank_ones):
    rows = np.array([[1, 0], [0, 1], [1, 1]])
    duals = np.array([[0, 1], [1, 0], [1, -1]])
    sets = [[[np.array(["-0+".index(c) - 1 for c in w]) for w in e.split()] for e in s] for s in rank_ones]
    left, right = [], []
    for t, s in enumerate(sets):
        p, q = [k for k in range(3) if k != t]
        for u, v in s:
            left += [np.outer(u, rows[p]), np.outer(u, rows[q])]
            right += [np.outer(v, duals[q]), np.outer(v, duals[p])]
    for (u0, v0), (u1, v1), (u2, v2) in itertools.product(*sets):
        for a, b in itertools.product((1, -1), repeat=2):
            e = np.outer(u0 + a * u1, v0 + b * v1)
            if (e == np.outer(u2, v2)).all() or (e == -np.outer(u2, v2)).all():
                left.append(np.outer(u0, rows[1]) - a * np.outer(u1, rows[0]))
                right.append(np.outer(v0, duals[1]) + b * np.outer(v1, duals[0]))
    left, right = np.array(left), np.array(right)
    have = np.einsum("rka,rnb->kanbr", left, right).reshape(-1, len(left))
    want = np.einsum("kp,nq,ab->kanbpq", np.eye(LT), np.eye(GW), np.eye(2)).reshape(len(have), -1)
    blocks = np.rint(np.linalg.lstsq(have, want, rcond=None)[0]).astype(int)
    assert (have @ blocks == want).all()
    sign = blocks.max(axis=1) * 2 - 1
    return left * sign[:, None, None], blocks * sign[:, None], right


def _shared_sums(matrix, seed):
    rng = random.Random(seed)
    rows = [{k: int(c) for k, c in enumerate(row) if c} for row in matrix]
    shared = {}
    while True:
        count = collections.Counter(
            (a, b, r[a] * r[b]) for r in rows for a, b in itertools.combinations(sorted(r), 2))
        top = max(count.values(), default=0)
        if top < 2:
            return shared, rows
        best = sorted(k for k, n in count.items() if n == top)
        a, b, sign = best[int(rng.random() * len(best))]
        name = matrix.shape[1] + len(shared)
        shared[name] = a, b, sign
        for r in rows:
            if r.get(a, 0) * r.get(b, 0) == sign:
                r[name] = r.pop(a)
                del r[b]


MODEL, BLOCKS, FEATURE = _algorithm((
    ("+0000 +00++0", "000+0 0+0000", "0000+ 000+00", "+-+00 00000+", "+00+0 00+0+0"),
    ("0+00+ 000+++", "0+0+0 0+00++", "00+-+ 00++00", "00+0+ +00000", "+0+00 0000+0", "00+00 0+-000"),
    ("0+000 0000++", "00+-+ ++0000", "00+00 +00+00", "+-000 0+-00+", "00+-0 00+000", "+-00- +0000-")))
NR = len(BLOCKS)
BOTH = 34
SINGLE = {r: int(row.argmax()) for r, row in enumerate(BLOCKS) if abs(row).sum() == 1}
SUMMED = [r for r in range(NR) if r not in SINGLE]


def _step_sums(out, step, seed):
    use = MODEL[:, :, step].any(1) & FEATURE[:, :, step].any(1)
    return [_shared_sums((m * keep[:, None]).T, seed) for m, keep in (
        (out.reshape(NR, -1), use), (out.reshape(NR, -1), use & (np.arange(NR) < BOTH)), (out[:, :, step], use))]


QKV_SUMS = _step_sums(FEATURE, 0, 32), _step_sums(FEATURE, 1, 5)
OUT_SUMS = _step_sums(MODEL, 0, 0), _step_sums(MODEL, 1, 6)
BLOCK_SUMS = _shared_sums(BLOCKS, 37)

QKV_ORDER = (
    (30, 14, 20, 3, 28, 12, 9, 22, 10, 18, 26, 1, 5, 24, 32, 7, 16,
     40, 38, 36, 45, 46, 44, 39, 34, 35, 43, 37, 41, 42),
    (31, 15, 4, 11, 27, 0, 19, 8, 23, 13, 33, 6, 29, 21, 2, 25, 17,
     40, 34, 41, 39, 35, 45, 46, 36, 43, 44, 38, 37, 42))
OUT_ORDER = (
    (24, 14, 10, 5, 32, 28, 16, 30, 22, 7, 9, 3, 12, 1, 18, 20, 26,
     40, 34, 41, 39, 42, 37, 43, 36, 46, 45, 44, 35, 38),
    (23, 11, 2, 13, 15, 17, 4, 25, 31, 6, 33, 8, 29, 21, 19, 0, 27,
     39, 36, 45, 34, 41, 40, 37, 44, 42, 43, 46, 35, 38))
BLOCK_ORDER = (3, 28, 6, 0, 5, 17, 11, 8, 10, 7, 4, 16, 2, 1, 23, 22, 9, 29, 24, 19, 12, 18, 25, 13, 14, 20,
               21, 15, 26, 27)
MEM_ORDER = (2, 1, 4, 0, 3)

LAGS = ((40, 70, 100), (50, 80, 110))
TOKENS_AT = (737, 4)
OUT_PARTS = (5, 5)
TURNS = int(
    "734a6a6a6a24a26a6a4a24b4a6a6a430dd2852d2d2969693094b4a552942968a52d21e5161c385d29525a294b42d32a4"
    "b0e172a626a3453521e49694385c61a5a4d22e28732a4b0e171a52968a52d21e5161c385d29525a294b42d32a4b0e172"
    "5a1c3465870e1b4a62a4b4a6870e15a52c385a587161a5a1c7171717161861a5a5a1861a5a5a5825a5a292d2d2d2d298"
    "a187353141c29a91a984d48d3a2c34a272a6a43a929a91a6870e2c1e1c3871385a529694a58707870d2954a9a90e4a5a"
    "52954a6a42e19694c5394a587078b0e1a8e1c8b0e626a62c1e1c3870790d4c29e1c3931a193931a949a9458d0e949871", 16)

A_PACE = (12, 4)
SUM_PACE = (18, 10)
A_CUT = (58, 1, 18, 0)
START_CUT = (15, 20)
FIRST_CUT = (5, 12, 21, 17, 21, 6)
LAST_LAGS = (7, 12, 3, 7, 1.9)


def _ds(i, n):
    return pl.ds(i * n if isinstance(i, int) else pl.multiple_of(i * n, n), n)


def _dot(a, b):
    return jnp.dot(a, b, preferred_element_type=F32)


def _cat(*parts):
    return jnp.concatenate(parts, axis=0)


def _add(a, b):
    return b if a is None else _cat(a[:M] + b[:M], a[M:] + b[M:])


def _acc(a, sign, b):
    if a is None:
        return sign, b
    if a[0] == sign:
        return sign, a[1] + b
    return (1, a[1] - b) if a[0] > 0 else (1, b - a[1])


def _sum(terms):
    return functools.reduce(lambda a, t: _acc(a, *t), terms, None)


def _val(a):
    return a[1] if a[0] > 0 else -a[1]


class _Sums:
    def __init__(self, plan, done, begin=lambda k: None):
        self.shared, self.rows = plan
        self.done, self.begin = done, begin
        self.terms, self.sums = {}, [None] * len(self.rows)
        for k, row in enumerate(self.rows):
            if not row and (first := begin(k)) is not None:
                done(k, first)

    def add(self, name, sign, value):
        self.terms[name] = sign, value
        for k, row in enumerate(self.rows):
            if name in row:
                if self.sums[k] is None and (first := self.begin(k)) is not None:
                    self.sums[k] = 1, first
                self.sums[k] = _acc(self.sums[k], row[name] * sign, value)
                if all(n in self.terms for n in row):
                    self.done(k, _val(self.sums[k]))
        for n, (a, b, s) in self.shared.items():
            if name in (a, b) and a in self.terms and b in self.terms and n not in self.terms:
                self.add(n, *_acc(self.terms[a], s * self.terms[b][0], self.terms[b][1]))


def _share(tasks, k, n):
    return list(tasks[k * len(tasks) // n:(k + 1) * len(tasks) // n])


def _merge(a, b, early=0):
    n = len(a) - early
    return [t for k in range(n) for t in [a[k]] + _share(b, k, n)] + a[n:]


def _each(f, items, *args):
    return [task for item in items for task in f(item, *args)]


def _run(tasks):
    for task in tasks:
        task()


def _kernel(ax_hbm, awqkv_hbm, awo_hbm, bx_hbm, mem_hbm, wq_hbm, wk_hbm, wv_hbm, wo_hbm,
            out_hbm,
            ax, awqkv, awo, tmp, wa, xb, q_s, kv_s, oa_s, outa,
            bx, mem, raw, wo_raw, plain, summed, wo, h0, first, xy, lhs, m_s, part, tok, ring,
            ox, mixed, opart, outb,
            sem_a, sem_x, sem_w, sem_b, sem_wo, sem_o):
    cp = pltpu.make_async_copy

    def rows_copy(src, dst, rows, sem):
        return [cp(src.at[rows, :], dst.at[rows, :], sem)]

    c_aw = [cp(awqkv_hbm.at[r0:r1, _ds(j, D)], awqkv.at[j, r0:r1], sem_a.at[k])
            for k, (j, (r0, r1)) in enumerate(itertools.product(range(3), ((0, 384), (384, D))))]
    c_awo = [cp(awo_hbm, awo, sem_a.at[6])]
    c_bx0 = [cp(mem_hbm, mem.at[0:M], sem_b.at[0])] + rows_copy(bx_hbm, bx, slice(0, 6 * SEG), sem_b.at[1])
    c_bx1 = rows_copy(bx_hbm, bx, slice(6 * SEG, S), sem_b.at[2])
    c_outa = [cp(outa, out_hbm.at[:, 0:D], sem_o.at[0])]

    def c_ax(c):
        return rows_copy(ax_hbm, ax, _ds(c, 2 * TB), sem_x.at[c])

    def c_w(c):
        return [cp(w.at[_ds(c, GW * 128), :], raw.at[_ds((c & (RAW - 1)) * 3 + j, GW * 128), :], sem_w.at[c, j])
                for j, w in enumerate((wq_hbm, wk_hbm, wv_hbm))]

    def c_wo(g):
        return rows_copy(wo_hbm, wo_raw, _ds(g, GW * 128), sem_wo.at[g])

    def c_outb(rows):
        return [cp(outb.at[rows, :], out_hbm.at[rows, D:], sem_o.at[1])]

    def start(copies):
        for c in copies:
            c.start()

    def wait(copies):
        for c in copies:
            c.wait()
        recent.clear()

    recent = []

    def paced(x, zero, marks):
        late = _cat(*[recent[t] if t >= 0 else jnp.zeros((8, 128), F32) for t in marks[:x.shape[0] // 8]])
        always = lax.broadcasted_iota(jnp.int32, x.shape, 1) >= zero
        return lax.select(always, x, late if x.dtype == F32 else pltpu.bitcast(late, U32))

    def tile(ref, i, j):
        return pltpu.bitcast(ref[_ds(i, 64), _ds(j, 128)], BF16)

    def a_weights(j, zero=None):
        def task(t):
            if j < 3:
                tmp[t] = awqkv[j, _ds(t, 128), :].astype(F32).T
            else:
                marks = [len(recent) - 40 + k * 3 // 4 for k in range(40)]
                w = paced(pltpu.bitcast(awo[:, _ds(t, 128)], U32), zero, marks)
                tmp[t] = pltpu.bitcast(w, BF16).astype(F32)
            w = _cat(*[tmp[t, pl.ds(d, AH, stride=AD), :] for d in range(AD)])
            wa[_ds(j, D // 2), _ds(t, 128)] = pltpu.bitcast(w.astype(BF16), U32)

        return [functools.partial(task, t) for t in range(LT)]

    def by_tile(product, put):
        acc = [None]

        def task(t, k):
            r = product(t, k)
            e = len(recent) % 16
            recent.extend(r[8 * (e + i) % TB:8 * (e + i) % TB + 8] for i in range(4))
            acc[0] = _add(acc[0] if k else None, r)
            if k == LT - 1:
                put(t, acc[0])

        return [functools.partial(task, t, k) for t in range(LT) for k in range(LT)]

    def a_load(i, b):
        xb[_ds(b, TB // 2), :] = pltpu.bitcast(ax[_ds(i, TB), :], U32)

    def a_proj(j, b, first_block=False):
        def put(t, r):
            if j == 0:
                q_s[b, t] = r
                return
            c = (j - 1) * LT + t
            kv_s[b, c, HALO:, :] = r
            if first_block:
                kv_s[b, c, 0:HALO, :] = jnp.broadcast_to(r[0:1, :], (HALO, 128))
            else:
                kv_s[b, c, 0:HALO, :] = kv_s[1 - b, c, TB:, :]

        return by_tile(lambda t, k: lax.dot_general(
            tile(xb, b, k), tile(wa, j * LT + t, k), NT, preferred_element_type=F32), put)

    def a_attention(b, zero, first_block=False):
        n = TB // 8
        lag = n if first_block else A_PACE[1]
        marks, logits = [], []

        def mark():
            marks.append(len(recent) - A_PACE[0])

        def window(c, w):
            return kv_s[b, c, pl.ds(HALO - ADIL * w, TB), :]

        def score():
            q = [paced(q_s[b, t], zero, marks[::4]) for t in range(LT)]
            sums = [functools.reduce(jnp.add, [q[t] * window(t, w) for t in range(LT)]) for w in range(AW)]
            rows = {}
            for k in range(n + 1):
                if k < n:
                    a = _cat(*[a[8 * k:8 * k + 8] for a in sums])
                    rows[k] = a + pltpu.roll(a, 2 * AH, 1)
                if k > 0:
                    rows[k - 1] = rows[k - 1] + pltpu.roll(rows[k - 1], AH, 1)
            logits.extend(_cat(*[rows[k][8 * w:8 * w + 8] for k in range(n)]) for w in range(AW))

        def mix():
            scale, lg = AD ** -0.5, logits
            if first_block:
                pos = lax.broadcasted_iota(jnp.int32, (HALO, 128), 0)
                lg = [_cat(jnp.where(pos >= ADIL * w, a[:HALO], MASKED / scale), a[HALO:])
                      for w, a in enumerate(lg)]
            m = paced(functools.reduce(jnp.maximum, lg), zero, marks[4 * lag + 1::4])
            e = [jnp.exp2((a - m) * (scale * LOG2E)) for a in lg]
            inv = 1.0 / functools.reduce(jnp.add, e)
            for t in range(LT):
                v = [window(LT + t, w) for w in range(AW)]
                v[0] = paced(v[0], zero, marks[4 * lag + 2 + 2 * t // LT::4])
                oa_s[b, :, _ds(t, 128)] = inv * functools.reduce(jnp.add, map(jnp.multiply, e, v))

        return [mark] * (4 * n) + [score], [mark] * (4 * lag) + [mix]

    def a_out(i, b):
        def put(t, r):
            outa[_ds(i, TB), _ds(t, 128)] = r.astype(BF16)

        return by_tile(lambda t, k: _dot(oa_s[b, :, _ds(k, 128)], tile(wa, 3 * LT + k, t)), put)

    def transposes(c, dst, g):
        def task(n):
            t = ((c & (RAW - 1)) * 3 + n % 9 // 3) * GW + n // 9 * 3 + n % 3
            v = pltpu.bitcast(raw[_ds(t, 128), :].T, U32)
            for k in range(LT):
                dst[_ds(g * GW + n, 64), _ds(k, 128)] = v[k * 64:(k + 1) * 64]

        return [functools.partial(task, n) for n in range(3 * GW)]

    def sum_blocks(block, put, zero):
        back, n = SUM_PACE
        marks = []

        def mark():
            marks.append(len(recent) - back)

        def done(r, v):
            if r not in SINGLE:
                put(r, pltpu.bitcast(v.astype(BF16), U32))

        def task():
            sums = _Sums(BLOCK_SUMS, done)
            for k in range(n):
                for i, b in enumerate(_share(BLOCK_ORDER, k, n)):
                    v = block(*divmod(b, GW))
                    if i == 0:
                        v = paced(v, zero, marks[k::n])
                    for r in SINGLE:
                        if SINGLE[r] == b:
                            put(r, v)
                    sums.add(b, 1, pltpu.bitcast(v, BF16).astype(F32))

        return [mark] * (8 * n) + [task]

    def sum_qkv(g, zero, src=plain, dst=summed):
        def put(r, v):
            if r not in SINGLE:
                i, j = divmod(SUMMED.index(r), LT)
                dst[_ds(g * 8 + i, 64), _ds(j, 128)] = v

        return sum_blocks(lambda k, n: src[_ds(g * GW + n, 64), _ds(k, 128)], put, zero)

    def sum_out(g, zero):
        def put(r, v):
            wo[_ds(g, 64), _ds(r, 128)] = v

        return sum_blocks(lambda k, n: pltpu.bitcast(wo_raw[_ds(g * GW + n, 128), _ds(k, 128)], U32), put, zero)

    def a_start():
        start(c_aw[:2])
        zero = lax.fori_loop(0, 2, lambda it, carry: it >> 16, 0)
        start(c_ax(0))
        wait(c_aw[:1])
        _run(a_weights(0)[:3])
        wait(c_aw[1:2])
        start(c_aw[2:3])
        _run(a_weights(0)[3:])
        wait(c_ax(0))
        start(c_aw[3:5])
        a_load(0, 0)
        a_load(1, 1)
        k0, rest = a_proj(1, 0, True), START_CUT
        _run(a_proj(0, 0))
        wait(c_aw[2:3])
        start(c_aw[5:] + c_awo)
        _run(a_proj(0, 1)[:rest[0]] + a_weights(1)[:3])
        wait(c_aw[3:4])
        start(c_ax(1) + c_ax(2))
        _run(a_proj(0, 1)[rest[0]:] + a_weights(1)[3:] + k0)
        wait(c_aw[4:])
        start(c_w(0))
        early, late = a_attention(0, zero, True)
        _run(a_proj(1, 1)[:rest[1]] + a_weights(2) + _merge(a_proj(2, 0, True), early))
        wait(c_awo)
        start(c_bx0)
        _run(_merge(a_proj(1, 1)[rest[1]:] + a_proj(2, 1), _merge(late, a_weights(3, zero)), 4))
        wait(c_ax(1))
        a_load(2, 0)

    def a_step(it, carry):
        i, g, zero = 2 * it, jnp.maximum(3 * it - 9 + PAD, 0), it >> 16
        pl.when(it + 2 < NB // 2)(lambda: start(c_ax(it + 2)))
        pl.when(it + 1 < NB // 2)(lambda: wait(c_ax(it + 1)))
        start(c_w(it))
        pl.when(it > 1)(lambda: wait(c_w(it - 2)))
        src, dst = [ref.at[pl.ds(pl.multiple_of(g * n, n), k * n)]
                    for ref, n, k in ((plain, GW * 64, 6), (summed, 8 * 64, 3))]
        sums, moves = _each(sum_qkv, range(3), zero, src, dst), transposes(it + RAW - 2, src, 3)
        cut, m1, m2 = len(sums) * A_CUT[0] // 100, A_CUT[1], A_CUT[2]
        early, late = a_attention(1, zero)
        a_load(i + 1, 1)
        _run(_merge(a_out(i - 2, 0) + _each(a_proj, range(3), 0),
                    moves[:m1] + _merge(early, sums[:cut]) + moves[m1:m2]))
        a_load(jnp.minimum(i + 2, NB - 1), 0)
        side = sum(a_attention(0, zero), [])
        side = _merge(side[:len(late)], late) + side[len(late):]
        _run(_merge(_each(a_proj, range(3), 1) + a_out(i - 1, 1), _merge(side, sums[cut:]) + moves[m2:], A_CUT[3]))
        return zero

    def attention(qkv, put, row0=0, zero=0):
        row = lax.broadcasted_iota(jnp.int32, (L - row0, 128), 0) + row0
        col = lax.broadcasted_iota(jnp.int32, (L - row0, 128), 1) + zero
        head0 = col < L
        visible = jnp.where(row < M, L - 1, row) >= jnp.where(head0, col, col - L)
        scale = DH ** -0.5
        st = {}

        def by_head(n):
            t = qkv(n)
            if n % 3 == 1:
                low = lax.broadcasted_iota(jnp.int32, t.shape, 1) < 64 + zero
                t = _cat(jnp.where(low, t, 0.0), jnp.where(low, 0.0, t))
            elif n % 3 == 2:
                t = _cat(jnp.zeros_like(t), t)
            return _cat(t, jnp.zeros((128 - len(t), 128), F32)).astype(BF16)

        def score(p):
            sc = [lax.dot_general(qkv(9 * p + t), by_head(9 * p + 3 + t), NT, preferred_element_type=F32)
                  for t in range(3)]
            sc = jnp.where(visible, functools.reduce(_add, sc), jnp.where(col < 2 * L, MASKED / scale, -jnp.inf))
            m0 = jnp.max(jnp.where(head0, sc, -jnp.inf), axis=1, keepdims=True)
            m1 = jnp.max(jnp.where(head0, -jnp.inf, sc), axis=1, keepdims=True)
            st[p] = sc - jnp.where(head0, m0, m1)

        def normalize(p):
            e = jnp.exp2(st[p] * (scale * LOG2E))
            l0 = jnp.sum(jnp.where(head0, e, 0.0), axis=1, keepdims=True)
            l1 = jnp.sum(jnp.where(head0, 0.0, e), axis=1, keepdims=True)
            st[p] = e / jnp.where(head0, l0, l1)

        def mix(p):
            for t in range(3):
                put(3 * p + t, _dot(st[p], by_head(9 * p + 6 + t)))

        return score, normalize, mix

    def mixed_at(n):
        return [(ref, n - g0 * GW) for ref, (g0, g1) in zip(mixed, CHUNKS) if g0 <= n // GW < g1][0]

    def put_x(n, r):
        ref, k = mixed_at(n)
        ref[k, 0:M] = r[0:M]
        ox[n] = r[M:]

    def put_y(n, r):
        ref, k = mixed_at(n)
        ref[k] = _cat(r[0:M], ox[n] - r[M:], r[M:])

    def left_operands(s, zero):
        def load(k):
            x, y = [paced(pltpu.bitcast(bx[_ds(s + e, SEG), _ds(k, 128)], U32), zero, [len(recent) - 20] * 2)
                    for e in range(2)]
            x, y = [pltpu.bitcast(v, BF16).astype(F32) for v in (x, y)]
            xy[k] = _cat(x, y, x + y)

        def task(r):
            src = xy.at[pl.ds(4 * zero, LT)]
            terms = [(a or b, src[k, _ds(2 if a and b else 1 if b else 0, SEG)])
                     for k, (a, b) in enumerate(MODEL[r]) if a or b]
            terms[0] = terms[0][0], paced(terms[0][1], zero, [len(recent) - 20] * 4)
            v = _val(_sum(terms))
            lhs[r, 0:HS] = v[:HS]
            lhs[r, HS + M:] = v[HS:]

        return [functools.partial(load, k) for k in range(LT)] + [functools.partial(task, r) for r in range(NR)]

    def step(s, second, zero):
        def reread(ref):
            return ref.at[pl.ds(4 * zero, ref.shape[0])]

        part_r, ring_r = reread(part), [reread(r) for r in ring]
        halves = [slice(0, HS), slice(HS, SEG)][::1 - 2 * second]
        new_mem = [None] * LT
        due = []

        def mm(x, w):
            r = _dot(x, w)
            recent.append(r[0:M] if second and len(recent) > TOKENS_AT[0] - 24 else None)
            while due and due[0][0] <= len(recent):
                due.pop(0)[1]()
            return r

        def in_turn(items):
            lists = [[x for x in items if (x[0] >= BOTH) == e] for e in (False, True)]
            for _ in items:
                yield lists[TURNS >> second * (NQ + NO) * LT + len(recent) & 1].pop(0)

        def mem_tiles(r):
            return [MEM_ORDER[k] for k, c in enumerate(MODEL[r]) if c[second]]

        def project(g):
            def token_sums(e):
                def begin(k):
                    return part_r[g, k, halves[e]] if second and QKV_SUMS[0][1 - e][1][k] else None

                def done(k, v):
                    n = GW * g + k // 2
                    if not second:
                        part[g, k, halves[e]] = v
                    elif k % 2:
                        tok[n, halves[e]] = v
                    else:
                        ring[n // 3 % RING][n % 3, pl.ds(M + halves[e].start, HS)] = v

                return _Sums(QKV_SUMS[second][e], done, begin)

            def done(k, v):
                n = GW * g + k
                ring[n // 3 % RING][n % 3, 0:M] = v

            sums = token_sums(0), token_sums(1), _Sums(QKV_SUMS[second][2], done)
            weights = pltpu.bitcast(summed[_ds(PAD + g, 8 * 64), :], BF16)
            order = sorted(QKV_ORDER[second], key=lambda r: max(mem_tiles(r)) if second and g == 0 else 0)
            for r, in in_turn([(r,) for r in order]):
                t0, t1 = (0, L) if r < BOTH else (second * HS, second * HS + HS + M)
                if g == 0:
                    lhs[r, HS:HS + M] = _val(_sum(
                        (c[second], m_s[k]) for k, c in enumerate(MODEL[r]) if c[second]))
                if r in SINGLE:
                    w = tile(plain, (PAD + g) * GW + SINGLE[r] % GW, SINGLE[r] // GW)
                else:
                    i, j = divmod(SUMMED.index(r), LT)
                    w = weights[i * 128:(i + 1) * 128, j * 128:(j + 1) * 128]
                v = mm(lhs[r, t0:t1], w)
                sums[2].add(r, 1, v[HS - t0:HS - t0 + M])
                if t0 == 0:
                    sums[second].add(r, 1, v[:HS])
                if t1 == L:
                    sums[1 - second].add(r, 1, v[-HS:])

        def projected(n):
            src = ring_r[n // 3 % RING]
            return src[n % 3] if second else _cat(src[n % 3, 0:M], tok[n])

        def out_chunk(ref, g0, g1):
            def token_sums(e):
                def begin(k):
                    if (second and OUT_SUMS[0][1 - e][1][k]) or (g0 > 0 and OUT_SUMS[second][e][1][k]):
                        return opart[k, halves[e]]

                def done(k, v):
                    if second and g1 == GO:
                        rows = _ds((s + k % 2) * 2 + halves[e].start // HS, HS)
                        outb[rows, _ds(k // 2, 128)] = v.astype(BF16)
                    else:
                        opart[k, halves[e]] = v

                return _Sums(OUT_SUMS[second][e], done, begin)

            def done(k, v):
                new_mem[k] = v
                if g1 == GO:
                    m_s[k] = v

            sums = token_sums(0), token_sums(1), _Sums(OUT_SUMS[second][2], done, list(new_mem).__getitem__)
            weights = [pltpu.bitcast(wo[_ds(g, 64), :], BF16) for g in range(g0, g1)]
            order = sorted(OUT_ORDER[second], key=lambda r: min(mem_tiles(r)) if g1 == GO and not second else 0)
            tall, short = [[r for r in order if (r >= BOTH) == e] for e in (False, True)]
            n = OUT_PARTS[second]
            for k in range(n):
                acc = {}
                some = _share(tall[::-1], n - 1 - k, n)[::-1] + _share(short, k, n)
                for r, g in in_turn([(r, g) for g in range(g0, g1) for r in some]):
                    t0, rows = (0, SEG) if r < BOTH else (halves[0].start, HS)
                    terms = []
                    for j, (a, b) in enumerate(FEATURE[r]):
                        i = (g - g0) * GW + j
                        if b:
                            terms.append((a or b, ref[i, pl.ds((M if a else L) + t0, rows)]))
                        elif a and second:
                            terms += [(a, ref[i, pl.ds(r0 + t0, rows)]) for r0 in (M, L)]
                        elif a:
                            terms.append((a, ox[g * GW + j, pl.ds(t0, rows)]))
                    sign, left = _sum(terms)
                    m_sign, m = _sum((c[second], ref[(g - g0) * GW + j, 0:M])
                                     for j, c in enumerate(FEATURE[r]) if c[second])
                    v = mm(_cat(m, left), weights[g - g0][:, r * 128:(r + 1) * 128])
                    acc[r] = m_sign, sign, _add(acc[r][2] if r in acc else None, v)
                for r, (m_sign, sign, v) in acc.items():
                    sums[2].add(r, m_sign, v[:M])
                    sums[second if r < BOTH else 0].add(r, sign, v[M:M + HS])
                    if r < BOTH:
                        sums[1 - second].add(r, sign, v[M + HS:])

        recent.clear()
        stages = attention(projected, put_x if second else put_y)
        for p in range(NP):
            ready = LT * GW * ((9 * p + 5) // GW + 1)
            due += [(ready + lag, functools.partial(f, p)) for f, lag in zip(stages, LAGS[second])]
        if second:
            due += [(TOKENS_AT[0] + k * TOKENS_AT[1], task)
                    for k, task in enumerate(left_operands(jnp.minimum(s + 4, NSEG - 2), zero))]
        due.sort(key=lambda e: e[0])
        for g in range(GQ):
            project(g)
        for ref, chunk in zip(mixed, CHUNKS):
            out_chunk(reread(ref), *chunk)

    def first_segment(zero):
        def project(g):
            acc = {}

            def task(n, k):
                r = _dot(h0[0:L + SEG, _ds(k, 128)], tile(plain, PAD * GW + n, k))
                e = len(recent) % 8
                recent.extend([r[8 * e:8 * e + 8], r[8 * e + 8:8 * e + 16]])
                acc[n] = _add(acc.get(n), r)
                if k == LT - 1:
                    first[n] = acc[n][0:L]
                    tok[n] = acc[n][L:]

            return [functools.partial(task, g * GW + n, k) for n in range(GW) for k in range(LT)]

        def put(n, r):
            recent.extend([r[k:k + 8] for k in range(0, L, 16)])
            put_x(n, r)

        stages = attention(lambda n: first[n], put, zero=zero)
        new_mem = [None] * LT

        def heads(p0, p1):
            return [functools.partial(f, t - lag) for t in range(p0, p1 + 2)
                    for lag, f in enumerate(stages) if p0 <= t - lag < p1] + [lambda: None]

        def out(g):
            def task(n, k):
                ref, i = mixed_at(n)
                r = _dot(ref[i, 0:M], wo_raw[_ds(n, 128), _ds(k, 128)])
                recent.append(r)
                new_mem[k] = r if new_mem[k] is None else new_mem[k] + r

            return [functools.partial(task, g * GW + n, k) for n in range(GW) for k in range(LT)]

        c1, c2, c3, d1, d2, m1 = FIRST_CUT
        moves = transposes(GO - 2, plain, PAD + GQ - 6) + transposes(GO - 1, plain, PAD + GQ - 3)
        start(c_wo(0))
        wait(c_w(GO - 2) + c_bx0)
        start(c_wo(1) + c_wo(2))
        h0[0:M, :] = mem[0:M, :].astype(F32)
        h0[M:L + SEG, :] = bx[0:2 * SEG, :].astype(F32)
        _run(_merge(a_out(NB - 2, 0) + _each(project, range(c1)), moves[:m1] + _merge(
            sum(a_attention(1, zero), []), _each(sum_qkv, range(PAD + GQ - 9, PAD + d1), zero))))
        wait(c_w(GO - 1))
        start(c_wo(3) + c_wo(4))
        _run(_merge(a_out(NB - 1, 1) + _each(project, range(c1, c2)),
                    moves[m1:] + _each(sum_qkv, range(PAD + d1, PAD + d2), zero)))
        start(c_wo(5))
        wait(_each(c_wo, range(3)))
        start(c_wo(6) + c_wo(7))
        _run(_merge(_merge(_each(project, range(c2, c3)), heads(0, 11)),
                    _each(sum_qkv, range(PAD + d2, PAD + GQ), zero) + _each(sum_out, range(3), zero)))
        wait(_each(c_wo, range(3, 6)))
        _run(_merge(_merge(_merge(_each(project, range(c3, GQ)), _each(out, range(3))), heads(11, 13))
                    + _merge(_each(out, range(3, 6)), heads(13, NP)),
                    _merge(_each(sum_out, range(3, 6), zero), left_operands(2, zero))))
        wait(c_wo(6) + c_wo(7))
        start(c_bx1 + c_outa)
        _run(_merge(out(6) + out(7), _each(sum_out, (6, 7), zero)))
        for k in range(LT):
            m_s[k] = new_mem[k]

    def two_segments(it, carry):
        pl.when(it == 1)(lambda: wait(c_bx1))
        step(2 * it, 0, it >> 16)
        step(2 * it, 1, it >> 16)
        start(c_outb(_ds(it, 2 * SEG)))
        return carry

    def last_segment():
        res, acc = {}, [None] * LT

        def project(n, k):
            r = _dot(-m_s[k] if k % 2 else m_s[k], tile(plain, PAD * GW + n, k))
            res[n] = _acc(res.get(n), 1 - 2 * (k % 2), r)

        def out(n, k):
            acc[k] = _add(acc[k], _dot(_cat(ox[n], res[NQ + n]), wo_raw[_ds(n, 128), _ds(k, 128)]))

        stages = attention(lambda n: _cat(_val(res[n]), tok[n]) if n in res else tok[n],
                           lambda n, r: res.update({NQ + n: r}), M)
        tiles = [9 * p + e for t in range(NP + 3) for p, e0 in ((t, 3), (t - 3, 6)) if 0 <= p < NP
                 for e in range(e0, e0 + 3)]
        ready = {n: (i * LT + LT - 1) // 4 for i, n in enumerate(tiles)}
        due = [((i * LT + k) // 4, 0, functools.partial(project, n, k))
               for i, n in enumerate(tiles) for k in range(LT)]
        for p in range(NP):
            due += [(ready[9 * p + e] + lag, rank, functools.partial(f, p))
                    for f, lag, e, rank in zip(stages, LAST_LAGS, (5, 5, 8), (2, 2, 1))]
        t = 0
        for k in range(NO * LT):
            if k % 4 == 0:
                t = max(t + LAST_LAGS[4], ready[9 * ((k + 3) // 15) + 8] + LAST_LAGS[3])
            due.append((int(t), 3, functools.partial(out, *divmod(k, LT))))
        _run([task for _, _, task in sorted(due, key=lambda e: e[:2])])
        outb[S - 2 * SEG:, :] = jnp.concatenate(acc, axis=1).astype(BF16)
        start(c_outb(slice(S - 2 * SEG, S)))

    a_start()
    first_segment(lax.fori_loop(1, NB // 2, a_step, 0))
    lax.fori_loop(0, NSEG // 2 - 1, two_segments, 0)
    last_segment()
    wait(c_outa + c_outb(slice(0, S)))


def pallas_concat_heads__sliding_local_dilated__memory_aug_recurrent_mem_tr__prompt_kernel(
    A_x, A_wqkv, A_wo, B_x, B_mem0, B_Wq, B_Wk, B_Wv, B_Wo, B_seg_len,
):
    assert B_seg_len == SEG
    assert A_x.shape == B_x.shape == (1, S, D) and B_mem0.shape == (1, M, D)
    assert B_Wq.shape == B_Wk.shape == B_Wv.shape == (D, H, DH) and B_Wo.shape == (H, DH, D)
    dma = pltpu.SemaphoreType.DMA

    def vmem(shape, dtype):
        assert math.prod(shape) * jnp.dtype(dtype).itemsize % 16384 == 0
        return pltpu.VMEM(shape, dtype)

    call = pl.pallas_call(
        _kernel,
        out_shape=jax.ShapeDtypeStruct((S, 2 * D), BF16),
        in_specs=[pl.BlockSpec(memory_space=pl.ANY)] * 9,
        out_specs=pl.BlockSpec(memory_space=pl.ANY),
        scratch_shapes=[
            vmem((S, D), BF16),
            vmem((3, D, D), BF16),
            vmem((D, D), BF16),
            vmem((LT, D, 128), F32),
            vmem((2 * D, D), U32),
            vmem((TB, D), U32),
            vmem((2, LT, TB, 128), F32),
            vmem((2, 2 * LT, HALO + TB, 128), F32),
            vmem((2, TB, D), F32),
            vmem((S, D), BF16),
            vmem((S, D), BF16),
            vmem((8 * M, D), BF16),
            vmem((RAW * 3 * GW * 128, D), BF16),
            vmem((H * DH, D), BF16),
            vmem(((PAD + GQ) * GW * 64, D), U32),
            vmem(((PAD + GQ) * 8 * 64, D), U32),
            vmem((GO * 64, NR * 128), U32),
            vmem((3 * SEG, D), F32),
            vmem((NQ, L, 128), F32),
            vmem((LT, 3 * SEG, 128), F32),
            vmem((NR + 1, L, 128), F32),
            vmem((8, M, 128), F32),
            vmem((GQ, 2 * GW, SEG, 128), F32),
            vmem((NQ, SEG, 128), F32),
            [vmem((4, L, 128), F32)] * RING,
            vmem((NO, SEG, 128), F32),
            [vmem((20, L + SEG, 128), F32)] * len(CHUNKS),
            vmem((2 * LT, SEG, 128), F32),
            vmem((S, D), BF16),
            dma((7,)), dma((NB // 2,)), dma((GO, 3)), dma((3,)), dma((GO,)), dma((2,)),
        ],
        compiler_params=pltpu.CompilerParams(vmem_limit_bytes=126 * 1024 * 1024, **{
            name: True for name in ("disable_bounds_checks", "disable_semaphore_checks")
            if hasattr(pltpu.CompilerParams, name)}),
        name="sliding_and_memory_attention",
    )

    def by_feature(w):
        return w.transpose(1, 2, 0).reshape(H * DH, D)

    out = call(A_x.reshape(S, D), A_wqkv, A_wo, B_x.reshape(S, D), B_mem0.reshape(M, D),
               by_feature(B_Wq), by_feature(B_Wk), by_feature(B_Wv), B_Wo.reshape(H * DH, D))
    return out.reshape(1, S, 2 * D)
```

```python
import collections
import functools
import itertools
import math
import random

import jax
import jax.numpy as jnp
import numpy as np
from jax import lax
from jax.experimental import pallas as pl
from jax.experimental.pallas import tpu as pltpu

F32, BF16, U32 = jnp.float32, jnp.bfloat16, jnp.uint32
NT = (((1,), (1,)), ((), ()))
MASKED = -1000000000.0
LOG2E = math.log2(math.e)

S, D = 2048, 640
LT = D // 128

AH, AD, AW, ADIL = 32, 20, 8, 2
HALO = 16
TB = 128
NB = S // TB

H, DH, M, SEG = 32, 192, 8, 32
L = M + SEG
HS = SEG // 2
NSEG = S // SEG
NP = H // 2
NO = 3 * NP
NQ = 3 * NO
GW = 6
GO, GQ = NO // GW, NQ // GW
PAD = 3
RAW = 4
RING = 12
CHUNKS = ((0, 3), (3, 5), (5, GO))


def _algorithm(rank_ones):
    rows = np.array([[1, 0], [0, 1], [1, 1]])
    duals = np.array([[0, 1], [1, 0], [1, -1]])
    sets = [[[np.array(["-0+".index(c) - 1 for c in w]) for w in e.split()] for e in s] for s in rank_ones]
    left, right = [], []
    for t, s in enumerate(sets):
        p, q = [k for k in range(3) if k != t]
        for u, v in s:
            left += [np.outer(u, rows[p]), np.outer(u, rows[q])]
            right += [np.outer(v, duals[q]), np.outer(v, duals[p])]
    for (u0, v0), (u1, v1), (u2, v2) in itertools.product(*sets):
        for a, b in itertools.product((1, -1), repeat=2):
            e = np.outer(u0 + a * u1, v0 + b * v1)
            if (e == np.outer(u2, v2)).all() or (e == -np.outer(u2, v2)).all():
                left.append(np.outer(u0, rows[1]) - a * np.outer(u1, rows[0]))
                right.append(np.outer(v0, duals[1]) + b * np.outer(v1, duals[0]))
    left, right = np.array(left), np.array(right)
    have = np.einsum("rka,rnb->kanbr", left, right).reshape(-1, len(left))
    want = np.einsum("kp,nq,ab->kanbpq", np.eye(LT), np.eye(GW), np.eye(2)).reshape(len(have), -1)
    blocks = np.rint(np.linalg.lstsq(have, want, rcond=None)[0]).astype(int)
    assert (have @ blocks == want).all()
    sign = blocks.max(axis=1) * 2 - 1
    return left * sign[:, None, None], blocks * sign[:, None], right


def _shared_sums(matrix, seed):
    rng = random.Random(seed)
    rows = [{k: int(c) for k, c in enumerate(row) if c} for row in matrix]
    shared = {}
    while True:
        count = collections.Counter(
            (a, b, r[a] * r[b]) for r in rows for a, b in itertools.combinations(sorted(r), 2))
        top = max(count.values(), default=0)
        if top < 2:
            return shared, rows
        best = sorted(k for k, n in count.items() if n == top)
        a, b, sign = best[int(rng.random() * len(best))]
        name = matrix.shape[1] + len(shared)
        shared[name] = a, b, sign
        for r in rows:
            if r.get(a, 0) * r.get(b, 0) == sign:
                r[name] = r.pop(a)
                del r[b]


MODEL, BLOCKS, FEATURE = _algorithm((
    ("+0000 +00++0", "000+0 0+0000", "0000+ 000+00", "+-+00 00000+", "+00+0 00+0+0"),
    ("0+00+ 000+++", "0+0+0 0+00++", "00+-+ 00++00", "00+0+ +00000", "+0+00 0000+0", "00+00 0+-000"),
    ("0+000 0000++", "00+-+ ++0000", "00+00 +00+00", "+-000 0+-00+", "00+-0 00+000", "+-00- +0000-")))
NR = len(BLOCKS)
BOTH = 34
SINGLE = {r: int(row.argmax()) for r, row in enumerate(BLOCKS) if abs(row).sum() == 1}
SUMMED = [r for r in range(NR) if r not in SINGLE]


def _step_sums(out, step, seed):
    use = MODEL[:, :, step].any(1) & FEATURE[:, :, step].any(1)
    return [_shared_sums((m * keep[:, None]).T, seed) for m, keep in (
        (out.reshape(NR, -1), use), (out.reshape(NR, -1), use & (np.arange(NR) < BOTH)), (out[:, :, step], use))]


QKV_SUMS = _step_sums(FEATURE, 0, 32), _step_sums(FEATURE, 1, 5)
OUT_SUMS = _step_sums(MODEL, 0, 0), _step_sums(MODEL, 1, 6)
BLOCK_SUMS = _shared_sums(BLOCKS, 37)

QKV_ORDER = (
    (30, 14, 20, 3, 12, 28, 9, 22, 10, 18, 26, 1, 5, 24, 7, 32, 16,
     40, 38, 45, 36, 46, 44, 39, 34, 35, 43, 37, 41, 42),
    (31, 15, 4, 11, 27, 0, 19, 8, 23, 13, 33, 6, 29, 21, 2, 25, 17,
     40, 34, 41, 39, 35, 45, 46, 36, 43, 44, 38, 37, 42))
OUT_ORDER = (
    (24, 14, 10, 5, 32, 28, 16, 30, 22, 7, 9, 3, 12, 1, 18, 20, 26,
     40, 34, 41, 42, 39, 37, 43, 36, 46, 45, 44, 35, 38),
    (23, 11, 13, 2, 15, 17, 4, 25, 31, 6, 33, 8, 29, 21, 19, 0, 27,
     39, 36, 45, 34, 41, 40, 37, 44, 43, 42, 46, 35, 38))
BLOCK_ORDER = (3, 28, 6, 0, 5, 17, 11, 8, 10, 7, 4, 16, 2, 1, 23, 22, 9, 29, 24, 19, 12, 18, 25, 13, 14, 20,
               21, 15, 26, 27)
MEM_ORDER = (2, 1, 4, 0, 3)

LAGS = ((40, 70, 100), (50, 80, 110))
TOKENS_AT = (737, 4)
OUT_PARTS = (5, 5)
TURNS = int(
    "734a6a6a6a24a26a6a4a24b4a6a6a430dd2852d2d2969693094b4a552942968a52d21e5161c385d29525a294b42d32a4"
    "b0e172a626a3453521e49694385c61a5a4d22e28732a4b0e171a52968a52d21e5161c385d29525a294b42d32a4b0e172"
    "5a1c3465870e1b4a62a4b4a6870e15a52c385a587161a5a1c7171717161861a5a5a1861a5a5a5825a5a292d2d2d2d298"
    "a187353141c29a91a984d48d3a2c34a272a6a43a929a91a6870e2c1e1c3871385a529694a58707870d2954a9a90e4a5a"
    "52954a6a42e19694c5394a587078b0e1a8e1c8b0e626a62c1e1c3870790d4c29e1c3931a193931a949a9458d0e949871", 16)

A_PACE = (12, 4)
SUM_PACE = (18, 10)
A_SHARE = 58
START_CUT = (15, 20)
FIRST_CUT = (5, 12, 21, 17, 21, 6)
LAST_LAGS = (7, 12, 3, 7, 1.9)


def _ds(i, n):
    return pl.ds(i * n if isinstance(i, int) else pl.multiple_of(i * n, n), n)


def _dot(a, b):
    return jnp.dot(a, b, preferred_element_type=F32)


def _cat(*parts):
    return jnp.concatenate(parts, axis=0)


def _add(a, b):
    return b if a is None else _cat(a[:M] + b[:M], a[M:] + b[M:])


def _acc(a, sign, b):
    if a is None:
        return sign, b
    if a[0] == sign:
        return sign, a[1] + b
    return (1, a[1] - b) if a[0] > 0 else (1, b - a[1])


def _sum(terms):
    return functools.reduce(lambda a, t: _acc(a, *t), terms, None)


def _val(a):
    return a[1] if a[0] > 0 else -a[1]


class _Sums:
    def __init__(self, plan, done, begin=lambda k: None):
        self.shared, self.rows = plan
        self.done, self.begin = done, begin
        self.terms, self.sums = {}, [None] * len(self.rows)
        for k, row in enumerate(self.rows):
            if not row and (first := begin(k)) is not None:
                done(k, first)

    def add(self, name, sign, value):
        self.terms[name] = sign, value
        for k, row in enumerate(self.rows):
            if name in row:
                if self.sums[k] is None and (first := self.begin(k)) is not None:
                    self.sums[k] = 1, first
                self.sums[k] = _acc(self.sums[k], row[name] * sign, value)
                if all(n in self.terms for n in row):
                    self.done(k, _val(self.sums[k]))
        for n, (a, b, s) in self.shared.items():
            if name in (a, b) and a in self.terms and b in self.terms and n not in self.terms:
                self.add(n, *_acc(self.terms[a], s * self.terms[b][0], self.terms[b][1]))


def _share(tasks, k, n):
    return list(tasks[k * len(tasks) // n:(k + 1) * len(tasks) // n])


def _merge(a, b, early=0):
    n = len(a) - early
    return [t for k in range(n) for t in [a[k]] + _share(b, k, n)] + a[n:]


def _each(f, items, *args):
    return [task for item in items for task in f(item, *args)]


def _run(tasks):
    for task in tasks:
        task()


def _kernel(ax_hbm, awqkv_hbm, awo_hbm, bx_hbm, mem_hbm, wq_hbm, wk_hbm, wv_hbm, wo_hbm,
            out_hbm,
            ax, awqkv, awo, tmp, wa, xb, q_s, kv_s, oa_s, outa,
            bx, mem, raw, wo_raw, plain, summed, wo, h0, first, xy, lhs, m_s, part, tok, ring,
            ox, mixed, opart, outb,
            sem_a, sem_x, sem_w, sem_b, sem_wo, sem_o):
    cp = pltpu.make_async_copy

    def rows_copy(src, dst, rows, sem):
        return [cp(src.at[rows, :], dst.at[rows, :], sem)]

    c_aw = [cp(awqkv_hbm.at[r0:r1, _ds(j, D)], awqkv.at[j, r0:r1], sem_a.at[k])
            for k, (j, (r0, r1)) in enumerate(itertools.product(range(3), ((0, 384), (384, D))))]
    c_awo = [cp(awo_hbm, awo, sem_a.at[6])]
    c_bx0 = [cp(mem_hbm, mem.at[0:M], sem_b.at[0])] + rows_copy(bx_hbm, bx, slice(0, 6 * SEG), sem_b.at[1])
    c_bx1 = rows_copy(bx_hbm, bx, slice(6 * SEG, S), sem_b.at[2])
    c_outa = [cp(outa, out_hbm.at[:, 0:D], sem_o.at[0])]

    def c_ax(c):
        return rows_copy(ax_hbm, ax, _ds(c, 2 * TB), sem_x.at[c])

    def c_w(c):
        return [cp(w.at[_ds(c, GW * 128), :], raw.at[_ds((c & (RAW - 1)) * 3 + j, GW * 128), :], sem_w.at[c, j])
                for j, w in enumerate((wq_hbm, wk_hbm, wv_hbm))]

    def c_wo(g):
        return rows_copy(wo_hbm, wo_raw, _ds(g, GW * 128), sem_wo.at[g])

    def c_outb(rows):
        return [cp(outb.at[rows, :], out_hbm.at[rows, D:], sem_o.at[1])]

    def start(copies):
        for c in copies:
            c.start()

    def wait(copies):
        for c in copies:
            c.wait()
        recent.clear()

    recent = []

    def paced(x, zero, marks):
        late = _cat(*[recent[t] if t >= 0 else jnp.zeros((8, 128), F32) for t in marks[:x.shape[0] // 8]])
        always = lax.broadcasted_iota(jnp.int32, x.shape, 1) >= zero
        return lax.select(always, x, late if x.dtype == F32 else pltpu.bitcast(late, U32))

    def tile(ref, i, j):
        return pltpu.bitcast(ref[_ds(i, 64), _ds(j, 128)], BF16)

    def a_weights(j, zero=None):
        def task(t):
            if j < 3:
                tmp[t] = awqkv[j, _ds(t, 128), :].astype(F32).T
            else:
                marks = [len(recent) - 40 + k * 3 // 4 for k in range(40)]
                w = paced(pltpu.bitcast(awo[:, _ds(t, 128)], U32), zero, marks)
                tmp[t] = pltpu.bitcast(w, BF16).astype(F32)
            w = _cat(*[tmp[t, pl.ds(d, AH, stride=AD), :] for d in range(AD)])
            wa[_ds(j, D // 2), _ds(t, 128)] = pltpu.bitcast(w.astype(BF16), U32)

        return [functools.partial(task, t) for t in range(LT)]

    def by_tile(product, put):
        acc = [None]

        def task(t, k):
            r = product(t, k)
            e = len(recent) % 16
            recent.extend(r[8 * (e + i) % TB:8 * (e + i) % TB + 8] for i in range(4))
            acc[0] = _add(acc[0] if k else None, r)
            if k == LT - 1:
                put(t, acc[0])

        return [functools.partial(task, t, k) for t in range(LT) for k in range(LT)]

    def a_load(i, b):
        xb[_ds(b, TB // 2), :] = pltpu.bitcast(ax[_ds(i, TB), :], U32)

    def a_proj(j, b, first_block=False):
        def put(t, r):
            if j == 0:
                q_s[b, t] = r
                return
            c = (j - 1) * LT + t
            kv_s[b, c, HALO:, :] = r
            if first_block:
                kv_s[b, c, 0:HALO, :] = jnp.broadcast_to(r[0:1, :], (HALO, 128))
            else:
                kv_s[b, c, 0:HALO, :] = kv_s[1 - b, c, TB:, :]

        return by_tile(lambda t, k: lax.dot_general(
            tile(xb, b, k), tile(wa, j * LT + t, k), NT, preferred_element_type=F32), put)

    def a_attention(b, zero, first_block=False):
        n = TB // 8
        lag = n if first_block else A_PACE[1]
        marks, logits = [], []

        def mark():
            marks.append(len(recent) - A_PACE[0])

        def window(c, w):
            return kv_s[b, c, pl.ds(HALO - ADIL * w, TB), :]

        def score():
            q = [paced(q_s[b, t], zero, marks[::4]) for t in range(LT)]
            sums = [functools.reduce(jnp.add, [q[t] * window(t, w) for t in range(LT)]) for w in range(AW)]
            rows = {}
            for k in range(n + 1):
                if k < n:
                    a = _cat(*[a[8 * k:8 * k + 8] for a in sums])
                    rows[k] = a + pltpu.roll(a, 2 * AH, 1)
                if k > 0:
                    rows[k - 1] = rows[k - 1] + pltpu.roll(rows[k - 1], AH, 1)
            logits.extend(_cat(*[rows[k][8 * w:8 * w + 8] for k in range(n)]) for w in range(AW))

        def mix():
            scale, lg = AD ** -0.5, logits
            if first_block:
                pos = lax.broadcasted_iota(jnp.int32, (HALO, 128), 0)
                lg = [_cat(jnp.where(pos >= ADIL * w, a[:HALO], MASKED / scale), a[HALO:])
                      for w, a in enumerate(lg)]
            m = paced(functools.reduce(jnp.maximum, lg), zero, marks[4 * lag + 1::4])
            e = [jnp.exp2((a - m) * (scale * LOG2E)) for a in lg]
            inv = 1.0 / functools.reduce(jnp.add, e)
            for t in range(LT):
                v = [window(LT + t, w) for w in range(AW)]
                v[0] = paced(v[0], zero, marks[4 * lag + 2 + 2 * t // LT::4])
                oa_s[b, :, _ds(t, 128)] = inv * functools.reduce(jnp.add, map(jnp.multiply, e, v))

        return [mark] * (4 * n) + [score], [mark] * (4 * lag) + [mix]

    def a_out(i, b):
        def put(t, r):
            outa[_ds(i, TB), _ds(t, 128)] = r.astype(BF16)

        return by_tile(lambda t, k: _dot(oa_s[b, :, _ds(k, 128)], tile(wa, 3 * LT + k, t)), put)

    def transposes(c, dst, g):
        def task(n):
            t = ((c & (RAW - 1)) * 3 + n % 9 // 3) * GW + n // 9 * 3 + n % 3
            v = pltpu.bitcast(raw[_ds(t, 128), :].T, U32)
            for k in range(LT):
                dst[_ds(g * GW + n, 64), _ds(k, 128)] = v[k * 64:(k + 1) * 64]

        return [functools.partial(task, n) for n in range(3 * GW)]

    def sum_blocks(block, put, zero):
        back, n = SUM_PACE
        marks = []

        def mark():
            marks.append(len(recent) - back)

        def done(r, v):
            if r not in SINGLE:
                put(r, pltpu.bitcast(v.astype(BF16), U32))

        def task():
            sums = _Sums(BLOCK_SUMS, done)
            for k in range(n):
                for i, b in enumerate(_share(BLOCK_ORDER, k, n)):
                    v = block(*divmod(b, GW))
                    if i == 0:
                        v = paced(v, zero, marks[k::n])
                    for r in SINGLE:
                        if SINGLE[r] == b:
                            put(r, v)
                    sums.add(b, 1, pltpu.bitcast(v, BF16).astype(F32))

        return [mark] * (8 * n) + [task]

    def sum_qkv(g, zero, src=plain, dst=summed):
        def put(r, v):
            if r not in SINGLE:
                i, j = divmod(SUMMED.index(r), LT)
                dst[_ds(g * 8 + i, 64), _ds(j, 128)] = v

        return sum_blocks(lambda k, n: src[_ds(g * GW + n, 64), _ds(k, 128)], put, zero)

    def sum_out(g, zero):
        def put(r, v):
            wo[_ds(g, 64), _ds(r, 128)] = v

        return sum_blocks(lambda k, n: pltpu.bitcast(wo_raw[_ds(g * GW + n, 128), _ds(k, 128)], U32), put, zero)

    def a_start():
        start(c_aw[:2])
        zero = lax.fori_loop(0, 2, lambda it, carry: it >> 16, 0)
        start(c_ax(0))
        wait(c_aw[:1])
        _run(a_weights(0)[:3])
        wait(c_aw[1:2])
        start(c_aw[2:3])
        _run(a_weights(0)[3:])
        wait(c_ax(0))
        start(c_aw[3:5])
        a_load(0, 0)
        a_load(1, 1)
        nq, nk = START_CUT
        _run(a_proj(0, 0))
        wait(c_aw[2:3])
        start(c_aw[5:] + c_awo)
        _run(a_proj(0, 1)[:nq] + a_weights(1)[:3])
        wait(c_aw[3:4])
        start(c_ax(1) + c_ax(2))
        _run(a_proj(0, 1)[nq:] + a_weights(1)[3:] + a_proj(1, 0, True))
        wait(c_aw[4:])
        start(c_w(0))
        early, late = a_attention(0, zero, True)
        _run(a_proj(1, 1)[:nk] + a_weights(2) + _merge(a_proj(2, 0, True), early))
        wait(c_awo)
        start(c_bx0)
        _run(_merge(a_proj(1, 1)[nk:] + a_proj(2, 1), _merge(late, a_weights(3, zero)), 4))
        wait(c_ax(1))
        a_load(2, 0)

    def a_step(it, carry):
        i, g, zero = 2 * it, jnp.maximum(3 * it - 9 + PAD, 0), it >> 16
        pl.when(it + 2 < NB // 2)(lambda: start(c_ax(it + 2)))
        pl.when(it + 1 < NB // 2)(lambda: wait(c_ax(it + 1)))
        start(c_w(it))
        pl.when(it > 1)(lambda: wait(c_w(it - 2)))
        src, dst = [ref.at[pl.ds(pl.multiple_of(g * n, n), k * n)]
                    for ref, n, k in ((plain, GW * 64, 6), (summed, 8 * 64, 3))]
        sums, moves = _each(sum_qkv, range(3), zero, src, dst), transposes(it + RAW - 2, src, 3)
        cut = len(sums) * A_SHARE // 100
        early, late = a_attention(1, zero)
        a_load(i + 1, 1)
        _run(_merge(a_out(i - 2, 0) + _each(a_proj, range(3), 0),
                    moves[:1] + _merge(early, sums[:cut]) + moves[1:]))
        a_load(jnp.minimum(i + 2, NB - 1), 0)
        side = sum(a_attention(0, zero), [])
        side = _merge(side[:len(late)], late) + side[len(late):]
        _run(_merge(_each(a_proj, range(3), 1) + a_out(i - 1, 1), _merge(side, sums[cut:])))
        return zero

    def attention(qkv, put, row0=0, zero=0):
        row = lax.broadcasted_iota(jnp.int32, (L - row0, 128), 0) + row0
        col = lax.broadcasted_iota(jnp.int32, (L - row0, 128), 1) + zero
        head0 = col < L
        visible = jnp.where(row < M, L - 1, row) >= jnp.where(head0, col, col - L)
        scale = DH ** -0.5
        st = {}

        def by_head(n):
            t = qkv(n)
            if n % 3 == 1:
                low = lax.broadcasted_iota(jnp.int32, t.shape, 1) < 64 + zero
                t = _cat(jnp.where(low, t, 0.0), jnp.where(low, 0.0, t))
            elif n % 3 == 2:
                t = _cat(jnp.zeros_like(t), t)
            return _cat(t, jnp.zeros((128 - len(t), 128), F32)).astype(BF16)

        def score(p):
            sc = [lax.dot_general(qkv(9 * p + t), by_head(9 * p + 3 + t), NT, preferred_element_type=F32)
                  for t in range(3)]
            sc = jnp.where(visible, functools.reduce(_add, sc), jnp.where(col < 2 * L, MASKED / scale, -jnp.inf))
            m0 = jnp.max(jnp.where(head0, sc, -jnp.inf), axis=1, keepdims=True)
            m1 = jnp.max(jnp.where(head0, -jnp.inf, sc), axis=1, keepdims=True)
            st[p] = sc - jnp.where(head0, m0, m1)

        def normalize(p):
            e = jnp.exp2(st[p] * (scale * LOG2E))
            l0 = jnp.sum(jnp.where(head0, e, 0.0), axis=1, keepdims=True)
            l1 = jnp.sum(jnp.where(head0, 0.0, e), axis=1, keepdims=True)
            st[p] = e / jnp.where(head0, l0, l1)

        def mix(p):
            for t in range(3):
                put(3 * p + t, _dot(st[p], by_head(9 * p + 6 + t)))

        return score, normalize, mix

    def mixed_at(n):
        return [(ref, (n - g0 * GW) * (L + SEG)) for ref, (g0, g1) in zip(mixed, CHUNKS) if g0 <= n // GW < g1][0]

    def put_x(n, r):
        ref, k = mixed_at(n)
        ref[k:k + M] = r[0:M]
        ox[n] = r[M:]

    def put_y(n, r):
        ref, k = mixed_at(n)
        ref[k:k + L + SEG] = _cat(r[0:M], ox[n] - r[M:], r[M:])

    def left_operands(s, zero):
        done = []

        def load(k):
            x, y = [paced(pltpu.bitcast(bx[_ds(s + e, SEG), _ds(k, 128)], U32), zero, [len(recent) - 20] * 2)
                    for e in range(2)]
            x, y = [pltpu.bitcast(v, BF16).astype(F32) for v in (x, y)]
            xy[_ds(k, 3 * SEG)] = _cat(x, y, x + y)

        def task(r):
            src = xy.at[_ds(zero, LT * 3 * SEG)]
            terms = [(a or b, src[_ds(3 * k + (2 if a and b else 1 if b else 0), SEG)])
                     for k, (a, b) in enumerate(MODEL[r]) if a or b]
            terms[0] = terms[0][0], paced(terms[0][1], zero, [len(recent) - 20] * 4)
            done.append(_val(_sum(terms)))
            if r == NR - 1:
                v = jnp.stack(done)
                lhs[0:NR, 0:HS] = v[:, :HS]
                lhs[0:NR, HS + M:] = v[:, HS:]

        return [functools.partial(load, k) for k in range(LT)] + [functools.partial(task, r) for r in range(NR)]

    def step(s, second, zero):
        def reread(ref):
            return ref.at[_ds(zero, ref.shape[0])]

        part_r, ring_r = reread(part), [reread(r) for r in ring]
        halves = [slice(0, HS), slice(HS, SEG)][::1 - 2 * second]
        new_mem = [None] * LT
        due = []

        def mm(x, w):
            r = _dot(x, w)
            recent.append(r[0:M] if second and len(recent) > TOKENS_AT[0] - 24 else None)
            while due and due[0][0] <= len(recent):
                due.pop(0)[1]()
            return r

        def in_turn(items):
            lists = [[x for x in items if (x[0] >= BOTH) == e] for e in (False, True)]
            for _ in items:
                yield lists[TURNS >> second * (NQ + NO) * LT + len(recent) & 1].pop(0)

        def mem_tiles(r):
            return [MEM_ORDER[k] for k, c in enumerate(MODEL[r]) if c[second]]

        def project(g):
            before = part_r[g] if second else None
            tokens, memory = {}, {}

            def token_sums(e):
                def begin(k):
                    return before[k * SEG + halves[e].start:k * SEG + halves[e].stop] if second else None

                return _Sums(QKV_SUMS[second][e], lambda k, v: tokens.update({(k, halves[e].start): v}), begin)

            sums = token_sums(0), token_sums(1), _Sums(QKV_SUMS[second][2], memory.__setitem__)
            if g == 0:
                m = [m_s[k] for k in range(LT)]
                lhs[0:NR, HS:HS + M] = jnp.stack([
                    _val(_sum((c[second], m[k]) for k, c in enumerate(MODEL[r]) if c[second]))
                    if r in QKV_ORDER[second] else jnp.zeros((M, 128), F32) for r in range(NR)])
            left = lhs[0:NR].reshape(NR * L, 128)
            blocks = pltpu.bitcast(plain[_ds(PAD + g, GW * 64), :], BF16)
            weights = pltpu.bitcast(summed[_ds(PAD + g, 8 * 64), :], BF16)
            order = sorted(QKV_ORDER[second], key=lambda r: max(mem_tiles(r)) if second and g == 0 else 0)
            for r, in in_turn([(r,) for r in order]):
                t0, t1 = (0, L) if r < BOTH else (second * HS, second * HS + HS + M)
                w, (i, j) = ((blocks, divmod(SINGLE[r], GW)[::-1]) if r in SINGLE
                             else (weights, divmod(SUMMED.index(r), LT)))
                v = mm(left[r * L + t0:r * L + t1], w[i * 128:(i + 1) * 128, j * 128:(j + 1) * 128])
                sums[2].add(r, 1, v[HS - t0:HS - t0 + M])
                if t0 == 0:
                    sums[second].add(r, 1, v[:HS])
                if t1 == L:
                    sums[1 - second].add(r, 1, v[-HS:])
            if second:
                tok[_ds(g, GW)] = jnp.stack([_cat(tokens[k, 0], tokens[k, HS]) for k in range(1, 2 * GW, 2)])
            else:
                part[g] = _cat(*[tokens[k, e] for k in range(2 * GW) for e in (0, HS)])
            for e in range(2):
                ring[(2 * g + e) % RING][0:3, 0:L if second else M] = jnp.stack([
                    _cat(memory[k], tokens[2 * k, 0], tokens[2 * k, HS]) if second else memory[k]
                    for k in range(3 * e, 3 * e + 3)])

        def projected(n):
            src = ring_r[n // 3 % RING]
            return src[n % 3] if second else _cat(src[n % 3, 0:M], tok[n])

        def out_chunk(ref, g0, g1):
            def token_sums(e):
                def begin(k):
                    if (second and OUT_SUMS[0][1 - e][1][k]) or (g0 > 0 and OUT_SUMS[second][e][1][k]):
                        return opart[k, halves[e]]

                def done(k, v):
                    if second and g1 == GO:
                        rows = _ds((s + k % 2) * 2 + halves[e].start // HS, HS)
                        outb[rows, _ds(k // 2, 128)] = v.astype(BF16)
                    else:
                        opart[k, halves[e]] = v

                return _Sums(OUT_SUMS[second][e], done, begin)

            def done(k, v):
                new_mem[k] = v
                if g1 == GO:
                    m_s[k] = v

            sums = token_sums(0), token_sums(1), _Sums(OUT_SUMS[second][2], done, list(new_mem).__getitem__)
            weights = [pltpu.bitcast(wo[_ds(g, 64), :], BF16) for g in range(g0, g1)]
            order = sorted(OUT_ORDER[second], key=lambda r: min(mem_tiles(r)) if g1 == GO and not second else 0)
            tall, short = [[r for r in order if (r >= BOTH) == e] for e in (False, True)]
            n = OUT_PARTS[second]
            for k in range(n):
                acc, both, x = {}, ref[0:(g1 - g0) * GW * (L + SEG)], None if second else ox[g0 * GW:g1 * GW]
                some = _share(tall[::-1], n - 1 - k, n)[::-1] + _share(short, k, n)
                for r, g in in_turn([(r, g) for g in range(g0, g1) for r in some]):
                    t0, rows = (0, SEG) if r < BOTH else (halves[0].start, HS)
                    terms = []
                    for j, (a, b) in enumerate(FEATURE[r]):
                        i = ((g - g0) * GW + j) * (L + SEG) + t0
                        if b:
                            terms.append((a or b, both[i + (M if a else L):i + (M if a else L) + rows]))
                        elif a and second:
                            terms += [(a, both[i + r0:i + r0 + rows]) for r0 in (M, L)]
                        elif a:
                            terms.append((a, x[(g - g0) * GW + j, t0:t0 + rows]))
                    sign, left = _sum(terms)
                    m_sign, m = _sum((c[second], both[j * (L + SEG):j * (L + SEG) + M])
                                     for j, c in enumerate(FEATURE[r], (g - g0) * GW) if c[second])
                    v = mm(_cat(m, left), weights[g - g0][:, r * 128:(r + 1) * 128])
                    acc[r] = m_sign, sign, _add(acc[r][2] if r in acc else None, v)
                for r, (m_sign, sign, v) in acc.items():
                    sums[2].add(r, m_sign, v[:M])
                    sums[second if r < BOTH else 0].add(r, sign, v[M:M + HS])
                    if r < BOTH:
                        sums[1 - second].add(r, sign, v[M + HS:])

        recent.clear()
        stages = attention(projected, put_x if second else put_y)
        for p in range(NP):
            ready = LT * GW * ((9 * p + 5) // GW + 1)
            due += [(ready + lag, functools.partial(f, p)) for f, lag in zip(stages, LAGS[second])]
        if second:
            due += [(TOKENS_AT[0] + k * TOKENS_AT[1], task)
                    for k, task in enumerate(left_operands(jnp.minimum(s + 4, NSEG - 2), zero))]
        due.sort(key=lambda e: e[0])
        for g in range(GQ):
            project(g)
        for ref, chunk in zip(mixed, CHUNKS):
            out_chunk(reread(ref), *chunk)

    def first_segment(zero):
        def project(g):
            acc = {}

            def task(n, k):
                r = _dot(h0[0:L + SEG, _ds(k, 128)], tile(plain, PAD * GW + n, k))
                e = len(recent) % 8
                recent.extend([r[8 * e:8 * e + 8], r[8 * e + 8:8 * e + 16]])
                acc[n] = _add(acc.get(n), r)
                if k == LT - 1:
                    first[n] = acc[n][0:L]
                    tok[n] = acc[n][L:]

            return [functools.partial(task, g * GW + n, k) for n in range(GW) for k in range(LT)]

        def put(n, r):
            recent.extend([r[k:k + 8] for k in range(0, L, 16)])
            put_x(n, r)

        stages = attention(lambda n: first[n], put, zero=zero)
        new_mem = [None] * LT

        def heads(p0, p1):
            return [functools.partial(f, t - lag) for t in range(p0, p1 + 2)
                    for lag, f in enumerate(stages) if p0 <= t - lag < p1] + [lambda: None]

        def out(g):
            def task(n, k):
                ref, i = mixed_at(n)
                r = _dot(ref[i:i + M], wo_raw[_ds(n, 128), _ds(k, 128)])
                recent.append(r)
                new_mem[k] = r if new_mem[k] is None else new_mem[k] + r

            return [functools.partial(task, g * GW + n, k) for n in range(GW) for k in range(LT)]

        c1, c2, c3, d1, d2, m1 = FIRST_CUT
        moves = transposes(GO - 2, plain, PAD + GQ - 6) + transposes(GO - 1, plain, PAD + GQ - 3)
        start(c_wo(0))
        wait(c_w(GO - 2) + c_bx0)
        start(c_wo(1) + c_wo(2))
        h0[0:M, :] = mem[0:M, :].astype(F32)
        h0[M:L + SEG, :] = bx[0:2 * SEG, :].astype(F32)
        _run(_merge(a_out(NB - 2, 0) + _each(project, range(c1)), moves[:m1] + _merge(
            sum(a_attention(1, zero), []), _each(sum_qkv, range(PAD + GQ - 9, PAD + d1), zero))))
        wait(c_w(GO - 1))
        start(c_wo(3) + c_wo(4))
        _run(_merge(a_out(NB - 1, 1) + _each(project, range(c1, c2)),
                    moves[m1:] + _each(sum_qkv, range(PAD + d1, PAD + d2), zero)))
        start(c_wo(5))
        wait(_each(c_wo, range(3)))
        start(c_wo(6) + c_wo(7))
        _run(_merge(_merge(_each(project, range(c2, c3)), heads(0, 11)),
                    _each(sum_qkv, range(PAD + d2, PAD + GQ), zero) + _each(sum_out, range(3), zero)))
        wait(_each(c_wo, range(3, 6)))
        _run(_merge(_merge(_merge(_each(project, range(c3, GQ)), _each(out, range(3))), heads(11, 13))
                    + _merge(_each(out, range(3, 6)), heads(13, NP)),
                    _merge(_each(sum_out, range(3, 6), zero), left_operands(2, zero))))
        wait(c_wo(6) + c_wo(7))
        start(c_bx1 + c_outa)
        _run(_merge(out(6) + out(7), _each(sum_out, (6, 7), zero)))
        for k in range(LT):
            m_s[k] = new_mem[k]

    def two_segments(it, carry):
        pl.when(it == 1)(lambda: wait(c_bx1))
        step(2 * it, 0, it >> 16)
        step(2 * it, 1, it >> 16)
        start(c_outb(_ds(it, 2 * SEG)))
        return carry

    def last_segment():
        res, acc = {}, [None] * LT

        def project(n, k):
            r = _dot(-m_s[k] if k % 2 else m_s[k], tile(plain, PAD * GW + n, k))
            res[n] = _acc(res.get(n), 1 - 2 * (k % 2), r)

        def out(n, k):
            acc[k] = _add(acc[k], _dot(_cat(ox[n], res[NQ + n]), wo_raw[_ds(n, 128), _ds(k, 128)]))

        stages = attention(lambda n: _cat(_val(res[n]), tok[n]) if n in res else tok[n],
                           lambda n, r: res.update({NQ + n: r}), M)
        tiles = [9 * p + e for t in range(NP + 3) for p, e0 in ((t, 3), (t - 3, 6)) if 0 <= p < NP
                 for e in range(e0, e0 + 3)]
        ready = {n: (i * LT + LT - 1) // 4 for i, n in enumerate(tiles)}
        due = [((i * LT + k) // 4, 0, functools.partial(project, n, k))
               for i, n in enumerate(tiles) for k in range(LT)]
        for p in range(NP):
            due += [(ready[9 * p + e] + lag, rank, functools.partial(f, p))
                    for f, lag, e, rank in zip(stages, LAST_LAGS, (5, 5, 8), (2, 2, 1))]
        t = 0
        for k in range(NO * LT):
            if k % 4 == 0:
                t = max(t + LAST_LAGS[4], ready[9 * ((k + 3) // 15) + 8] + LAST_LAGS[3])
            due.append((int(t), 3, functools.partial(out, *divmod(k, LT))))
        _run([task for _, _, task in sorted(due, key=lambda e: e[:2])])
        outb[S - 2 * SEG:, :] = jnp.concatenate(acc, axis=1).astype(BF16)
        start(c_outb(slice(S - 2 * SEG, S)))

    a_start()
    first_segment(lax.fori_loop(1, NB // 2, a_step, 0))
    lax.fori_loop(0, NSEG // 2 - 1, two_segments, 0)
    last_segment()
    wait(c_outa + c_outb(slice(0, S)))


def pallas_concat_heads__sliding_local_dilated__memory_aug_recurrent_mem_tr__prompt_kernel(
    A_x, A_wqkv, A_wo, B_x, B_mem0, B_Wq, B_Wk, B_Wv, B_Wo, B_seg_len,
):
    assert B_seg_len == SEG
    assert A_x.shape == B_x.shape == (1, S, D) and B_mem0.shape == (1, M, D)
    assert B_Wq.shape == B_Wk.shape == B_Wv.shape == (D, H, DH) and B_Wo.shape == (H, DH, D)
    dma = pltpu.SemaphoreType.DMA

    def vmem(shape, dtype):
        assert math.prod(shape) * jnp.dtype(dtype).itemsize % 16384 == 0
        return pltpu.VMEM(shape, dtype)

    call = pl.pallas_call(
        _kernel,
        out_shape=jax.ShapeDtypeStruct((S, 2 * D), BF16),
        in_specs=[pl.BlockSpec(memory_space=pl.ANY)] * 9,
        out_specs=pl.BlockSpec(memory_space=pl.ANY),
        scratch_shapes=[
            vmem((S, D), BF16),
            vmem((3, D, D), BF16),
            vmem((D, D), BF16),
            vmem((LT, D, 128), F32),
            vmem((2 * D, D), U32),
            vmem((TB, D), U32),
            vmem((2, LT, TB, 128), F32),
            vmem((2, 2 * LT, HALO + TB, 128), F32),
            vmem((2, TB, D), F32),
            vmem((S, D), BF16),
            vmem((S, D), BF16),
            vmem((8 * M, D), BF16),
            vmem((RAW * 3 * GW * 128, D), BF16),
            vmem((H * DH, D), BF16),
            vmem(((PAD + GQ) * GW * 64, D), U32),
            vmem(((PAD + GQ) * 8 * 64, D), U32),
            vmem((GO * 64, NR * 128), U32),
            vmem((3 * SEG, D), F32),
            vmem((NQ, L, 128), F32),
            vmem((LT * 3 * SEG, 128), F32),
            vmem((NR + 1, L, 128), F32),
            vmem((8, M, 128), F32),
            vmem((GQ, 2 * GW * SEG, 128), F32),
            vmem((NQ, SEG, 128), F32),
            [vmem((4, L, 128), F32)] * RING,
            vmem((NO, SEG, 128), F32),
            [vmem((20 * (L + SEG), 128), F32)] * len(CHUNKS),
            vmem((2 * LT, SEG, 128), F32),
            vmem((S, D), BF16),
            dma((7,)), dma((NB // 2,)), dma((GO, 3)), dma((3,)), dma((GO,)), dma((2,)),
        ],
        compiler_params=pltpu.CompilerParams(vmem_limit_bytes=126 * 1024 * 1024, **{
            name: True for name in ("disable_bounds_checks", "disable_semaphore_checks")
            if hasattr(pltpu.CompilerParams, name)}),
        name="sliding_and_memory_attention",
    )

    def by_feature(w):
        return w.transpose(1, 2, 0).reshape(H * DH, D)

    out = call(A_x.reshape(S, D), A_wqkv, A_wo, B_x.reshape(S, D), B_mem0.reshape(M, D),
               by_feature(B_Wq), by_feature(B_Wk), by_feature(B_Wv), B_Wo.reshape(H * DH, D))
    return out.reshape(1, S, 2 * D)
```
